```python
import jax
import jax.numpy as jnp

def _softmax(x, axis=-1):
    return jax.nn.softmax(x, axis=axis)

def _gelu(x):
    return jax.nn.gelu(x, approximate=True)

def _silu(x):
    return jax.nn.silu(x)

def _sigmoid(x):
    return jax.nn.sigmoid(x)

def _layernorm(x, axis=-1, eps=1e-05):
    m = jnp.mean(x, axis=axis, keepdims=True)
    v = jnp.var(x, axis=axis, keepdims=True)
    return (x - m) / jnp.sqrt(v + eps)

def _scatter_add(tgt, idx, src, axis=0):
    return tgt.at[idx].add(src)

def _segment_sum(src, seg, n):
    return jax.ops.segment_sum(src, seg, n)

class _Rng:

    def __init__(self, key):
        self._k = key

    def _next(self):
        self._k, sub = jax.random.split(self._k)
        return sub

    def normal(self, shape):
        return jax.random.normal(self._next(), shape, dtype=jnp.bfloat16)

    def randint(self, lo, hi, shape):
        return jax.random.randint(self._next(), shape, lo, hi, dtype=jnp.int32)

    def uniform(self, shape, lo=0.0, hi=1.0):
        return jax.random.uniform(self._next(), shape, jnp.bfloat16, lo, hi)

    def permutation(self, n):
        return jax.random.permutation(self._next(), n)
kernel_name = 'sequential_preLN__memory_aug_infini_attn__moe_arch_mod__prompt'

def setup_inputs():
    _rng = _Rng(jax.random.key(int.from_bytes(__import__("os").urandom(4), "little")))
    _w = lambda a: (lambda t: t.astype(jnp.bfloat16) if jnp.issubdtype(t.dtype, jnp.floating) else t)(jnp.asarray(a))

    def _A_setup():
        B, S, D, H = (1, 2048, 576, 32)
        N = 4
        L = max(1, S // N)
        sc = D ** (-0.5)
        return {'x': _w((lambda *s: _rng.normal(s) * 0.05)(B, N * L, D)), 'wq': _w((lambda *s: _rng.normal(s) * 0.05)(D, D) * sc), 'wk': _w((lambda *s: _rng.normal(s) * 0.05)(D, D) * sc), 'wv': _w((lambda *s: _rng.normal(s) * 0.05)(D, D) * sc), 'wo': _w((lambda *s: _rng.normal(s) * 0.05)(D, D) * sc), 'beta': _w((lambda *s: _rng.normal(s) * 0.05)(H))}
    _A_in = _A_setup()

    def _B_setup():
        B, S, D, F, C = (1, 2048, 576, 4608, 1)
        return {'x': _w((lambda *s: _rng.normal(s) * 0.05)(B, S, D)), 'w_r': _w((lambda *s: _rng.normal(s) * 0.05)(D)), 'w_gate': _w((lambda *s: _rng.normal(s) * 0.05)(D, F)), 'w_up': _w((lambda *s: _rng.normal(s) * 0.05)(D, F)), 'w_down': _w((lambda *s: _rng.normal(s) * 0.05)(F, D))}
    _B_in = _B_setup()
    return {'A_x': _A_in['x'], 'A_wq': _A_in['wq'], 'A_wk': _A_in['wk'], 'A_wv': _A_in['wv'], 'A_wo': _A_in['wo'], 'A_beta': _A_in['beta'], 'B_x': _B_in['x'], 'B_w_r': _B_in['w_r'], 'B_w_gate': _B_in['w_gate'], 'B_w_up': _B_in['w_up'], 'B_w_down': _B_in['w_down']}

def reference(A_x, A_wq, A_wk, A_wv, A_wo, A_beta, B_x, B_w_r, B_w_gate, B_w_up, B_w_down):

    def _A_ref(x, wq, wk, wv, wo, beta):
        B, S, D = x.shape
        H = 32
        Dh = D // H
        N = 4
        L = S // N
        q = (lambda x, *d: x.transpose(*d))((x @ wq).reshape(B, S, H, Dh), 0, 2, 1, 3).reshape(B, H, N, L, Dh)
        k = (lambda x, *d: x.transpose(*d))((x @ wk).reshape(B, S, H, Dh), 0, 2, 1, 3).reshape(B, H, N, L, Dh)
        v = (lambda x, *d: x.transpose(*d))((x @ wv).reshape(B, S, H, Dh), 0, 2, 1, 3).reshape(B, H, N, L, Dh)
        phi = lambda t: jnp.where(t > 0, t + 1.0, jnp.exp(t))
        scale = Dh ** (-0.5)
        ar = jnp.arange(L)
        mask = (lambda x, dt: x.astype(dt))(ar[:, None] < ar[None, :], x.dtype) * -1000000000.0
        g = _sigmoid(beta).reshape(1, H, 1, 1)
        M = jnp.einsum('bhd,bhe->bhde', q[:, :, 0, 0, :] * 0.0, q[:, :, 0, 0, :] * 0.0)
        z = q[:, :, 0, 0, :] * 0.0
        outs = []
        for s in range(N):
            qs, ks, vs = (q[:, :, s].copy(), k[:, :, s].copy(), v[:, :, s].copy())
            logits = jnp.einsum('bhqd,bhkd->bhqk', qs, ks) * scale + mask
            p = _softmax(logits, axis=-1)
            a_dot = jnp.einsum('bhqk,bhkd->bhqd', p, vs)
            pq = phi(qs)
            num = jnp.einsum('bhld,bhde->bhle', pq, M)
            den = jnp.einsum('bhld,bhd->bhl', pq, z)[..., None] + 1e-06
            a_mem = num / den
            o = g * a_mem + (1.0 - g) * a_dot
            outs.append(o)
            pk = phi(ks)
            M = M + jnp.einsum('bhld,bhle->bhde', pk, vs)
            z = z + jnp.einsum('bhld->bhd', pk)
        o = (lambda x, *d: x.transpose(*d))(jnp.stack(outs, 2).reshape(B, H, S, Dh), 0, 2, 1, 3).reshape(B, S, D)
        return o @ wo

    def _B_ref(x, w_r, w_gate, w_up, w_down):
        B, S, D = x.shape
        C = 1
        r = x @ w_r
        idx = jnp.argsort(-r, axis=-1)[:, :C]
        idx_e = jnp.repeat(idx.reshape(B, C, 1), D, axis=2)
        x_sel = jnp.take_along_axis(x, idx_e, axis=1)
        g = _silu(x_sel @ w_gate)
        u = x_sel @ w_up
        y = g * u @ w_down
        r_sel = _sigmoid(jnp.take_along_axis(r, idx, axis=1))
        y = y * r_sel.reshape(B, C, 1)
        b_off = (jnp.arange(B) * S).reshape(B, 1)
        flat_idx = (idx + b_off).reshape(B * C)
        zero = (x * 0.0).reshape(B * S, D)
        upd = _scatter_add(zero, flat_idx, y.reshape(B * C, D), axis=0)
        return x + upd.reshape(B, S, D)
    x = A_x
    h = x + _A_ref(_layernorm(x, axis=-1), A_wq, A_wk, A_wv, A_wo, A_beta)
    h2 = h + _B_ref(_layernorm(h, axis=-1), B_w_r, B_w_gate, B_w_up, B_w_down)
    return h2
```

```python
import jax
import jax.numpy as jnp
from jax import lax
import jax.experimental.pallas as pl
import jax.experimental.pallas.tpu as pltpu

S = 2048
D = 576
H = 32
DH = 18
NSEG = 4
L = 512
NT = S // 128
F = 4608
HPW = 7
NW = 5
WL = HPW * DH
RS = 24
MROWS = 176
QKV_ROWS = 3 * D + 64
LOG2E = 1.4426950408889634
NEG = -1e9 * LOG2E
QSCALE = (DH ** -0.5) * LOG2E
EPS = 1e-5

f32 = jnp.float32
bf16 = jnp.bfloat16
u32 = jnp.uint32


def _nh(w):
    return HPW if w < NW - 1 else H - HPW * (NW - 1)


def _pack(x):
    return pltpu.bitcast(x.astype(bf16), u32)


def _unpack(x):
    return pltpu.bitcast(x, bf16)


def _phi(t):
    return jnp.where(t > 0, t + 1.0, jnp.exp(t))


def _layernorm_t(x):
    m = jnp.sum(x, axis=0, keepdims=True) * (1.0 / D)
    xc = x - m
    v = jnp.sum(xc * xc, axis=0, keepdims=True) * (1.0 / D)
    return xc * lax.rsqrt(v + EPS)


def _sigmoid(x):
    return 1.0 / (1.0 + jnp.exp(-x))


def _kernel(xT_hbm, wq_hbm, wk_hbm, wv_hbm, wo_hbm, beta_ref, wr_ref, wg_hbm, wu_hbm, wdT_hbm,
            out_hbm,
            x_v, wq_v, wk_v, wv_v, wo_v, wg_v, wu_v, wdT_v,
            wT, woT, g_s, wr_s,
            xn_s, k_s, phikT_s, qv_s, qT_s, phiqT_s, vT_s, mt_s, mtb_s,
            s_scr, m_scr, oT_s, out_v, hn_s, r_s,
            sem_x, sem_w, sem_o):
    def x_copy(s):
        return pltpu.make_async_copy(xT_hbm.at[:, pl.ds(s * L, L)], x_v.at[s], sem_x.at[s])

    def o_copy(t):
        return pltpu.make_async_copy(out_v.at[t], out_hbm.at[:, pl.ds(pl.multiple_of(t * 128, 128), 128)],
                                     sem_o.at[t])

    w_copies = [pltpu.make_async_copy(src, dst, sem_w.at[i]) for i, (src, dst) in enumerate(
        [(wq_hbm, wq_v), (wv_hbm, wv_v), (wk_hbm, wk_v), (wo_hbm, wo_v),
         (wg_hbm, wg_v), (wu_hbm, wu_v), (wdT_hbm, wdT_v)])]
    x_copy(0).start()
    for c in w_copies[:3]:
        c.start()
    for s in range(1, NSEG):
        x_copy(s).start()
    for c in w_copies[3:]:
        c.start()

    beta = beta_ref[...].astype(f32).reshape(1, H)
    hrow = lax.broadcasted_iota(jnp.int32, (8 * NW, H), 0)
    hcol = lax.broadcasted_iota(jnp.int32, (8 * NW, H), 1)
    sel = (hcol == HPW * (hrow >> 3) + (hrow & 7)) & ((hrow & 7) < HPW)
    bcol = jnp.sum(jnp.where(sel, beta, 0.0), axis=1, keepdims=True)
    g_s[...] = jnp.broadcast_to(_sigmoid(bcol), (8 * NW, 128)).reshape(NW, 8, 128)
    wr_row = wr_ref[...].astype(f32).reshape(1, D)
    wr_pad = jnp.concatenate([wr_row, jnp.zeros((1, 64), f32)], axis=1)
    wr_s[...] = jnp.broadcast_to(wr_pad, (128, D + 64)).T

    mt_s[...] = jnp.zeros(mt_s.shape, f32)
    mtb_s[...] = jnp.zeros(mtb_s.shape, u32)
    vT_s[...] = jnp.zeros(vT_s.shape, u32)
    qv_s[:, 3 * D:QKV_ROWS, :] = jnp.zeros((4, QKV_ROWS - 3 * D, 128), f32)

    for i in range(3):
        w_copies[i].wait()
        wT[D * i:D * (i + 1), :] = (wq_v, wv_v, wk_v)[i][...].T
    w_copies[3].wait()
    woT[...] = wo_v[...].T

    def phase_a(w, nh, j, buf):
        n = 128 * (j + 1)
        rows = lax.broadcasted_iota(jnp.int32, (64, 128), 0)
        qw = qT_s[w, j]
        qbd = jnp.concatenate(
            [jnp.where((rows >= 9 * a) & (rows < 9 * a + 9), qw, jnp.uint32(0)) for a in range(nh)], axis=1)
        s = jnp.dot(_unpack(k_s[w, 0:n // 2, :]), _unpack(qbd), preferred_element_type=f32)
        kr = lax.broadcasted_iota(jnp.int32, (128, 128), 0)
        qc = lax.broadcasted_iota(jnp.int32, (128, 128), 1)
        causal = kr <= qc
        sd = jnp.concatenate(
            [jnp.where(causal, s[n - 128:n, 128 * a:128 * (a + 1)], NEG) for a in range(nh)], axis=1)
        s_scr[buf, n - 128:n, 0:128 * nh] = sd
        m = jnp.max(sd, axis=0, keepdims=True)
        if j > 0:
            s_scr[buf, 0:n - 128, 0:128 * nh] = s[0:n - 128]
            m = jnp.maximum(m, jnp.max(s[0:n - 128], axis=0, keepdims=True))
        m_scr[buf, :, 0:128 * nh] = jnp.broadcast_to(m, (8, 128 * nh))

    def phase_b(w, nh, j, buf):
        n = 128 * (j + 1)
        am = jnp.dot(_unpack(mtb_s[w]), _unpack(phiqT_s[w, j]), preferred_element_type=f32)
        for a in range(nh):
            m = m_scr[buf, 0:1, 128 * a:128 * (a + 1)]
            p = jnp.exp2(s_scr[buf, 0:n, 128 * a:128 * (a + 1)] - m).astype(bf16)
            vt = jnp.concatenate([_unpack(vT_s[w, t, 12 * a:12 * a + 16, :]) for t in range(j + 1)], axis=1)
            o = jnp.dot(vt, p, preferred_element_type=f32)
            g = g_s[w, a:a + 1, :]
            ama = am[RS * a:RS * (a + 1)]
            od = o[0:RS] * ((1.0 - g) / o[DH:DH + 1])
            om = ama * (g / (ama[DH:DH + 1] + 1e-6))
            oT_s[j, pl.ds(WL * w + DH * a, DH), :] = (od + om)[0:DH]

    def mem_update(w, nh):
        vt = jnp.concatenate([_unpack(vT_s[w, t]) for t in range(4)], axis=1)
        pk = jnp.concatenate([_unpack(phikT_s[w, t]) for t in range(4)], axis=1)
        upd = lax.dot_general(vt, pk, (((1,), (1,)), ((), ())), preferred_element_type=f32)
        mt = mt_s[w] + upd
        mt_s[w] = mt
        r = lax.broadcasted_iota(jnp.int32, (MROWS, 128), 0)
        c = lax.broadcasted_iota(jnp.int32, (MROWS, 128), 1)
        keep = jnp.zeros((MROWS, 128), jnp.bool_)
        for a in range(nh):
            keep = keep | ((r >= RS * a) & (r < RS * (a + 1)) & (c >= DH * a) & (c < DH * (a + 1)))
        mtb_s[w] = _pack(jnp.where(keep, mt, 0.0))

    def window(w, nh):
        order = [3, 2, 1, 0]
        phase_a(w, nh, order[0], 0)
        for t in range(4):
            if t < 3:
                phase_a(w, nh, order[t + 1], (t + 1) % 2)
            phase_b(w, nh, order[t], t % 2)
        mem_update(w, nh)

    def segment(seg, carry):
        x_copy(seg).wait()
        xn_s[...] = _layernorm_t(x_v[seg].astype(f32)).astype(bf16)
        qv = jnp.dot(wT[...], xn_s[...], preferred_element_type=f32)
        for t in range(4):
            qv_s[t, 0:3 * D, :] = qv[:, 128 * t:128 * (t + 1)]
        r24 = lax.broadcasted_iota(jnp.int32, (RS, 128), 0)
        ones_row = jnp.where(r24 == DH, 1.0, 0.0).astype(f32)
        for t in range(4):
            for w in range(NW):
                q = qv_s[t, WL * w:WL * w + 128, :]
                qT_s[w, t] = _pack(q * QSCALE)
                phiqT_s[w, t] = _pack(_phi(q))
                kk = qv_s[t, 2 * D + WL * w:2 * D + WL * w + 128, :]
                k_s[w, 64 * t:64 * (t + 1), :] = pltpu.bitcast(kk.astype(bf16).T, u32)
                phikT_s[w, t] = _pack(_phi(kk))
                nh = _nh(w)
                vs = [jnp.where(r24 < DH, qv_s[t, D + DH * (HPW * w + a):D + DH * (HPW * w + a) + RS, :], ones_row)
                      for a in range(nh)]
                if nh % 2:
                    vs.append(jnp.zeros((8, 128), f32))
                vv = _pack(jnp.concatenate(vs, axis=0))
                vT_s[w, t, 0:vv.shape[0], :] = vv

        def wbody(w, c):
            window(w, HPW)
            return c
        lax.fori_loop(0, NW - 1, wbody, 0)
        window(NW - 1, _nh(NW - 1))

        oT = jnp.concatenate([oT_s[t] for t in range(4)], axis=1).astype(bf16)
        attn = jnp.dot(woT[...], oT, preferred_element_type=f32)
        h = x_v[seg].astype(f32) + attn
        hn = _layernorm_t(h)
        o = (h + hn).astype(bf16)
        wr = wr_s[0:D, :]
        for t in range(4):
            hn_t = hn[:, 128 * t:128 * (t + 1)]
            hn_s[4 * seg + t] = hn_t
            out_v[4 * seg + t] = o[:, 128 * t:128 * (t + 1)]
            r_s[pl.ds(4 * seg + t, 1), :] = jnp.sum(hn_t * wr, axis=0, keepdims=True)
            o_copy(4 * seg + t).start()
        return carry

    lax.fori_loop(0, NSEG, segment, 0)

    r = r_s[...]
    rmax = jnp.max(r)
    tok = (lax.broadcasted_iota(jnp.int32, (NT, 128), 0) * 128
           + lax.broadcasted_iota(jnp.int32, (NT, 128), 1))
    idx = jnp.minimum(jnp.min(jnp.where(r == rmax, tok, S)), S - 1)
    tile = idx >> 7
    lane = idx & 127
    lanes = lax.broadcasted_iota(jnp.int32, (D, 128), 1)
    hsel = jnp.where(lanes == lane, hn_s[tile], 0.0)
    hsel = jnp.concatenate([hsel, jnp.zeros((64, 128), f32)], axis=0)
    xrow = jnp.sum(hsel.T, axis=0, keepdims=True)[:, 0:D]
    for c in w_copies[4:]:
        c.wait()
    xs = jnp.broadcast_to(xrow, (16, D)).astype(bf16)
    gate = jnp.dot(xs, wg_v[...], preferred_element_type=f32)
    up = jnp.dot(xs, wu_v[...], preferred_element_type=f32)
    act = (gate * _sigmoid(gate) * up).astype(bf16)
    y = lax.dot_general(act, wdT_v[...], (((1,), (1,)), ((), ())), preferred_element_type=f32)
    y = y[0:1] * _sigmoid(jnp.full((1, 1), rmax, f32))
    ypad = jnp.concatenate([y, jnp.zeros((1, 64), f32)], axis=1)
    ycol = jnp.broadcast_to(ypad, (128, D + 64)).T[0:D]
    for t in range(NT):
        o_copy(t).wait()
    blk = out_v[tile].astype(f32)
    out_v[tile] = jnp.where(lanes == lane, blk + ycol, blk).astype(bf16)
    fix = o_copy(tile)
    fix.start()
    fix.wait()


@jax.jit
def pallas_sequential_preLN__memory_aug_infini_attn__moe_arch_mod__prompt_kernel(
    A_x: jax.Array,
    A_wq: jax.Array,
    A_wk: jax.Array,
    A_wv: jax.Array,
    A_wo: jax.Array,
    A_beta: jax.Array,
    B_x: jax.Array,
    B_w_r: jax.Array,
    B_w_gate: jax.Array,
    B_w_up: jax.Array,
    B_w_down: jax.Array,
):
    del B_x
    xT = A_x.reshape(S, D).T
    wdT = B_w_down.T

    hbm = pl.BlockSpec(memory_space=pltpu.HBM)
    vmem = pl.BlockSpec(memory_space=pltpu.VMEM)
    scratch = [
        pltpu.VMEM((NSEG, D, L), bf16),
        pltpu.VMEM((D, D), bf16),
        pltpu.VMEM((D, D), bf16),
        pltpu.VMEM((D, D), bf16),
        pltpu.VMEM((D, D), bf16),
        pltpu.VMEM((D, F), bf16),
        pltpu.VMEM((D, F), bf16),
        pltpu.VMEM((D, F), bf16),
        pltpu.VMEM((3 * D, D), bf16),
        pltpu.VMEM((D, D), bf16),
        pltpu.VMEM((NW, 8, 128), f32),
        pltpu.VMEM((D + 64, 128), f32),
        pltpu.VMEM((D, L), bf16),
        pltpu.VMEM((NW, L // 2, 128), u32),
        pltpu.VMEM((NW, 4, 64, 128), u32),
        pltpu.VMEM((4, QKV_ROWS, 128), f32),
        pltpu.VMEM((NW, 4, 64, 128), u32),
        pltpu.VMEM((NW, 4, 64, 128), u32),
        pltpu.VMEM((NW, 4, MROWS // 2, 128), u32),
        pltpu.VMEM((NW, MROWS, 128), f32),
        pltpu.VMEM((NW, MROWS // 2, 128), u32),
        pltpu.VMEM((2, L, 128 * HPW), f32),
        pltpu.VMEM((2, 8, 128 * HPW), f32),
        pltpu.VMEM((4, D, 128), f32),
        pltpu.VMEM((NT, D, 128), bf16),
        pltpu.VMEM((NT, D, 128), f32),
        pltpu.VMEM((NT, 128), f32),
        pltpu.SemaphoreType.DMA((NSEG,)),
        pltpu.SemaphoreType.DMA((7,)),
        pltpu.SemaphoreType.DMA((NT,)),
    ]
    outT = pl.pallas_call(
        _kernel,
        out_shape=jax.ShapeDtypeStruct((D, S), bf16),
        in_specs=[hbm, hbm, hbm, hbm, hbm, vmem, vmem, hbm, hbm, hbm],
        out_specs=hbm,
        scratch_shapes=scratch,
        compiler_params=pltpu.CompilerParams(vmem_limit_bytes=100 * 1024 * 1024),
    )(xT, A_wq, A_wk, A_wv, A_wo, A_beta, B_w_r, B_w_gate, B_w_up, B_w_down.T)
    return outT.T.reshape(1, S, D)
```

```python
import jax
import jax.numpy as jnp
from jax import lax
import jax.experimental.pallas as pl
import jax.experimental.pallas.tpu as pltpu

S = 2048
D = 576
H = 32
DH = 18
NSEG = 4
L = 512
NT = S // 128
F = 4608
HPW = 7
NW = 5
WL = HPW * DH
RS = 24
MROWS = 176
QKV_ROWS = D + 64
LOG2E = 1.4426950408889634
NEG = -1e9 * LOG2E
QSCALE = (DH ** -0.5) * LOG2E
EPS = 1e-5

import contextlib
import os
_PROF = bool(os.environ.get("PROF"))


def _scope(name):
    return jax.named_scope(name) if _PROF else contextlib.nullcontext()


f32 = jnp.float32
bf16 = jnp.bfloat16
u32 = jnp.uint32


def _nh(w):
    return HPW if w < NW - 1 else H - HPW * (NW - 1)


def _pack(x):
    return pltpu.bitcast(x.astype(bf16), u32)


def _unpack(x):
    return pltpu.bitcast(x, bf16)


def _phi(t):
    return jnp.where(t > 0, t + 1.0, jnp.exp(t))


def _ln_stats(x):
    c = x[0:1]
    d = x - c
    mu = jnp.sum(d, axis=0, keepdims=True) * (1.0 / D)
    m2 = jnp.sum(d * d, axis=0, keepdims=True) * (1.0 / D)
    var = jnp.maximum(m2 - mu * mu, 0.0)
    return c + mu, lax.rsqrt(var + EPS)


def _sigmoid(x):
    return 1.0 / (1.0 + jnp.exp(-x))


def _kernel(xT_hbm, wq_hbm, wk_hbm, wv_hbm, wo_hbm, beta_ref, wr_ref, wg_hbm, wu_hbm, wdT_hbm,
            out_hbm,
            x_v, wq_v, wk_v, wv_v, wo_v, wg_v, wu_v, wdT_v,
            wT, woT, g_s, wr_s,
            xn_s, k_s, phikT_s, qT_s, phiqT_s, vT_s, mt_s, mtb_s, am_s,
            s_scr, m_scr, oT_s, out_v, h_s, st_s, r_s,
            sem_x, sem_w, sem_o):
    def x_copy(s):
        return pltpu.make_async_copy(xT_hbm.at[:, pl.ds(s * L, L)], x_v.at[s], sem_x.at[s])

    def o_copy(t):
        return pltpu.make_async_copy(out_v.at[t], out_hbm.at[:, pl.ds(pl.multiple_of(t * 128, 128), 128)],
                                     sem_o.at[t])

    w_copies = [pltpu.make_async_copy(src, dst, sem_w.at[i]) for i, (src, dst) in enumerate(
        [(wk_hbm, wk_v), (wv_hbm, wv_v), (wq_hbm, wq_v), (wo_hbm, wo_v),
         (wg_hbm, wg_v), (wu_hbm, wu_v), (wdT_hbm, wdT_v)])]

    def ln1_tile(seg, t):
        cols = pl.ds(pl.multiple_of(t * 128, 128), 128)
        mean, rstd = _ln_stats(x_v[seg, :, cols].astype(f32))
        xn_s[t] = ((x_v[seg, :, cols].astype(f32) - mean) * rstd).astype(bf16)

    def proj(i):
        xn = jnp.concatenate([xn_s[t] for t in range(4)], axis=1)
        r = jnp.dot(wT[D * i:D * (i + 1), :], xn, preferred_element_type=f32)
        return jnp.concatenate([r, jnp.zeros((64, L), f32)], axis=0)

    def post_k(r):
        for t in range(4):
            for w in range(NW):
                kk = r[WL * w:WL * w + 128, 128 * t:128 * (t + 1)]
                k_s[w, 64 * t:64 * (t + 1), :] = pltpu.bitcast(kk.astype(bf16).T, u32)
                phikT_s[w, t] = _pack(_phi(kk))

    def post_v(r):
        r24 = lax.broadcasted_iota(jnp.int32, (RS, 128), 0)
        ones_row = jnp.where(r24 == DH, 1.0, 0.0).astype(f32)
        for t in range(4):
            for w in range(NW):
                nh = _nh(w)
                vs = [jnp.where(r24 < DH,
                                r[DH * (HPW * w + a):DH * (HPW * w + a) + RS, 128 * t:128 * (t + 1)], ones_row)
                      for a in range(nh)]
                if nh % 2:
                    vs.append(jnp.zeros((8, 128), f32))
                vv = _pack(jnp.concatenate(vs, axis=0))
                vT_s[w, t, 0:vv.shape[0], :] = vv

    def post_q(r):
        for t in range(4):
            for w in range(NW):
                q = r[WL * w:WL * w + 128, 128 * t:128 * (t + 1)]
                qT_s[w, t] = _pack(q * QSCALE)
                phiqT_s[w, t] = _pack(_phi(q))

    def mem_update():
        r = lax.broadcasted_iota(jnp.int32, (MROWS, 128), 0)
        c = lax.broadcasted_iota(jnp.int32, (MROWS, 128), 1)
        for w in range(NW):
            vt = jnp.concatenate([_unpack(vT_s[w, t]) for t in range(4)], axis=1)
            pk = jnp.concatenate([_unpack(phikT_s[w, t]) for t in range(4)], axis=1)
            upd = lax.dot_general(vt, pk, (((1,), (1,)), ((), ())), preferred_element_type=f32)
            mt = mt_s[w] + upd
            mt_s[w] = mt
            keep = jnp.zeros((MROWS, 128), jnp.bool_)
            for a in range(_nh(w)):
                keep = keep | ((r >= RS * a) & (r < RS * (a + 1)) & (c >= DH * a) & (c < DH * (a + 1)))
            mtb_s[w] = _pack(jnp.where(keep, mt, 0.0))

    def mem_retrieve():
        for w in range(NW):
            for j in range(4):
                am = jnp.dot(_unpack(mtb_s[w]), _unpack(phiqT_s[w, j]), preferred_element_type=f32)
                for a in range(_nh(w)):
                    ama = am[RS * a:RS * (a + 1)]
                    g = g_s[w, a:a + 1, :]
                    om = ama * (g / (ama[DH:DH + 1] + 1e-6))
                    am_s[j, WL * w + DH * a:WL * w + DH * (a + 1), :] = om[0:DH]

    def phase_a(w, nh, j, buf):
        n = 128 * (j + 1)
        rows = lax.broadcasted_iota(jnp.int32, (64, 128), 0)
        qw = qT_s[w, j]
        qbd = jnp.concatenate(
            [jnp.where((rows >= 9 * a) & (rows < 9 * a + 9), qw, jnp.uint32(0)) for a in range(nh)], axis=1)
        s = jnp.dot(_unpack(k_s[w, 0:n // 2, :]), _unpack(qbd), preferred_element_type=f32)
        kr = lax.broadcasted_iota(jnp.int32, (128, 128), 0)
        qc = lax.broadcasted_iota(jnp.int32, (128, 128), 1)
        causal = kr <= qc
        sd = jnp.concatenate(
            [jnp.where(causal, s[n - 128:n, 128 * a:128 * (a + 1)], NEG) for a in range(nh)], axis=1)
        s_scr[buf, n - 128:n, 0:128 * nh] = sd
        m = jnp.max(sd, axis=0, keepdims=True)
        if j > 0:
            s_scr[buf, 0:n - 128, 0:128 * nh] = s[0:n - 128]
            m = jnp.maximum(m, jnp.max(s[0:n - 128], axis=0, keepdims=True))
        m_scr[buf, :, 0:128 * nh] = jnp.broadcast_to(m, (8, 128 * nh))

    def phase_b(w, nh, j, buf):
        n = 128 * (j + 1)
        for a in range(nh):
            m = m_scr[buf, 0:1, 128 * a:128 * (a + 1)]
            p = jnp.exp2(s_scr[buf, 0:n, 128 * a:128 * (a + 1)] - m).astype(bf16)
            vt = jnp.concatenate([_unpack(vT_s[w, t, 12 * a:12 * a + 16, :]) for t in range(j + 1)], axis=1)
            o = jnp.dot(vt, p, preferred_element_type=f32)
            g = g_s[w, a:a + 1, :]
            od = o[0:RS] * ((1.0 - g) / o[DH:DH + 1])
            row0 = WL * w + DH * a
            oT_s[j, pl.ds(row0, DH), :] = (od + am_s[j, pl.ds(row0, RS), :])[0:DH]

    def window(w, nh, nxt):
        order = [3, 2, 1, 0]
        for t in range(4):
            if t < 3:
                phase_a(w, nh, order[t + 1], (t + 1) % 2)
            elif nxt is not None:
                phase_a(nxt, HPW, order[0], 0)
            phase_b(w, nh, order[t], t % 2)

    def outproj(seg):
        oT = jnp.concatenate([oT_s[t] for t in range(4)], axis=1).astype(bf16)
        attn = jnp.dot(woT[...], oT, preferred_element_type=f32)
        wr = wr_s[0:D, :]
        for t in range(4):
            cols = slice(128 * t, 128 * (t + 1))
            tile = 4 * seg + t
            h = x_v[seg, :, cols].astype(f32) + attn[:, cols]
            h_s[tile] = h
            mean, rstd = _ln_stats(h)
            st_s[tile, 0:1, :] = mean
            st_s[tile, 1:2, :] = rstd
            h = h_s[tile]
            hn = (h - mean) * rstd
            out_v[tile] = (h + hn).astype(bf16)
            r_s[pl.ds(tile, 1), :] = jnp.sum(hn * wr, axis=0, keepdims=True)

    def project_segment():
        post_k(proj(0))
        post_v(proj(1))
        post_q(proj(2))

    with _scope("setup"):
        w_copies[0].start()
        x_copy(0).start()
        w_copies[1].start()
        w_copies[2].start()
        beta = beta_ref[...].astype(f32).reshape(1, H)
        hrow = lax.broadcasted_iota(jnp.int32, (8 * NW, H), 0)
        hcol = lax.broadcasted_iota(jnp.int32, (8 * NW, H), 1)
        sel = (hcol == HPW * (hrow >> 3) + (hrow & 7)) & ((hrow & 7) < HPW)
        bcol = jnp.sum(jnp.where(sel, beta, 0.0), axis=1, keepdims=True)
        g_s[...] = jnp.broadcast_to(_sigmoid(bcol), (8 * NW, 128)).reshape(NW, 8, 128)
        wr_row = wr_ref[...].astype(f32).reshape(1, D)
        wr_pad = jnp.concatenate([wr_row, jnp.zeros((1, 64), f32)], axis=1)
        wr_s[...] = jnp.broadcast_to(wr_pad, (128, D + 64)).T

        mt_s[...] = jnp.zeros(mt_s.shape, f32)
        vT_s[...] = jnp.zeros(vT_s.shape, u32)
        am_s[...] = jnp.zeros(am_s.shape, f32)

        w_copies[0].wait()
        x_copy(0).wait()
        wT[0:D, :] = wk_v[...].T
        for t in range(4):
            ln1_tile(0, t)
    with _scope("proj0"):
        w_copies[1].wait()
        for s in range(1, NSEG):
            x_copy(s).start()
        w_copies[3].start()
        post_k(proj(0))
        wT[D:2 * D, :] = wv_v[...].T
        w_copies[2].wait()
        for c in w_copies[4:]:
            c.start()
        post_v(proj(1))
        wT[2 * D:3 * D, :] = wq_v[...].T
        w_copies[3].wait()
        post_q(proj(2))
        woT[...] = wo_v[...].T
        phase_a(0, HPW, 3, 0)
        for s in range(1, NSEG):
            x_copy(s).wait()

    def segment(seg, carry):
        nseg = jnp.minimum(seg + 1, NSEG - 1)

        def wbody(w, c):
            ln1_tile(nseg, w)
            window(w, HPW, w + 1)
            return c
        with _scope("win7"):
            lax.fori_loop(0, NW - 1, wbody, 0)
        with _scope("win4"):
            window(NW - 1, _nh(NW - 1), None)

        @pl.when(seg < NSEG - 1)
        def _():
            with _scope("mid"):
                mem_update()
                outproj(seg)
                project_segment()
                mem_retrieve()
                phase_a(0, HPW, 3, 0)
                for t in range(4):
                    o_copy(4 * seg + t).start()
        return carry

    lax.fori_loop(0, NSEG, segment, 0)
    with _scope("last_out"):
        outproj(NSEG - 1)
        for t in range(4):
            o_copy(4 * (NSEG - 1) + t).start()

    with _scope("ffn"):
        r = r_s[...]
        rmax = jnp.max(r)
        tok = (lax.broadcasted_iota(jnp.int32, (NT, 128), 0) * 128
               + lax.broadcasted_iota(jnp.int32, (NT, 128), 1))
        idx = jnp.minimum(jnp.min(jnp.where(r == rmax, tok, S)), S - 1)
        tile = idx >> 7
        lane = idx & 127
        lanes = lax.broadcasted_iota(jnp.int32, (D, 128), 1)
        hn = (h_s[tile] - st_s[tile, 0:1, :]) * st_s[tile, 1:2, :]
        hsel = jnp.where(lanes == lane, hn, 0.0)
        hsel = jnp.concatenate([hsel, jnp.zeros((64, 128), f32)], axis=0)
        xrow = jnp.sum(hsel.T, axis=0, keepdims=True)[:, 0:D]
        for c in w_copies[4:]:
            c.wait()
        xs = jnp.broadcast_to(xrow, (16, D)).astype(bf16)
        gate = jnp.dot(xs, wg_v[...], preferred_element_type=f32)
        up = jnp.dot(xs, wu_v[...], preferred_element_type=f32)
        act = (gate * _sigmoid(gate) * up).astype(bf16)
        y = lax.dot_general(act, wdT_v[...], (((1,), (1,)), ((), ())), preferred_element_type=f32)
        y = y[0:1] * _sigmoid(jnp.full((1, 1), rmax, f32))
        ypad = jnp.concatenate([y, jnp.zeros((1, 64), f32)], axis=1)
        ycol = jnp.broadcast_to(ypad, (128, D + 64)).T[0:D]
        for t in range(NT):
            o_copy(t).wait()
        blk = out_v[tile].astype(f32)
        out_v[tile] = jnp.where(lanes == lane, blk + ycol, blk).astype(bf16)
        fix = o_copy(tile)
        fix.start()
        fix.wait()


@jax.jit
def pallas_sequential_preLN__memory_aug_infini_attn__moe_arch_mod__prompt_kernel(
    A_x: jax.Array,
    A_wq: jax.Array,
    A_wk: jax.Array,
    A_wv: jax.Array,
    A_wo: jax.Array,
    A_beta: jax.Array,
    B_x: jax.Array,
    B_w_r: jax.Array,
    B_w_gate: jax.Array,
    B_w_up: jax.Array,
    B_w_down: jax.Array,
):
    del B_x
    xT = A_x.reshape(S, D).T
    wdT = B_w_down.T

    hbm = pl.BlockSpec(memory_space=pltpu.HBM)
    vmem = pl.BlockSpec(memory_space=pltpu.VMEM)
    scratch = [
        pltpu.VMEM((NSEG, D, L), bf16),
        pltpu.VMEM((D, D), bf16),
        pltpu.VMEM((D, D), bf16),
        pltpu.VMEM((D, D), bf16),
        pltpu.VMEM((D, D), bf16),
        pltpu.VMEM((D, F), bf16),
        pltpu.VMEM((D, F), bf16),
        pltpu.VMEM((D, F), bf16),
        pltpu.VMEM((3 * D, D), bf16),
        pltpu.VMEM((D, D), bf16),
        pltpu.VMEM((NW, 8, 128), f32),
        pltpu.VMEM((D + 64, 128), f32),
        pltpu.VMEM((4, D, 128), bf16),
        pltpu.VMEM((NW, L // 2, 128), u32),
        pltpu.VMEM((NW, 4, 64, 128), u32),
        pltpu.VMEM((NW, 4, 64, 128), u32),
        pltpu.VMEM((NW, 4, 64, 128), u32),
        pltpu.VMEM((NW, 4, MROWS // 2, 128), u32),
        pltpu.VMEM((NW, MROWS, 128), f32),
        pltpu.VMEM((NW, MROWS // 2, 128), u32),
        pltpu.VMEM((4, D + 8, 128), f32),
        pltpu.VMEM((2, L, 128 * HPW), f32),
        pltpu.VMEM((2, 8, 128 * HPW), f32),
        pltpu.VMEM((4, D, 128), f32),
        pltpu.VMEM((NT, D, 128), bf16),
        pltpu.VMEM((NT, D, 128), f32),
        pltpu.VMEM((NT, 8, 128), f32),
        pltpu.VMEM((NT, 128), f32),
        pltpu.SemaphoreType.DMA((NSEG,)),
        pltpu.SemaphoreType.DMA((7,)),
        pltpu.SemaphoreType.DMA((NT,)),
    ]
    outT = pl.pallas_call(
        _kernel,
        out_shape=jax.ShapeDtypeStruct((D, S), bf16),
        in_specs=[hbm, hbm, hbm, hbm, hbm, vmem, vmem, hbm, hbm, hbm],
        out_specs=hbm,
        scratch_shapes=scratch,
        compiler_params=pltpu.CompilerParams(vmem_limit_bytes=100 * 1024 * 1024),
    )(xT, A_wq, A_wk, A_wv, A_wo, A_beta, B_w_r, B_w_gate, B_w_up, B_w_down.T)
    return outT.T.reshape(1, S, D)
```

```python
import jax
import jax.numpy as jnp
from jax import lax
import jax.experimental.pallas as pl
import jax.experimental.pallas.tpu as pltpu

S = 2048
D = 576
H = 32
DH = 18
NSEG = 4
L = 512
NT = S // 128
F = 4608
HPW = 7
NW = 5
WL = HPW * DH
RS = 24
MROWS = 176
QKV_ROWS = D + 64
LOG2E = 1.4426950408889634
NEG = -1e9 * LOG2E
QSCALE = (DH ** -0.5) * LOG2E
EPS = 1e-5

import contextlib
import os
_PROF = bool(os.environ.get("PROF"))


def _scope(name):
    return jax.named_scope(name) if _PROF else contextlib.nullcontext()


f32 = jnp.float32
bf16 = jnp.bfloat16
u32 = jnp.uint32


def _nh(w):
    return HPW if w < NW - 1 else H - HPW * (NW - 1)


def _pack(x):
    return pltpu.bitcast(x.astype(bf16), u32)


def _unpack(x):
    return pltpu.bitcast(x, bf16)


def _phi(t):
    return jnp.where(t > 0, t + 1.0, jnp.exp(t))


def _ln_stats(x):
    c = x[0:1]
    d = x - c
    mu = jnp.sum(d, axis=0, keepdims=True) * (1.0 / D)
    m2 = jnp.sum(d * d, axis=0, keepdims=True) * (1.0 / D)
    var = jnp.maximum(m2 - mu * mu, 0.0)
    return c + mu, lax.rsqrt(var + EPS)


def _sigmoid(x):
    return 1.0 / (1.0 + jnp.exp(-x))


def _kernel(xT_hbm, wq_hbm, wk_hbm, wv_hbm, wo_hbm, beta_ref, wr_ref, wg_hbm, wu_hbm, wdT_hbm,
            out_hbm,
            x_v, wq_v, wk_v, wv_v, wo_v, wg_v, wu_v, wdT_v,
            wT, woT, g_s, wr_s,
            xn_s, k_s, phikT_s, qT_s, phiqT_s, vT_s, mt_s, mtb_s, am_s,
            s_scr, m_scr, oT_s, out_v, h_s, st_s, r_s,
            sem_x, sem_w, sem_o):
    def x_copy(s):
        return pltpu.make_async_copy(xT_hbm.at[:, pl.ds(s * L, L)], x_v.at[s], sem_x.at[s])

    def o_copy(t):
        return pltpu.make_async_copy(out_v.at[t], out_hbm.at[:, pl.ds(pl.multiple_of(t * 128, 128), 128)],
                                     sem_o.at[t])

    w_copies = [pltpu.make_async_copy(src, dst, sem_w.at[i]) for i, (src, dst) in enumerate(
        [(wk_hbm, wk_v), (wv_hbm, wv_v), (wq_hbm, wq_v), (wo_hbm, wo_v),
         (wg_hbm, wg_v), (wu_hbm, wu_v), (wdT_hbm, wdT_v)])]

    def ln1_tile(seg, t):
        cols = pl.ds(pl.multiple_of(t * 128, 128), 128)
        mean, rstd = _ln_stats(x_v[seg, :, cols].astype(f32))
        xn_s[t] = ((x_v[seg, :, cols].astype(f32) - mean) * rstd).astype(bf16)

    def proj(i):
        xn = jnp.concatenate([xn_s[t] for t in range(4)], axis=1)
        r = jnp.dot(wT[D * i:D * (i + 1), :], xn, preferred_element_type=f32)
        return jnp.concatenate([r, jnp.zeros((64, L), f32)], axis=0)

    def post_k(r):
        for t in range(4):
            for w in range(NW):
                kk = r[WL * w:WL * w + 128, 128 * t:128 * (t + 1)]
                k_s[w, 64 * t:64 * (t + 1), :] = pltpu.bitcast(kk.astype(bf16).T, u32)
                phikT_s[w, t] = _pack(_phi(kk))

    def post_v(r):
        r24 = lax.broadcasted_iota(jnp.int32, (RS, 128), 0)
        ones_row = jnp.where(r24 == DH, 1.0, 0.0).astype(f32)
        for t in range(4):
            for w in range(NW):
                nh = _nh(w)
                vs = [jnp.where(r24 < DH,
                                r[DH * (HPW * w + a):DH * (HPW * w + a) + RS, 128 * t:128 * (t + 1)], ones_row)
                      for a in range(nh)]
                if nh % 2:
                    vs.append(jnp.zeros((8, 128), f32))
                vv = _pack(jnp.concatenate(vs, axis=0))
                vT_s[w, t, 0:vv.shape[0], :] = vv

    def post_q(r):
        for t in range(4):
            for w in range(NW):
                q = r[WL * w:WL * w + 128, 128 * t:128 * (t + 1)]
                qT_s[w, t] = _pack(q * QSCALE)
                phiqT_s[w, t] = _pack(_phi(q))

    def mem_update():
        r = lax.broadcasted_iota(jnp.int32, (MROWS, 128), 0)
        c = lax.broadcasted_iota(jnp.int32, (MROWS, 128), 1)
        for w in range(NW):
            vt = jnp.concatenate([_unpack(vT_s[w, t]) for t in range(4)], axis=1)
            pk = jnp.concatenate([_unpack(phikT_s[w, t]) for t in range(4)], axis=1)
            upd = lax.dot_general(vt, pk, (((1,), (1,)), ((), ())), preferred_element_type=f32)
            mt = mt_s[w] + upd
            mt_s[w] = mt
            keep = jnp.zeros((MROWS, 128), jnp.bool_)
            for a in range(_nh(w)):
                keep = keep | ((r >= RS * a) & (r < RS * (a + 1)) & (c >= DH * a) & (c < DH * (a + 1)))
            mtb_s[w] = _pack(jnp.where(keep, mt, 0.0))

    def mem_retrieve():
        for w in range(NW):
            for j in range(4):
                am = jnp.dot(_unpack(mtb_s[w]), _unpack(phiqT_s[w, j]), preferred_element_type=f32)
                for a in range(_nh(w)):
                    ama = am[RS * a:RS * (a + 1)]
                    g = g_s[w, a:a + 1, :]
                    om = ama * (g / (ama[DH:DH + 1] + 1e-6))
                    am_s[j, WL * w + DH * a:WL * w + DH * (a + 1), :] = om[0:DH]

    def phase_a(w, nh, j, buf):
        n = 128 * (j + 1)
        rows = lax.broadcasted_iota(jnp.int32, (64, 128), 0)
        qw = qT_s[w, j]
        qbd = jnp.concatenate(
            [jnp.where((rows >= 9 * a) & (rows < 9 * a + 9), qw, jnp.uint32(0)) for a in range(nh)], axis=1)
        s = jnp.dot(_unpack(k_s[w, 0:n // 2, :]), _unpack(qbd), preferred_element_type=f32)
        kr = lax.broadcasted_iota(jnp.int32, (128, 128), 0)
        qc = lax.broadcasted_iota(jnp.int32, (128, 128), 1)
        causal = kr <= qc
        sd = jnp.concatenate(
            [jnp.where(causal, s[n - 128:n, 128 * a:128 * (a + 1)], NEG) for a in range(nh)], axis=1)
        s_scr[buf, n - 128:n, 0:128 * nh] = sd
        m = jnp.max(sd, axis=0, keepdims=True)
        if j > 0:
            s_scr[buf, 0:n - 128, 0:128 * nh] = s[0:n - 128]
            m = jnp.maximum(m, jnp.max(s[0:n - 128], axis=0, keepdims=True))
        m_scr[buf, :, 0:128 * nh] = jnp.broadcast_to(m, (8, 128 * nh))

    def phase_b(w, nh, j, buf):
        n = 128 * (j + 1)
        for a in range(nh):
            m = m_scr[buf, 0:1, 128 * a:128 * (a + 1)]
            p = jnp.exp2(s_scr[buf, 0:n, 128 * a:128 * (a + 1)] - m).astype(bf16)
            vt = jnp.concatenate([_unpack(vT_s[w, t, 12 * a:12 * a + 16, :]) for t in range(j + 1)], axis=1)
            o = jnp.dot(vt, p, preferred_element_type=f32)
            g = g_s[w, a:a + 1, :]
            od = o[0:RS] * ((1.0 - g) / o[DH:DH + 1])
            row0 = WL * w + DH * a
            oT_s[j, pl.ds(row0, DH), :] = (od + am_s[j, pl.ds(row0, RS), :])[0:DH]

    def window(w, nh, nxt):
        order = [3, 2, 1, 0]
        for t in range(4):
            if t < 3:
                phase_a(w, nh, order[t + 1], (t + 1) % 2)
            elif nxt is not None:
                phase_a(nxt, _nh(nxt), order[0], 0)
            phase_b(w, nh, order[t], t % 2)

    def outproj(seg):
        oT = jnp.concatenate([oT_s[t] for t in range(4)], axis=1).astype(bf16)
        attn = jnp.dot(woT[...], oT, preferred_element_type=f32)
        wr = wr_s[0:D, :]
        for t in range(4):
            cols = slice(128 * t, 128 * (t + 1))
            tile = 4 * seg + t
            h = x_v[seg, :, cols].astype(f32) + attn[:, cols]
            h_s[tile] = h
            mean, rstd = _ln_stats(h)
            st_s[tile, 0:1, :] = mean
            st_s[tile, 1:2, :] = rstd
            h = h_s[tile]
            hn = (h - mean) * rstd
            out_v[tile] = (h + hn).astype(bf16)
            r_s[pl.ds(tile, 1), :] = jnp.sum(hn * wr, axis=0, keepdims=True)

    def project_segment():
        post_k(proj(0))
        post_v(proj(1))
        post_q(proj(2))

    with _scope("setup"):
        w_copies[0].start()
        x_copy(0).start()
        beta = beta_ref[...].astype(f32).reshape(1, H)
        hrow = lax.broadcasted_iota(jnp.int32, (8 * NW, H), 0)
        hcol = lax.broadcasted_iota(jnp.int32, (8 * NW, H), 1)
        sel = (hcol == HPW * (hrow >> 3) + (hrow & 7)) & ((hrow & 7) < HPW)
        bcol = jnp.sum(jnp.where(sel, beta, 0.0), axis=1, keepdims=True)
        g_s[...] = jnp.broadcast_to(_sigmoid(bcol), (8 * NW, 128)).reshape(NW, 8, 128)
        wr_row = wr_ref[...].astype(f32).reshape(1, D)
        wr_pad = jnp.concatenate([wr_row, jnp.zeros((1, 64), f32)], axis=1)
        wr_s[...] = jnp.broadcast_to(wr_pad, (128, D + 64)).T

        mt_s[...] = jnp.zeros(mt_s.shape, f32)
        vT_s[...] = jnp.zeros(vT_s.shape, u32)
        am_s[...] = jnp.zeros(am_s.shape, f32)

        w_copies[0].wait()
        w_copies[1].start()
        wT[0:D, :] = wk_v[...].T
        x_copy(0).wait()
        w_copies[2].start()
        for t in range(4):
            ln1_tile(0, t)
    with _scope("proj0"):
        w_copies[1].wait()
        w_copies[3].start()
        post_k(proj(0))
        wT[D:2 * D, :] = wv_v[...].T
        w_copies[2].wait()
        for s in range(1, NSEG):
            x_copy(s).start()
        post_v(proj(1))
        wT[2 * D:3 * D, :] = wq_v[...].T
        w_copies[3].wait()
        for c in w_copies[4:]:
            c.start()
        post_q(proj(2))
        woT[...] = wo_v[...].T
        phase_a(0, HPW, 3, 0)
        for s in range(1, NSEG):
            x_copy(s).wait()

    def segment(seg, carry):
        nseg = jnp.minimum(seg + 1, NSEG - 1)

        with _scope("windows"):
            for w in range(NW):
                if w < 4:
                    ln1_tile(nseg, w)
                window(w, _nh(w), w + 1 if w + 1 < NW else None)

        @pl.when(seg < NSEG - 1)
        def _():
            with _scope("mid"):
                mem_update()
                outproj(seg)
                project_segment()
                mem_retrieve()
                phase_a(0, HPW, 3, 0)
                for t in range(4):
                    o_copy(4 * seg + t).start()
        return carry

    lax.fori_loop(0, NSEG, segment, 0)
    with _scope("last_out"):
        outproj(NSEG - 1)
        for t in range(4):
            o_copy(4 * (NSEG - 1) + t).start()

    with _scope("ffn"):
        r = r_s[...]
        rmax = jnp.max(r)
        tok = (lax.broadcasted_iota(jnp.int32, (NT, 128), 0) * 128
               + lax.broadcasted_iota(jnp.int32, (NT, 128), 1))
        idx = jnp.minimum(jnp.min(jnp.where(r == rmax, tok, S)), S - 1)
        tile = idx >> 7
        lane = idx & 127
        lanes = lax.broadcasted_iota(jnp.int32, (D, 128), 1)
        hn = (h_s[tile] - st_s[tile, 0:1, :]) * st_s[tile, 1:2, :]
        hsel = jnp.where(lanes == lane, hn, 0.0)
        hsel = jnp.concatenate([hsel, jnp.zeros((64, 128), f32)], axis=0)
        xrow = jnp.sum(hsel.T, axis=0, keepdims=True)[:, 0:D]
        for c in w_copies[4:]:
            c.wait()
        xs = jnp.broadcast_to(xrow, (16, D)).astype(bf16)
        gate = jnp.dot(xs, wg_v[...], preferred_element_type=f32)
        up = jnp.dot(xs, wu_v[...], preferred_element_type=f32)
        act = (gate * _sigmoid(gate) * up).astype(bf16)
        y = lax.dot_general(act, wdT_v[...], (((1,), (1,)), ((), ())), preferred_element_type=f32)
        y = y[0:1] * _sigmoid(jnp.full((1, 1), rmax, f32))
        ypad = jnp.concatenate([y, jnp.zeros((1, 64), f32)], axis=1)
        ycol = jnp.broadcast_to(ypad, (128, D + 64)).T[0:D]
        for t in range(NT):
            o_copy(t).wait()
        blk = out_v[tile].astype(f32)
        out_v[tile] = jnp.where(lanes == lane, blk + ycol, blk).astype(bf16)
        fix = o_copy(tile)
        fix.start()
        fix.wait()


@jax.jit
def pallas_sequential_preLN__memory_aug_infini_attn__moe_arch_mod__prompt_kernel(
    A_x: jax.Array,
    A_wq: jax.Array,
    A_wk: jax.Array,
    A_wv: jax.Array,
    A_wo: jax.Array,
    A_beta: jax.Array,
    B_x: jax.Array,
    B_w_r: jax.Array,
    B_w_gate: jax.Array,
    B_w_up: jax.Array,
    B_w_down: jax.Array,
):
    del B_x
    xT = A_x.reshape(S, D).T
    wdT = B_w_down.T

    hbm = pl.BlockSpec(memory_space=pltpu.HBM)
    vmem = pl.BlockSpec(memory_space=pltpu.VMEM)
    scratch = [
        pltpu.VMEM((NSEG, D, L), bf16),
        pltpu.VMEM((D, D), bf16),
        pltpu.VMEM((D, D), bf16),
        pltpu.VMEM((D, D), bf16),
        pltpu.VMEM((D, D), bf16),
        pltpu.VMEM((D, F), bf16),
        pltpu.VMEM((D, F), bf16),
        pltpu.VMEM((D, F), bf16),
        pltpu.VMEM((3 * D, D), bf16),
        pltpu.VMEM((D, D), bf16),
        pltpu.VMEM((NW, 8, 128), f32),
        pltpu.VMEM((D + 64, 128), f32),
        pltpu.VMEM((4, D, 128), bf16),
        pltpu.VMEM((NW, L // 2, 128), u32),
        pltpu.VMEM((NW, 4, 64, 128), u32),
        pltpu.VMEM((NW, 4, 64, 128), u32),
        pltpu.VMEM((NW, 4, 64, 128), u32),
        pltpu.VMEM((NW, 4, MROWS // 2, 128), u32),
        pltpu.VMEM((NW, MROWS, 128), f32),
        pltpu.VMEM((NW, MROWS // 2, 128), u32),
        pltpu.VMEM((4, D + 8, 128), f32),
        pltpu.VMEM((2, L, 128 * HPW), f32),
        pltpu.VMEM((2, 8, 128 * HPW), f32),
        pltpu.VMEM((4, D, 128), f32),
        pltpu.VMEM((NT, D, 128), bf16),
        pltpu.VMEM((NT, D, 128), f32),
        pltpu.VMEM((NT, 8, 128), f32),
        pltpu.VMEM((NT, 128), f32),
        pltpu.SemaphoreType.DMA((NSEG,)),
        pltpu.SemaphoreType.DMA((7,)),
        pltpu.SemaphoreType.DMA((NT,)),
    ]
    outT = pl.pallas_call(
        _kernel,
        out_shape=jax.ShapeDtypeStruct((D, S), bf16),
        in_specs=[hbm, hbm, hbm, hbm, hbm, vmem, vmem, hbm, hbm, hbm],
        out_specs=hbm,
        scratch_shapes=scratch,
        compiler_params=pltpu.CompilerParams(vmem_limit_bytes=100 * 1024 * 1024),
    )(xT, A_wq, A_wk, A_wv, A_wo, A_beta, B_w_r, B_w_gate, B_w_up, B_w_down.T)
    return outT.T.reshape(1, S, D)
```

```python
import jax
import jax.numpy as jnp
from jax import lax
import jax.experimental.pallas as pl
import jax.experimental.pallas.tpu as pltpu

S = 2048
D = 576
H = 32
DH = 18
NSEG = 4
L = 512
NT = S // 128
F = 4608
HPW = 7
NW = 5
WL = HPW * DH
RS = 24
MROWS = 176
QKV_ROWS = D + 64
LOG2E = 1.4426950408889634
NEG = -1e9 * LOG2E
QSCALE = (DH ** -0.5) * LOG2E
EPS = 1e-5

import contextlib
import os
_PROF = bool(os.environ.get("PROF"))


def _scope(name):
    return jax.named_scope(name) if _PROF else contextlib.nullcontext()


f32 = jnp.float32
bf16 = jnp.bfloat16
u32 = jnp.uint32


def _nh(w):
    return HPW if w < NW - 1 else H - HPW * (NW - 1)


def _pack(x):
    return pltpu.bitcast(x.astype(bf16), u32)


def _unpack(x):
    return pltpu.bitcast(x, bf16)


def _phi(t):
    return jnp.where(t > 0, t + 1.0, jnp.exp(t))


def _colsum(x, nacc=4):
    n = x.shape[0] // 8
    accs = [x[8 * i:8 * (i + 1)] for i in range(nacc)]
    for i in range(nacc, n):
        accs[i % nacc] = accs[i % nacc] + x[8 * i:8 * (i + 1)]
    while len(accs) > 1:
        accs = [accs[i] + accs[i + 1] for i in range(0, len(accs), 2)]
    return jnp.sum(accs[0], axis=0, keepdims=True)


def _ln_stats(x):
    c = x[0:1]
    d = x - c
    mu = _colsum(d) * (1.0 / D)
    m2 = _colsum(d * d) * (1.0 / D)
    var = jnp.maximum(m2 - mu * mu, 0.0)
    return c + mu, lax.rsqrt(var + EPS)


def _sigmoid(x):
    return 1.0 / (1.0 + jnp.exp(-x))


def _kernel(xT_hbm, wq_hbm, wk_hbm, wv_hbm, wo_hbm, beta_ref, wr_ref, wg_hbm, wu_hbm, wdT_hbm,
            out_hbm,
            x_v, wq_v, wk_v, wv_v, wo_v, wg_v, wu_v, wdT_v,
            wT, woT, g_s, wr_s,
            xn_s, k_s, phikT_s, qT_s, phiqT_s, vT_s, mt_s, mtb_s, am_s,
            s_scr, m_scr, oT_s, out_v, h_s, st_s, r_s,
            sem_x, sem_w, sem_o):
    def x_copy(s):
        return pltpu.make_async_copy(xT_hbm.at[:, pl.ds(s * L, L)], x_v.at[s], sem_x.at[s])

    def o_copy(t):
        return pltpu.make_async_copy(out_v.at[t], out_hbm.at[:, pl.ds(pl.multiple_of(t * 128, 128), 128)],
                                     sem_o.at[t])

    w_copies = [pltpu.make_async_copy(src, dst, sem_w.at[i]) for i, (src, dst) in enumerate(
        [(wk_hbm, wk_v), (wv_hbm, wv_v), (wq_hbm, wq_v), (wo_hbm, wo_v),
         (wg_hbm, wg_v), (wu_hbm, wu_v), (wdT_hbm, wdT_v)])]

    def ln1_tile(seg, t):
        cols = pl.ds(pl.multiple_of(t * 128, 128), 128)
        mean, rstd = _ln_stats(x_v[seg, :, cols].astype(f32))
        pltpu.touch(x_v)
        xn_s[t] = ((x_v[seg, :, cols].astype(f32) - mean) * rstd).astype(bf16)

    def proj(i):
        xn = jnp.concatenate([xn_s[t] for t in range(4)], axis=1)
        r = jnp.dot(wT[D * i:D * (i + 1), :], xn, preferred_element_type=f32)
        return jnp.concatenate([r, jnp.zeros((64, L), f32)], axis=0)

    def post_k(r):
        for t in range(4):
            for w in range(NW):
                kk = r[WL * w:WL * w + 128, 128 * t:128 * (t + 1)]
                k_s[w, 64 * t:64 * (t + 1), :] = pltpu.bitcast(kk.astype(bf16).T, u32)
                phikT_s[w, t] = _pack(_phi(kk))

    def post_v(r):
        r24 = lax.broadcasted_iota(jnp.int32, (RS, 128), 0)
        ones_row = jnp.where(r24 == DH, 1.0, 0.0).astype(f32)
        for t in range(4):
            for w in range(NW):
                nh = _nh(w)
                vs = [jnp.where(r24 < DH,
                                r[DH * (HPW * w + a):DH * (HPW * w + a) + RS, 128 * t:128 * (t + 1)], ones_row)
                      for a in range(nh)]
                if nh % 2:
                    vs.append(jnp.zeros((8, 128), f32))
                vv = _pack(jnp.concatenate(vs, axis=0))
                vT_s[w, t, 0:vv.shape[0], :] = vv

    def post_q(r):
        for t in range(4):
            for w in range(NW):
                q = r[WL * w:WL * w + 128, 128 * t:128 * (t + 1)]
                qT_s[w, t] = _pack(q * QSCALE)
                phiqT_s[w, t] = _pack(_phi(q))

    def mem_update():
        r = lax.broadcasted_iota(jnp.int32, (MROWS, 128), 0)
        c = lax.broadcasted_iota(jnp.int32, (MROWS, 128), 1)
        for w in range(NW):
            vt = jnp.concatenate([_unpack(vT_s[w, t]) for t in range(4)], axis=1)
            pk = jnp.concatenate([_unpack(phikT_s[w, t]) for t in range(4)], axis=1)
            upd = lax.dot_general(vt, pk, (((1,), (1,)), ((), ())), preferred_element_type=f32)
            mt = mt_s[w] + upd
            mt_s[w] = mt
            keep = jnp.zeros((MROWS, 128), jnp.bool_)
            for a in range(_nh(w)):
                keep = keep | ((r >= RS * a) & (r < RS * (a + 1)) & (c >= DH * a) & (c < DH * (a + 1)))
            mtb_s[w] = _pack(jnp.where(keep, mt, 0.0))

    def mem_retrieve():
        for w in range(NW):
            for j in range(4):
                am = jnp.dot(_unpack(mtb_s[w]), _unpack(phiqT_s[w, j]), preferred_element_type=f32)
                for a in range(_nh(w)):
                    ama = am[RS * a:RS * (a + 1)]
                    g = g_s[w, a:a + 1, :]
                    om = ama * (g / (ama[DH:DH + 1] + 1e-6))
                    am_s[j, WL * w + DH * a:WL * w + DH * (a + 1), :] = om[0:DH]

    def phase_a(w, nh, j, buf):
        n = 128 * (j + 1)
        rows = lax.broadcasted_iota(jnp.int32, (64, 128), 0)
        qw = qT_s[w, j]
        qbd = jnp.concatenate(
            [jnp.where((rows >= 9 * a) & (rows < 9 * a + 9), qw, jnp.uint32(0)) for a in range(nh)], axis=1)
        s = jnp.dot(_unpack(k_s[w, 0:n // 2, :]), _unpack(qbd), preferred_element_type=f32)
        kr = lax.broadcasted_iota(jnp.int32, (128, 128), 0)
        qc = lax.broadcasted_iota(jnp.int32, (128, 128), 1)
        causal = kr <= qc
        sd = jnp.concatenate(
            [jnp.where(causal, s[n - 128:n, 128 * a:128 * (a + 1)], NEG) for a in range(nh)], axis=1)
        s_scr[buf, n - 128:n, 0:128 * nh] = sd
        m = jnp.max(sd, axis=0, keepdims=True)
        if j > 0:
            s_scr[buf, 0:n - 128, 0:128 * nh] = s[0:n - 128]
            m = jnp.maximum(m, jnp.max(s[0:n - 128], axis=0, keepdims=True))
        m_scr[buf, :, 0:128 * nh] = jnp.broadcast_to(m, (8, 128 * nh))

    def phase_b(w, nh, j, buf):
        n = 128 * (j + 1)
        for a in range(nh):
            m = m_scr[buf, 0:1, 128 * a:128 * (a + 1)]
            p = jnp.exp2(s_scr[buf, 0:n, 128 * a:128 * (a + 1)] - m).astype(bf16)
            vt = jnp.concatenate([_unpack(vT_s[w, t, 12 * a:12 * a + 16, :]) for t in range(j + 1)], axis=1)
            o = jnp.dot(vt, p, preferred_element_type=f32)
            g = g_s[w, a:a + 1, :]
            od = o[0:RS] * ((1.0 - g) / o[DH:DH + 1])
            row0 = WL * w + DH * a
            oT_s[j, pl.ds(row0, DH), :] = (od + am_s[j, pl.ds(row0, RS), :])[0:DH]

    def window(w, nh, nxt):
        order = [3, 2, 1, 0]
        for t in range(4):
            if t < 3:
                phase_a(w, nh, order[t + 1], (t + 1) % 2)
            elif nxt is not None:
                phase_a(nxt, _nh(nxt), order[0], 0)
            phase_b(w, nh, order[t], t % 2)

    def outproj(seg):
        oT = jnp.concatenate([oT_s[t] for t in range(4)], axis=1).astype(bf16)
        attn = jnp.dot(woT[...], oT, preferred_element_type=f32)
        wr = wr_s[0:D, :]
        for t in range(4):
            cols = slice(128 * t, 128 * (t + 1))
            tile = 4 * seg + t
            h = x_v[seg, :, cols].astype(f32) + attn[:, cols]
            h_s[tile] = h
            mean, rstd = _ln_stats(h)
            st_s[tile, 0:1, :] = mean
            st_s[tile, 1:2, :] = rstd
            pltpu.touch(h_s)
            h = h_s[tile]
            hn = (h - mean) * rstd
            r_s[pl.ds(tile, 1), :] = _colsum(hn * wr)
            out_v[tile] = (h + hn).astype(bf16)

    def project_segment():
        post_k(proj(0))
        post_v(proj(1))
        post_q(proj(2))

    with _scope("setup"):
        w_copies[0].start()
        x_copy(0).start()
        beta = beta_ref[...].astype(f32).reshape(1, H)
        hrow = lax.broadcasted_iota(jnp.int32, (8 * NW, H), 0)
        hcol = lax.broadcasted_iota(jnp.int32, (8 * NW, H), 1)
        sel = (hcol == HPW * (hrow >> 3) + (hrow & 7)) & ((hrow & 7) < HPW)
        bcol = jnp.sum(jnp.where(sel, beta, 0.0), axis=1, keepdims=True)
        g_s[...] = jnp.broadcast_to(_sigmoid(bcol), (8 * NW, 128)).reshape(NW, 8, 128)
        wr_row = wr_ref[...].astype(f32).reshape(1, D)
        wr_pad = jnp.concatenate([wr_row, jnp.zeros((1, 64), f32)], axis=1)
        wr_s[...] = jnp.broadcast_to(wr_pad, (128, D + 64)).T

        mt_s[...] = jnp.zeros(mt_s.shape, f32)
        vT_s[...] = jnp.zeros(vT_s.shape, u32)
        am_s[...] = jnp.zeros(am_s.shape, f32)

        w_copies[0].wait()
        w_copies[1].start()
        wT[0:D, :] = wk_v[...].T
        x_copy(0).wait()
        w_copies[2].start()
        for t in range(4):
            ln1_tile(0, t)
    with _scope("proj0"):
        w_copies[1].wait()
        w_copies[3].start()
        post_k(proj(0))
        wT[D:2 * D, :] = wv_v[...].T
        w_copies[2].wait()
        for s in range(1, NSEG):
            x_copy(s).start()
        post_v(proj(1))
        wT[2 * D:3 * D, :] = wq_v[...].T
        w_copies[3].wait()
        for c in w_copies[4:]:
            c.start()
        post_q(proj(2))
        woT[...] = wo_v[...].T
        phase_a(0, HPW, 3, 0)
        for s in range(1, NSEG):
            x_copy(s).wait()

    def segment(seg, carry):
        nseg = jnp.minimum(seg + 1, NSEG - 1)

        with _scope("windows"):
            for w in range(NW):
                if w < 4:
                    ln1_tile(nseg, w)
                window(w, _nh(w), w + 1 if w + 1 < NW else None)

        @pl.when(seg < NSEG - 1)
        def _():
            with _scope("mid"):
                mem_update()
                outproj(seg)
                project_segment()
                mem_retrieve()
                phase_a(0, HPW, 3, 0)
                for t in range(4):
                    o_copy(4 * seg + t).start()
        return carry

    lax.fori_loop(0, NSEG, segment, 0)
    with _scope("last_out"):
        outproj(NSEG - 1)
        for t in range(4):
            o_copy(4 * (NSEG - 1) + t).start()

    with _scope("ffn"):
        r = r_s[...]
        rmax = jnp.max(r)
        tok = (lax.broadcasted_iota(jnp.int32, (NT, 128), 0) * 128
               + lax.broadcasted_iota(jnp.int32, (NT, 128), 1))
        idx = jnp.minimum(jnp.min(jnp.where(r == rmax, tok, S)), S - 1)
        tile = idx >> 7
        lane = idx & 127
        lanes = lax.broadcasted_iota(jnp.int32, (D, 128), 1)
        hn = (h_s[tile] - st_s[tile, 0:1, :]) * st_s[tile, 1:2, :]
        hsel = jnp.where(lanes == lane, hn, 0.0)
        hsel = jnp.concatenate([hsel, jnp.zeros((64, 128), f32)], axis=0)
        xrow = jnp.sum(hsel.T, axis=0, keepdims=True)[:, 0:D]
        for c in w_copies[4:]:
            c.wait()
        xs = jnp.broadcast_to(xrow, (16, D)).astype(bf16)
        gate = jnp.dot(xs, wg_v[...], preferred_element_type=f32)
        up = jnp.dot(xs, wu_v[...], preferred_element_type=f32)
        act = (gate * _sigmoid(gate) * up).astype(bf16)
        y = lax.dot_general(act, wdT_v[...], (((1,), (1,)), ((), ())), preferred_element_type=f32)
        y = y[0:1] * _sigmoid(jnp.full((1, 1), rmax, f32))
        ypad = jnp.concatenate([y, jnp.zeros((1, 64), f32)], axis=1)
        ycol = jnp.broadcast_to(ypad, (128, D + 64)).T[0:D]
        for t in range(NT):
            o_copy(t).wait()
        blk = out_v[tile].astype(f32)
        out_v[tile] = jnp.where(lanes == lane, blk + ycol, blk).astype(bf16)
        fix = o_copy(tile)
        fix.start()
        fix.wait()


@jax.jit
def pallas_sequential_preLN__memory_aug_infini_attn__moe_arch_mod__prompt_kernel(
    A_x: jax.Array,
    A_wq: jax.Array,
    A_wk: jax.Array,
    A_wv: jax.Array,
    A_wo: jax.Array,
    A_beta: jax.Array,
    B_x: jax.Array,
    B_w_r: jax.Array,
    B_w_gate: jax.Array,
    B_w_up: jax.Array,
    B_w_down: jax.Array,
):
    del B_x
    xT = A_x.reshape(S, D).T
    wdT = B_w_down.T

    hbm = pl.BlockSpec(memory_space=pltpu.HBM)
    vmem = pl.BlockSpec(memory_space=pltpu.VMEM)
    scratch = [
        pltpu.VMEM((NSEG, D, L), bf16),
        pltpu.VMEM((D, D), bf16),
        pltpu.VMEM((D, D), bf16),
        pltpu.VMEM((D, D), bf16),
        pltpu.VMEM((D, D), bf16),
        pltpu.VMEM((D, F), bf16),
        pltpu.VMEM((D, F), bf16),
        pltpu.VMEM((D, F), bf16),
        pltpu.VMEM((3 * D, D), bf16),
        pltpu.VMEM((D, D), bf16),
        pltpu.VMEM((NW, 8, 128), f32),
        pltpu.VMEM((D + 64, 128), f32),
        pltpu.VMEM((4, D, 128), bf16),
        pltpu.VMEM((NW, L // 2, 128), u32),
        pltpu.VMEM((NW, 4, 64, 128), u32),
        pltpu.VMEM((NW, 4, 64, 128), u32),
        pltpu.VMEM((NW, 4, 64, 128), u32),
        pltpu.VMEM((NW, 4, MROWS // 2, 128), u32),
        pltpu.VMEM((NW, MROWS, 128), f32),
        pltpu.VMEM((NW, MROWS // 2, 128), u32),
        pltpu.VMEM((4, D + 8, 128), f32),
        pltpu.VMEM((2, L, 128 * HPW), f32),
        pltpu.VMEM((2, 8, 128 * HPW), f32),
        pltpu.VMEM((4, D, 128), f32),
        pltpu.VMEM((NT, D, 128), bf16),
        pltpu.VMEM((NT, D, 128), f32),
        pltpu.VMEM((NT, 8, 128), f32),
        pltpu.VMEM((NT, 128), f32),
        pltpu.SemaphoreType.DMA((NSEG,)),
        pltpu.SemaphoreType.DMA((7,)),
        pltpu.SemaphoreType.DMA((NT,)),
    ]
    outT = pl.pallas_call(
        _kernel,
        out_shape=jax.ShapeDtypeStruct((D, S), bf16),
        in_specs=[hbm, hbm, hbm, hbm, hbm, vmem, vmem, hbm, hbm, hbm],
        out_specs=hbm,
        scratch_shapes=scratch,
        compiler_params=pltpu.CompilerParams(vmem_limit_bytes=100 * 1024 * 1024),
    )(xT, A_wq, A_wk, A_wv, A_wo, A_beta, B_w_r, B_w_gate, B_w_up, B_w_down.T)
    return outT.T.reshape(1, S, D)
```

```python
import jax
import jax.numpy as jnp
from jax import lax
import jax.experimental.pallas as pl
import jax.experimental.pallas.tpu as pltpu

S = 2048
D = 576
H = 32
DH = 18
NSEG = 4
L = 512
NT = S // 128
F = 4608
HPW = 7
NW = 5
WL = HPW * DH
RS = 24
MROWS = 176
QKV_ROWS = D + 64
LOG2E = 1.4426950408889634
NEG = -1e9 * LOG2E
QSCALE = (DH ** -0.5) * LOG2E
EPS = 1e-5

import contextlib
import os
_PROF = bool(os.environ.get("PROF"))


def _scope(name):
    return jax.named_scope(name) if _PROF else contextlib.nullcontext()


f32 = jnp.float32
bf16 = jnp.bfloat16
u32 = jnp.uint32


def _nh(w):
    return HPW if w < NW - 1 else H - HPW * (NW - 1)


def _pack(x):
    return pltpu.bitcast(x.astype(bf16), u32)


def _unpack(x):
    return pltpu.bitcast(x, bf16)


def _phi(t):
    return jnp.where(t > 0, t + 1.0, jnp.exp(t))


RC = 16
NCH = D // RC


class _Acc:
    def __init__(self, n=2):
        self.parts = [None] * n
        self.i = 0

    def add(self, x):
        k = self.i % len(self.parts)
        self.parts[k] = x if self.parts[k] is None else self.parts[k] + x
        self.i += 1

    def total(self):
        t = self.parts[0]
        for p in self.parts[1:]:
            t = t + p
        return jnp.sum(t, axis=0, keepdims=True)


def _ln_stats(chunk):
    x0 = chunk(0)
    c = x0[0:1]
    s1, s2 = _Acc(), _Acc()
    for i in range(NCH):
        d = (x0 if i == 0 else chunk(i)) - c
        s1.add(d)
        s2.add(d * d)
    mu = s1.total() * (1.0 / D)
    var = jnp.maximum(s2.total() * (1.0 / D) - mu * mu, 0.0)
    return c + mu, lax.rsqrt(var + EPS)


def _sigmoid(x):
    return 1.0 / (1.0 + jnp.exp(-x))


def _kernel(xT_hbm, wq_hbm, wk_hbm, wv_hbm, wo_hbm, beta_ref, wr_ref, wg_hbm, wu_hbm, wdT_hbm,
            out_hbm,
            x_v, wq_v, wk_v, wv_v, wo_v, wg_v, wu_v, wdT_v,
            wT, woT, g_s, wr_s,
            xn_s, k_s, phikT_s, qT_s, phiqT_s, vT_s, mt_s, mtb_s, am_s,
            s_scr, m_scr, oT_s, out_v, h_s, st_s, r_s,
            sem_x, sem_w, sem_o):
    def x_copy(s):
        return pltpu.make_async_copy(xT_hbm.at[:, pl.ds(s * L, L)], x_v.at[s], sem_x.at[s])

    def o_copy(t):
        return pltpu.make_async_copy(out_v.at[t], out_hbm.at[:, pl.ds(pl.multiple_of(t * 128, 128), 128)],
                                     sem_o.at[t])

    w_copies = [pltpu.make_async_copy(src, dst, sem_w.at[i]) for i, (src, dst) in enumerate(
        [(wk_hbm, wk_v), (wv_hbm, wv_v), (wq_hbm, wq_v), (wo_hbm, wo_v),
         (wg_hbm, wg_v), (wu_hbm, wu_v), (wdT_hbm, wdT_v)])]

    def ln1_tile(seg, t):
        cols = pl.ds(pl.multiple_of(t * 128, 128), 128)

        def chunk(i):
            return x_v[seg, RC * i:RC * (i + 1), cols].astype(f32)
        mean, rstd = _ln_stats(chunk)
        pltpu.touch(x_v)
        for i in range(NCH):
            xn_s[t, RC * i:RC * (i + 1), :] = ((chunk(i) - mean) * rstd).astype(bf16)

    def proj(i):
        xn = jnp.concatenate([xn_s[t] for t in range(4)], axis=1)
        r = jnp.dot(wT[D * i:D * (i + 1), :], xn, preferred_element_type=f32)
        return jnp.concatenate([r, jnp.zeros((64, L), f32)], axis=0)

    def post_k(r):
        for t in range(4):
            for w in range(NW):
                kk = r[WL * w:WL * w + 128, 128 * t:128 * (t + 1)]
                k_s[w, 64 * t:64 * (t + 1), :] = pltpu.bitcast(kk.astype(bf16).T, u32)
                phikT_s[w, t] = _pack(_phi(kk))

    def post_v(r):
        r24 = lax.broadcasted_iota(jnp.int32, (RS, 128), 0)
        ones_row = jnp.where(r24 == DH, 1.0, 0.0).astype(f32)
        for t in range(4):
            for w in range(NW):
                nh = _nh(w)
                vs = [jnp.where(r24 < DH,
                                r[DH * (HPW * w + a):DH * (HPW * w + a) + RS, 128 * t:128 * (t + 1)], ones_row)
                      for a in range(nh)]
                if nh % 2:
                    vs.append(jnp.zeros((8, 128), f32))
                vv = _pack(jnp.concatenate(vs, axis=0))
                vT_s[w, t, 0:vv.shape[0], :] = vv

    def post_q(r):
        for t in range(4):
            for w in range(NW):
                q = r[WL * w:WL * w + 128, 128 * t:128 * (t + 1)]
                qT_s[w, t] = _pack(q * QSCALE)
                phiqT_s[w, t] = _pack(_phi(q))

    def mem_update():
        r = lax.broadcasted_iota(jnp.int32, (MROWS, 128), 0)
        c = lax.broadcasted_iota(jnp.int32, (MROWS, 128), 1)
        for w in range(NW):
            vt = jnp.concatenate([_unpack(vT_s[w, t]) for t in range(4)], axis=1)
            pk = jnp.concatenate([_unpack(phikT_s[w, t]) for t in range(4)], axis=1)
            upd = lax.dot_general(vt, pk, (((1,), (1,)), ((), ())), preferred_element_type=f32)
            mt = mt_s[w] + upd
            mt_s[w] = mt
            keep = jnp.zeros((MROWS, 128), jnp.bool_)
            for a in range(_nh(w)):
                keep = keep | ((r >= RS * a) & (r < RS * (a + 1)) & (c >= DH * a) & (c < DH * (a + 1)))
            mtb_s[w] = _pack(jnp.where(keep, mt, 0.0))

    def mem_retrieve():
        for w in range(NW):
            for j in range(4):
                am = jnp.dot(_unpack(mtb_s[w]), _unpack(phiqT_s[w, j]), preferred_element_type=f32)
                for a in range(_nh(w)):
                    ama = am[RS * a:RS * (a + 1)]
                    g = g_s[w, a:a + 1, :]
                    om = ama * (g / (ama[DH:DH + 1] + 1e-6))
                    am_s[j, WL * w + DH * a:WL * w + DH * (a + 1), :] = om[0:DH]

    def phase_a(w, nh, j, buf):
        n = 128 * (j + 1)
        rows = lax.broadcasted_iota(jnp.int32, (64, 128), 0)
        qw = qT_s[w, j]
        qbd = jnp.concatenate(
            [jnp.where((rows >= 9 * a) & (rows < 9 * a + 9), qw, jnp.uint32(0)) for a in range(nh)], axis=1)
        s = jnp.dot(_unpack(k_s[w, 0:n // 2, :]), _unpack(qbd), preferred_element_type=f32)
        kr = lax.broadcasted_iota(jnp.int32, (128, 128), 0)
        qc = lax.broadcasted_iota(jnp.int32, (128, 128), 1)
        causal = kr <= qc
        sd = jnp.concatenate(
            [jnp.where(causal, s[n - 128:n, 128 * a:128 * (a + 1)], NEG) for a in range(nh)], axis=1)
        s_scr[buf, n - 128:n, 0:128 * nh] = sd
        m = jnp.max(sd, axis=0, keepdims=True)
        if j > 0:
            s_scr[buf, 0:n - 128, 0:128 * nh] = s[0:n - 128]
            m = jnp.maximum(m, jnp.max(s[0:n - 128], axis=0, keepdims=True))
        m_scr[buf, :, 0:128 * nh] = jnp.broadcast_to(m, (8, 128 * nh))

    def phase_b(w, nh, j, buf):
        n = 128 * (j + 1)
        for a in range(nh):
            m = m_scr[buf, 0:1, 128 * a:128 * (a + 1)]
            p = jnp.exp2(s_scr[buf, 0:n, 128 * a:128 * (a + 1)] - m).astype(bf16)
            vt = jnp.concatenate([_unpack(vT_s[w, t, 12 * a:12 * a + 16, :]) for t in range(j + 1)], axis=1)
            o = jnp.dot(vt, p, preferred_element_type=f32)
            g = g_s[w, a:a + 1, :]
            od = o[0:RS] * ((1.0 - g) / o[DH:DH + 1])
            row0 = WL * w + DH * a
            oT_s[j, pl.ds(row0, DH), :] = (od + am_s[j, pl.ds(row0, RS), :])[0:DH]

    def window(w, nh, nxt):
        order = [3, 2, 1, 0]
        for t in range(4):
            if t < 3:
                phase_a(w, nh, order[t + 1], (t + 1) % 2)
            elif nxt is not None:
                phase_a(nxt, _nh(nxt), order[0], 0)
            phase_b(w, nh, order[t], t % 2)

    def outproj(seg):
        oT = jnp.concatenate([oT_s[t] for t in range(4)], axis=1).astype(bf16)
        attn = jnp.dot(woT[...], oT, preferred_element_type=f32)
        for t in range(4):
            cols = slice(128 * t, 128 * (t + 1))
            tile = 4 * seg + t

            def chunk(i):
                rows = slice(RC * i, RC * (i + 1))
                h = x_v[seg, rows, cols].astype(f32) + attn[rows, cols]
                h_s[tile, rows, :] = h
                return h
            mean, rstd = _ln_stats(chunk)
            st_s[tile, 0:1, :] = mean
            st_s[tile, 1:2, :] = rstd
            pltpu.touch(h_s)
            racc = _Acc()
            for i in range(NCH):
                rows = slice(RC * i, RC * (i + 1))
                h = h_s[tile, rows, :]
                hn = (h - mean) * rstd
                out_v[tile, rows, :] = (h + hn).astype(bf16)
                racc.add(hn * wr_s[rows, :])
            r_s[pl.ds(tile, 1), :] = racc.total()

    def project_segment():
        post_k(proj(0))
        post_v(proj(1))
        post_q(proj(2))

    with _scope("setup"):
        w_copies[0].start()
        x_copy(0).start()
        beta = beta_ref[...].astype(f32).reshape(1, H)
        hrow = lax.broadcasted_iota(jnp.int32, (8 * NW, H), 0)
        hcol = lax.broadcasted_iota(jnp.int32, (8 * NW, H), 1)
        sel = (hcol == HPW * (hrow >> 3) + (hrow & 7)) & ((hrow & 7) < HPW)
        bcol = jnp.sum(jnp.where(sel, beta, 0.0), axis=1, keepdims=True)
        g_s[...] = jnp.broadcast_to(_sigmoid(bcol), (8 * NW, 128)).reshape(NW, 8, 128)
        wr_row = wr_ref[...].astype(f32).reshape(1, D)
        wr_pad = jnp.concatenate([wr_row, jnp.zeros((1, 64), f32)], axis=1)
        wr_s[...] = jnp.broadcast_to(wr_pad, (128, D + 64)).T

        mt_s[...] = jnp.zeros(mt_s.shape, f32)
        vT_s[...] = jnp.zeros(vT_s.shape, u32)
        am_s[...] = jnp.zeros(am_s.shape, f32)

        w_copies[0].wait()
        w_copies[1].start()
        wT[0:D, :] = wk_v[...].T
        x_copy(0).wait()
        w_copies[2].start()
        for t in range(4):
            ln1_tile(0, t)
    with _scope("proj0"):
        w_copies[1].wait()
        w_copies[3].start()
        post_k(proj(0))
        wT[D:2 * D, :] = wv_v[...].T
        w_copies[2].wait()
        for s in range(1, NSEG):
            x_copy(s).start()
        post_v(proj(1))
        wT[2 * D:3 * D, :] = wq_v[...].T
        w_copies[3].wait()
        for c in w_copies[4:]:
            c.start()
        post_q(proj(2))
        woT[...] = wo_v[...].T
        phase_a(0, HPW, 3, 0)
        for s in range(1, NSEG):
            x_copy(s).wait()

    def segment(seg, carry):
        nseg = jnp.minimum(seg + 1, NSEG - 1)

        with _scope("windows"):
            for w in range(NW):
                if w < 4:
                    ln1_tile(nseg, w)
                window(w, _nh(w), w + 1 if w + 1 < NW else None)

        @pl.when(seg < NSEG - 1)
        def _():
            with _scope("mid"):
                mem_update()
                outproj(seg)
                project_segment()
                mem_retrieve()
                phase_a(0, HPW, 3, 0)
                for t in range(4):
                    o_copy(4 * seg + t).start()
        return carry

    lax.fori_loop(0, NSEG, segment, 0)
    with _scope("last_out"):
        outproj(NSEG - 1)
        for t in range(4):
            o_copy(4 * (NSEG - 1) + t).start()

    with _scope("ffn"):
        r = r_s[...]
        rmax = jnp.max(r)
        tok = (lax.broadcasted_iota(jnp.int32, (NT, 128), 0) * 128
               + lax.broadcasted_iota(jnp.int32, (NT, 128), 1))
        idx = jnp.minimum(jnp.min(jnp.where(r == rmax, tok, S)), S - 1)
        tile = idx >> 7
        lane = idx & 127
        lanes = lax.broadcasted_iota(jnp.int32, (D, 128), 1)
        hn = (h_s[tile] - st_s[tile, 0:1, :]) * st_s[tile, 1:2, :]
        hsel = jnp.where(lanes == lane, hn, 0.0)
        hsel = jnp.concatenate([hsel, jnp.zeros((64, 128), f32)], axis=0)
        xrow = jnp.sum(hsel.T, axis=0, keepdims=True)[:, 0:D]
        for c in w_copies[4:]:
            c.wait()
        xs = jnp.broadcast_to(xrow, (16, D)).astype(bf16)
        gate = jnp.dot(xs, wg_v[...], preferred_element_type=f32)
        up = jnp.dot(xs, wu_v[...], preferred_element_type=f32)
        act = (gate * _sigmoid(gate) * up).astype(bf16)
        y = lax.dot_general(act, wdT_v[...], (((1,), (1,)), ((), ())), preferred_element_type=f32)
        y = y[0:1] * _sigmoid(jnp.full((1, 1), rmax, f32))
        ypad = jnp.concatenate([y, jnp.zeros((1, 64), f32)], axis=1)
        ycol = jnp.broadcast_to(ypad, (128, D + 64)).T[0:D]
        for t in range(NT):
            o_copy(t).wait()
        blk = out_v[tile].astype(f32)
        out_v[tile] = jnp.where(lanes == lane, blk + ycol, blk).astype(bf16)
        fix = o_copy(tile)
        fix.start()
        fix.wait()


@jax.jit
def pallas_sequential_preLN__memory_aug_infini_attn__moe_arch_mod__prompt_kernel(
    A_x: jax.Array,
    A_wq: jax.Array,
    A_wk: jax.Array,
    A_wv: jax.Array,
    A_wo: jax.Array,
    A_beta: jax.Array,
    B_x: jax.Array,
    B_w_r: jax.Array,
    B_w_gate: jax.Array,
    B_w_up: jax.Array,
    B_w_down: jax.Array,
):
    del B_x
    xT = A_x.reshape(S, D).T
    wdT = B_w_down.T

    hbm = pl.BlockSpec(memory_space=pltpu.HBM)
    vmem = pl.BlockSpec(memory_space=pltpu.VMEM)
    scratch = [
        pltpu.VMEM((NSEG, D, L), bf16),
        pltpu.VMEM((D, D), bf16),
        pltpu.VMEM((D, D), bf16),
        pltpu.VMEM((D, D), bf16),
        pltpu.VMEM((D, D), bf16),
        pltpu.VMEM((D, F), bf16),
        pltpu.VMEM((D, F), bf16),
        pltpu.VMEM((D, F), bf16),
        pltpu.VMEM((3 * D, D), bf16),
        pltpu.VMEM((D, D), bf16),
        pltpu.VMEM((NW, 8, 128), f32),
        pltpu.VMEM((D + 64, 128), f32),
        pltpu.VMEM((4, D, 128), bf16),
        pltpu.VMEM((NW, L // 2, 128), u32),
        pltpu.VMEM((NW, 4, 64, 128), u32),
        pltpu.VMEM((NW, 4, 64, 128), u32),
        pltpu.VMEM((NW, 4, 64, 128), u32),
        pltpu.VMEM((NW, 4, MROWS // 2, 128), u32),
        pltpu.VMEM((NW, MROWS, 128), f32),
        pltpu.VMEM((NW, MROWS // 2, 128), u32),
        pltpu.VMEM((4, D + 8, 128), f32),
        pltpu.VMEM((2, L, 128 * HPW), f32),
        pltpu.VMEM((2, 8, 128 * HPW), f32),
        pltpu.VMEM((4, D, 128), f32),
        pltpu.VMEM((NT, D, 128), bf16),
        pltpu.VMEM((NT, D, 128), f32),
        pltpu.VMEM((NT, 8, 128), f32),
        pltpu.VMEM((NT, 128), f32),
        pltpu.SemaphoreType.DMA((NSEG,)),
        pltpu.SemaphoreType.DMA((7,)),
        pltpu.SemaphoreType.DMA((NT,)),
    ]
    outT = pl.pallas_call(
        _kernel,
        out_shape=jax.ShapeDtypeStruct((D, S), bf16),
        in_specs=[hbm, hbm, hbm, hbm, hbm, vmem, vmem, hbm, hbm, hbm],
        out_specs=hbm,
        scratch_shapes=scratch,
        compiler_params=pltpu.CompilerParams(vmem_limit_bytes=100 * 1024 * 1024),
    )(xT, A_wq, A_wk, A_wv, A_wo, A_beta, B_w_r, B_w_gate, B_w_up, B_w_down.T)
    return outT.T.reshape(1, S, D)
```

```python
import jax
import jax.numpy as jnp
from jax import lax
import jax.experimental.pallas as pl
import jax.experimental.pallas.tpu as pltpu

S = 2048
D = 576
H = 32
DH = 18
NSEG = 4
L = 512
NT = S // 128
F = 4608
HPW = 7
NW = 5
WL = HPW * DH
RS = 24
MROWS = 176
QKV_ROWS = D + 64
LOG2E = 1.4426950408889634
NEG = -1e9 * LOG2E
QSCALE = (DH ** -0.5) * LOG2E
EPS = 1e-5

import contextlib
import os
_PROF = bool(os.environ.get("PROF"))


def _scope(name):
    return jax.named_scope(name) if _PROF else contextlib.nullcontext()


f32 = jnp.float32
bf16 = jnp.bfloat16
u32 = jnp.uint32


def _nh(w):
    return HPW if w < NW - 1 else H - HPW * (NW - 1)


def _pack(x):
    return pltpu.bitcast(x.astype(bf16), u32)


def _unpack(x):
    return pltpu.bitcast(x, bf16)


def _phi(t):
    return jnp.where(t > 0, t + 1.0, jnp.exp(t))


RC = 16
NCH = D // RC


class _Acc:
    def __init__(self, n=2):
        self.parts = [None] * n
        self.i = 0

    def add(self, x):
        k = self.i % len(self.parts)
        self.parts[k] = x if self.parts[k] is None else self.parts[k] + x
        self.i += 1

    def total(self):
        t = self.parts[0]
        for p in self.parts[1:]:
            t = t + p
        return jnp.sum(t, axis=0, keepdims=True)


def _ln_stats(chunk):
    x0 = chunk(0)
    c = x0[0:1]
    s1, s2 = _Acc(), _Acc()
    for i in range(NCH):
        d = (x0 if i == 0 else chunk(i)) - c
        s1.add(d)
        s2.add(d * d)
    mu = s1.total() * (1.0 / D)
    var = jnp.maximum(s2.total() * (1.0 / D) - mu * mu, 0.0)
    return c + mu, lax.rsqrt(var + EPS)


def _sigmoid(x):
    return 1.0 / (1.0 + jnp.exp(-x))


def _kernel(xT_hbm, wq_hbm, wk_hbm, wv_hbm, wo_hbm, beta_ref, wr_ref, wg_hbm, wu_hbm, wdT_hbm,
            out_hbm,
            x_v, wq_v, wk_v, wv_v, wo_v, wg_v, wu_v, wdT_v,
            wT, woT, wd_s, g_s, wr_s,
            xn_s, k_s, phikT_s, qT_s, phiqT_s, vT_s, mt_s, mtb_s, am_s,
            s_scr, m_scr, oT_s, out_v, h_s, st_s, r_s,
            sem_x, sem_w, sem_o):
    def x_copy(s):
        return pltpu.make_async_copy(xT_hbm.at[:, pl.ds(s * L, L)], x_v.at[s], sem_x.at[s])

    def o_copy(t):
        return pltpu.make_async_copy(out_v.at[t], out_hbm.at[:, pl.ds(pl.multiple_of(t * 128, 128), 128)],
                                     sem_o.at[t])

    w_copies = [pltpu.make_async_copy(src, dst, sem_w.at[i]) for i, (src, dst) in enumerate(
        [(wk_hbm, wk_v), (wv_hbm, wv_v), (wq_hbm, wq_v), (wo_hbm, wo_v),
         (wdT_hbm, wdT_v), (wg_hbm, wg_v), (wu_hbm, wu_v)])]

    def ln1_tile(seg, t):
        cols = pl.ds(pl.multiple_of(t * 128, 128), 128)

        def chunk(i):
            return x_v[seg, RC * i:RC * (i + 1), cols].astype(f32)
        mean, rstd = _ln_stats(chunk)
        pltpu.touch(x_v)
        for i in range(NCH):
            xn_s[t, RC * i:RC * (i + 1), :] = ((chunk(i) - mean) * rstd).astype(bf16)

    def proj(i):
        xn = jnp.concatenate([xn_s[t] for t in range(4)], axis=1)
        r = jnp.dot(wT[D * i:D * (i + 1), :], xn, preferred_element_type=f32)
        return jnp.concatenate([r, jnp.zeros((64, L), f32)], axis=0)

    def post_k(r):
        for t in range(4):
            for w in range(NW):
                kk = r[WL * w:WL * w + 128, 128 * t:128 * (t + 1)]
                k_s[w, 64 * t:64 * (t + 1), :] = pltpu.bitcast(kk.astype(bf16).T, u32)
                phikT_s[w, t] = _pack(_phi(kk))

    def post_v(r):
        r24 = lax.broadcasted_iota(jnp.int32, (RS, 128), 0)
        ones_row = jnp.where(r24 == DH, 1.0, 0.0).astype(f32)
        for t in range(4):
            for w in range(NW):
                nh = _nh(w)
                vs = [jnp.where(r24 < DH,
                                r[DH * (HPW * w + a):DH * (HPW * w + a) + RS, 128 * t:128 * (t + 1)], ones_row)
                      for a in range(nh)]
                if nh % 2:
                    vs.append(jnp.zeros((8, 128), f32))
                vv = _pack(jnp.concatenate(vs, axis=0))
                vT_s[w, t, 0:vv.shape[0], :] = vv

    def post_q(r):
        for t in range(4):
            for w in range(NW):
                q = r[WL * w:WL * w + 128, 128 * t:128 * (t + 1)]
                qT_s[w, t] = _pack(q * QSCALE)
                phiqT_s[w, t] = _pack(_phi(q))

    def mem_update():
        r = lax.broadcasted_iota(jnp.int32, (MROWS, 128), 0)
        c = lax.broadcasted_iota(jnp.int32, (MROWS, 128), 1)
        for w in range(NW):
            vt = jnp.concatenate([_unpack(vT_s[w, t]) for t in range(4)], axis=1)
            pk = jnp.concatenate([_unpack(phikT_s[w, t]) for t in range(4)], axis=1)
            upd = lax.dot_general(vt, pk, (((1,), (1,)), ((), ())), preferred_element_type=f32)
            mt = mt_s[w] + upd
            mt_s[w] = mt
            keep = jnp.zeros((MROWS, 128), jnp.bool_)
            for a in range(_nh(w)):
                keep = keep | ((r >= RS * a) & (r < RS * (a + 1)) & (c >= DH * a) & (c < DH * (a + 1)))
            mtb_s[w] = _pack(jnp.where(keep, mt, 0.0))

    def mem_retrieve():
        for w in range(NW):
            for j in range(4):
                am = jnp.dot(_unpack(mtb_s[w]), _unpack(phiqT_s[w, j]), preferred_element_type=f32)
                for a in range(_nh(w)):
                    ama = am[RS * a:RS * (a + 1)]
                    g = g_s[w, a:a + 1, :]
                    om = ama * (g / (ama[DH:DH + 1] + 1e-6))
                    am_s[j, WL * w + DH * a:WL * w + DH * (a + 1), :] = om[0:DH]

    def phase_a(w, nh, j, buf):
        n = 128 * (j + 1)
        rows = lax.broadcasted_iota(jnp.int32, (64, 128), 0)
        qw = qT_s[w, j]
        qbd = jnp.concatenate(
            [jnp.where((rows >= 9 * a) & (rows < 9 * a + 9), qw, jnp.uint32(0)) for a in range(nh)], axis=1)
        s = jnp.dot(_unpack(k_s[w, 0:n // 2, :]), _unpack(qbd), preferred_element_type=f32)
        kr = lax.broadcasted_iota(jnp.int32, (128, 128), 0)
        qc = lax.broadcasted_iota(jnp.int32, (128, 128), 1)
        causal = kr <= qc
        sd = jnp.concatenate(
            [jnp.where(causal, s[n - 128:n, 128 * a:128 * (a + 1)], NEG) for a in range(nh)], axis=1)
        s_scr[buf, n - 128:n, 0:128 * nh] = sd
        m = jnp.max(sd, axis=0, keepdims=True)
        if j > 0:
            s_scr[buf, 0:n - 128, 0:128 * nh] = s[0:n - 128]
            m = jnp.maximum(m, jnp.max(s[0:n - 128], axis=0, keepdims=True))
        m_scr[buf, :, 0:128 * nh] = jnp.broadcast_to(m, (8, 128 * nh))

    def phase_b(w, nh, j, buf):
        n = 128 * (j + 1)
        for a in range(nh):
            m = m_scr[buf, 0:1, 128 * a:128 * (a + 1)]
            p = jnp.exp2(s_scr[buf, 0:n, 128 * a:128 * (a + 1)] - m).astype(bf16)
            vt = jnp.concatenate([_unpack(vT_s[w, t, 12 * a:12 * a + 16, :]) for t in range(j + 1)], axis=1)
            o = jnp.dot(vt, p, preferred_element_type=f32)
            g = g_s[w, a:a + 1, :]
            od = o[0:RS] * ((1.0 - g) / o[DH:DH + 1])
            row0 = WL * w + DH * a
            oT_s[j, pl.ds(row0, DH), :] = (od + am_s[j, pl.ds(row0, RS), :])[0:DH]

    def window(w, nh, nxt):
        order = [3, 2, 1, 0]
        for t in range(4):
            if t < 3:
                phase_a(w, nh, order[t + 1], (t + 1) % 2)
            elif nxt is not None:
                phase_a(nxt, _nh(nxt), order[0], 0)
            phase_b(w, nh, order[t], t % 2)

    def outproj(seg):
        oT = jnp.concatenate([oT_s[t] for t in range(4)], axis=1).astype(bf16)
        attn = jnp.dot(woT[...], oT, preferred_element_type=f32)
        for t in range(4):
            cols = slice(128 * t, 128 * (t + 1))
            tile = 4 * seg + t

            def chunk(i):
                rows = slice(RC * i, RC * (i + 1))
                h = x_v[seg, rows, cols].astype(f32) + attn[rows, cols]
                h_s[tile, rows, :] = h
                return h
            mean, rstd = _ln_stats(chunk)
            st_s[tile, 0:1, :] = mean
            st_s[tile, 1:2, :] = rstd
            pltpu.touch(h_s)
            racc = _Acc()
            for i in range(NCH):
                rows = slice(RC * i, RC * (i + 1))
                h = h_s[tile, rows, :]
                hn = (h - mean) * rstd
                out_v[tile, rows, :] = (h + hn).astype(bf16)
                racc.add(hn * wr_s[rows, :])
            r_s[pl.ds(tile, 1), :] = racc.total()

    def transpose_wd(seg):
        nblk = F // 128 // (NSEG - 1)
        for i in range(nblk):
            c0 = pl.multiple_of((seg * nblk + i) * 128, 128)
            wd_s[pl.ds(c0, 128), :] = wdT_v[:, pl.ds(c0, 128)].T

    def project_segment():
        post_k(proj(0))
        post_v(proj(1))
        post_q(proj(2))

    with _scope("setup"):
        w_copies[0].start()
        x_copy(0).start()
        beta = beta_ref[...].astype(f32).reshape(1, H)
        hrow = lax.broadcasted_iota(jnp.int32, (8 * NW, H), 0)
        hcol = lax.broadcasted_iota(jnp.int32, (8 * NW, H), 1)
        sel = (hcol == HPW * (hrow >> 3) + (hrow & 7)) & ((hrow & 7) < HPW)
        bcol = jnp.sum(jnp.where(sel, beta, 0.0), axis=1, keepdims=True)
        g_s[...] = jnp.broadcast_to(_sigmoid(bcol), (8 * NW, 128)).reshape(NW, 8, 128)
        wr_row = wr_ref[...].astype(f32).reshape(1, D)
        wr_pad = jnp.concatenate([wr_row, jnp.zeros((1, 64), f32)], axis=1)
        wr_s[...] = jnp.broadcast_to(wr_pad, (128, D + 64)).T

        mt_s[...] = jnp.zeros(mt_s.shape, f32)
        vT_s[...] = jnp.zeros(vT_s.shape, u32)
        am_s[...] = jnp.zeros(am_s.shape, f32)

        w_copies[0].wait()
        w_copies[1].start()
        wT[0:D, :] = wk_v[...].T
        x_copy(0).wait()
        w_copies[2].start()
        for t in range(4):
            ln1_tile(0, t)
    with _scope("proj0"):
        w_copies[1].wait()
        w_copies[3].start()
        post_k(proj(0))
        wT[D:2 * D, :] = wv_v[...].T
        w_copies[2].wait()
        for s in range(1, NSEG):
            x_copy(s).start()
        post_v(proj(1))
        wT[2 * D:3 * D, :] = wq_v[...].T
        w_copies[3].wait()
        for c in w_copies[4:]:
            c.start()
        post_q(proj(2))
        woT[...] = wo_v[...].T
        phase_a(0, HPW, 3, 0)
        for s in range(1, NSEG):
            x_copy(s).wait()

    def segment(seg, carry):
        nseg = jnp.minimum(seg + 1, NSEG - 1)

        with _scope("windows"):
            for w in range(NW):
                if w < 4:
                    ln1_tile(nseg, w)
                window(w, _nh(w), w + 1 if w + 1 < NW else None)

        @pl.when(seg < NSEG - 1)
        def _():
            @pl.when(seg == 0)
            def _():
                w_copies[4].wait()

            with _scope("mid"):
                transpose_wd(seg)
                mem_update()
                outproj(seg)
                project_segment()
                mem_retrieve()
                phase_a(0, HPW, 3, 0)
                for t in range(4):
                    o_copy(4 * seg + t).start()
        return carry

    lax.fori_loop(0, NSEG, segment, 0)
    with _scope("last_out"):
        outproj(NSEG - 1)
        for t in range(4):
            o_copy(4 * (NSEG - 1) + t).start()

    with _scope("ffn"):
        r = r_s[...]
        rmax = jnp.max(r)
        tok = (lax.broadcasted_iota(jnp.int32, (NT, 128), 0) * 128
               + lax.broadcasted_iota(jnp.int32, (NT, 128), 1))
        idx = jnp.minimum(jnp.min(jnp.where(r == rmax, tok, S)), S - 1)
        tile = idx >> 7
        lane = idx & 127
        hn = ((h_s[tile] - st_s[tile, 0:1, :]) * st_s[tile, 1:2, :]).astype(bf16)
        onehot = jnp.where(lax.broadcasted_iota(jnp.int32, (16, 128), 1) == lane, 1.0, 0.0).astype(bf16)
        xs = lax.dot_general(onehot, hn, (((1,), (1,)), ((), ())), preferred_element_type=f32)
        for c in w_copies[5:]:
            c.wait()
        xm = xs[:, 0:512].astype(bf16)
        xr = xs[:, 512:D]
        row = lax.broadcasted_iota(jnp.int32, (16, 64), 0)
        x2 = jnp.concatenate([jnp.where(row == 0, xr, 0.0), jnp.where(row == 1, xr, 0.0)], axis=1).astype(bf16)
        wrem = jnp.concatenate([wg_v[512:D, :], wu_v[512:D, :]], axis=0)
        rem = jnp.dot(x2, wrem, preferred_element_type=f32)
        gate = jnp.dot(xm, wg_v[0:512, :], preferred_element_type=f32)[0:1] + rem[0:1]
        up = jnp.dot(xm, wu_v[0:512, :], preferred_element_type=f32)[0:1] + rem[1:2]
        act = jnp.broadcast_to(gate * _sigmoid(gate) * up, (16, F)).astype(bf16)
        y = jnp.dot(act, wd_s[...], preferred_element_type=f32)
        y = y[0:1] * _sigmoid(jnp.full((1, 1), rmax, f32))
        ypad = jnp.concatenate([y, jnp.zeros((1, 64), f32)], axis=1)
        ycol = jnp.broadcast_to(ypad, (128, D + 64)).T[0:D]
        for t in range(NT):
            o_copy(t).wait()
        lanes = lax.broadcasted_iota(jnp.int32, (D, 128), 1)
        blk = out_v[tile].astype(f32)
        out_v[tile] = jnp.where(lanes == lane, blk + ycol, blk).astype(bf16)
        fix = o_copy(tile)
        fix.start()
        fix.wait()


@jax.jit
def pallas_sequential_preLN__memory_aug_infini_attn__moe_arch_mod__prompt_kernel(
    A_x: jax.Array,
    A_wq: jax.Array,
    A_wk: jax.Array,
    A_wv: jax.Array,
    A_wo: jax.Array,
    A_beta: jax.Array,
    B_x: jax.Array,
    B_w_r: jax.Array,
    B_w_gate: jax.Array,
    B_w_up: jax.Array,
    B_w_down: jax.Array,
):
    del B_x
    xT = A_x.reshape(S, D).T
    wdT = B_w_down.T

    hbm = pl.BlockSpec(memory_space=pltpu.HBM)
    vmem = pl.BlockSpec(memory_space=pltpu.VMEM)
    scratch = [
        pltpu.VMEM((NSEG, D, L), bf16),
        pltpu.VMEM((D, D), bf16),
        pltpu.VMEM((D, D), bf16),
        pltpu.VMEM((D, D), bf16),
        pltpu.VMEM((D, D), bf16),
        pltpu.VMEM((D, F), bf16),
        pltpu.VMEM((D, F), bf16),
        pltpu.VMEM((D, F), bf16),
        pltpu.VMEM((3 * D, D), bf16),
        pltpu.VMEM((D, D), bf16),
        pltpu.VMEM((F, D), bf16),
        pltpu.VMEM((NW, 8, 128), f32),
        pltpu.VMEM((D + 64, 128), f32),
        pltpu.VMEM((4, D, 128), bf16),
        pltpu.VMEM((NW, L // 2, 128), u32),
        pltpu.VMEM((NW, 4, 64, 128), u32),
        pltpu.VMEM((NW, 4, 64, 128), u32),
        pltpu.VMEM((NW, 4, 64, 128), u32),
        pltpu.VMEM((NW, 4, MROWS // 2, 128), u32),
        pltpu.VMEM((NW, MROWS, 128), f32),
        pltpu.VMEM((NW, MROWS // 2, 128), u32),
        pltpu.VMEM((4, D + 8, 128), f32),
        pltpu.VMEM((2, L, 128 * HPW), f32),
        pltpu.VMEM((2, 8, 128 * HPW), f32),
        pltpu.VMEM((4, D, 128), f32),
        pltpu.VMEM((NT, D, 128), bf16),
        pltpu.VMEM((NT, D, 128), f32),
        pltpu.VMEM((NT, 8, 128), f32),
        pltpu.VMEM((NT, 128), f32),
        pltpu.SemaphoreType.DMA((NSEG,)),
        pltpu.SemaphoreType.DMA((7,)),
        pltpu.SemaphoreType.DMA((NT,)),
    ]
    outT = pl.pallas_call(
        _kernel,
        out_shape=jax.ShapeDtypeStruct((D, S), bf16),
        in_specs=[hbm, hbm, hbm, hbm, hbm, vmem, vmem, hbm, hbm, hbm],
        out_specs=hbm,
        scratch_shapes=scratch,
        compiler_params=pltpu.CompilerParams(vmem_limit_bytes=100 * 1024 * 1024),
    )(xT, A_wq, A_wk, A_wv, A_wo, A_beta, B_w_r, B_w_gate, B_w_up, B_w_down.T)
    return outT.T.reshape(1, S, D)
```

```python
import jax
import jax.numpy as jnp
from jax import lax
import jax.experimental.pallas as pl
import jax.experimental.pallas.tpu as pltpu

S = 2048
D = 576
H = 32
DH = 18
NSEG = 4
L = 512
NT = S // 128
F = 4608
HPW = 7
NW = 5
WL = HPW * DH
RS = 24
MROWS = 176
QKV_ROWS = D + 64
LOG2E = 1.4426950408889634
NEG = -1e9 * LOG2E
QSCALE = (DH ** -0.5) * LOG2E
EPS = 1e-5

import contextlib
import os
_PROF = bool(os.environ.get("PROF"))


def _scope(name):
    return jax.named_scope(name) if _PROF else contextlib.nullcontext()


f32 = jnp.float32
bf16 = jnp.bfloat16
u32 = jnp.uint32


def _nh(w):
    return HPW if w < NW - 1 else H - HPW * (NW - 1)


def _pack(x):
    return pltpu.bitcast(x.astype(bf16), u32)


def _unpack(x):
    return pltpu.bitcast(x, bf16)


def _phi(t):
    return jnp.where(t > 0, t + 1.0, jnp.exp(t))


RC = 16
NCH = D // RC


class _Acc:
    def __init__(self, n=2):
        self.parts = [None] * n
        self.i = 0

    def add(self, x):
        k = self.i % len(self.parts)
        self.parts[k] = x if self.parts[k] is None else self.parts[k] + x
        self.i += 1

    def total(self):
        t = self.parts[0]
        for p in self.parts[1:]:
            t = t + p
        return jnp.sum(t, axis=0, keepdims=True)


def _ln_stats(chunk):
    x0 = chunk(0)
    c = x0[0:1]
    s1, s2 = _Acc(), _Acc()
    for i in range(NCH):
        d = (x0 if i == 0 else chunk(i)) - c
        s1.add(d)
        s2.add(d * d)
    mu = s1.total() * (1.0 / D)
    var = jnp.maximum(s2.total() * (1.0 / D) - mu * mu, 0.0)
    return c + mu, lax.rsqrt(var + EPS)


def _sigmoid(x):
    return 1.0 / (1.0 + jnp.exp(-x))


def _kernel(xT_hbm, wq_hbm, wk_hbm, wv_hbm, wo_hbm, beta_ref, wr_ref, wg_hbm, wu_hbm, wdT_hbm,
            out_hbm,
            x_v, wq_v, wk_v, wv_v, wo_v, wg_v, wu_v, wdT_v,
            wT, woT, wd_s, g_s, wr_s,
            xn_s, k_s, phikT_s, qT_s, phiqT_s, vT_s, mt_s, mtb_s, am_s,
            s_scr, m_scr, oT_s, out_v, h_s, st_s, r_s,
            sem_x, sem_w, sem_o):
    def x_copy(s):
        return pltpu.make_async_copy(xT_hbm.at[:, pl.ds(s * L, L)], x_v.at[s], sem_x.at[s])

    def o_copy(t):
        return pltpu.make_async_copy(out_v.at[t], out_hbm.at[:, pl.ds(pl.multiple_of(t * 128, 128), 128)],
                                     sem_o.at[t])

    w_copies = [pltpu.make_async_copy(src, dst, sem_w.at[i]) for i, (src, dst) in enumerate(
        [(wk_hbm, wk_v), (wv_hbm, wv_v), (wq_hbm, wq_v), (wo_hbm, wo_v),
         (wdT_hbm, wdT_v), (wg_hbm, wg_v), (wu_hbm, wu_v)])]

    def ln1_tile(seg, t):
        cols = pl.ds(pl.multiple_of(t * 128, 128), 128)

        def chunk(i):
            return x_v[seg, RC * i:RC * (i + 1), cols].astype(f32)
        mean, rstd = _ln_stats(chunk)
        pltpu.touch(x_v)
        for i in range(NCH):
            xn_s[t, RC * i:RC * (i + 1), :] = ((chunk(i) - mean) * rstd).astype(bf16)

    def proj(i):
        xn = jnp.concatenate([xn_s[t] for t in range(4)], axis=1)
        r = jnp.dot(wT[D * i:D * (i + 1), :], xn, preferred_element_type=f32)
        return jnp.concatenate([r, jnp.zeros((64, L), f32)], axis=0)

    def post_k(r):
        for t in range(4):
            for w in range(NW):
                kk = r[WL * w:WL * w + 128, 128 * t:128 * (t + 1)]
                k_s[w, 64 * t:64 * (t + 1), :] = pltpu.bitcast(kk.astype(bf16).T, u32)
                phikT_s[w, t] = _pack(_phi(kk))

    def post_v(r):
        r24 = lax.broadcasted_iota(jnp.int32, (RS, 128), 0)
        ones_row = jnp.where(r24 == DH, 1.0, 0.0).astype(f32)
        for t in range(4):
            for w in range(NW):
                nh = _nh(w)
                vs = [jnp.where(r24 < DH,
                                r[DH * (HPW * w + a):DH * (HPW * w + a) + RS, 128 * t:128 * (t + 1)], ones_row)
                      for a in range(nh)]
                if nh % 2:
                    vs.append(jnp.zeros((8, 128), f32))
                vv = _pack(jnp.concatenate(vs, axis=0))
                vT_s[w, t, 0:vv.shape[0], :] = vv

    def post_q(r):
        for t in range(4):
            for w in range(NW):
                q = r[WL * w:WL * w + 128, 128 * t:128 * (t + 1)]
                qT_s[w, t] = _pack(q * QSCALE)
                phiqT_s[w, t] = _pack(_phi(q))

    def mem_update():
        r = lax.broadcasted_iota(jnp.int32, (MROWS, 128), 0)
        c = lax.broadcasted_iota(jnp.int32, (MROWS, 128), 1)
        for w in range(NW):
            vt = jnp.concatenate([_unpack(vT_s[w, t]) for t in range(4)], axis=1)
            pk = jnp.concatenate([_unpack(phikT_s[w, t]) for t in range(4)], axis=1)
            upd = lax.dot_general(vt, pk, (((1,), (1,)), ((), ())), preferred_element_type=f32)
            mt = mt_s[w] + upd
            mt_s[w] = mt
            keep = jnp.zeros((MROWS, 128), jnp.bool_)
            for a in range(_nh(w)):
                keep = keep | ((r >= RS * a) & (r < RS * (a + 1)) & (c >= DH * a) & (c < DH * (a + 1)))
            mtb_s[w] = _pack(jnp.where(keep, mt, 0.0))

    def mem_retrieve():
        for w in range(NW):
            for j in range(4):
                am = jnp.dot(_unpack(mtb_s[w]), _unpack(phiqT_s[w, j]), preferred_element_type=f32)
                for a in range(_nh(w)):
                    ama = am[RS * a:RS * (a + 1)]
                    g = g_s[w, a:a + 1, :]
                    om = ama * (g / (ama[DH:DH + 1] + 1e-6))
                    am_s[j, WL * w + DH * a:WL * w + DH * (a + 1), :] = om[0:DH]

    def phase_a(w, nh, j, buf):
        n = 128 * (j + 1)
        rows = lax.broadcasted_iota(jnp.int32, (64, 128), 0)
        qw = qT_s[w, j]
        qbd = jnp.concatenate(
            [jnp.where((rows >= 9 * a) & (rows < 9 * a + 9), qw, jnp.uint32(0)) for a in range(nh)], axis=1)
        s = jnp.dot(_unpack(k_s[w, 0:n // 2, :]), _unpack(qbd), preferred_element_type=f32)
        kr = lax.broadcasted_iota(jnp.int32, (128, 128), 0)
        qc = lax.broadcasted_iota(jnp.int32, (128, 128), 1)
        causal = kr <= qc
        sd = jnp.concatenate(
            [jnp.where(causal, s[n - 128:n, 128 * a:128 * (a + 1)], NEG) for a in range(nh)], axis=1)
        s_scr[buf, n - 128:n, 0:128 * nh] = sd
        m = jnp.max(sd, axis=0, keepdims=True)
        if j > 0:
            s_scr[buf, 0:n - 128, 0:128 * nh] = s[0:n - 128]
            m = jnp.maximum(m, jnp.max(s[0:n - 128], axis=0, keepdims=True))
        m_scr[buf, :, 0:128 * nh] = jnp.broadcast_to(m, (8, 128 * nh))

    def phase_b(w, nh, j, buf):
        n = 128 * (j + 1)
        for a in range(nh):
            m = m_scr[buf, 0:1, 128 * a:128 * (a + 1)]
            p = jnp.exp2(s_scr[buf, 0:n, 128 * a:128 * (a + 1)] - m).astype(bf16)
            vt = jnp.concatenate([_unpack(vT_s[w, t, 12 * a:12 * a + 16, :]) for t in range(j + 1)], axis=1)
            o = jnp.dot(vt, p, preferred_element_type=f32)
            g = g_s[w, a:a + 1, :]
            od = o[0:RS] * ((1.0 - g) / o[DH:DH + 1])
            row0 = WL * w + DH * a
            oT_s[j, pl.ds(row0, DH), :] = (od + am_s[j, pl.ds(row0, RS), :])[0:DH]

    def window(w, nh, nxt):
        order = [3, 2, 1, 0]
        for t in range(4):
            if t < 3:
                phase_a(w, nh, order[t + 1], (t + 1) % 2)
            elif nxt is not None:
                phase_a(nxt, _nh(nxt), order[0], 0)
            phase_b(w, nh, order[t], t % 2)

    def outproj(seg):
        oT = jnp.concatenate([oT_s[t] for t in range(4)], axis=1).astype(bf16)
        attn = jnp.dot(woT[...], oT, preferred_element_type=f32)
        for t in range(4):
            cols = slice(128 * t, 128 * (t + 1))
            tile = 4 * seg + t
            c = None
            s1, s2, s3 = _Acc(), _Acc(), _Acc()
            for i in range(NCH):
                rows = slice(RC * i, RC * (i + 1))
                h = x_v[seg, rows, cols].astype(f32) + attn[rows, cols]
                h_s[tile, rows, :] = h
                if c is None:
                    c = h[0:1]
                d = h - c
                s1.add(d)
                s2.add(d * d)
                s3.add(d * wr_s[rows, :])
            mu = s1.total() * (1.0 / D)
            var = jnp.maximum(s2.total() * (1.0 / D) - mu * mu, 0.0)
            rstd = lax.rsqrt(var + EPS)
            mean = c + mu
            st_s[tile, 0:1, :] = mean
            st_s[tile, 1:2, :] = rstd
            r_s[pl.ds(tile, 1), :] = (s3.total() - mu * wr_s[D:D + 1, :]) * rstd
            pltpu.touch(h_s)
            ga = 1.0 + rstd
            gb = mean * rstd
            for i in range(NCH):
                rows = slice(RC * i, RC * (i + 1))
                out_v[tile, rows, :] = (h_s[tile, rows, :] * ga - gb).astype(bf16)

    def transpose_wd(seg):
        nblk = F // 128 // (NSEG - 1)
        for i in range(nblk):
            c0 = pl.multiple_of((seg * nblk + i) * 128, 128)
            wd_s[pl.ds(c0, 128), :] = wdT_v[:, pl.ds(c0, 128)].T

    def project_segment():
        post_k(proj(0))
        post_v(proj(1))
        post_q(proj(2))

    with _scope("setup"):
        w_copies[0].start()
        x_copy(0).start()
        beta = beta_ref[...].astype(f32).reshape(1, H)
        hrow = lax.broadcasted_iota(jnp.int32, (8 * NW, H), 0)
        hcol = lax.broadcasted_iota(jnp.int32, (8 * NW, H), 1)
        sel = (hcol == HPW * (hrow >> 3) + (hrow & 7)) & ((hrow & 7) < HPW)
        bcol = jnp.sum(jnp.where(sel, beta, 0.0), axis=1, keepdims=True)
        g_s[...] = jnp.broadcast_to(_sigmoid(bcol), (8 * NW, 128)).reshape(NW, 8, 128)
        wr_row = wr_ref[...].astype(f32).reshape(1, D)
        wr_pad = jnp.concatenate([wr_row, jnp.zeros((1, 64), f32)], axis=1)
        wr_s[...] = jnp.broadcast_to(wr_pad, (128, D + 64)).T
        wr_s[D:D + 1, :] = jnp.broadcast_to(jnp.sum(wr_row, axis=1, keepdims=True), (1, 128))

        mt_s[...] = jnp.zeros(mt_s.shape, f32)
        vT_s[...] = jnp.zeros(vT_s.shape, u32)
        am_s[...] = jnp.zeros(am_s.shape, f32)

        w_copies[0].wait()
        w_copies[1].start()
        wT[0:D, :] = wk_v[...].T
        x_copy(0).wait()
        w_copies[2].start()
        for t in range(4):
            ln1_tile(0, t)
    with _scope("proj0"):
        w_copies[1].wait()
        w_copies[3].start()
        post_k(proj(0))
        wT[D:2 * D, :] = wv_v[...].T
        w_copies[2].wait()
        for s in range(1, NSEG):
            x_copy(s).start()
        post_v(proj(1))
        wT[2 * D:3 * D, :] = wq_v[...].T
        w_copies[3].wait()
        for c in w_copies[4:]:
            c.start()
        post_q(proj(2))
        woT[...] = wo_v[...].T
        phase_a(0, HPW, 3, 0)
        for s in range(1, NSEG):
            x_copy(s).wait()

    def segment(seg, carry):
        nseg = jnp.minimum(seg + 1, NSEG - 1)

        with _scope("windows"):
            for w in range(NW):
                if w < 4:
                    ln1_tile(nseg, w)
                window(w, _nh(w), w + 1 if w + 1 < NW else None)

        @pl.when(seg < NSEG - 1)
        def _():
            @pl.when(seg == 0)
            def _():
                w_copies[4].wait()

            with _scope("mid"):
                transpose_wd(seg)
                mem_update()
                outproj(seg)
                project_segment()
                mem_retrieve()
                phase_a(0, HPW, 3, 0)
                for t in range(4):
                    o_copy(4 * seg + t).start()
        return carry

    lax.fori_loop(0, NSEG, segment, 0)
    with _scope("last_out"):
        outproj(NSEG - 1)
        for t in range(4):
            o_copy(4 * (NSEG - 1) + t).start()

    with _scope("ffn"):
        r = r_s[...]
        rmax = jnp.max(r)
        tok = (lax.broadcasted_iota(jnp.int32, (NT, 128), 0) * 128
               + lax.broadcasted_iota(jnp.int32, (NT, 128), 1))
        idx = jnp.minimum(jnp.min(jnp.where(r == rmax, tok, S)), S - 1)
        tile = idx >> 7
        lane = idx & 127
        hn = ((h_s[tile] - st_s[tile, 0:1, :]) * st_s[tile, 1:2, :]).astype(bf16)
        onehot = jnp.where(lax.broadcasted_iota(jnp.int32, (16, 128), 1) == lane, 1.0, 0.0).astype(bf16)
        xs = lax.dot_general(onehot, hn, (((1,), (1,)), ((), ())), preferred_element_type=f32)
        for c in w_copies[5:]:
            c.wait()
        xm = xs[:, 0:512].astype(bf16)
        xr = xs[:, 512:D]
        row = lax.broadcasted_iota(jnp.int32, (16, 64), 0)
        x2 = jnp.concatenate([jnp.where(row == 0, xr, 0.0), jnp.where(row == 1, xr, 0.0)], axis=1).astype(bf16)
        wrem = jnp.concatenate([wg_v[512:D, :], wu_v[512:D, :]], axis=0)
        rem = jnp.dot(x2, wrem, preferred_element_type=f32)
        gate = jnp.dot(xm, wg_v[0:512, :], preferred_element_type=f32)[0:1] + rem[0:1]
        up = jnp.dot(xm, wu_v[0:512, :], preferred_element_type=f32)[0:1] + rem[1:2]
        act = jnp.broadcast_to(gate * _sigmoid(gate) * up, (16, F)).astype(bf16)
        y = jnp.dot(act, wd_s[...], preferred_element_type=f32)
        y = y[0:1] * _sigmoid(jnp.full((1, 1), rmax, f32))
        ypad = jnp.concatenate([y, jnp.zeros((1, 64), f32)], axis=1)
        ycol = jnp.broadcast_to(ypad, (128, D + 64)).T[0:D]
        for t in range(NT):
            o_copy(t).wait()
        lanes = lax.broadcasted_iota(jnp.int32, (D, 128), 1)
        blk = out_v[tile].astype(f32)
        out_v[tile] = jnp.where(lanes == lane, blk + ycol, blk).astype(bf16)
        fix = o_copy(tile)
        fix.start()
        fix.wait()


@jax.jit
def pallas_sequential_preLN__memory_aug_infini_attn__moe_arch_mod__prompt_kernel(
    A_x: jax.Array,
    A_wq: jax.Array,
    A_wk: jax.Array,
    A_wv: jax.Array,
    A_wo: jax.Array,
    A_beta: jax.Array,
    B_x: jax.Array,
    B_w_r: jax.Array,
    B_w_gate: jax.Array,
    B_w_up: jax.Array,
    B_w_down: jax.Array,
):
    del B_x
    xT = A_x.reshape(S, D).T
    wdT = B_w_down.T

    hbm = pl.BlockSpec(memory_space=pltpu.HBM)
    vmem = pl.BlockSpec(memory_space=pltpu.VMEM)
    scratch = [
        pltpu.VMEM((NSEG, D, L), bf16),
        pltpu.VMEM((D, D), bf16),
        pltpu.VMEM((D, D), bf16),
        pltpu.VMEM((D, D), bf16),
        pltpu.VMEM((D, D), bf16),
        pltpu.VMEM((D, F), bf16),
        pltpu.VMEM((D, F), bf16),
        pltpu.VMEM((D, F), bf16),
        pltpu.VMEM((3 * D, D), bf16),
        pltpu.VMEM((D, D), bf16),
        pltpu.VMEM((F, D), bf16),
        pltpu.VMEM((NW, 8, 128), f32),
        pltpu.VMEM((D + 64, 128), f32),
        pltpu.VMEM((4, D, 128), bf16),
        pltpu.VMEM((NW, L // 2, 128), u32),
        pltpu.VMEM((NW, 4, 64, 128), u32),
        pltpu.VMEM((NW, 4, 64, 128), u32),
        pltpu.VMEM((NW, 4, 64, 128), u32),
        pltpu.VMEM((NW, 4, MROWS // 2, 128), u32),
        pltpu.VMEM((NW, MROWS, 128), f32),
        pltpu.VMEM((NW, MROWS // 2, 128), u32),
        pltpu.VMEM((4, D + 8, 128), f32),
        pltpu.VMEM((2, L, 128 * HPW), f32),
        pltpu.VMEM((2, 8, 128 * HPW), f32),
        pltpu.VMEM((4, D, 128), f32),
        pltpu.VMEM((NT, D, 128), bf16),
        pltpu.VMEM((NT, D, 128), f32),
        pltpu.VMEM((NT, 8, 128), f32),
        pltpu.VMEM((NT, 128), f32),
        pltpu.SemaphoreType.DMA((NSEG,)),
        pltpu.SemaphoreType.DMA((7,)),
        pltpu.SemaphoreType.DMA((NT,)),
    ]
    outT = pl.pallas_call(
        _kernel,
        out_shape=jax.ShapeDtypeStruct((D, S), bf16),
        in_specs=[hbm, hbm, hbm, hbm, hbm, vmem, vmem, hbm, hbm, hbm],
        out_specs=hbm,
        scratch_shapes=scratch,
        compiler_params=pltpu.CompilerParams(vmem_limit_bytes=100 * 1024 * 1024),
    )(xT, A_wq, A_wk, A_wv, A_wo, A_beta, B_w_r, B_w_gate, B_w_up, B_w_down.T)
    return outT.T.reshape(1, S, D)
```

```python
import jax
import jax.numpy as jnp
from jax import lax
import jax.experimental.pallas as pl
import jax.experimental.pallas.tpu as pltpu

S = 2048
D = 576
H = 32
DH = 18
NSEG = 4
L = 512
NT = S // 128
F = 4608
HPW = 7
NW = 5
WL = HPW * DH
RS = 20
MROWS = 144
VWORDS = 80
QKV_ROWS = D + 64
LOG2E = 1.4426950408889634
NEG = -1e9 * LOG2E
QSCALE = (DH ** -0.5) * LOG2E
EPS = 1e-5

import contextlib
import os
_PROF = bool(os.environ.get("PROF"))


def _scope(name):
    return jax.named_scope(name) if _PROF else contextlib.nullcontext()


f32 = jnp.float32
bf16 = jnp.bfloat16
u32 = jnp.uint32


def _nh(w):
    return HPW if w < NW - 1 else H - HPW * (NW - 1)


def _pack(x):
    return pltpu.bitcast(x.astype(bf16), u32)


def _unpack(x):
    return pltpu.bitcast(x, bf16)


def _phi(t):
    return jnp.where(t > 0, t + 1.0, jnp.exp(t))


RC = 16
NCH = D // RC


class _Acc:
    def __init__(self, n=2):
        self.parts = [None] * n
        self.i = 0

    def add(self, x):
        k = self.i % len(self.parts)
        self.parts[k] = x if self.parts[k] is None else self.parts[k] + x
        self.i += 1

    def total(self):
        t = self.parts[0]
        for p in self.parts[1:]:
            t = t + p
        return jnp.sum(t, axis=0, keepdims=True)


def _ln_stats(chunk):
    x0 = chunk(0)
    c = x0[0:1]
    s1, s2 = _Acc(), _Acc()
    for i in range(NCH):
        d = (x0 if i == 0 else chunk(i)) - c
        s1.add(d)
        s2.add(d * d)
    mu = s1.total() * (1.0 / D)
    var = jnp.maximum(s2.total() * (1.0 / D) - mu * mu, 0.0)
    return c + mu, lax.rsqrt(var + EPS)


def _sigmoid(x):
    return 1.0 / (1.0 + jnp.exp(-x))


def _kernel(xT_hbm, wq_hbm, wk_hbm, wv_hbm, wo_hbm, beta_ref, wr_ref, wg_hbm, wu_hbm, wdT_hbm,
            out_hbm,
            x_v, wq_v, wk_v, wv_v, wo_v, wg_v, wu_v, wdT_v,
            wT, woT, wd_s, g_s, wr_s,
            xn_s, k_s, phikT_s, qT_s, phiqT_s, vT_s, mt_s, mtb_s, am_s,
            s_scr, m_scr, oT_s, out_v, h_s, st_s, r_s,
            sem_x, sem_w, sem_o):
    def x_copy(s):
        return pltpu.make_async_copy(xT_hbm.at[:, pl.ds(s * L, L)], x_v.at[s], sem_x.at[s])

    def o_copy(t):
        return pltpu.make_async_copy(out_v.at[t], out_hbm.at[:, pl.ds(pl.multiple_of(t * 128, 128), 128)],
                                     sem_o.at[t])

    w_copies = [pltpu.make_async_copy(src, dst, sem_w.at[i]) for i, (src, dst) in enumerate(
        [(wk_hbm, wk_v), (wv_hbm, wv_v), (wq_hbm, wq_v), (wo_hbm, wo_v),
         (wdT_hbm, wdT_v), (wg_hbm, wg_v), (wu_hbm, wu_v)])]

    def ln1_tile(seg, t):
        cols = pl.ds(pl.multiple_of(t * 128, 128), 128)

        def chunk(i):
            return x_v[seg, RC * i:RC * (i + 1), cols].astype(f32)
        mean, rstd = _ln_stats(chunk)
        pltpu.touch(x_v)
        for i in range(NCH):
            xn_s[t, RC * i:RC * (i + 1), :] = ((chunk(i) - mean) * rstd).astype(bf16)

    def proj(i):
        xn = jnp.concatenate([xn_s[t] for t in range(4)], axis=1)
        r = jnp.dot(wT[D * i:D * (i + 1), :], xn, preferred_element_type=f32)
        return jnp.concatenate([r, jnp.zeros((64, L), f32)], axis=0)

    def post_k(r):
        for t in range(4):
            for w in range(NW):
                kk = r[WL * w:WL * w + 128, 128 * t:128 * (t + 1)]
                k_s[w, 64 * t:64 * (t + 1), :] = pltpu.bitcast(kk.astype(bf16).T, u32)
                phikT_s[w, t] = _pack(_phi(kk))

    def post_v(r):
        rr = lax.broadcasted_iota(jnp.int32, (RS, 128), 0)
        ones_row = jnp.where(rr == DH, 1.0, 0.0).astype(f32)
        for t in range(4):
            for w in range(NW):
                nh = _nh(w)
                vs = [jnp.where(rr < DH,
                                r[DH * (HPW * w + a):DH * (HPW * w + a) + RS, 128 * t:128 * (t + 1)], ones_row)
                      for a in range(nh)]
                if (nh * RS) % 16:
                    vs.append(jnp.zeros((16 - (nh * RS) % 16, 128), f32))
                vv = _pack(jnp.concatenate(vs, axis=0))
                vT_s[w, t, 0:vv.shape[0], :] = vv

    def post_q(r):
        for t in range(4):
            for w in range(NW):
                q = r[WL * w:WL * w + 128, 128 * t:128 * (t + 1)]
                qT_s[w, t] = _pack(q * QSCALE)
                phiqT_s[w, t] = _pack(_phi(q))

    def mem_update():
        r = lax.broadcasted_iota(jnp.int32, (MROWS, 128), 0)
        c = lax.broadcasted_iota(jnp.int32, (MROWS, 128), 1)
        for w in range(NW):
            vt = jnp.concatenate([_unpack(vT_s[w, t, 0:MROWS // 2, :]) for t in range(4)], axis=1)
            pk = jnp.concatenate([_unpack(phikT_s[w, t]) for t in range(4)], axis=1)
            upd = lax.dot_general(vt, pk, (((1,), (1,)), ((), ())), preferred_element_type=f32)
            mt = mt_s[w] + upd
            mt_s[w] = mt
            keep = jnp.zeros((MROWS, 128), jnp.bool_)
            for a in range(_nh(w)):
                keep = keep | ((r >= RS * a) & (r < RS * (a + 1)) & (c >= DH * a) & (c < DH * (a + 1)))
            mtb_s[w] = _pack(jnp.where(keep, mt, 0.0))

    def mem_retrieve():
        for w in range(NW):
            for j in range(4):
                am = jnp.dot(_unpack(mtb_s[w]), _unpack(phiqT_s[w, j]), preferred_element_type=f32)
                for a in range(_nh(w)):
                    ama = am[RS * a:RS * a + 24]
                    g = g_s[w, a:a + 1, :]
                    om = ama * (g / (ama[DH:DH + 1] + 1e-6))
                    am_s[j, WL * w + DH * a:WL * w + DH * (a + 1), :] = om[0:DH]

    def phase_a(w, nh, j, buf):
        n = 128 * (j + 1)
        rows = lax.broadcasted_iota(jnp.int32, (64, 128), 0)
        qw = qT_s[w, j]
        qbd = jnp.concatenate(
            [jnp.where((rows >= 9 * a) & (rows < 9 * a + 9), qw, jnp.uint32(0)) for a in range(nh)], axis=1)
        s = jnp.dot(_unpack(k_s[w, 0:n // 2, :]), _unpack(qbd), preferred_element_type=f32)
        kr = lax.broadcasted_iota(jnp.int32, (128, 128), 0)
        qc = lax.broadcasted_iota(jnp.int32, (128, 128), 1)
        causal = kr <= qc
        sd = jnp.concatenate(
            [jnp.where(causal, s[n - 128:n, 128 * a:128 * (a + 1)], NEG) for a in range(nh)], axis=1)
        s_scr[buf, n - 128:n, 0:128 * nh] = sd
        m = jnp.max(sd, axis=0, keepdims=True)
        if j > 0:
            s_scr[buf, 0:n - 128, 0:128 * nh] = s[0:n - 128]
            m = jnp.maximum(m, jnp.max(s[0:n - 128], axis=0, keepdims=True))
        m_scr[buf, :, 0:128 * nh] = jnp.broadcast_to(m, (8, 128 * nh))

    def phase_b(w, nh, j, buf):
        n = 128 * (j + 1)
        for a in range(nh):
            m = m_scr[buf, 0:1, 128 * a:128 * (a + 1)]
            p = jnp.exp2(s_scr[buf, 0:n, 128 * a:128 * (a + 1)] - m).astype(bf16)
            vt = jnp.concatenate([_unpack(vT_s[w, t, (RS // 2) * a:(RS // 2) * a + 16, :]) for t in range(j + 1)], axis=1)
            o = jnp.dot(vt, p, preferred_element_type=f32)
            g = g_s[w, a:a + 1, :]
            od = o[0:24] * ((1.0 - g) / o[DH:DH + 1])
            row0 = WL * w + DH * a
            oT_s[j, pl.ds(row0, DH), :] = (od + am_s[j, pl.ds(row0, 24), :])[0:DH]

    def window(w, nh, nxt):
        order = [3, 2, 1, 0]
        for t in range(4):
            if t < 3:
                phase_a(w, nh, order[t + 1], (t + 1) % 2)
            elif nxt is not None:
                phase_a(nxt, _nh(nxt), order[0], 0)
            phase_b(w, nh, order[t], t % 2)

    def outproj(seg):
        oT = jnp.concatenate([oT_s[t] for t in range(4)], axis=1).astype(bf16)
        attn = jnp.dot(woT[...], oT, preferred_element_type=f32)
        for t in range(4):
            cols = slice(128 * t, 128 * (t + 1))
            tile = 4 * seg + t
            c = None
            s1, s2, s3 = _Acc(), _Acc(), _Acc()
            for i in range(NCH):
                rows = slice(RC * i, RC * (i + 1))
                h = x_v[seg, rows, cols].astype(f32) + attn[rows, cols]
                h_s[tile, rows, :] = h
                if c is None:
                    c = h[0:1]
                d = h - c
                s1.add(d)
                s2.add(d * d)
                s3.add(d * wr_s[rows, :])
            mu = s1.total() * (1.0 / D)
            var = jnp.maximum(s2.total() * (1.0 / D) - mu * mu, 0.0)
            rstd = lax.rsqrt(var + EPS)
            mean = c + mu
            st_s[tile, 0:1, :] = mean
            st_s[tile, 1:2, :] = rstd
            r_s[pl.ds(tile, 1), :] = (s3.total() - mu * wr_s[D:D + 1, :]) * rstd
            pltpu.touch(h_s)
            ga = 1.0 + rstd
            gb = mean * rstd
            for i in range(NCH):
                rows = slice(RC * i, RC * (i + 1))
                out_v[tile, rows, :] = (h_s[tile, rows, :] * ga - gb).astype(bf16)

    def transpose_wd(seg):
        nblk = F // 128 // (NSEG - 1)
        for i in range(nblk):
            c0 = pl.multiple_of((seg * nblk + i) * 128, 128)
            wd_s[pl.ds(c0, 128), :] = wdT_v[:, pl.ds(c0, 128)].T

    def project_segment():
        post_k(proj(0))
        post_v(proj(1))
        post_q(proj(2))

    with _scope("setup"):
        w_copies[0].start()
        x_copy(0).start()
        beta = beta_ref[...].astype(f32).reshape(1, H)
        hrow = lax.broadcasted_iota(jnp.int32, (8 * NW, H), 0)
        hcol = lax.broadcasted_iota(jnp.int32, (8 * NW, H), 1)
        sel = (hcol == HPW * (hrow >> 3) + (hrow & 7)) & ((hrow & 7) < HPW)
        bcol = jnp.sum(jnp.where(sel, beta, 0.0), axis=1, keepdims=True)
        g_s[...] = jnp.broadcast_to(_sigmoid(bcol), (8 * NW, 128)).reshape(NW, 8, 128)
        wr_row = wr_ref[...].astype(f32).reshape(1, D)
        wr_pad = jnp.concatenate([wr_row, jnp.zeros((1, 64), f32)], axis=1)
        wr_s[...] = jnp.broadcast_to(wr_pad, (128, D + 64)).T
        wr_s[D:D + 1, :] = jnp.broadcast_to(jnp.sum(wr_row, axis=1, keepdims=True), (1, 128))

        mt_s[...] = jnp.zeros(mt_s.shape, f32)
        vT_s[...] = jnp.zeros(vT_s.shape, u32)
        am_s[...] = jnp.zeros(am_s.shape, f32)

        w_copies[0].wait()
        w_copies[1].start()
        wT[0:D, :] = wk_v[...].T
        x_copy(0).wait()
        w_copies[2].start()
        for t in range(4):
            ln1_tile(0, t)
    with _scope("proj0"):
        w_copies[1].wait()
        w_copies[3].start()
        post_k(proj(0))
        wT[D:2 * D, :] = wv_v[...].T
        w_copies[2].wait()
        for s in range(1, NSEG):
            x_copy(s).start()
        post_v(proj(1))
        wT[2 * D:3 * D, :] = wq_v[...].T
        w_copies[3].wait()
        for c in w_copies[4:]:
            c.start()
        post_q(proj(2))
        woT[...] = wo_v[...].T
        phase_a(0, HPW, 3, 0)
        for s in range(1, NSEG):
            x_copy(s).wait()

    def segment(seg, carry):
        nseg = jnp.minimum(seg + 1, NSEG - 1)

        with _scope("windows"):
            for w in range(NW):
                if w < 4:
                    ln1_tile(nseg, w)
                window(w, _nh(w), w + 1 if w + 1 < NW else None)

        @pl.when(seg < NSEG - 1)
        def _():
            @pl.when(seg == 0)
            def _():
                w_copies[4].wait()

            with _scope("mid"):
                transpose_wd(seg)
                mem_update()
                outproj(seg)
                project_segment()
                mem_retrieve()
                phase_a(0, HPW, 3, 0)
                for t in range(4):
                    o_copy(4 * seg + t).start()
        return carry

    lax.fori_loop(0, NSEG, segment, 0)
    with _scope("last_out"):
        outproj(NSEG - 1)
        for t in range(4):
            o_copy(4 * (NSEG - 1) + t).start()

    with _scope("ffn"):
        r = r_s[...]
        rmax = jnp.max(r)
        tok = (lax.broadcasted_iota(jnp.int32, (NT, 128), 0) * 128
               + lax.broadcasted_iota(jnp.int32, (NT, 128), 1))
        idx = jnp.minimum(jnp.min(jnp.where(r == rmax, tok, S)), S - 1)
        tile = idx >> 7
        lane = idx & 127
        hn = ((h_s[tile] - st_s[tile, 0:1, :]) * st_s[tile, 1:2, :]).astype(bf16)
        onehot = jnp.where(lax.broadcasted_iota(jnp.int32, (16, 128), 1) == lane, 1.0, 0.0).astype(bf16)
        xs = lax.dot_general(onehot, hn, (((1,), (1,)), ((), ())), preferred_element_type=f32)
        for c in w_copies[5:]:
            c.wait()
        xm = xs[:, 0:512].astype(bf16)
        xr = xs[:, 512:D]
        row = lax.broadcasted_iota(jnp.int32, (16, 64), 0)
        x2 = jnp.concatenate([jnp.where(row == 0, xr, 0.0), jnp.where(row == 1, xr, 0.0)], axis=1).astype(bf16)
        wrem = jnp.concatenate([wg_v[512:D, :], wu_v[512:D, :]], axis=0)
        rem = jnp.dot(x2, wrem, preferred_element_type=f32)
        gate = jnp.dot(xm, wg_v[0:512, :], preferred_element_type=f32)[0:1] + rem[0:1]
        up = jnp.dot(xm, wu_v[0:512, :], preferred_element_type=f32)[0:1] + rem[1:2]
        act = jnp.broadcast_to(gate * _sigmoid(gate) * up, (16, F)).astype(bf16)
        y = jnp.dot(act, wd_s[...], preferred_element_type=f32)
        y = y[0:1] * _sigmoid(jnp.full((1, 1), rmax, f32))
        ypad = jnp.concatenate([y, jnp.zeros((1, 64), f32)], axis=1)
        ycol = jnp.broadcast_to(ypad, (128, D + 64)).T[0:D]
        for t in range(NT):
            o_copy(t).wait()
        lanes = lax.broadcasted_iota(jnp.int32, (D, 128), 1)
        blk = out_v[tile].astype(f32)
        out_v[tile] = jnp.where(lanes == lane, blk + ycol, blk).astype(bf16)
        fix = o_copy(tile)
        fix.start()
        fix.wait()


@jax.jit
def pallas_sequential_preLN__memory_aug_infini_attn__moe_arch_mod__prompt_kernel(
    A_x: jax.Array,
    A_wq: jax.Array,
    A_wk: jax.Array,
    A_wv: jax.Array,
    A_wo: jax.Array,
    A_beta: jax.Array,
    B_x: jax.Array,
    B_w_r: jax.Array,
    B_w_gate: jax.Array,
    B_w_up: jax.Array,
    B_w_down: jax.Array,
):
    del B_x
    xT = A_x.reshape(S, D).T
    wdT = B_w_down.T

    hbm = pl.BlockSpec(memory_space=pltpu.HBM)
    vmem = pl.BlockSpec(memory_space=pltpu.VMEM)
    scratch = [
        pltpu.VMEM((NSEG, D, L), bf16),
        pltpu.VMEM((D, D), bf16),
        pltpu.VMEM((D, D), bf16),
        pltpu.VMEM((D, D), bf16),
        pltpu.VMEM((D, D), bf16),
        pltpu.VMEM((D, F), bf16),
        pltpu.VMEM((D, F), bf16),
        pltpu.VMEM((D, F), bf16),
        pltpu.VMEM((3 * D, D), bf16),
        pltpu.VMEM((D, D), bf16),
        pltpu.VMEM((F, D), bf16),
        pltpu.VMEM((NW, 8, 128), f32),
        pltpu.VMEM((D + 64, 128), f32),
        pltpu.VMEM((4, D, 128), bf16),
        pltpu.VMEM((NW, L // 2, 128), u32),
        pltpu.VMEM((NW, 4, 64, 128), u32),
        pltpu.VMEM((NW, 4, 64, 128), u32),
        pltpu.VMEM((NW, 4, 64, 128), u32),
        pltpu.VMEM((NW, 4, VWORDS, 128), u32),
        pltpu.VMEM((NW, MROWS, 128), f32),
        pltpu.VMEM((NW, MROWS // 2, 128), u32),
        pltpu.VMEM((4, D + 8, 128), f32),
        pltpu.VMEM((2, L, 128 * HPW), f32),
        pltpu.VMEM((2, 8, 128 * HPW), f32),
        pltpu.VMEM((4, D, 128), f32),
        pltpu.VMEM((NT, D, 128), bf16),
        pltpu.VMEM((NT, D, 128), f32),
        pltpu.VMEM((NT, 8, 128), f32),
        pltpu.VMEM((NT, 128), f32),
        pltpu.SemaphoreType.DMA((NSEG,)),
        pltpu.SemaphoreType.DMA((7,)),
        pltpu.SemaphoreType.DMA((NT,)),
    ]
    outT = pl.pallas_call(
        _kernel,
        out_shape=jax.ShapeDtypeStruct((D, S), bf16),
        in_specs=[hbm, hbm, hbm, hbm, hbm, vmem, vmem, hbm, hbm, hbm],
        out_specs=hbm,
        scratch_shapes=scratch,
        compiler_params=pltpu.CompilerParams(vmem_limit_bytes=100 * 1024 * 1024),
    )(xT, A_wq, A_wk, A_wv, A_wo, A_beta, B_w_r, B_w_gate, B_w_up, B_w_down.T)
    return outT.T.reshape(1, S, D)
```

```python
import jax
import jax.numpy as jnp
from jax import lax
import jax.experimental.pallas as pl
import jax.experimental.pallas.tpu as pltpu

S = 2048
D = 576
H = 32
DH = 18
NSEG = 4
L = 512
NT = S // 128
F = 4608
HPW = 7
NW = 5
WL = HPW * DH
RS = 20
MROWS = 144
VWORDS = 80
QKV_ROWS = D + 64
LOG2E = 1.4426950408889634
NEG = -1e9 * LOG2E
QSCALE = (DH ** -0.5) * LOG2E
EPS = 1e-5

import contextlib
import os
_PROF = bool(os.environ.get("PROF"))


def _scope(name):
    return jax.named_scope(name) if _PROF else contextlib.nullcontext()


f32 = jnp.float32
bf16 = jnp.bfloat16
u32 = jnp.uint32


def _nh(w):
    return HPW if w < NW - 1 else H - HPW * (NW - 1)


def _pack(x):
    return pltpu.bitcast(x.astype(bf16), u32)


def _unpack(x):
    return pltpu.bitcast(x, bf16)


def _phi(t):
    return jnp.where(t > 0, t + 1.0, jnp.exp(t))


RC = 16
NCH = D // RC


class _Acc:
    def __init__(self, n=2):
        self.parts = [None] * n
        self.i = 0

    def add(self, x):
        k = self.i % len(self.parts)
        self.parts[k] = x if self.parts[k] is None else self.parts[k] + x
        self.i += 1

    def total(self):
        t = self.parts[0]
        for p in self.parts[1:]:
            t = t + p
        return jnp.sum(t, axis=0, keepdims=True)


def _ln_stats(chunk):
    x0 = chunk(0)
    c = x0[0:1]
    s1, s2 = _Acc(), _Acc()
    for i in range(NCH):
        d = (x0 if i == 0 else chunk(i)) - c
        s1.add(d)
        s2.add(d * d)
    mu = s1.total() * (1.0 / D)
    var = jnp.maximum(s2.total() * (1.0 / D) - mu * mu, 0.0)
    return c + mu, lax.rsqrt(var + EPS)


def _sigmoid(x):
    return 1.0 / (1.0 + jnp.exp(-x))


def _kernel(xT_hbm, wq_hbm, wk_hbm, wv_hbm, wo_hbm, beta_ref, wr_ref, wg_hbm, wu_hbm, wdT_hbm,
            out_hbm,
            x_v, wq_v, wk_v, wv_v, wo_v, wg_v, wu_v, wdT_v,
            wT, woT, wd_s, g_s, wr_s,
            xn_s, k_s, phikT_s, qT_s, phiqT_s, vT_s, mt_s, mtb_s, am_s,
            s_scr, m_scr, oT_s, out_v, h_s, st_s, r_s,
            sem_x, sem_w, sem_o):
    def x_copy(s):
        return pltpu.make_async_copy(xT_hbm.at[:, pl.ds(s * L, L)], x_v.at[s], sem_x.at[s])

    def o_copy(t):
        return pltpu.make_async_copy(out_v.at[t], out_hbm.at[:, pl.ds(pl.multiple_of(t * 128, 128), 128)],
                                     sem_o.at[t])

    w_copies = [pltpu.make_async_copy(src, dst, sem_w.at[i]) for i, (src, dst) in enumerate(
        [(wk_hbm, wk_v), (wq_hbm, wq_v), (wv_hbm, wv_v), (wo_hbm, wo_v),
         (wdT_hbm, wdT_v), (wg_hbm, wg_v), (wu_hbm, wu_v)])]

    def ln1_tile(seg, t):
        cols = pl.ds(pl.multiple_of(t * 128, 128), 128)

        def chunk(i):
            return x_v[seg, RC * i:RC * (i + 1), cols].astype(f32)
        mean, rstd = _ln_stats(chunk)
        for i in range(NCH):
            xn_s[t, RC * i:RC * (i + 1), :] = ((chunk(i) - mean) * rstd).astype(bf16)

    def proj(i):
        xn = jnp.concatenate([xn_s[t] for t in range(4)], axis=1)
        r = jnp.dot(wT[D * i:D * (i + 1), :], xn, preferred_element_type=f32)
        return jnp.concatenate([r, jnp.zeros((64, L), f32)], axis=0)

    def post_k(r):
        for t in range(4):
            for w in range(NW):
                kk = r[WL * w:WL * w + 128, 128 * t:128 * (t + 1)]
                k_s[w, 64 * t:64 * (t + 1), :] = pltpu.bitcast(kk.astype(bf16).T, u32)
                phikT_s[w, t] = _pack(_phi(kk))

    def post_v(r):
        rr = lax.broadcasted_iota(jnp.int32, (RS, 128), 0)
        ones_row = jnp.where(rr == DH, 1.0, 0.0).astype(f32)
        for t in range(4):
            for w in range(NW):
                nh = _nh(w)
                vs = [jnp.where(rr < DH,
                                r[DH * (HPW * w + a):DH * (HPW * w + a) + RS, 128 * t:128 * (t + 1)], ones_row)
                      for a in range(nh)]
                if (nh * RS) % 16:
                    vs.append(jnp.zeros((16 - (nh * RS) % 16, 128), f32))
                vv = _pack(jnp.concatenate(vs, axis=0))
                vT_s[w, t, 0:vv.shape[0], :] = vv

    def post_q(r):
        for t in range(4):
            for w in range(NW):
                q = r[WL * w:WL * w + 128, 128 * t:128 * (t + 1)]
                qT_s[w, t] = _pack(q * QSCALE)
                phiqT_s[w, t] = _pack(_phi(q))

    def mem_update():
        r = lax.broadcasted_iota(jnp.int32, (MROWS, 128), 0)
        c = lax.broadcasted_iota(jnp.int32, (MROWS, 128), 1)
        for w in range(NW):
            vt = jnp.concatenate([_unpack(vT_s[w, t, 0:MROWS // 2, :]) for t in range(4)], axis=1)
            pk = jnp.concatenate([_unpack(phikT_s[w, t]) for t in range(4)], axis=1)
            upd = lax.dot_general(vt, pk, (((1,), (1,)), ((), ())), preferred_element_type=f32)
            mt = mt_s[w] + upd
            mt_s[w] = mt
            keep = jnp.zeros((MROWS, 128), jnp.bool_)
            for a in range(_nh(w)):
                keep = keep | ((r >= RS * a) & (r < RS * (a + 1)) & (c >= DH * a) & (c < DH * (a + 1)))
            mtb_s[w] = _pack(jnp.where(keep, mt, 0.0))

    def mem_retrieve():
        for w in range(NW):
            for j in range(4):
                am = jnp.dot(_unpack(mtb_s[w]), _unpack(phiqT_s[w, j]), preferred_element_type=f32)
                for a in range(_nh(w)):
                    ama = am[RS * a:RS * a + 24]
                    g = g_s[w, a:a + 1, :]
                    om = ama * (g / (ama[DH:DH + 1] + 1e-6))
                    am_s[j, WL * w + DH * a:WL * w + DH * (a + 1), :] = om[0:DH]

    def phase_a(w, nh, j, buf):
        n = 128 * (j + 1)
        rows = lax.broadcasted_iota(jnp.int32, (64, 128), 0)
        qw = qT_s[w, j]
        qbd = jnp.concatenate(
            [jnp.where((rows >= 9 * a) & (rows < 9 * a + 9), qw, jnp.uint32(0)) for a in range(nh)], axis=1)
        s = jnp.dot(_unpack(k_s[w, 0:n // 2, :]), _unpack(qbd), preferred_element_type=f32)
        kr = lax.broadcasted_iota(jnp.int32, (128, 128), 0)
        qc = lax.broadcasted_iota(jnp.int32, (128, 128), 1)
        causal = kr <= qc
        sd = jnp.concatenate(
            [jnp.where(causal, s[n - 128:n, 128 * a:128 * (a + 1)], NEG) for a in range(nh)], axis=1)
        s_scr[buf, n - 128:n, 0:128 * nh] = sd
        m = jnp.max(sd, axis=0, keepdims=True)
        if j > 0:
            s_scr[buf, 0:n - 128, 0:128 * nh] = s[0:n - 128]
            m = jnp.maximum(m, jnp.max(s[0:n - 128], axis=0, keepdims=True))
        m_scr[buf, :, 0:128 * nh] = jnp.broadcast_to(m, (8, 128 * nh))

    def phase_b(w, nh, j, buf):
        n = 128 * (j + 1)
        for a in range(nh):
            m = m_scr[buf, 0:1, 128 * a:128 * (a + 1)]
            p = jnp.exp2(s_scr[buf, 0:n, 128 * a:128 * (a + 1)] - m).astype(bf16)
            vt = jnp.concatenate([_unpack(vT_s[w, t, (RS // 2) * a:(RS // 2) * a + 16, :]) for t in range(j + 1)], axis=1)
            o = jnp.dot(vt, p, preferred_element_type=f32)
            g = g_s[w, a:a + 1, :]
            od = o[0:24] * ((1.0 - g) / o[DH:DH + 1])
            row0 = WL * w + DH * a
            oT_s[j, pl.ds(row0, DH), :] = (od + am_s[j, pl.ds(row0, 24), :])[0:DH]

    def window(w, nh, nxt):
        order = [3, 2, 1, 0]
        for t in range(4):
            if t < 3:
                phase_a(w, nh, order[t + 1], (t + 1) % 2)
            elif nxt is not None:
                phase_a(nxt, _nh(nxt), order[0], 0)
            phase_b(w, nh, order[t], t % 2)

    def outproj(seg):
        oT = jnp.concatenate([oT_s[t] for t in range(4)], axis=1).astype(bf16)
        attn = jnp.dot(woT[...], oT, preferred_element_type=f32)
        for t in range(4):
            cols = slice(128 * t, 128 * (t + 1))
            tile = 4 * seg + t
            c = None
            s1, s2, s3 = _Acc(), _Acc(), _Acc()
            for i in range(NCH):
                rows = slice(RC * i, RC * (i + 1))
                h = x_v[seg, rows, cols].astype(f32) + attn[rows, cols]
                h_s[tile, rows, :] = h
                if c is None:
                    c = h[0:1]
                d = h - c
                s1.add(d)
                s2.add(d * d)
                s3.add(d * wr_s[rows, :])
            mu = s1.total() * (1.0 / D)
            var = jnp.maximum(s2.total() * (1.0 / D) - mu * mu, 0.0)
            rstd = lax.rsqrt(var + EPS)
            mean = c + mu
            st_s[tile, 0:1, :] = mean
            st_s[tile, 1:2, :] = rstd
            r_s[pl.ds(tile, 1), :] = (s3.total() - mu * wr_s[D:D + 1, :]) * rstd
            ga = 1.0 + rstd
            gb = mean * rstd
            for i in range(NCH):
                rows = slice(RC * i, RC * (i + 1))
                out_v[tile, rows, :] = (h_s[tile, rows, :] * ga - gb).astype(bf16)

    def transpose_wd(seg):
        nblk = F // 128 // (NSEG - 1)
        for i in range(nblk):
            c0 = pl.multiple_of((seg * nblk + i) * 128, 128)
            wd_s[pl.ds(c0, 128), :] = wdT_v[:, pl.ds(c0, 128)].T

    def project_segment():
        post_k(proj(0))
        post_q(proj(1))
        post_v(proj(2))

    with _scope("setup"):
        w_copies[0].start()
        x_copy(0).start()
        beta = beta_ref[...].astype(f32).reshape(1, H)
        hrow = lax.broadcasted_iota(jnp.int32, (8 * NW, H), 0)
        hcol = lax.broadcasted_iota(jnp.int32, (8 * NW, H), 1)
        sel = (hcol == HPW * (hrow >> 3) + (hrow & 7)) & ((hrow & 7) < HPW)
        bcol = jnp.sum(jnp.where(sel, beta, 0.0), axis=1, keepdims=True)
        g_s[...] = jnp.broadcast_to(_sigmoid(bcol), (8 * NW, 128)).reshape(NW, 8, 128)
        wr_row = wr_ref[...].astype(f32).reshape(1, D)
        wr_pad = jnp.concatenate([wr_row, jnp.zeros((1, 64), f32)], axis=1)
        wr_s[...] = jnp.broadcast_to(wr_pad, (128, D + 64)).T
        wr_s[D:D + 1, :] = jnp.broadcast_to(jnp.sum(wr_row, axis=1, keepdims=True), (1, 128))

        mt_s[...] = jnp.zeros(mt_s.shape, f32)
        vT_s[...] = jnp.zeros(vT_s.shape, u32)
        am_s[...] = jnp.zeros(am_s.shape, f32)

        w_copies[0].wait()
        w_copies[1].start()
        wT[0:D, :] = wk_v[...].T
        x_copy(0).wait()
        w_copies[2].start()
        for t in range(4):
            ln1_tile(0, t)
    with _scope("proj0"):
        w_copies[1].wait()
        w_copies[3].start()
        post_k(proj(0))
        wT[D:2 * D, :] = wq_v[...].T
        w_copies[2].wait()
        for s in range(1, NSEG):
            x_copy(s).start()
        post_q(proj(1))
        wT[2 * D:3 * D, :] = wv_v[...].T
        w_copies[3].wait()
        for c in w_copies[4:]:
            c.start()
        post_v(proj(2))
        woT[...] = wo_v[...].T
        phase_a(0, HPW, 3, 0)
        for s in range(1, NSEG):
            x_copy(s).wait()

    def segment(seg, carry):
        nseg = jnp.minimum(seg + 1, NSEG - 1)

        with _scope("windows"):
            for w in range(NW):
                if w < 4:
                    ln1_tile(nseg, w)
                window(w, _nh(w), w + 1 if w + 1 < NW else None)

        @pl.when(seg < NSEG - 1)
        def _():
            @pl.when(seg == 0)
            def _():
                w_copies[4].wait()

            with _scope("mid"):
                transpose_wd(seg)
                mem_update()
                outproj(seg)
                project_segment()
                mem_retrieve()
                phase_a(0, HPW, 3, 0)
                for t in range(4):
                    o_copy(4 * seg + t).start()
        return carry

    lax.fori_loop(0, NSEG, segment, 0)
    with _scope("last_out"):
        outproj(NSEG - 1)
        for t in range(4):
            o_copy(4 * (NSEG - 1) + t).start()

    with _scope("ffn"):
        r = r_s[...]
        rmax = jnp.max(r)
        tok = (lax.broadcasted_iota(jnp.int32, (NT, 128), 0) * 128
               + lax.broadcasted_iota(jnp.int32, (NT, 128), 1))
        idx = jnp.minimum(jnp.min(jnp.where(r == rmax, tok, S)), S - 1)
        tile = idx >> 7
        lane = idx & 127
        hn = ((h_s[tile] - st_s[tile, 0:1, :]) * st_s[tile, 1:2, :]).astype(bf16)
        onehot = jnp.where(lax.broadcasted_iota(jnp.int32, (16, 128), 1) == lane, 1.0, 0.0).astype(bf16)
        xs = lax.dot_general(onehot, hn, (((1,), (1,)), ((), ())), preferred_element_type=f32)
        for c in w_copies[5:]:
            c.wait()
        xm = xs[:, 0:512].astype(bf16)
        xr = xs[:, 512:D]
        row = lax.broadcasted_iota(jnp.int32, (16, 64), 0)
        x2 = jnp.concatenate([jnp.where(row == 0, xr, 0.0), jnp.where(row == 1, xr, 0.0)], axis=1).astype(bf16)
        wrem = jnp.concatenate([wg_v[512:D, :], wu_v[512:D, :]], axis=0)
        rem = jnp.dot(x2, wrem, preferred_element_type=f32)
        gate = jnp.dot(xm, wg_v[0:512, :], preferred_element_type=f32)[0:1] + rem[0:1]
        up = jnp.dot(xm, wu_v[0:512, :], preferred_element_type=f32)[0:1] + rem[1:2]
        act = jnp.broadcast_to(gate * _sigmoid(gate) * up, (16, F)).astype(bf16)
        y = jnp.dot(act, wd_s[...], preferred_element_type=f32)
        y = y[0:1] * _sigmoid(jnp.full((1, 1), rmax, f32))
        ypad = jnp.concatenate([y, jnp.zeros((1, 64), f32)], axis=1)
        ycol = jnp.broadcast_to(ypad, (128, D + 64)).T[0:D]
        for t in range(NT):
            o_copy(t).wait()
        lanes = lax.broadcasted_iota(jnp.int32, (D, 128), 1)
        blk = out_v[tile].astype(f32)
        out_v[tile] = jnp.where(lanes == lane, blk + ycol, blk).astype(bf16)
        fix = o_copy(tile)
        fix.start()
        fix.wait()


@jax.jit
def pallas_sequential_preLN__memory_aug_infini_attn__moe_arch_mod__prompt_kernel(
    A_x: jax.Array,
    A_wq: jax.Array,
    A_wk: jax.Array,
    A_wv: jax.Array,
    A_wo: jax.Array,
    A_beta: jax.Array,
    B_x: jax.Array,
    B_w_r: jax.Array,
    B_w_gate: jax.Array,
    B_w_up: jax.Array,
    B_w_down: jax.Array,
):
    del B_x
    xT = A_x.reshape(S, D).T
    wdT = B_w_down.T

    hbm = pl.BlockSpec(memory_space=pltpu.HBM)
    vmem = pl.BlockSpec(memory_space=pltpu.VMEM)
    scratch = [
        pltpu.VMEM((NSEG, D, L), bf16),
        pltpu.VMEM((D, D), bf16),
        pltpu.VMEM((D, D), bf16),
        pltpu.VMEM((D, D), bf16),
        pltpu.VMEM((D, D), bf16),
        pltpu.VMEM((D, F), bf16),
        pltpu.VMEM((D, F), bf16),
        pltpu.VMEM((D, F), bf16),
        pltpu.VMEM((3 * D, D), bf16),
        pltpu.VMEM((D, D), bf16),
        pltpu.VMEM((F, D), bf16),
        pltpu.VMEM((NW, 8, 128), f32),
        pltpu.VMEM((D + 64, 128), f32),
        pltpu.VMEM((4, D, 128), bf16),
        pltpu.VMEM((NW, L // 2, 128), u32),
        pltpu.VMEM((NW, 4, 64, 128), u32),
        pltpu.VMEM((NW, 4, 64, 128), u32),
        pltpu.VMEM((NW, 4, 64, 128), u32),
        pltpu.VMEM((NW, 4, VWORDS, 128), u32),
        pltpu.VMEM((NW, MROWS, 128), f32),
        pltpu.VMEM((NW, MROWS // 2, 128), u32),
        pltpu.VMEM((4, D + 8, 128), f32),
        pltpu.VMEM((2, L, 128 * HPW), f32),
        pltpu.VMEM((2, 8, 128 * HPW), f32),
        pltpu.VMEM((4, D, 128), f32),
        pltpu.VMEM((NT, D, 128), bf16),
        pltpu.VMEM((NT, D, 128), f32),
        pltpu.VMEM((NT, 8, 128), f32),
        pltpu.VMEM((NT, 128), f32),
        pltpu.SemaphoreType.DMA((NSEG,)),
        pltpu.SemaphoreType.DMA((7,)),
        pltpu.SemaphoreType.DMA((NT,)),
    ]
    outT = pl.pallas_call(
        _kernel,
        out_shape=jax.ShapeDtypeStruct((D, S), bf16),
        in_specs=[hbm, hbm, hbm, hbm, hbm, vmem, vmem, hbm, hbm, hbm],
        out_specs=hbm,
        scratch_shapes=scratch,
        compiler_params=pltpu.CompilerParams(vmem_limit_bytes=100 * 1024 * 1024),
    )(xT, A_wq, A_wk, A_wv, A_wo, A_beta, B_w_r, B_w_gate, B_w_up, B_w_down.T)
    return outT.T.reshape(1, S, D)
```

```python
import jax
import jax.numpy as jnp
from jax import lax
import jax.experimental.pallas as pl
import jax.experimental.pallas.tpu as pltpu

S = 2048
D = 576
H = 32
DH = 18
NSEG = 4
L = 512
NT = S // 128
F = 4608
HPW = 7
NW = 5
WL = HPW * DH
RS = 20
MROWS = 144
VWORDS = 80
QKV_ROWS = D + 64
LOG2E = 1.4426950408889634
NEG = -1e9 * LOG2E
QSCALE = (DH ** -0.5) * LOG2E
EPS = 1e-5
KSPLIT = int(__import__('os').environ.get('KSPLIT', '288'))
import os
MID_ORDER = os.environ.get('MID_ORDER', 'uokqvra')
WFILL = int(os.environ.get('WFILL', '0'))

import contextlib
import os
_PROF = bool(os.environ.get("PROF"))


def _scope(name):
    return jax.named_scope(name) if _PROF else contextlib.nullcontext()


f32 = jnp.float32
bf16 = jnp.bfloat16
u32 = jnp.uint32


def _nh(w):
    return HPW if w < NW - 1 else H - HPW * (NW - 1)


def _pack(x):
    return pltpu.bitcast(x.astype(bf16), u32)


def _unpack(x):
    return pltpu.bitcast(x, bf16)


def _phi(t):
    return jnp.where(t > 0, t + 1.0, jnp.exp(t))


RC = 16
NCH = D // RC


class _Acc:
    def __init__(self, n=2):
        self.parts = [None] * n
        self.i = 0

    def add(self, x):
        k = self.i % len(self.parts)
        self.parts[k] = x if self.parts[k] is None else self.parts[k] + x
        self.i += 1

    def total(self):
        t = self.parts[0]
        for p in self.parts[1:]:
            t = t + p
        return jnp.sum(t, axis=0, keepdims=True)


def _ln_stats(chunk):
    x0 = chunk(0)
    c = x0[0:1]
    s1, s2 = _Acc(), _Acc()
    for i in range(NCH):
        d = (x0 if i == 0 else chunk(i)) - c
        s1.add(d)
        s2.add(d * d)
    mu = s1.total() * (1.0 / D)
    var = jnp.maximum(s2.total() * (1.0 / D) - mu * mu, 0.0)
    return c + mu, lax.rsqrt(var + EPS)


def _sigmoid(x):
    return 1.0 / (1.0 + jnp.exp(-x))


def _kernel(xT_hbm, wq_hbm, wk_hbm, wv_hbm, wo_hbm, beta_ref, wr_ref, wg_hbm, wu_hbm, wdT_hbm,
            out_hbm,
            x_v, wq_v, wk_v, wv_v, wo_v, wg_v, wu_v, wdT_v,
            wT, woT, wd_s, g_s, wr_s,
            xn_s, k_s, phikT_s, qT_s, phiqT_s, vT_s, mt_s, mtb_s, am_s,
            s_scr, m_scr, oT_s, out_v, h_s, st_s, r_s,
            sem_x, sem_w, sem_o):
    def x_copy(s):
        return pltpu.make_async_copy(xT_hbm.at[:, pl.ds(s * L, L)], x_v.at[s], sem_x.at[s])

    def o_copy(t):
        return pltpu.make_async_copy(out_v.at[t], out_hbm.at[:, pl.ds(pl.multiple_of(t * 128, 128), 128)],
                                     sem_o.at[t])

    w_copies = [pltpu.make_async_copy(src, dst, sem_w.at[i]) for i, (src, dst) in enumerate(
        [(wk_hbm, wk_v), (wq_hbm, wq_v), (wv_hbm, wv_v), (wo_hbm, wo_v),
         (wdT_hbm, wdT_v), (wg_hbm, wg_v), (wu_hbm, wu_v)])]

    def ln1_tile(seg, t):
        cols = pl.ds(pl.multiple_of(t * 128, 128), 128)

        def chunk(i):
            return x_v[seg, RC * i:RC * (i + 1), cols].astype(f32)
        mean, rstd = _ln_stats(chunk)
        for i in range(NCH):
            xn_s[t, RC * i:RC * (i + 1), :] = ((chunk(i) - mean) * rstd).astype(bf16)

    def proj_rows(lo, hi):
        xn = jnp.concatenate([xn_s[t] for t in range(4)], axis=1)
        return jnp.dot(wT[lo:hi, :], xn, preferred_element_type=f32)

    def proj(i, head=None):
        lo = D * i if head is None else D * i + head.shape[0]
        parts = [] if head is None else [head]
        parts += [proj_rows(lo, D * (i + 1)), jnp.zeros((64, L), f32)]
        return jnp.concatenate(parts, axis=0)

    def post_k(r):
        for t in range(4):
            for w in range(NW):
                kk = r[WL * w:WL * w + 128, 128 * t:128 * (t + 1)]
                k_s[w, 64 * t:64 * (t + 1), :] = pltpu.bitcast(kk.astype(bf16).T, u32)
                phikT_s[w, t] = _pack(_phi(kk))

    def post_v(r):
        rr = lax.broadcasted_iota(jnp.int32, (RS, 128), 0)
        ones_row = jnp.where(rr == DH, 1.0, 0.0).astype(f32)
        for t in range(4):
            for w in range(NW):
                nh = _nh(w)
                vs = [jnp.where(rr < DH,
                                r[DH * (HPW * w + a):DH * (HPW * w + a) + RS, 128 * t:128 * (t + 1)], ones_row)
                      for a in range(nh)]
                if (nh * RS) % 16:
                    vs.append(jnp.zeros((16 - (nh * RS) % 16, 128), f32))
                vv = _pack(jnp.concatenate(vs, axis=0))
                vT_s[w, t, 0:vv.shape[0], :] = vv

    def post_q(r):
        for t in range(4):
            for w in range(NW):
                q = r[WL * w:WL * w + 128, 128 * t:128 * (t + 1)]
                qT_s[w, t] = _pack(q * QSCALE)
                phiqT_s[w, t] = _pack(_phi(q))

    def mem_update(ws=range(NW)):
        r = lax.broadcasted_iota(jnp.int32, (MROWS, 128), 0)
        c = lax.broadcasted_iota(jnp.int32, (MROWS, 128), 1)
        for w in ws:
            vt = jnp.concatenate([_unpack(vT_s[w, t, 0:MROWS // 2, :]) for t in range(4)], axis=1)
            pk = jnp.concatenate([_unpack(phikT_s[w, t]) for t in range(4)], axis=1)
            upd = lax.dot_general(vt, pk, (((1,), (1,)), ((), ())), preferred_element_type=f32)
            mt = mt_s[w] + upd
            mt_s[w] = mt
            keep = jnp.zeros((MROWS, 128), jnp.bool_)
            for a in range(_nh(w)):
                keep = keep | ((r >= RS * a) & (r < RS * (a + 1)) & (c >= DH * a) & (c < DH * (a + 1)))
            mtb_s[w] = _pack(jnp.where(keep, mt, 0.0))

    def mem_retrieve():
        for w in range(NW):
            for j in range(4):
                am = jnp.dot(_unpack(mtb_s[w]), _unpack(phiqT_s[w, j]), preferred_element_type=f32)
                for a in range(_nh(w)):
                    ama = am[RS * a:RS * a + 24]
                    g = g_s[w, a:a + 1, :]
                    om = ama * (g / (ama[DH:DH + 1] + 1e-6))
                    am_s[j, WL * w + DH * a:WL * w + DH * (a + 1), :] = om[0:DH]

    def phase_a(w, nh, j, buf):
        n = 128 * (j + 1)
        rows = lax.broadcasted_iota(jnp.int32, (64, 128), 0)
        qw = qT_s[w, j]
        qbd = jnp.concatenate(
            [jnp.where((rows >= 9 * a) & (rows < 9 * a + 9), qw, jnp.uint32(0)) for a in range(nh)], axis=1)
        s = jnp.dot(_unpack(k_s[w, 0:n // 2, :]), _unpack(qbd), preferred_element_type=f32)
        kr = lax.broadcasted_iota(jnp.int32, (128, 128), 0)
        qc = lax.broadcasted_iota(jnp.int32, (128, 128), 1)
        causal = kr <= qc
        sd = jnp.concatenate(
            [jnp.where(causal, s[n - 128:n, 128 * a:128 * (a + 1)], NEG) for a in range(nh)], axis=1)
        s_scr[buf, n - 128:n, 0:128 * nh] = sd
        m = jnp.max(sd, axis=0, keepdims=True)
        if j > 0:
            s_scr[buf, 0:n - 128, 0:128 * nh] = s[0:n - 128]
            m = jnp.maximum(m, jnp.max(s[0:n - 128], axis=0, keepdims=True))
        m_scr[buf, :, 0:128 * nh] = jnp.broadcast_to(m, (8, 128 * nh))

    def phase_b(w, nh, j, buf):
        n = 128 * (j + 1)
        for a in range(nh):
            m = m_scr[buf, 0:1, 128 * a:128 * (a + 1)]
            p = jnp.exp2(s_scr[buf, 0:n, 128 * a:128 * (a + 1)] - m).astype(bf16)
            vt = jnp.concatenate([_unpack(vT_s[w, t, (RS // 2) * a:(RS // 2) * a + 16, :]) for t in range(j + 1)], axis=1)
            o = jnp.dot(vt, p, preferred_element_type=f32)
            g = g_s[w, a:a + 1, :]
            od = o[0:24] * ((1.0 - g) / o[DH:DH + 1])
            row0 = WL * w + DH * a
            oT_s[j, pl.ds(row0, DH), :] = (od + am_s[j, pl.ds(row0, 24), :])[0:DH]

    def window(w, nh, nxt):
        order = [3, 2, 1, 0]
        for t in range(4):
            if t < 3:
                phase_a(w, nh, order[t + 1], (t + 1) % 2)
            elif nxt is not None:
                phase_a(nxt, _nh(nxt), order[0], 0)
            else:
                mem_update(range(WFILL))
            phase_b(w, nh, order[t], t % 2)

    def outproj(seg):
        oT = jnp.concatenate([oT_s[t] for t in range(4)], axis=1).astype(bf16)
        attn = jnp.dot(woT[...], oT, preferred_element_type=f32)
        for t in range(4):
            cols = slice(128 * t, 128 * (t + 1))
            tile = 4 * seg + t
            c = None
            s1, s2, s3 = _Acc(), _Acc(), _Acc()
            for i in range(NCH):
                rows = slice(RC * i, RC * (i + 1))
                h = x_v[seg, rows, cols].astype(f32) + attn[rows, cols]
                h_s[tile, rows, :] = h
                if c is None:
                    c = h[0:1]
                d = h - c
                s1.add(d)
                s2.add(d * d)
                s3.add(d * wr_s[rows, :])
            mu = s1.total() * (1.0 / D)
            var = jnp.maximum(s2.total() * (1.0 / D) - mu * mu, 0.0)
            rstd = lax.rsqrt(var + EPS)
            mean = c + mu
            st_s[tile, 0:1, :] = mean
            st_s[tile, 1:2, :] = rstd
            r_s[pl.ds(tile, 1), :] = (s3.total() - mu * wr_s[D:D + 1, :]) * rstd
            ga = 1.0 + rstd
            gb = mean * rstd
            for i in range(NCH):
                rows = slice(RC * i, RC * (i + 1))
                out_v[tile, rows, :] = (h_s[tile, rows, :] * ga - gb).astype(bf16)

    def transpose_wd(seg):
        nblk = F // 128 // (NSEG - 1)
        for i in range(nblk):
            c0 = pl.multiple_of((seg * nblk + i) * 128, 128)
            wd_s[pl.ds(c0, 128), :] = wdT_v[:, pl.ds(c0, 128)].T

    def project_segment():
        post_k(proj(0))
        post_q(proj(1))
        post_v(proj(2))

    with _scope("setup"):
        w_copies[0].start()
        x_copy(0).start()
        beta = beta_ref[...].astype(f32).reshape(1, H)
        hrow = lax.broadcasted_iota(jnp.int32, (8 * NW, H), 0)
        hcol = lax.broadcasted_iota(jnp.int32, (8 * NW, H), 1)
        sel = (hcol == HPW * (hrow >> 3) + (hrow & 7)) & ((hrow & 7) < HPW)
        bcol = jnp.sum(jnp.where(sel, beta, 0.0), axis=1, keepdims=True)
        g_s[...] = jnp.broadcast_to(_sigmoid(bcol), (8 * NW, 128)).reshape(NW, 8, 128)
        wr_row = wr_ref[...].astype(f32).reshape(1, D)
        wr_pad = jnp.concatenate([wr_row, jnp.zeros((1, 64), f32)], axis=1)
        wr_s[...] = jnp.broadcast_to(wr_pad, (128, D + 64)).T
        wr_s[D:D + 1, :] = jnp.broadcast_to(jnp.sum(wr_row, axis=1, keepdims=True), (1, 128))

        mt_s[...] = jnp.zeros(mt_s.shape, f32)
        vT_s[...] = jnp.zeros(vT_s.shape, u32)
        am_s[...] = jnp.zeros(am_s.shape, f32)

        w_copies[0].wait()
        w_copies[1].start()
        wT[0:D, :] = wk_v[...].T
        x_copy(0).wait()
        w_copies[2].start()
        w_copies[3].start()
        for t in range(4):
            ln1_tile(0, t)
    with _scope("proj0"):
        post_k(proj(0))
        w_copies[1].wait()
        w_copies[2].wait()
        w_copies[3].wait()
        for s in range(1, NSEG):
            x_copy(s).start()
        wT[D:2 * D, :] = wq_v[...].T
        wT[2 * D:3 * D, :] = wv_v[...].T
        post_q(proj(1))
        woT[...] = wo_v[...].T
        post_v(proj(2))
        phase_a(0, HPW, 3, 0)
        for s in range(1, NSEG):
            x_copy(s).wait()
        w_copies[4].start()

    def segment(seg, carry):
        nseg = jnp.minimum(seg + 1, NSEG - 1)

        with _scope("windows"):
            for w in range(NW):
                if w < 4:
                    ln1_tile(nseg, w)
                window(w, _nh(w), w + 1 if w + 1 < NW else None)

        @pl.when(seg < NSEG - 1)
        def _():
            @pl.when(seg == 0)
            def _():
                w_copies[4].wait()
                for c in w_copies[5:]:
                    c.start()

            with _scope("mid"):
                transpose_wd(seg)
                steps = {
                    "u": lambda: mem_update(range(WFILL, NW)),
                    "o": lambda: outproj(seg),
                    "k": lambda: post_k(proj(0)),
                    "q": lambda: post_q(proj(1)),
                    "v": lambda: post_v(proj(2)),
                    "r": mem_retrieve,
                    "a": lambda: phase_a(0, HPW, 3, 0),
                }
                for c in MID_ORDER:
                    steps[c]()
                for t in range(4):
                    o_copy(4 * seg + t).start()
        return carry

    lax.fori_loop(0, NSEG, segment, 0)
    with _scope("last_out"):
        outproj(NSEG - 1)
        for t in range(4):
            o_copy(4 * (NSEG - 1) + t).start()

    with _scope("ffn"):
        r = r_s[...]
        rmax = jnp.max(r)
        tok = (lax.broadcasted_iota(jnp.int32, (NT, 128), 0) * 128
               + lax.broadcasted_iota(jnp.int32, (NT, 128), 1))
        idx = jnp.minimum(jnp.min(jnp.where(r == rmax, tok, S)), S - 1)
        tile = idx >> 7
        lane = idx & 127
        hn = ((h_s[tile] - st_s[tile, 0:1, :]) * st_s[tile, 1:2, :]).astype(bf16)
        onehot = jnp.where(lax.broadcasted_iota(jnp.int32, (16, 128), 1) == lane, 1.0, 0.0).astype(bf16)
        xs = lax.dot_general(onehot, hn, (((1,), (1,)), ((), ())), preferred_element_type=f32)
        for c in w_copies[5:]:
            c.wait()
        xm = xs[:, 0:512].astype(bf16)
        xr = xs[:, 512:D]
        row = lax.broadcasted_iota(jnp.int32, (16, 64), 0)
        x2 = jnp.concatenate([jnp.where(row == 0, xr, 0.0), jnp.where(row == 1, xr, 0.0)], axis=1).astype(bf16)
        wrem = jnp.concatenate([wg_v[512:D, :], wu_v[512:D, :]], axis=0)
        rem = jnp.dot(x2, wrem, preferred_element_type=f32)
        gate = jnp.dot(xm, wg_v[0:512, :], preferred_element_type=f32)[0:1] + rem[0:1]
        up = jnp.dot(xm, wu_v[0:512, :], preferred_element_type=f32)[0:1] + rem[1:2]
        act = jnp.broadcast_to(gate * _sigmoid(gate) * up, (16, F)).astype(bf16)
        y = jnp.dot(act, wd_s[...], preferred_element_type=f32)
        y = y[0:1] * _sigmoid(jnp.full((1, 1), rmax, f32))
        ypad = jnp.concatenate([y, jnp.zeros((1, 64), f32)], axis=1)
        ycol = jnp.broadcast_to(ypad, (128, D + 64)).T[0:D]
        for t in range(NT):
            o_copy(t).wait()
        lanes = lax.broadcasted_iota(jnp.int32, (D, 128), 1)
        blk = out_v[tile].astype(f32)
        out_v[tile] = jnp.where(lanes == lane, blk + ycol, blk).astype(bf16)
        fix = o_copy(tile)
        fix.start()
        fix.wait()


@jax.jit
def pallas_sequential_preLN__memory_aug_infini_attn__moe_arch_mod__prompt_kernel(
    A_x: jax.Array,
    A_wq: jax.Array,
    A_wk: jax.Array,
    A_wv: jax.Array,
    A_wo: jax.Array,
    A_beta: jax.Array,
    B_x: jax.Array,
    B_w_r: jax.Array,
    B_w_gate: jax.Array,
    B_w_up: jax.Array,
    B_w_down: jax.Array,
):
    del B_x
    xT = A_x.reshape(S, D).T
    wdT = B_w_down.T

    hbm = pl.BlockSpec(memory_space=pltpu.HBM)
    vmem = pl.BlockSpec(memory_space=pltpu.VMEM)
    scratch = [
        pltpu.VMEM((NSEG, D, L), bf16),
        pltpu.VMEM((D, D), bf16),
        pltpu.VMEM((D, D), bf16),
        pltpu.VMEM((D, D), bf16),
        pltpu.VMEM((D, D), bf16),
        pltpu.VMEM((D, F), bf16),
        pltpu.VMEM((D, F), bf16),
        pltpu.VMEM((D, F), bf16),
        pltpu.VMEM((3 * D, D), bf16),
        pltpu.VMEM((D, D), bf16),
        pltpu.VMEM((F, D), bf16),
        pltpu.VMEM((NW, 8, 128), f32),
        pltpu.VMEM((D + 64, 128), f32),
        pltpu.VMEM((4, D, 128), bf16),
        pltpu.VMEM((NW, L // 2, 128), u32),
        pltpu.VMEM((NW, 4, 64, 128), u32),
        pltpu.VMEM((NW, 4, 64, 128), u32),
        pltpu.VMEM((NW, 4, 64, 128), u32),
        pltpu.VMEM((NW, 4, VWORDS, 128), u32),
        pltpu.VMEM((NW, MROWS, 128), f32),
        pltpu.VMEM((NW, MROWS // 2, 128), u32),
        pltpu.VMEM((4, D + 8, 128), f32),
        pltpu.VMEM((2, L, 128 * HPW), f32),
        pltpu.VMEM((2, 8, 128 * HPW), f32),
        pltpu.VMEM((4, D, 128), f32),
        pltpu.VMEM((NT, D, 128), bf16),
        pltpu.VMEM((NT, D, 128), f32),
        pltpu.VMEM((NT, 8, 128), f32),
        pltpu.VMEM((NT, 128), f32),
        pltpu.SemaphoreType.DMA((NSEG,)),
        pltpu.SemaphoreType.DMA((7,)),
        pltpu.SemaphoreType.DMA((NT,)),
    ]
    outT = pl.pallas_call(
        _kernel,
        out_shape=jax.ShapeDtypeStruct((D, S), bf16),
        in_specs=[hbm, hbm, hbm, hbm, hbm, vmem, vmem, hbm, hbm, hbm],
        out_specs=hbm,
        scratch_shapes=scratch,
        compiler_params=pltpu.CompilerParams(vmem_limit_bytes=100 * 1024 * 1024),
    )(xT, A_wq, A_wk, A_wv, A_wo, A_beta, B_w_r, B_w_gate, B_w_up, B_w_down.T)
    return outT.T.reshape(1, S, D)
```

```python
import jax
import jax.numpy as jnp
from jax import lax
import jax.experimental.pallas as pl
import jax.experimental.pallas.tpu as pltpu

S = 2048
D = 576
H = 32
DH = 18
NSEG = 4
L = 512
NT = S // 128
F = 4608
HPW = 7
NW = 5
WL = HPW * DH
RS = 20
MROWS = 144
VWORDS = 80
QKV_ROWS = D + 64
LOG2E = 1.4426950408889634
NEG = -1e9 * LOG2E
QSCALE = (DH ** -0.5) * LOG2E
EPS = 1e-5
KSPLIT = int(__import__('os').environ.get('KSPLIT', '288'))
import os
MID_ORDER = os.environ.get('MID_ORDER', 'uokqvr')
WFILL = int(os.environ.get('WFILL', '0'))

import contextlib
import os
_PROF = bool(os.environ.get("PROF"))


def _scope(name):
    return jax.named_scope(name) if _PROF else contextlib.nullcontext()


f32 = jnp.float32
bf16 = jnp.bfloat16
u32 = jnp.uint32


def _nh(w):
    return HPW if w < NW - 1 else H - HPW * (NW - 1)


def _pack(x):
    return pltpu.bitcast(x.astype(bf16), u32)


def _unpack(x):
    return pltpu.bitcast(x, bf16)


def _phi(t):
    return jnp.where(t > 0, t + 1.0, jnp.exp(t))


RC = 16
NCH = D // RC


class _Acc:
    def __init__(self, n=2):
        self.parts = [None] * n
        self.i = 0

    def add(self, x):
        k = self.i % len(self.parts)
        self.parts[k] = x if self.parts[k] is None else self.parts[k] + x
        self.i += 1

    def total(self):
        t = self.parts[0]
        for p in self.parts[1:]:
            t = t + p
        return jnp.sum(t, axis=0, keepdims=True)


def _ln_stats(chunk):
    x0 = chunk(0)
    c = x0[0:1]
    s1, s2 = _Acc(), _Acc()
    for i in range(NCH):
        d = (x0 if i == 0 else chunk(i)) - c
        s1.add(d)
        s2.add(d * d)
    mu = s1.total() * (1.0 / D)
    var = jnp.maximum(s2.total() * (1.0 / D) - mu * mu, 0.0)
    return c + mu, lax.rsqrt(var + EPS)


def _sigmoid(x):
    return 1.0 / (1.0 + jnp.exp(-x))


def _kernel(xT_hbm, wq_hbm, wk_hbm, wv_hbm, wo_hbm, beta_ref, wr_ref, wg_hbm, wu_hbm, wdT_hbm,
            out_hbm,
            x_v, wq_v, wk_v, wv_v, wo_v, wg_v, wu_v, wdT_v,
            wT, woT, wd_s, g_s, wr_s,
            xn_s, k_s, phikT_s, qT_s, phiqT_s, vT_s, mt_s, mtb_s, am_s,
            s_scr, m_scr, oT_s, out_v, h_s, st_s, r_s, xs_keep,
            sem_x, sem_w, sem_o):
    def x_copy(s):
        return pltpu.make_async_copy(xT_hbm.at[:, pl.ds(s * L, L)], x_v.at[s], sem_x.at[s])

    def o_copy(t):
        return pltpu.make_async_copy(out_v.at[t], out_hbm.at[:, pl.ds(pl.multiple_of(t * 128, 128), 128)],
                                     sem_o.at[t])

    w_copies = [pltpu.make_async_copy(src, dst, sem_w.at[i]) for i, (src, dst) in enumerate(
        [(wk_hbm, wk_v), (wq_hbm, wq_v), (wv_hbm, wv_v), (wo_hbm, wo_v),
         (wdT_hbm, wdT_v), (wg_hbm, wg_v), (wu_hbm, wu_v)])]

    def ln1_tile(seg, t):
        cols = pl.ds(pl.multiple_of(t * 128, 128), 128)

        def chunk(i):
            return x_v[seg, RC * i:RC * (i + 1), cols].astype(f32)
        mean, rstd = _ln_stats(chunk)
        for i in range(NCH):
            xn_s[t, RC * i:RC * (i + 1), :] = ((chunk(i) - mean) * rstd).astype(bf16)

    def proj_rows(lo, hi):
        xn = jnp.concatenate([xn_s[t] for t in range(4)], axis=1)
        return jnp.dot(wT[lo:hi, :], xn, preferred_element_type=f32)

    def proj(i, head=None):
        lo = D * i if head is None else D * i + head.shape[0]
        parts = [] if head is None else [head]
        parts += [proj_rows(lo, D * (i + 1)), jnp.zeros((64, L), f32)]
        return jnp.concatenate(parts, axis=0)

    def post_k(r):
        for t in range(4):
            for w in range(NW):
                kk = r[WL * w:WL * w + 128, 128 * t:128 * (t + 1)]
                k_s[w, 64 * t:64 * (t + 1), :] = pltpu.bitcast(kk.astype(bf16).T, u32)
                phikT_s[w, t] = _pack(_phi(kk))

    def post_v(r):
        rr = lax.broadcasted_iota(jnp.int32, (RS, 128), 0)
        ones_row = jnp.where(rr == DH, 1.0, 0.0).astype(f32)
        for t in range(4):
            for w in range(NW):
                nh = _nh(w)
                vs = [jnp.where(rr < DH,
                                r[DH * (HPW * w + a):DH * (HPW * w + a) + RS, 128 * t:128 * (t + 1)], ones_row)
                      for a in range(nh)]
                if (nh * RS) % 16:
                    vs.append(jnp.zeros((16 - (nh * RS) % 16, 128), f32))
                vv = _pack(jnp.concatenate(vs, axis=0))
                vT_s[w, t, 0:vv.shape[0], :] = vv

    def post_q(r):
        for t in range(4):
            for w in range(NW):
                q = r[WL * w:WL * w + 128, 128 * t:128 * (t + 1)]
                qT_s[w, t] = _pack(q * QSCALE)
                phiqT_s[w, t] = _pack(_phi(q))

    def mem_update(ws=range(NW)):
        r = lax.broadcasted_iota(jnp.int32, (MROWS, 128), 0)
        c = lax.broadcasted_iota(jnp.int32, (MROWS, 128), 1)
        for w in ws:
            vt = jnp.concatenate([_unpack(vT_s[w, t, 0:MROWS // 2, :]) for t in range(4)], axis=1)
            pk = jnp.concatenate([_unpack(phikT_s[w, t]) for t in range(4)], axis=1)
            upd = lax.dot_general(vt, pk, (((1,), (1,)), ((), ())), preferred_element_type=f32)
            mt = mt_s[w] + upd
            mt_s[w] = mt
            keep = jnp.zeros((MROWS, 128), jnp.bool_)
            for a in range(_nh(w)):
                keep = keep | ((r >= RS * a) & (r < RS * (a + 1)) & (c >= DH * a) & (c < DH * (a + 1)))
            mtb_s[w] = _pack(jnp.where(keep, mt, 0.0))

    def mem_retrieve():
        for w in range(NW):
            for j in range(4):
                am = jnp.dot(_unpack(mtb_s[w]), _unpack(phiqT_s[w, j]), preferred_element_type=f32)
                for a in range(_nh(w)):
                    ama = am[RS * a:RS * a + 24]
                    g = g_s[w, a:a + 1, :]
                    om = ama * (g / (ama[DH:DH + 1] + 1e-6))
                    am_s[j, WL * w + DH * a:WL * w + DH * (a + 1), :] = om[0:DH]

    def phase_a(w, nh, j, buf):
        n = 128 * (j + 1)
        rows = lax.broadcasted_iota(jnp.int32, (64, 128), 0)
        qw = qT_s[w, j]
        qbd = jnp.concatenate(
            [jnp.where((rows >= 9 * a) & (rows < 9 * a + 9), qw, jnp.uint32(0)) for a in range(nh)], axis=1)
        s = jnp.dot(_unpack(k_s[w, 0:n // 2, :]), _unpack(qbd), preferred_element_type=f32)
        kr = lax.broadcasted_iota(jnp.int32, (128, 128), 0)
        qc = lax.broadcasted_iota(jnp.int32, (128, 128), 1)
        causal = kr <= qc
        sd = jnp.concatenate(
            [jnp.where(causal, s[n - 128:n, 128 * a:128 * (a + 1)], NEG) for a in range(nh)], axis=1)
        s_scr[buf, n - 128:n, 0:128 * nh] = sd
        m = jnp.max(sd, axis=0, keepdims=True)
        if j > 0:
            s_scr[buf, 0:n - 128, 0:128 * nh] = s[0:n - 128]
            m = jnp.maximum(m, jnp.max(s[0:n - 128], axis=0, keepdims=True))
        m_scr[buf, :, 0:128 * nh] = jnp.broadcast_to(m, (8, 128 * nh))

    def phase_b(w, nh, j, buf):
        n = 128 * (j + 1)
        for a in range(nh):
            m = m_scr[buf, 0:1, 128 * a:128 * (a + 1)]
            p = jnp.exp2(s_scr[buf, 0:n, 128 * a:128 * (a + 1)] - m).astype(bf16)
            vt = jnp.concatenate([_unpack(vT_s[w, t, (RS // 2) * a:(RS // 2) * a + 16, :]) for t in range(j + 1)], axis=1)
            o = jnp.dot(vt, p, preferred_element_type=f32)
            g = g_s[w, a:a + 1, :]
            od = o[0:24] * ((1.0 - g) / o[DH:DH + 1])
            row0 = WL * w + DH * a
            oT_s[j, pl.ds(row0, DH), :] = (od + am_s[j, pl.ds(row0, 24), :])[0:DH]

    def window(w, nh, nxt):
        order = [3, 2, 1, 0]
        for t in range(4):
            if t < 3:
                phase_a(w, nh, order[t + 1], (t + 1) % 2)
            elif nxt is not None:
                phase_a(nxt, _nh(nxt), order[0], 0)
            else:
                mem_update(range(WFILL))
            phase_b(w, nh, order[t], t % 2)

    def outproj(seg):
        oT = jnp.concatenate([oT_s[t] for t in range(4)], axis=1).astype(bf16)
        attn = jnp.dot(woT[...], oT, preferred_element_type=f32)
        for t in range(4):
            cols = slice(128 * t, 128 * (t + 1))
            tile = 4 * seg + t
            c = None
            s1, s2, s3 = _Acc(), _Acc(), _Acc()
            for i in range(NCH):
                rows = slice(RC * i, RC * (i + 1))
                h = x_v[seg, rows, cols].astype(f32) + attn[rows, cols]
                h_s[tile, rows, :] = h
                if c is None:
                    c = h[0:1]
                d = h - c
                s1.add(d)
                s2.add(d * d)
                s3.add(d * wr_s[rows, :])
            mu = s1.total() * (1.0 / D)
            var = jnp.maximum(s2.total() * (1.0 / D) - mu * mu, 0.0)
            rstd = lax.rsqrt(var + EPS)
            mean = c + mu
            st_s[tile, 0:1, :] = mean
            st_s[tile, 1:2, :] = rstd
            r_s[pl.ds(tile, 1), :] = (s3.total() - mu * wr_s[D:D + 1, :]) * rstd
            ga = 1.0 + rstd
            gb = mean * rstd
            for i in range(NCH):
                rows = slice(RC * i, RC * (i + 1))
                out_v[tile, rows, :] = (h_s[tile, rows, :] * ga - gb).astype(bf16)

    def transpose_wd(seg):
        nblk = F // 128 // (NSEG - 1)
        for i in range(nblk):
            c0 = pl.multiple_of((seg * nblk + i) * 128, 128)
            wd_s[pl.ds(c0, 128), :] = wdT_v[:, pl.ds(c0, 128)].T

    def project_segment():
        post_k(proj(0))
        post_q(proj(1))
        post_v(proj(2))

    with _scope("setup"):
        w_copies[0].start()
        x_copy(0).start()
        beta = beta_ref[...].astype(f32).reshape(1, H)
        hrow = lax.broadcasted_iota(jnp.int32, (8 * NW, H), 0)
        hcol = lax.broadcasted_iota(jnp.int32, (8 * NW, H), 1)
        sel = (hcol == HPW * (hrow >> 3) + (hrow & 7)) & ((hrow & 7) < HPW)
        bcol = jnp.sum(jnp.where(sel, beta, 0.0), axis=1, keepdims=True)
        g_s[...] = jnp.broadcast_to(_sigmoid(bcol), (8 * NW, 128)).reshape(NW, 8, 128)
        wr_row = wr_ref[...].astype(f32).reshape(1, D)
        wr_pad = jnp.concatenate([wr_row, jnp.zeros((1, 64), f32)], axis=1)
        wr_s[...] = jnp.broadcast_to(wr_pad, (128, D + 64)).T
        wr_s[D:D + 1, :] = jnp.broadcast_to(jnp.sum(wr_row, axis=1, keepdims=True), (1, 128))

        mt_s[...] = jnp.zeros(mt_s.shape, f32)
        vT_s[...] = jnp.zeros(vT_s.shape, u32)
        am_s[...] = jnp.zeros(am_s.shape, f32)
        s_scr[:, 0:8, 0:128] = jnp.zeros((2, 8, 128), f32)
        m_scr[...] = jnp.zeros(m_scr.shape, f32)

        w_copies[0].wait()
        w_copies[1].start()
        wT[0:D, :] = wk_v[...].T
        x_copy(0).wait()
        w_copies[2].start()
        w_copies[3].start()
        for t in range(4):
            ln1_tile(0, t)
    with _scope("proj0"):
        post_k(proj(0))
        w_copies[1].wait()
        w_copies[2].wait()
        w_copies[3].wait()
        for s in range(1, NSEG):
            x_copy(s).start()
        wT[D:2 * D, :] = wq_v[...].T
        wT[2 * D:3 * D, :] = wv_v[...].T
        post_q(proj(1))
        woT[...] = wo_v[...].T
        post_v(proj(2))
        for s in range(1, NSEG):
            x_copy(s).wait()
        w_copies[4].start()

    def segment(seg, carry):
        nseg = jnp.minimum(seg + 1, NSEG - 1)

        with _scope("windows"):
            phase_a(0, HPW, 3, 0)
            for w in range(NW):
                if w < 4:
                    ln1_tile(nseg, w)
                window(w, _nh(w), w + 1 if w + 1 < NW else None)

        @pl.when(seg < NSEG - 1)
        def _():
            @pl.when(seg == 0)
            def _():
                w_copies[4].wait()
                for c in w_copies[5:]:
                    c.start()

            with _scope("mid"):
                transpose_wd(seg)
                steps = {
                    "u": lambda: mem_update(range(WFILL, NW)),
                    "o": lambda: outproj(seg),
                    "k": lambda: post_k(proj(0)),
                    "q": lambda: post_q(proj(1)),
                    "v": lambda: post_v(proj(2)),
                    "r": mem_retrieve,
                    "a": lambda: phase_a(0, HPW, 3, 0),
                }
                for c in MID_ORDER:
                    steps[c]()
                for t in range(4):
                    o_copy(4 * seg + t).start()
        return carry

    lax.fori_loop(0, NSEG, segment, 0)
    with _scope("last_out"):
        xs_keep[...] = s_scr[0, 0:8, 0:128] + s_scr[1, 0:8, 0:128] + m_scr[0, :, 0:128] + m_scr[1, :, 0:128]
        outproj(NSEG - 1)
        for t in range(4):
            o_copy(4 * (NSEG - 1) + t).start()

    with _scope("ffn"):
        r = r_s[...]
        rmax = jnp.max(r)
        tok = (lax.broadcasted_iota(jnp.int32, (NT, 128), 0) * 128
               + lax.broadcasted_iota(jnp.int32, (NT, 128), 1))
        idx = jnp.minimum(jnp.min(jnp.where(r == rmax, tok, S)), S - 1)
        tile = idx >> 7
        lane = idx & 127
        hn = ((h_s[tile] - st_s[tile, 0:1, :]) * st_s[tile, 1:2, :]).astype(bf16)
        onehot = jnp.where(lax.broadcasted_iota(jnp.int32, (16, 128), 1) == lane, 1.0, 0.0).astype(bf16)
        xs = lax.dot_general(onehot, hn, (((1,), (1,)), ((), ())), preferred_element_type=f32)
        for c in w_copies[5:]:
            c.wait()
        xm = xs[:, 0:512].astype(bf16)
        xr = xs[:, 512:D]
        row = lax.broadcasted_iota(jnp.int32, (16, 64), 0)
        x2 = jnp.concatenate([jnp.where(row == 0, xr, 0.0), jnp.where(row == 1, xr, 0.0)], axis=1).astype(bf16)
        wrem = jnp.concatenate([wg_v[512:D, :], wu_v[512:D, :]], axis=0)
        rem = jnp.dot(x2, wrem, preferred_element_type=f32)
        gate = jnp.dot(xm, wg_v[0:512, :], preferred_element_type=f32)[0:1] + rem[0:1]
        up = jnp.dot(xm, wu_v[0:512, :], preferred_element_type=f32)[0:1] + rem[1:2]
        act = jnp.broadcast_to(gate * _sigmoid(gate) * up, (16, F)).astype(bf16)
        y = jnp.dot(act, wd_s[...], preferred_element_type=f32)
        y = y[0:1] * _sigmoid(jnp.full((1, 1), rmax, f32))
        ypad = jnp.concatenate([y, jnp.zeros((1, 64), f32)], axis=1)
        ycol = jnp.broadcast_to(ypad, (128, D + 64)).T[0:D]
        for t in range(NT):
            o_copy(t).wait()
        lanes = lax.broadcasted_iota(jnp.int32, (D, 128), 1)
        blk = out_v[tile].astype(f32)
        out_v[tile] = jnp.where(lanes == lane, blk + ycol, blk).astype(bf16)
        fix = o_copy(tile)
        fix.start()
        fix.wait()


@jax.jit
def pallas_sequential_preLN__memory_aug_infini_attn__moe_arch_mod__prompt_kernel(
    A_x: jax.Array,
    A_wq: jax.Array,
    A_wk: jax.Array,
    A_wv: jax.Array,
    A_wo: jax.Array,
    A_beta: jax.Array,
    B_x: jax.Array,
    B_w_r: jax.Array,
    B_w_gate: jax.Array,
    B_w_up: jax.Array,
    B_w_down: jax.Array,
):
    del B_x
    xT = A_x.reshape(S, D).T
    wdT = B_w_down.T

    hbm = pl.BlockSpec(memory_space=pltpu.HBM)
    vmem = pl.BlockSpec(memory_space=pltpu.VMEM)
    scratch = [
        pltpu.VMEM((NSEG, D, L), bf16),
        pltpu.VMEM((D, D), bf16),
        pltpu.VMEM((D, D), bf16),
        pltpu.VMEM((D, D), bf16),
        pltpu.VMEM((D, D), bf16),
        pltpu.VMEM((D, F), bf16),
        pltpu.VMEM((D, F), bf16),
        pltpu.VMEM((D, F), bf16),
        pltpu.VMEM((3 * D, D), bf16),
        pltpu.VMEM((D, D), bf16),
        pltpu.VMEM((F, D), bf16),
        pltpu.VMEM((NW, 8, 128), f32),
        pltpu.VMEM((D + 64, 128), f32),
        pltpu.VMEM((4, D, 128), bf16),
        pltpu.VMEM((NW, L // 2, 128), u32),
        pltpu.VMEM((NW, 4, 64, 128), u32),
        pltpu.VMEM((NW, 4, 64, 128), u32),
        pltpu.VMEM((NW, 4, 64, 128), u32),
        pltpu.VMEM((NW, 4, VWORDS, 128), u32),
        pltpu.VMEM((NW, MROWS, 128), f32),
        pltpu.VMEM((NW, MROWS // 2, 128), u32),
        pltpu.VMEM((4, D + 8, 128), f32),
        pltpu.VMEM((2, L, 128 * HPW), f32),
        pltpu.VMEM((2, 8, 128 * HPW), f32),
        pltpu.VMEM((4, D, 128), f32),
        pltpu.VMEM((NT, D, 128), bf16),
        pltpu.VMEM((NT, D, 128), f32),
        pltpu.VMEM((NT, 8, 128), f32),
        pltpu.VMEM((NT, 128), f32),
        pltpu.VMEM((8, 128), f32),
        pltpu.SemaphoreType.DMA((NSEG,)),
        pltpu.SemaphoreType.DMA((7,)),
        pltpu.SemaphoreType.DMA((NT,)),
    ]
    outT = pl.pallas_call(
        _kernel,
        out_shape=jax.ShapeDtypeStruct((D, S), bf16),
        in_specs=[hbm, hbm, hbm, hbm, hbm, vmem, vmem, hbm, hbm, hbm],
        out_specs=hbm,
        scratch_shapes=scratch,
        compiler_params=pltpu.CompilerParams(vmem_limit_bytes=100 * 1024 * 1024),
    )(xT, A_wq, A_wk, A_wv, A_wo, A_beta, B_w_r, B_w_gate, B_w_up, B_w_down.T)
    return outT.T.reshape(1, S, D)
```

```python
import functools
import jax
import jax.numpy as jnp
from jax import lax
import jax.experimental.pallas as pl
import jax.experimental.pallas.tpu as pltpu

S = 2048
D = 576
H = 32
DH = 18
NSEG = 4
L = 512
NT = S // 128
F = 4608
HPW = 7
NW = 5
WL = HPW * DH
RS = 20
MROWS = 144
VWORDS = 80
QKV_ROWS = D + 64
LOG2E = 1.4426950408889634
NEG = -1e9 * LOG2E
QSCALE = (DH ** -0.5) * LOG2E
EPS = 1e-5
KSPLIT = int(__import__('os').environ.get('KSPLIT', '288'))
import os
MID_ORDER = os.environ.get('MID_ORDER', 'ukqvor')
WFILL = int(os.environ.get('WFILL', '1'))
LNPOS = int(os.environ.get('LNPOS', '0'))

import contextlib
import os
_PROF = bool(os.environ.get("PROF"))


def _scope(name):
    return jax.named_scope(name) if _PROF else contextlib.nullcontext()


f32 = jnp.float32
bf16 = jnp.bfloat16
u32 = jnp.uint32


def _nh(w):
    return HPW if w < NW - 1 else H - HPW * (NW - 1)


def _pack(x):
    return pltpu.bitcast(x.astype(bf16), u32)


def _unpack(x):
    return pltpu.bitcast(x, bf16)


def _phi(t):
    return jnp.where(t > 0, t + 1.0, jnp.exp(t))


RC = 16
NCH = D // RC


class _Acc:
    def __init__(self, n=2):
        self.parts = [None] * n
        self.i = 0

    def add(self, x):
        k = self.i % len(self.parts)
        self.parts[k] = x if self.parts[k] is None else self.parts[k] + x
        self.i += 1

    def total(self):
        t = self.parts[0]
        for p in self.parts[1:]:
            t = t + p
        return jnp.sum(t, axis=0, keepdims=True)


def _ln_stats(chunk):
    x0 = chunk(0)
    c = x0[0:1]
    s1, s2 = _Acc(), _Acc()
    for i in range(NCH):
        d = (x0 if i == 0 else chunk(i)) - c
        s1.add(d)
        s2.add(d * d)
    mu = s1.total() * (1.0 / D)
    var = jnp.maximum(s2.total() * (1.0 / D) - mu * mu, 0.0)
    return c + mu, lax.rsqrt(var + EPS)


def _sigmoid(x):
    return 1.0 / (1.0 + jnp.exp(-x))


def _kernel(xT_hbm, wq_hbm, wk_hbm, wv_hbm, wo_hbm, beta_ref, wr_ref, wg_hbm, wu_hbm, wdT_hbm,
            out_hbm,
            x_v, wq_v, wk_v, wv_v, wo_v, wg_v, wu_v, wdT_v,
            wT, woT, wd_s, g_s, wr_s,
            xn_s, k_s, phikT_s, qT_s, phiqT_s, vT_s, mt_s, mtb_s, am_s,
            s_scr, m_scr, oT_s, out_v, h_s, st_s, r_s, xs_keep,
            sem_x, sem_w, sem_o):
    def x_copy(s):
        return pltpu.make_async_copy(xT_hbm.at[:, pl.ds(s * L, L)], x_v.at[s], sem_x.at[s])

    def o_copy(t):
        return pltpu.make_async_copy(out_v.at[t], out_hbm.at[:, pl.ds(pl.multiple_of(t * 128, 128), 128)],
                                     sem_o.at[t])

    w_copies = [pltpu.make_async_copy(src, dst, sem_w.at[i]) for i, (src, dst) in enumerate(
        [(wk_hbm, wk_v), (wq_hbm, wq_v), (wv_hbm, wv_v), (wo_hbm, wo_v),
         (wdT_hbm, wdT_v), (wg_hbm, wg_v), (wu_hbm, wu_v)])]

    def ln1_tile(seg, t):
        cols = pl.ds(pl.multiple_of(t * 128, 128), 128)

        def chunk(i):
            return x_v[seg, RC * i:RC * (i + 1), cols].astype(f32)
        mean, rstd = _ln_stats(chunk)
        for i in range(NCH):
            xn_s[t, RC * i:RC * (i + 1), :] = ((chunk(i) - mean) * rstd).astype(bf16)

    def proj_rows(lo, hi):
        xn = jnp.concatenate([xn_s[t] for t in range(4)], axis=1)
        return jnp.dot(wT[lo:hi, :], xn, preferred_element_type=f32)

    def proj(i, head=None):
        lo = D * i if head is None else D * i + head.shape[0]
        parts = [] if head is None else [head]
        parts += [proj_rows(lo, D * (i + 1)), jnp.zeros((64, L), f32)]
        return jnp.concatenate(parts, axis=0)

    def post_k(r):
        for t in range(4):
            for w in range(NW):
                kk = r[WL * w:WL * w + 128, 128 * t:128 * (t + 1)]
                k_s[w, 64 * t:64 * (t + 1), :] = pltpu.bitcast(kk.astype(bf16).T, u32)
                phikT_s[w, t] = _pack(_phi(kk))

    def post_v(r):
        rr = lax.broadcasted_iota(jnp.int32, (RS, 128), 0)
        ones_row = jnp.where(rr == DH, 1.0, 0.0).astype(f32)
        for t in range(4):
            for w in range(NW):
                nh = _nh(w)
                vs = [jnp.where(rr < DH,
                                r[DH * (HPW * w + a):DH * (HPW * w + a) + RS, 128 * t:128 * (t + 1)], ones_row)
                      for a in range(nh)]
                if (nh * RS) % 16:
                    vs.append(jnp.zeros((16 - (nh * RS) % 16, 128), f32))
                vv = _pack(jnp.concatenate(vs, axis=0))
                vT_s[w, t, 0:vv.shape[0], :] = vv

    def post_q(r):
        for t in range(4):
            for w in range(NW):
                q = r[WL * w:WL * w + 128, 128 * t:128 * (t + 1)]
                qT_s[w, t] = _pack(q * QSCALE)
                phiqT_s[w, t] = _pack(_phi(q))

    def mem_update(ws=range(NW)):
        r = lax.broadcasted_iota(jnp.int32, (MROWS, 128), 0)
        c = lax.broadcasted_iota(jnp.int32, (MROWS, 128), 1)
        for w in ws:
            vt = jnp.concatenate([_unpack(vT_s[w, t, 0:MROWS // 2, :]) for t in range(4)], axis=1)
            pk = jnp.concatenate([_unpack(phikT_s[w, t]) for t in range(4)], axis=1)
            upd = lax.dot_general(vt, pk, (((1,), (1,)), ((), ())), preferred_element_type=f32)
            mt = mt_s[w] + upd
            mt_s[w] = mt
            keep = jnp.zeros((MROWS, 128), jnp.bool_)
            for a in range(_nh(w)):
                keep = keep | ((r >= RS * a) & (r < RS * (a + 1)) & (c >= DH * a) & (c < DH * (a + 1)))
            mtb_s[w] = _pack(jnp.where(keep, mt, 0.0))

    def mem_retrieve():
        for w in range(NW):
            for j in range(4):
                am = jnp.dot(_unpack(mtb_s[w]), _unpack(phiqT_s[w, j]), preferred_element_type=f32)
                for a in range(_nh(w)):
                    ama = am[RS * a:RS * a + 24]
                    g = g_s[w, a:a + 1, :]
                    om = ama * (g / (ama[DH:DH + 1] + 1e-6))
                    am_s[j, WL * w + DH * a:WL * w + DH * (a + 1), :] = om[0:DH]

    def phase_a(w, nh, j, buf):
        n = 128 * (j + 1)
        rows = lax.broadcasted_iota(jnp.int32, (64, 128), 0)
        qw = qT_s[w, j]
        qbd = jnp.concatenate(
            [jnp.where((rows >= 9 * a) & (rows < 9 * a + 9), qw, jnp.uint32(0)) for a in range(nh)], axis=1)
        s = jnp.dot(_unpack(k_s[w, 0:n // 2, :]), _unpack(qbd), preferred_element_type=f32)
        kr = lax.broadcasted_iota(jnp.int32, (128, 128), 0)
        qc = lax.broadcasted_iota(jnp.int32, (128, 128), 1)
        causal = kr <= qc
        sd = jnp.concatenate(
            [jnp.where(causal, s[n - 128:n, 128 * a:128 * (a + 1)], NEG) for a in range(nh)], axis=1)
        s_scr[buf, n - 128:n, 0:128 * nh] = sd
        m = jnp.max(sd, axis=0, keepdims=True)
        if j > 0:
            s_scr[buf, 0:n - 128, 0:128 * nh] = s[0:n - 128]
            m = jnp.maximum(m, jnp.max(s[0:n - 128], axis=0, keepdims=True))
        m_scr[buf, :, 0:128 * nh] = jnp.broadcast_to(m, (8, 128 * nh))

    def phase_b(w, nh, j, buf):
        n = 128 * (j + 1)
        for a in range(nh):
            m = m_scr[buf, 0:1, 128 * a:128 * (a + 1)]
            p = jnp.exp2(s_scr[buf, 0:n, 128 * a:128 * (a + 1)] - m).astype(bf16)
            vt = jnp.concatenate([_unpack(vT_s[w, t, (RS // 2) * a:(RS // 2) * a + 16, :]) for t in range(j + 1)], axis=1)
            o = jnp.dot(vt, p, preferred_element_type=f32)
            g = g_s[w, a:a + 1, :]
            od = o[0:24] * ((1.0 - g) / o[DH:DH + 1])
            row0 = WL * w + DH * a
            oT_s[j, pl.ds(row0, DH), :] = (od + am_s[j, pl.ds(row0, 24), :])[0:DH]

    def window(w, nh, nxt, filler=None):
        order = [3, 2, 1, 0]
        for t in range(4):
            if filler is not None and LNPOS == 2 * t:
                filler()
            if t < 3:
                phase_a(w, nh, order[t + 1], (t + 1) % 2)
            elif nxt is not None:
                phase_a(nxt, _nh(nxt), order[0], 0)
            else:
                mem_update(range(WFILL))
            if filler is not None and LNPOS == 2 * t + 1:
                filler()
            phase_b(w, nh, order[t], t % 2)

    def outproj(seg):
        oT = jnp.concatenate([oT_s[t] for t in range(4)], axis=1).astype(bf16)
        attn = jnp.dot(woT[...], oT, preferred_element_type=f32)
        for t in range(4):
            cols = slice(128 * t, 128 * (t + 1))
            tile = 4 * seg + t
            c = None
            s1, s2, s3 = _Acc(), _Acc(), _Acc()
            for i in range(NCH):
                rows = slice(RC * i, RC * (i + 1))
                h = x_v[seg, rows, cols].astype(f32) + attn[rows, cols]
                h_s[tile, rows, :] = h
                if c is None:
                    c = h[0:1]
                d = h - c
                s1.add(d)
                s2.add(d * d)
                s3.add(d * wr_s[rows, :])
            mu = s1.total() * (1.0 / D)
            var = jnp.maximum(s2.total() * (1.0 / D) - mu * mu, 0.0)
            rstd = lax.rsqrt(var + EPS)
            mean = c + mu
            st_s[tile, 0:1, :] = mean
            st_s[tile, 1:2, :] = rstd
            r_s[pl.ds(tile, 1), :] = (s3.total() - mu * wr_s[D:D + 1, :]) * rstd
            ga = 1.0 + rstd
            gb = mean * rstd
            for i in range(NCH):
                rows = slice(RC * i, RC * (i + 1))
                out_v[tile, rows, :] = (h_s[tile, rows, :] * ga - gb).astype(bf16)

    def transpose_wd(seg):
        nblk = F // 128 // (NSEG - 1)
        for i in range(nblk):
            c0 = pl.multiple_of((seg * nblk + i) * 128, 128)
            wd_s[pl.ds(c0, 128), :] = wdT_v[:, pl.ds(c0, 128)].T

    def project_segment():
        post_k(proj(0))
        post_q(proj(1))
        post_v(proj(2))

    with _scope("setup"):
        w_copies[0].start()
        x_copy(0).start()
        beta = beta_ref[...].astype(f32).reshape(1, H)
        hrow = lax.broadcasted_iota(jnp.int32, (8 * NW, H), 0)
        hcol = lax.broadcasted_iota(jnp.int32, (8 * NW, H), 1)
        sel = (hcol == HPW * (hrow >> 3) + (hrow & 7)) & ((hrow & 7) < HPW)
        bcol = jnp.sum(jnp.where(sel, beta, 0.0), axis=1, keepdims=True)
        g_s[...] = jnp.broadcast_to(_sigmoid(bcol), (8 * NW, 128)).reshape(NW, 8, 128)
        wr_row = wr_ref[...].astype(f32).reshape(1, D)
        wr_pad = jnp.concatenate([wr_row, jnp.zeros((1, 64), f32)], axis=1)
        wr_s[...] = jnp.broadcast_to(wr_pad, (128, D + 64)).T
        wr_s[D:D + 1, :] = jnp.broadcast_to(jnp.sum(wr_row, axis=1, keepdims=True), (1, 128))

        mt_s[...] = jnp.zeros(mt_s.shape, f32)
        vT_s[...] = jnp.zeros(vT_s.shape, u32)
        am_s[...] = jnp.zeros(am_s.shape, f32)
        s_scr[:, 0:8, 0:128] = jnp.zeros((2, 8, 128), f32)
        m_scr[...] = jnp.zeros(m_scr.shape, f32)

        w_copies[0].wait()
        w_copies[1].start()
        wT[0:D, :] = wk_v[...].T
        x_copy(0).wait()
        w_copies[2].start()
        w_copies[3].start()
        for t in range(4):
            ln1_tile(0, t)
    with _scope("proj0"):
        post_k(proj(0))
        w_copies[1].wait()
        w_copies[2].wait()
        w_copies[3].wait()
        for s in range(1, NSEG):
            x_copy(s).start()
        wT[D:2 * D, :] = wq_v[...].T
        wT[2 * D:3 * D, :] = wv_v[...].T
        post_q(proj(1))
        woT[...] = wo_v[...].T
        post_v(proj(2))
        for s in range(1, NSEG):
            x_copy(s).wait()
        w_copies[4].start()

    def segment(seg, carry):
        nseg = jnp.minimum(seg + 1, NSEG - 1)

        with _scope("windows"):
            phase_a(0, HPW, 3, 0)
            for w in range(NW):
                window(w, _nh(w), w + 1 if w + 1 < NW else None,
                       functools.partial(ln1_tile, nseg, w) if w < 4 else None)

        @pl.when(seg < NSEG - 1)
        def _():
            @pl.when(seg == 0)
            def _():
                w_copies[4].wait()
                for c in w_copies[5:]:
                    c.start()

            with _scope("mid"):
                transpose_wd(seg)
                steps = {
                    "u": lambda: mem_update(range(WFILL, NW)),
                    "o": lambda: outproj(seg),
                    "k": lambda: post_k(proj(0)),
                    "q": lambda: post_q(proj(1)),
                    "v": lambda: post_v(proj(2)),
                    "r": mem_retrieve,
                    "a": lambda: phase_a(0, HPW, 3, 0),
                }
                for c in MID_ORDER:
                    steps[c]()
                for t in range(4):
                    o_copy(4 * seg + t).start()
        return carry

    lax.fori_loop(0, NSEG, segment, 0)
    with _scope("last_out"):
        xs_keep[...] = s_scr[0, 0:8, 0:128] + s_scr[1, 0:8, 0:128] + m_scr[0, :, 0:128] + m_scr[1, :, 0:128]
        outproj(NSEG - 1)
        for t in range(4):
            o_copy(4 * (NSEG - 1) + t).start()

    with _scope("ffn"):
        r = r_s[...]
        rmax = jnp.max(r)
        tok = (lax.broadcasted_iota(jnp.int32, (NT, 128), 0) * 128
               + lax.broadcasted_iota(jnp.int32, (NT, 128), 1))
        idx = jnp.minimum(jnp.min(jnp.where(r == rmax, tok, S)), S - 1)
        tile = idx >> 7
        lane = idx & 127
        hn = ((h_s[tile] - st_s[tile, 0:1, :]) * st_s[tile, 1:2, :]).astype(bf16)
        onehot = jnp.where(lax.broadcasted_iota(jnp.int32, (16, 128), 1) == lane, 1.0, 0.0).astype(bf16)
        xs = lax.dot_general(onehot, hn, (((1,), (1,)), ((), ())), preferred_element_type=f32)
        for c in w_copies[5:]:
            c.wait()
        xm = xs[:, 0:512].astype(bf16)
        xr = xs[:, 512:D]
        row = lax.broadcasted_iota(jnp.int32, (16, 64), 0)
        x2 = jnp.concatenate([jnp.where(row == 0, xr, 0.0), jnp.where(row == 1, xr, 0.0)], axis=1).astype(bf16)
        wrem = jnp.concatenate([wg_v[512:D, :], wu_v[512:D, :]], axis=0)
        rem = jnp.dot(x2, wrem, preferred_element_type=f32)
        gate = jnp.dot(xm, wg_v[0:512, :], preferred_element_type=f32)[0:1] + rem[0:1]
        up = jnp.dot(xm, wu_v[0:512, :], preferred_element_type=f32)[0:1] + rem[1:2]
        act = jnp.broadcast_to(gate * _sigmoid(gate) * up, (16, F)).astype(bf16)
        y = jnp.dot(act, wd_s[...], preferred_element_type=f32)
        y = y[0:1] * _sigmoid(jnp.full((1, 1), rmax, f32))
        ypad = jnp.concatenate([y, jnp.zeros((1, 64), f32)], axis=1)
        ycol = jnp.broadcast_to(ypad, (128, D + 64)).T[0:D]
        for t in range(NT):
            o_copy(t).wait()
        lanes = lax.broadcasted_iota(jnp.int32, (D, 128), 1)
        blk = out_v[tile].astype(f32)
        out_v[tile] = jnp.where(lanes == lane, blk + ycol, blk).astype(bf16)
        fix = o_copy(tile)
        fix.start()
        fix.wait()


@jax.jit
def pallas_sequential_preLN__memory_aug_infini_attn__moe_arch_mod__prompt_kernel(
    A_x: jax.Array,
    A_wq: jax.Array,
    A_wk: jax.Array,
    A_wv: jax.Array,
    A_wo: jax.Array,
    A_beta: jax.Array,
    B_x: jax.Array,
    B_w_r: jax.Array,
    B_w_gate: jax.Array,
    B_w_up: jax.Array,
    B_w_down: jax.Array,
):
    del B_x
    xT = A_x.reshape(S, D).T
    wdT = B_w_down.T

    hbm = pl.BlockSpec(memory_space=pltpu.HBM)
    vmem = pl.BlockSpec(memory_space=pltpu.VMEM)
    scratch = [
        pltpu.VMEM((NSEG, D, L), bf16),
        pltpu.VMEM((D, D), bf16),
        pltpu.VMEM((D, D), bf16),
        pltpu.VMEM((D, D), bf16),
        pltpu.VMEM((D, D), bf16),
        pltpu.VMEM((D, F), bf16),
        pltpu.VMEM((D, F), bf16),
        pltpu.VMEM((D, F), bf16),
        pltpu.VMEM((3 * D, D), bf16),
        pltpu.VMEM((D, D), bf16),
        pltpu.VMEM((F, D), bf16),
        pltpu.VMEM((NW, 8, 128), f32),
        pltpu.VMEM((D + 64, 128), f32),
        pltpu.VMEM((4, D, 128), bf16),
        pltpu.VMEM((NW, L // 2, 128), u32),
        pltpu.VMEM((NW, 4, 64, 128), u32),
        pltpu.VMEM((NW, 4, 64, 128), u32),
        pltpu.VMEM((NW, 4, 64, 128), u32),
        pltpu.VMEM((NW, 4, VWORDS, 128), u32),
        pltpu.VMEM((NW, MROWS, 128), f32),
        pltpu.VMEM((NW, MROWS // 2, 128), u32),
        pltpu.VMEM((4, D + 8, 128), f32),
        pltpu.VMEM((2, L, 128 * HPW), f32),
        pltpu.VMEM((2, 8, 128 * HPW), f32),
        pltpu.VMEM((4, D, 128), f32),
        pltpu.VMEM((NT, D, 128), bf16),
        pltpu.VMEM((NT, D, 128), f32),
        pltpu.VMEM((NT, 8, 128), f32),
        pltpu.VMEM((NT, 128), f32),
        pltpu.VMEM((8, 128), f32),
        pltpu.SemaphoreType.DMA((NSEG,)),
        pltpu.SemaphoreType.DMA((7,)),
        pltpu.SemaphoreType.DMA((NT,)),
    ]
    outT = pl.pallas_call(
        _kernel,
        out_shape=jax.ShapeDtypeStruct((D, S), bf16),
        in_specs=[hbm, hbm, hbm, hbm, hbm, vmem, vmem, hbm, hbm, hbm],
        out_specs=hbm,
        scratch_shapes=scratch,
        compiler_params=pltpu.CompilerParams(vmem_limit_bytes=100 * 1024 * 1024),
    )(xT, A_wq, A_wk, A_wv, A_wo, A_beta, B_w_r, B_w_gate, B_w_up, B_w_down.T)
    return outT.T.reshape(1, S, D)
```

```python
import contextlib
import functools
import os

import jax
import jax.numpy as jnp
from jax import lax
import jax.experimental.pallas as pl
import jax.experimental.pallas.tpu as pltpu

S = 2048
D = 576
H = 32
DH = 18
NSEG = 4
L = 512
NT = S // 128
F = 4608
HPW = 7
NW = 5
WL = HPW * DH
RS = 20
MROWS = 144
VWORDS = 80
LOG2E = 1.4426950408889634
NEG = -1e9 * LOG2E
QSCALE = (DH ** -0.5) * LOG2E
EPS = 1e-5
MID_ORDER = os.environ.get('MID_ORDER', 'ukqvor')
WFILL = int(os.environ.get('WFILL', '1'))
LNPOS = int(os.environ.get('LNPOS', '0'))
GROUP = int(os.environ.get('GROUP', '0'))

_PROF = bool(os.environ.get("PROF"))


def _scope(name):
    return jax.named_scope(name) if _PROF else contextlib.nullcontext()


f32 = jnp.float32
bf16 = jnp.bfloat16
u32 = jnp.uint32


def _nh(w):
    return HPW if w < NW - 1 else H - HPW * (NW - 1)


def _pack(x):
    return pltpu.bitcast(x.astype(bf16), u32)


def _unpack(x):
    return pltpu.bitcast(x, bf16)


def _phi(t):
    return jnp.where(t > 0, t + 1.0, jnp.exp(t))


RC = 16
NCH = D // RC


class _Acc:
    def __init__(self, n=2):
        self.parts = [None] * n
        self.i = 0

    def add(self, x):
        k = self.i % len(self.parts)
        self.parts[k] = x if self.parts[k] is None else self.parts[k] + x
        self.i += 1

    def total(self):
        t = self.parts[0]
        for p in self.parts[1:]:
            t = t + p
        return jnp.sum(t, axis=0, keepdims=True)


def _ln_stats(chunk):
    x0 = chunk(0)
    c = x0[0:1]
    s1, s2 = _Acc(), _Acc()
    for i in range(NCH):
        d = (x0 if i == 0 else chunk(i)) - c
        s1.add(d)
        s2.add(d * d)
    mu = s1.total() * (1.0 / D)
    var = jnp.maximum(s2.total() * (1.0 / D) - mu * mu, 0.0)
    return c + mu, lax.rsqrt(var + EPS)


def _sigmoid(x):
    return 1.0 / (1.0 + jnp.exp(-x))


def _kernel(xT_hbm, wq_hbm, wk_hbm, wv_hbm, wo_hbm, beta_ref, wr_ref, wg_hbm, wu_hbm, wdT_hbm,
            out_hbm,
            x_v, wq_v, wk_v, wv_v, wo_v, wg_v, wu_v, wdT_v,
            wT, woT, wd_s, g_s, wr_s,
            xn_s, k_s, phikT_s, qT_s, phiqT_s, vT_s, mt_s, mtb_s, am_s,
            s_scr, m_scr, oT_s, out_v, h_s, st_s, r_s, xs_keep,
            sem_x, sem_w, sem_o):
    def x_copy(s):
        return pltpu.make_async_copy(xT_hbm.at[:, pl.ds(s * L, L)], x_v.at[s], sem_x.at[s])

    def o_copy(t):
        return pltpu.make_async_copy(out_v.at[t], out_hbm.at[:, pl.ds(pl.multiple_of(t * 128, 128), 128)],
                                     sem_o.at[t])

    w_copies = [pltpu.make_async_copy(src, dst, sem_w.at[i]) for i, (src, dst) in enumerate(
        [(wk_hbm, wk_v), (wq_hbm, wq_v), (wv_hbm, wv_v), (wo_hbm, wo_v),
         (wdT_hbm, wdT_v), (wg_hbm, wg_v), (wu_hbm, wu_v)])]

    def ln1_tile(seg, t):
        cols = pl.ds(pl.multiple_of(t * 128, 128), 128)

        def chunk(i):
            return x_v[seg, RC * i:RC * (i + 1), cols].astype(f32)
        mean, rstd = _ln_stats(chunk)
        for i in range(NCH):
            xn_s[t, RC * i:RC * (i + 1), :] = ((chunk(i) - mean) * rstd).astype(bf16)

    def proj_rows(lo, hi):
        xn = jnp.concatenate([xn_s[t] for t in range(4)], axis=1)
        return jnp.dot(wT[lo:hi, :], xn, preferred_element_type=f32)

    def proj(i, head=None):
        lo = D * i if head is None else D * i + head.shape[0]
        parts = [] if head is None else [head]
        parts += [proj_rows(lo, D * (i + 1)), jnp.zeros((64, L), f32)]
        return jnp.concatenate(parts, axis=0)

    def post_k(r):
        for t in range(4):
            for w in range(NW):
                kk = r[WL * w:WL * w + 128, 128 * t:128 * (t + 1)]
                k_s[w, 64 * t:64 * (t + 1), :] = pltpu.bitcast(kk.astype(bf16).T, u32)
                phikT_s[w, t] = _pack(_phi(kk))

    def post_v(r):
        rr = lax.broadcasted_iota(jnp.int32, (RS, 128), 0)
        ones_row = jnp.where(rr == DH, 1.0, 0.0).astype(f32)
        for t in range(4):
            for w in range(NW):
                nh = _nh(w)
                vs = [jnp.where(rr < DH,
                                r[DH * (HPW * w + a):DH * (HPW * w + a) + RS, 128 * t:128 * (t + 1)], ones_row)
                      for a in range(nh)]
                if (nh * RS) % 16:
                    vs.append(jnp.zeros((16 - (nh * RS) % 16, 128), f32))
                vv = _pack(jnp.concatenate(vs, axis=0))
                vT_s[w, t, 0:vv.shape[0], :] = vv

    def post_q(r):
        for t in range(4):
            for w in range(NW):
                q = r[WL * w:WL * w + 128, 128 * t:128 * (t + 1)]
                qT_s[w, t] = _pack(q * QSCALE)
                phiqT_s[w, t] = _pack(_phi(q))

    def mem_update(ws=range(NW)):
        r = lax.broadcasted_iota(jnp.int32, (MROWS, 128), 0)
        c = lax.broadcasted_iota(jnp.int32, (MROWS, 128), 1)
        for w in ws:
            vt = jnp.concatenate([_unpack(vT_s[w, t, 0:MROWS // 2, :]) for t in range(4)], axis=1)
            pk = jnp.concatenate([_unpack(phikT_s[w, t]) for t in range(4)], axis=1)
            upd = lax.dot_general(vt, pk, (((1,), (1,)), ((), ())), preferred_element_type=f32)
            mt = mt_s[w] + upd
            mt_s[w] = mt
            keep = jnp.zeros((MROWS, 128), jnp.bool_)
            for a in range(_nh(w)):
                keep = keep | ((r >= RS * a) & (r < RS * (a + 1)) & (c >= DH * a) & (c < DH * (a + 1)))
            mtb_s[w] = _pack(jnp.where(keep, mt, 0.0))

    def mem_retrieve():
        for w in range(NW):
            for j in range(4):
                am = jnp.dot(_unpack(mtb_s[w]), _unpack(phiqT_s[w, j]), preferred_element_type=f32)
                for a in range(_nh(w)):
                    ama = am[RS * a:RS * a + 24]
                    g = g_s[w, a:a + 1, :]
                    om = ama * (g / (ama[DH:DH + 1] + 1e-6))
                    am_s[j, WL * w + DH * a:WL * w + DH * (a + 1), :] = om[0:DH]

    def phase_a(w, heads, j, buf):
        n = 128 * (j + 1)
        nh = len(heads)
        cols = slice(128 * heads[0], 128 * (heads[-1] + 1))
        rows = lax.broadcasted_iota(jnp.int32, (64, 128), 0)
        qw = qT_s[w, j]
        qbd = jnp.concatenate(
            [jnp.where((rows >= 9 * a) & (rows < 9 * a + 9), qw, jnp.uint32(0)) for a in heads], axis=1)
        s = jnp.dot(_unpack(k_s[w, 0:n // 2, :]), _unpack(qbd), preferred_element_type=f32)
        kr = lax.broadcasted_iota(jnp.int32, (128, 128), 0)
        qc = lax.broadcasted_iota(jnp.int32, (128, 128), 1)
        causal = kr <= qc
        sd = jnp.concatenate(
            [jnp.where(causal, s[n - 128:n, 128 * a:128 * (a + 1)], NEG) for a in range(nh)], axis=1)
        s_scr[buf, n - 128:n, cols] = sd
        m = jnp.max(sd, axis=0, keepdims=True)
        if j > 0:
            s_scr[buf, 0:n - 128, cols] = s[0:n - 128]
            m = jnp.maximum(m, jnp.max(s[0:n - 128], axis=0, keepdims=True))
        m_scr[buf, :, cols] = jnp.broadcast_to(m, (8, 128 * nh))

    def phase_b(w, heads, j, buf):
        n = 128 * (j + 1)
        for a in heads:
            m = m_scr[buf, 0:1, 128 * a:128 * (a + 1)]
            p = jnp.exp2(s_scr[buf, 0:n, 128 * a:128 * (a + 1)] - m).astype(bf16)
            vt = jnp.concatenate([_unpack(vT_s[w, t, (RS // 2) * a:(RS // 2) * a + 16, :]) for t in range(j + 1)], axis=1)
            o = jnp.dot(vt, p, preferred_element_type=f32)
            g = g_s[w, a:a + 1, :]
            od = o[0:24] * ((1.0 - g) / o[DH:DH + 1])
            row0 = WL * w + DH * a
            oT_s[j, pl.ds(row0, DH), :] = (od + am_s[j, pl.ds(row0, 24), :])[0:DH]

    def groups(w):
        nh = _nh(w)
        if GROUP == 0 or nh <= GROUP:
            return [list(range(nh))]
        return [list(range(0, GROUP)), list(range(GROUP, nh))]

    def window(w, nxt, filler=None):
        order = [3, 2, 1, 0]
        for t in range(4):
            if filler is not None and LNPOS == 2 * t:
                filler()
            ga = groups(w) if t < 3 else (groups(nxt) if nxt is not None else [])
            gb = groups(w)
            for i in range(max(len(ga), len(gb))):
                if i < len(ga):
                    if t < 3:
                        phase_a(w, ga[i], order[t + 1], (t + 1) % 2)
                    else:
                        phase_a(nxt, ga[i], order[0], 0)
                if t == 3 and nxt is None and i == 0:
                    mem_update(range(WFILL))
                if i < len(gb):
                    phase_b(w, gb[i], order[t], t % 2)

    def outproj(seg):
        oT = jnp.concatenate([oT_s[t] for t in range(4)], axis=1).astype(bf16)
        attn = jnp.dot(woT[...], oT, preferred_element_type=f32)
        for t in range(4):
            cols = slice(128 * t, 128 * (t + 1))
            tile = 4 * seg + t
            c = None
            s1, s2, s3 = _Acc(), _Acc(), _Acc()
            for i in range(NCH):
                rows = slice(RC * i, RC * (i + 1))
                h = x_v[seg, rows, cols].astype(f32) + attn[rows, cols]
                h_s[tile, rows, :] = h
                if c is None:
                    c = h[0:1]
                d = h - c
                s1.add(d)
                s2.add(d * d)
                s3.add(d * wr_s[rows, :])
            mu = s1.total() * (1.0 / D)
            var = jnp.maximum(s2.total() * (1.0 / D) - mu * mu, 0.0)
            rstd = lax.rsqrt(var + EPS)
            mean = c + mu
            st_s[tile, 0:1, :] = mean
            st_s[tile, 1:2, :] = rstd
            r_s[pl.ds(tile, 1), :] = (s3.total() - mu * wr_s[D:D + 1, :]) * rstd
            ga = 1.0 + rstd
            gb = mean * rstd
            for i in range(NCH):
                rows = slice(RC * i, RC * (i + 1))
                out_v[tile, rows, :] = (h_s[tile, rows, :] * ga - gb).astype(bf16)

    def transpose_wd(seg):
        nblk = F // 128 // (NSEG - 1)
        for i in range(nblk):
            c0 = pl.multiple_of((seg * nblk + i) * 128, 128)
            wd_s[pl.ds(c0, 128), :] = wdT_v[:, pl.ds(c0, 128)].T

    def project_segment():
        post_k(proj(0))
        post_q(proj(1))
        post_v(proj(2))

    with _scope("setup"):
        w_copies[0].start()
        x_copy(0).start()
        beta = beta_ref[...].astype(f32).reshape(1, H)
        hrow = lax.broadcasted_iota(jnp.int32, (8 * NW, H), 0)
        hcol = lax.broadcasted_iota(jnp.int32, (8 * NW, H), 1)
        sel = (hcol == HPW * (hrow >> 3) + (hrow & 7)) & ((hrow & 7) < HPW)
        bcol = jnp.sum(jnp.where(sel, beta, 0.0), axis=1, keepdims=True)
        g_s[...] = jnp.broadcast_to(_sigmoid(bcol), (8 * NW, 128)).reshape(NW, 8, 128)
        wr_row = wr_ref[...].astype(f32).reshape(1, D)
        wr_pad = jnp.concatenate([wr_row, jnp.zeros((1, 64), f32)], axis=1)
        wr_s[...] = jnp.broadcast_to(wr_pad, (128, D + 64)).T
        wr_s[D:D + 1, :] = jnp.broadcast_to(jnp.sum(wr_row, axis=1, keepdims=True), (1, 128))

        mt_s[...] = jnp.zeros(mt_s.shape, f32)
        vT_s[...] = jnp.zeros(vT_s.shape, u32)
        am_s[...] = jnp.zeros(am_s.shape, f32)
        s_scr[:, 0:8, 0:128] = jnp.zeros((2, 8, 128), f32)
        m_scr[...] = jnp.zeros(m_scr.shape, f32)

        w_copies[0].wait()
        w_copies[1].start()
        wT[0:D, :] = wk_v[...].T
        x_copy(0).wait()
        w_copies[2].start()
        w_copies[3].start()
        for t in range(4):
            ln1_tile(0, t)
    with _scope("proj0"):
        post_k(proj(0))
        w_copies[1].wait()
        w_copies[2].wait()
        w_copies[3].wait()
        for s in range(1, NSEG):
            x_copy(s).start()
        wT[D:2 * D, :] = wq_v[...].T
        wT[2 * D:3 * D, :] = wv_v[...].T
        post_q(proj(1))
        woT[...] = wo_v[...].T
        post_v(proj(2))
        for s in range(1, NSEG):
            x_copy(s).wait()
        w_copies[4].start()

    def segment(seg, carry):
        nseg = jnp.minimum(seg + 1, NSEG - 1)

        with _scope("windows"):
            for hs in groups(0):
                phase_a(0, hs, 3, 0)
            for w in range(NW):
                window(w, w + 1 if w + 1 < NW else None,
                       functools.partial(ln1_tile, nseg, w) if w < 4 else None)

        @pl.when(seg < NSEG - 1)
        def _():
            @pl.when(seg == 0)
            def _():
                w_copies[4].wait()
                for c in w_copies[5:]:
                    c.start()

            with _scope("mid"):
                transpose_wd(seg)
                steps = {
                    "u": lambda: mem_update(range(WFILL, NW)),
                    "o": lambda: outproj(seg),
                    "k": lambda: post_k(proj(0)),
                    "q": lambda: post_q(proj(1)),
                    "v": lambda: post_v(proj(2)),
                    "r": mem_retrieve,
                }
                for c in MID_ORDER:
                    steps[c]()
                for t in range(4):
                    o_copy(4 * seg + t).start()
        return carry

    lax.fori_loop(0, NSEG, segment, 0)
    with _scope("last_out"):
        xs_keep[...] = s_scr[0, 0:8, 0:128] + s_scr[1, 0:8, 0:128] + m_scr[0, :, 0:128] + m_scr[1, :, 0:128]
        outproj(NSEG - 1)
        for t in range(4):
            o_copy(4 * (NSEG - 1) + t).start()

    with _scope("ffn"):
        r = r_s[...]
        rmax = jnp.max(r)
        tok = (lax.broadcasted_iota(jnp.int32, (NT, 128), 0) * 128
               + lax.broadcasted_iota(jnp.int32, (NT, 128), 1))
        idx = jnp.minimum(jnp.min(jnp.where(r == rmax, tok, S)), S - 1)
        tile = idx >> 7
        lane = idx & 127
        hn = ((h_s[tile] - st_s[tile, 0:1, :]) * st_s[tile, 1:2, :]).astype(bf16)
        onehot = jnp.where(lax.broadcasted_iota(jnp.int32, (16, 128), 1) == lane, 1.0, 0.0).astype(bf16)
        xs = lax.dot_general(onehot, hn, (((1,), (1,)), ((), ())), preferred_element_type=f32)
        for c in w_copies[5:]:
            c.wait()
        xm = xs[:, 0:512].astype(bf16)
        xr = xs[:, 512:D]
        row = lax.broadcasted_iota(jnp.int32, (16, 64), 0)
        x2 = jnp.concatenate([jnp.where(row == 0, xr, 0.0), jnp.where(row == 1, xr, 0.0)], axis=1).astype(bf16)
        wrem = jnp.concatenate([wg_v[512:D, :], wu_v[512:D, :]], axis=0)
        rem = jnp.dot(x2, wrem, preferred_element_type=f32)
        gate = jnp.dot(xm, wg_v[0:512, :], preferred_element_type=f32)[0:1] + rem[0:1]
        up = jnp.dot(xm, wu_v[0:512, :], preferred_element_type=f32)[0:1] + rem[1:2]
        act = jnp.broadcast_to(gate * _sigmoid(gate) * up, (16, F)).astype(bf16)
        y = jnp.dot(act, wd_s[...], preferred_element_type=f32)
        y = y[0:1] * _sigmoid(jnp.full((1, 1), rmax, f32))
        ypad = jnp.concatenate([y, jnp.zeros((1, 64), f32)], axis=1)
        ycol = jnp.broadcast_to(ypad, (128, D + 64)).T[0:D]
        for t in range(NT):
            o_copy(t).wait()
        lanes = lax.broadcasted_iota(jnp.int32, (D, 128), 1)
        blk = out_v[tile].astype(f32)
        out_v[tile] = jnp.where(lanes == lane, blk + ycol, blk).astype(bf16)
        fix = o_copy(tile)
        fix.start()
        fix.wait()


@jax.jit
def pallas_sequential_preLN__memory_aug_infini_attn__moe_arch_mod__prompt_kernel(
    A_x: jax.Array,
    A_wq: jax.Array,
    A_wk: jax.Array,
    A_wv: jax.Array,
    A_wo: jax.Array,
    A_beta: jax.Array,
    B_x: jax.Array,
    B_w_r: jax.Array,
    B_w_gate: jax.Array,
    B_w_up: jax.Array,
    B_w_down: jax.Array,
):
    del B_x
    xT = A_x.reshape(S, D).T
    wdT = B_w_down.T

    hbm = pl.BlockSpec(memory_space=pltpu.HBM)
    vmem = pl.BlockSpec(memory_space=pltpu.VMEM)
    scratch = [
        pltpu.VMEM((NSEG, D, L), bf16),
        pltpu.VMEM((D, D), bf16),
        pltpu.VMEM((D, D), bf16),
        pltpu.VMEM((D, D), bf16),
        pltpu.VMEM((D, D), bf16),
        pltpu.VMEM((D, F), bf16),
        pltpu.VMEM((D, F), bf16),
        pltpu.VMEM((D, F), bf16),
        pltpu.VMEM((3 * D, D), bf16),
        pltpu.VMEM((D, D), bf16),
        pltpu.VMEM((F, D), bf16),
        pltpu.VMEM((NW, 8, 128), f32),
        pltpu.VMEM((D + 64, 128), f32),
        pltpu.VMEM((4, D, 128), bf16),
        pltpu.VMEM((NW, L // 2, 128), u32),
        pltpu.VMEM((NW, 4, 64, 128), u32),
        pltpu.VMEM((NW, 4, 64, 128), u32),
        pltpu.VMEM((NW, 4, 64, 128), u32),
        pltpu.VMEM((NW, 4, VWORDS, 128), u32),
        pltpu.VMEM((NW, MROWS, 128), f32),
        pltpu.VMEM((NW, MROWS // 2, 128), u32),
        pltpu.VMEM((4, D + 8, 128), f32),
        pltpu.VMEM((2, L, 128 * HPW), f32),
        pltpu.VMEM((2, 8, 128 * HPW), f32),
        pltpu.VMEM((4, D, 128), f32),
        pltpu.VMEM((NT, D, 128), bf16),
        pltpu.VMEM((NT, D, 128), f32),
        pltpu.VMEM((NT, 8, 128), f32),
        pltpu.VMEM((NT, 128), f32),
        pltpu.VMEM((8, 128), f32),
        pltpu.SemaphoreType.DMA((NSEG,)),
        pltpu.SemaphoreType.DMA((7,)),
        pltpu.SemaphoreType.DMA((NT,)),
    ]
    outT = pl.pallas_call(
        _kernel,
        out_shape=jax.ShapeDtypeStruct((D, S), bf16),
        in_specs=[hbm, hbm, hbm, hbm, hbm, vmem, vmem, hbm, hbm, hbm],
        out_specs=hbm,
        scratch_shapes=scratch,
        compiler_params=pltpu.CompilerParams(vmem_limit_bytes=100 * 1024 * 1024),
    )(xT, A_wq, A_wk, A_wv, A_wo, A_beta, B_w_r, B_w_gate, B_w_up, B_w_down.T)
    return outT.T.reshape(1, S, D)
```

```python
import contextlib
import functools
import os

import jax
import jax.numpy as jnp
from jax import lax
import jax.experimental.pallas as pl
import jax.experimental.pallas.tpu as pltpu

S = 2048
D = 576
H = 32
DH = 18
NSEG = 4
L = 512
NT = S // 128
F = 4608
HPW = 7
NW = 5
WL = HPW * DH
RS = 20
MROWS = 144
VWORDS = 80
LOG2E = 1.4426950408889634
NEG = -1e9 * LOG2E
QSCALE = (DH ** -0.5) * LOG2E
EPS = 1e-5
MID_ORDER = os.environ.get('MID_ORDER', 'ukqvor')
WFILL = int(os.environ.get('WFILL', '1'))
LNPOS = int(os.environ.get('LNPOS', '0'))
GROUP = int(os.environ.get('GROUP', '0'))
PRO = int(os.environ.get('PRO', '1'))
OSPLIT = int(os.environ.get('OSPLIT', '0'))
LNIN = int(os.environ.get('LNIN', '4'))

_PROF = bool(os.environ.get("PROF"))


def _scope(name):
    return jax.named_scope(name) if _PROF else contextlib.nullcontext()


f32 = jnp.float32
bf16 = jnp.bfloat16
u32 = jnp.uint32


def _nh(w):
    return HPW if w < NW - 1 else H - HPW * (NW - 1)


def _pack(x):
    return pltpu.bitcast(x.astype(bf16), u32)


def _unpack(x):
    return pltpu.bitcast(x, bf16)


def _phi(t):
    return jnp.where(t > 0, t + 1.0, jnp.exp(t))


RC = 16
NCH = D // RC


class _Acc:
    def __init__(self, n=2):
        self.parts = [None] * n
        self.i = 0

    def add(self, x):
        k = self.i % len(self.parts)
        self.parts[k] = x if self.parts[k] is None else self.parts[k] + x
        self.i += 1

    def total(self):
        t = self.parts[0]
        for p in self.parts[1:]:
            t = t + p
        return jnp.sum(t, axis=0, keepdims=True)


def _ln_stats(chunk):
    x0 = chunk(0)
    c = x0[0:1]
    s1, s2 = _Acc(), _Acc()
    for i in range(NCH):
        d = (x0 if i == 0 else chunk(i)) - c
        s1.add(d)
        s2.add(d * d)
    mu = s1.total() * (1.0 / D)
    var = jnp.maximum(s2.total() * (1.0 / D) - mu * mu, 0.0)
    return c + mu, lax.rsqrt(var + EPS)


def _sigmoid(x):
    return 1.0 / (1.0 + jnp.exp(-x))


def _kernel(xT_hbm, wq_hbm, wk_hbm, wv_hbm, wo_hbm, beta_ref, wr_ref, wg_hbm, wu_hbm, wdT_hbm,
            out_hbm,
            x_v, wq_v, wk_v, wv_v, wo_v, wg_v, wu_v, wdT_v,
            wT, woT, wd_s, g_s, wr_s,
            xn_s, k_s, phikT_s, qT_s, phiqT_s, vT_s, mt_s, mtb_s, am_s,
            s_scr, m_scr, oT_s, out_v, h_s, st_s, r_s, xs_keep,
            sem_x, sem_w, sem_o):
    def x_copy(s):
        return pltpu.make_async_copy(xT_hbm.at[:, pl.ds(s * L, L)], x_v.at[s], sem_x.at[s])

    def o_copy(t):
        return pltpu.make_async_copy(out_v.at[t], out_hbm.at[:, pl.ds(pl.multiple_of(t * 128, 128), 128)],
                                     sem_o.at[t])

    w_copies = [pltpu.make_async_copy(src, dst, sem_w.at[i]) for i, (src, dst) in enumerate(
        [(wk_hbm, wk_v), (wq_hbm, wq_v), (wv_hbm, wv_v), (wo_hbm, wo_v),
         (wdT_hbm, wdT_v), (wg_hbm, wg_v), (wu_hbm, wu_v)])]

    def ln1_tile(seg, t):
        cols = pl.ds(pl.multiple_of(t * 128, 128), 128)

        def chunk(i):
            return x_v[seg, RC * i:RC * (i + 1), cols].astype(f32)
        mean, rstd = _ln_stats(chunk)
        for i in range(NCH):
            xn_s[t, RC * i:RC * (i + 1), :] = ((chunk(i) - mean) * rstd).astype(bf16)

    def proj_rows(lo, hi):
        xn = jnp.concatenate([xn_s[t] for t in range(4)], axis=1)
        return jnp.dot(wT[lo:hi, :], xn, preferred_element_type=f32)

    def proj(i, head=None):
        lo = D * i if head is None else D * i + head.shape[0]
        parts = [] if head is None else [head]
        parts += [proj_rows(lo, D * (i + 1)), jnp.zeros((64, L), f32)]
        return jnp.concatenate(parts, axis=0)

    def post_k(r):
        for t in range(4):
            for w in range(NW):
                kk = r[WL * w:WL * w + 128, 128 * t:128 * (t + 1)]
                k_s[w, 64 * t:64 * (t + 1), :] = pltpu.bitcast(kk.astype(bf16).T, u32)
                phikT_s[w, t] = _pack(_phi(kk))

    def post_v(r):
        rr = lax.broadcasted_iota(jnp.int32, (RS, 128), 0)
        ones_row = jnp.where(rr == DH, 1.0, 0.0).astype(f32)
        for t in range(4):
            for w in range(NW):
                nh = _nh(w)
                vs = [jnp.where(rr < DH,
                                r[DH * (HPW * w + a):DH * (HPW * w + a) + RS, 128 * t:128 * (t + 1)], ones_row)
                      for a in range(nh)]
                if (nh * RS) % 16:
                    vs.append(jnp.zeros((16 - (nh * RS) % 16, 128), f32))
                vv = _pack(jnp.concatenate(vs, axis=0))
                vT_s[w, t, 0:vv.shape[0], :] = vv

    def post_q(r):
        for t in range(4):
            for w in range(NW):
                q = r[WL * w:WL * w + 128, 128 * t:128 * (t + 1)]
                qT_s[w, t] = _pack(q * QSCALE)
                phiqT_s[w, t] = _pack(_phi(q))

    def mem_update(ws=range(NW)):
        r = lax.broadcasted_iota(jnp.int32, (MROWS, 128), 0)
        c = lax.broadcasted_iota(jnp.int32, (MROWS, 128), 1)
        for w in ws:
            vt = jnp.concatenate([_unpack(vT_s[w, t, 0:MROWS // 2, :]) for t in range(4)], axis=1)
            pk = jnp.concatenate([_unpack(phikT_s[w, t]) for t in range(4)], axis=1)
            upd = lax.dot_general(vt, pk, (((1,), (1,)), ((), ())), preferred_element_type=f32)
            mt = mt_s[w] + upd
            mt_s[w] = mt
            keep = jnp.zeros((MROWS, 128), jnp.bool_)
            for a in range(_nh(w)):
                keep = keep | ((r >= RS * a) & (r < RS * (a + 1)) & (c >= DH * a) & (c < DH * (a + 1)))
            mtb_s[w] = _pack(jnp.where(keep, mt, 0.0))

    def mem_retrieve():
        for w in range(NW):
            for j in range(4):
                am = jnp.dot(_unpack(mtb_s[w]), _unpack(phiqT_s[w, j]), preferred_element_type=f32)
                for a in range(_nh(w)):
                    ama = am[RS * a:RS * a + 24]
                    g = g_s[w, a:a + 1, :]
                    om = ama * (g / (ama[DH:DH + 1] + 1e-6))
                    am_s[j, WL * w + DH * a:WL * w + DH * (a + 1), :] = om[0:DH]

    def phase_a(w, heads, j, buf):
        n = 128 * (j + 1)
        nh = len(heads)
        cols = slice(128 * heads[0], 128 * (heads[-1] + 1))
        rows = lax.broadcasted_iota(jnp.int32, (64, 128), 0)
        qw = qT_s[w, j]
        qbd = jnp.concatenate(
            [jnp.where((rows >= 9 * a) & (rows < 9 * a + 9), qw, jnp.uint32(0)) for a in heads], axis=1)
        s = jnp.dot(_unpack(k_s[w, 0:n // 2, :]), _unpack(qbd), preferred_element_type=f32)
        kr = lax.broadcasted_iota(jnp.int32, (128, 128), 0)
        qc = lax.broadcasted_iota(jnp.int32, (128, 128), 1)
        causal = kr <= qc
        sd = jnp.concatenate(
            [jnp.where(causal, s[n - 128:n, 128 * a:128 * (a + 1)], NEG) for a in range(nh)], axis=1)
        s_scr[buf, n - 128:n, cols] = sd
        m = jnp.max(sd, axis=0, keepdims=True)
        if j > 0:
            s_scr[buf, 0:n - 128, cols] = s[0:n - 128]
            m = jnp.maximum(m, jnp.max(s[0:n - 128], axis=0, keepdims=True))
        m_scr[buf, :, cols] = jnp.broadcast_to(m, (8, 128 * nh))

    def phase_b(w, heads, j, buf):
        n = 128 * (j + 1)
        for a in heads:
            m = m_scr[buf, 0:1, 128 * a:128 * (a + 1)]
            p = jnp.exp2(s_scr[buf, 0:n, 128 * a:128 * (a + 1)] - m).astype(bf16)
            vt = jnp.concatenate([_unpack(vT_s[w, t, (RS // 2) * a:(RS // 2) * a + 16, :]) for t in range(j + 1)], axis=1)
            o = jnp.dot(vt, p, preferred_element_type=f32)
            g = g_s[w, a:a + 1, :]
            od = o[0:24] * ((1.0 - g) / o[DH:DH + 1])
            row0 = WL * w + DH * a
            oT_s[j, pl.ds(row0, DH), :] = (od + am_s[j, pl.ds(row0, 24), :])[0:DH]

    def groups(w):
        nh = _nh(w)
        if GROUP == 0 or nh <= GROUP:
            return [list(range(nh))]
        return [list(range(0, GROUP)), list(range(GROUP, nh))]

    def window(w, nxt, filler=None):
        order = [3, 2, 1, 0]
        for t in range(4):
            if filler is not None and LNPOS == 2 * t:
                filler()
            ga = groups(w) if t < 3 else (groups(nxt) if nxt is not None else [])
            gb = groups(w)
            for i in range(max(len(ga), len(gb))):
                if i < len(ga):
                    if t < 3:
                        phase_a(w, ga[i], order[t + 1], (t + 1) % 2)
                    else:
                        phase_a(nxt, ga[i], order[0], 0)
                if t == 3 and nxt is None and i == 0:
                    mem_update(range(WFILL))
                if i < len(gb):
                    phase_b(w, gb[i], order[t], t % 2)

    def outproj(seg):
        oT = jnp.concatenate([oT_s[t] for t in range(4)], axis=1).astype(bf16)
        if OSPLIT:
            rem = jnp.dot(woT[:, 512:D], oT[512:D], preferred_element_type=f32)
            attn = rem + jnp.dot(woT[:, 0:512], oT[0:512], preferred_element_type=f32)
        else:
            attn = jnp.dot(woT[...], oT, preferred_element_type=f32)
        for t in range(4):
            cols = slice(128 * t, 128 * (t + 1))
            tile = 4 * seg + t
            c = None
            s1, s2, s3 = _Acc(), _Acc(), _Acc()
            for i in range(NCH):
                rows = slice(RC * i, RC * (i + 1))
                h = x_v[seg, rows, cols].astype(f32) + attn[rows, cols]
                h_s[tile, rows, :] = h
                if c is None:
                    c = h[0:1]
                d = h - c
                s1.add(d)
                s2.add(d * d)
                s3.add(d * wr_s[rows, :])
            mu = s1.total() * (1.0 / D)
            var = jnp.maximum(s2.total() * (1.0 / D) - mu * mu, 0.0)
            rstd = lax.rsqrt(var + EPS)
            mean = c + mu
            st_s[tile, 0:1, :] = mean
            st_s[tile, 1:2, :] = rstd
            r_s[pl.ds(tile, 1), :] = (s3.total() - mu * wr_s[D:D + 1, :]) * rstd
            ga = 1.0 + rstd
            gb = mean * rstd
            for i in range(NCH):
                rows = slice(RC * i, RC * (i + 1))
                out_v[tile, rows, :] = (h_s[tile, rows, :] * ga - gb).astype(bf16)

    def transpose_wd(seg):
        nblk = F // 128 // (NSEG - 1)
        for i in range(nblk):
            c0 = pl.multiple_of((seg * nblk + i) * 128, 128)
            wd_s[pl.ds(c0, 128), :] = wdT_v[:, pl.ds(c0, 128)].T

    def project_segment():
        post_k(proj(0))
        post_q(proj(1))
        post_v(proj(2))

    with _scope("setup"):
        x_copy(0).start()
        if PRO == 0:
            w_copies[0].start()
        beta = beta_ref[...].astype(f32).reshape(1, H)
        hrow = lax.broadcasted_iota(jnp.int32, (8 * NW, H), 0)
        hcol = lax.broadcasted_iota(jnp.int32, (8 * NW, H), 1)
        sel = (hcol == HPW * (hrow >> 3) + (hrow & 7)) & ((hrow & 7) < HPW)
        bcol = jnp.sum(jnp.where(sel, beta, 0.0), axis=1, keepdims=True)
        g_s[...] = jnp.broadcast_to(_sigmoid(bcol), (8 * NW, 128)).reshape(NW, 8, 128)
        wr_row = wr_ref[...].astype(f32).reshape(1, D)
        wr_pad = jnp.concatenate([wr_row, jnp.zeros((1, 64), f32)], axis=1)
        wr_s[...] = jnp.broadcast_to(wr_pad, (128, D + 64)).T
        wr_s[D:D + 1, :] = jnp.broadcast_to(jnp.sum(wr_row, axis=1, keepdims=True), (1, 128))

        if PRO == 1:
            w_copies[0].start()
        mt_s[...] = jnp.zeros(mt_s.shape, f32)
        vT_s[...] = jnp.zeros(vT_s.shape, u32)
        am_s[...] = jnp.zeros(am_s.shape, f32)
        s_scr[:, 0:8, 0:128] = jnp.zeros((2, 8, 128), f32)
        m_scr[...] = jnp.zeros(m_scr.shape, f32)

        if PRO == 2:
            w_copies[0].start()
        x_copy(0).wait()
        w_copies[1].start()
        for t in range(4):
            ln1_tile(0, t)
    with _scope("proj0"):
        w_copies[0].wait()
        w_copies[2].start()
        wT[0:D, :] = wk_v[...].T
        post_k(proj(0))
        w_copies[1].wait()
        w_copies[2].wait()
        w_copies[3].start()
        for s in range(1, NSEG):
            x_copy(s).start()
        wT[D:2 * D, :] = wq_v[...].T
        wT[2 * D:3 * D, :] = wv_v[...].T
        post_q(proj(1))
        post_v(proj(2))
        w_copies[3].wait()
        for s in range(1, NSEG):
            x_copy(s).wait()
        w_copies[4].start()

    def segment(seg, carry):
        nseg = jnp.minimum(seg + 1, NSEG - 1)

        with _scope("windows"):
            for hs in groups(0):
                phase_a(0, hs, 3, 0)
            for w in range(NW):
                window(w, w + 1 if w + 1 < NW else None,
                       functools.partial(ln1_tile, nseg, w) if w < LNIN else None)
            for t in range(LNIN, 4):
                ln1_tile(nseg, t)

        @pl.when(seg < NSEG - 1)
        def _():
            @pl.when(seg == 0)
            def _():
                w_copies[4].wait()
                for c in w_copies[5:]:
                    c.start()

            with _scope("mid"):
                woT[...] = wo_v[...].T
                transpose_wd(seg)
                steps = {
                    "u": lambda: mem_update(range(WFILL, NW)),
                    "o": lambda: outproj(seg),
                    "k": lambda: post_k(proj(0)),
                    "q": lambda: post_q(proj(1)),
                    "v": lambda: post_v(proj(2)),
                    "r": mem_retrieve,
                }
                for c in MID_ORDER:
                    steps[c]()
                for t in range(4):
                    o_copy(4 * seg + t).start()
        return carry

    lax.fori_loop(0, NSEG, segment, 0)
    with _scope("last_out"):
        xs_keep[...] = s_scr[0, 0:8, 0:128] + s_scr[1, 0:8, 0:128] + m_scr[0, :, 0:128] + m_scr[1, :, 0:128]
        outproj(NSEG - 1)
        for t in range(4):
            o_copy(4 * (NSEG - 1) + t).start()

    with _scope("ffn"):
        r = r_s[...]
        rmax = jnp.max(r)
        tok = (lax.broadcasted_iota(jnp.int32, (NT, 128), 0) * 128
               + lax.broadcasted_iota(jnp.int32, (NT, 128), 1))
        idx = jnp.minimum(jnp.min(jnp.where(r == rmax, tok, S)), S - 1)
        tile = idx >> 7
        lane = idx & 127
        hn = ((h_s[tile] - st_s[tile, 0:1, :]) * st_s[tile, 1:2, :]).astype(bf16)
        onehot = jnp.where(lax.broadcasted_iota(jnp.int32, (16, 128), 1) == lane, 1.0, 0.0).astype(bf16)
        xs = lax.dot_general(onehot, hn, (((1,), (1,)), ((), ())), preferred_element_type=f32)
        for c in w_copies[5:]:
            c.wait()
        xm = xs[:, 0:512].astype(bf16)
        xr = xs[:, 512:D]
        row = lax.broadcasted_iota(jnp.int32, (16, 64), 0)
        x2 = jnp.concatenate([jnp.where(row == 0, xr, 0.0), jnp.where(row == 1, xr, 0.0)], axis=1).astype(bf16)
        wrem = jnp.concatenate([wg_v[512:D, :], wu_v[512:D, :]], axis=0)
        rem = jnp.dot(x2, wrem, preferred_element_type=f32)
        gate = jnp.dot(xm, wg_v[0:512, :], preferred_element_type=f32)[0:1] + rem[0:1]
        up = jnp.dot(xm, wu_v[0:512, :], preferred_element_type=f32)[0:1] + rem[1:2]
        act = jnp.broadcast_to(gate * _sigmoid(gate) * up, (16, F)).astype(bf16)
        y = jnp.dot(act, wd_s[...], preferred_element_type=f32)
        y = y[0:1] * _sigmoid(jnp.full((1, 1), rmax, f32))
        ypad = jnp.concatenate([y, jnp.zeros((1, 64), f32)], axis=1)
        ycol = jnp.broadcast_to(ypad, (128, D + 64)).T[0:D]
        for t in range(NT):
            o_copy(t).wait()
        lanes = lax.broadcasted_iota(jnp.int32, (D, 128), 1)
        blk = out_v[tile].astype(f32)
        out_v[tile] = jnp.where(lanes == lane, blk + ycol, blk).astype(bf16)
        fix = o_copy(tile)
        fix.start()
        fix.wait()


@jax.jit
def pallas_sequential_preLN__memory_aug_infini_attn__moe_arch_mod__prompt_kernel(
    A_x: jax.Array,
    A_wq: jax.Array,
    A_wk: jax.Array,
    A_wv: jax.Array,
    A_wo: jax.Array,
    A_beta: jax.Array,
    B_x: jax.Array,
    B_w_r: jax.Array,
    B_w_gate: jax.Array,
    B_w_up: jax.Array,
    B_w_down: jax.Array,
):
    del B_x
    xT = A_x.reshape(S, D).T
    wdT = B_w_down.T

    hbm = pl.BlockSpec(memory_space=pltpu.HBM)
    vmem = pl.BlockSpec(memory_space=pltpu.VMEM)
    scratch = [
        pltpu.VMEM((NSEG, D, L), bf16),
        pltpu.VMEM((D, D), bf16),
        pltpu.VMEM((D, D), bf16),
        pltpu.VMEM((D, D), bf16),
        pltpu.VMEM((D, D), bf16),
        pltpu.VMEM((D, F), bf16),
        pltpu.VMEM((D, F), bf16),
        pltpu.VMEM((D, F), bf16),
        pltpu.VMEM((3 * D, D), bf16),
        pltpu.VMEM((D, D), bf16),
        pltpu.VMEM((F, D), bf16),
        pltpu.VMEM((NW, 8, 128), f32),
        pltpu.VMEM((D + 64, 128), f32),
        pltpu.VMEM((4, D, 128), bf16),
        pltpu.VMEM((NW, L // 2, 128), u32),
        pltpu.VMEM((NW, 4, 64, 128), u32),
        pltpu.VMEM((NW, 4, 64, 128), u32),
        pltpu.VMEM((NW, 4, 64, 128), u32),
        pltpu.VMEM((NW, 4, VWORDS, 128), u32),
        pltpu.VMEM((NW, MROWS, 128), f32),
        pltpu.VMEM((NW, MROWS // 2, 128), u32),
        pltpu.VMEM((4, D + 8, 128), f32),
        pltpu.VMEM((2, L, 128 * HPW), f32),
        pltpu.VMEM((2, 8, 128 * HPW), f32),
        pltpu.VMEM((4, D, 128), f32),
        pltpu.VMEM((NT, D, 128), bf16),
        pltpu.VMEM((NT, D, 128), f32),
        pltpu.VMEM((NT, 8, 128), f32),
        pltpu.VMEM((NT, 128), f32),
        pltpu.VMEM((8, 128), f32),
        pltpu.SemaphoreType.DMA((NSEG,)),
        pltpu.SemaphoreType.DMA((7,)),
        pltpu.SemaphoreType.DMA((NT,)),
    ]
    outT = pl.pallas_call(
        _kernel,
        out_shape=jax.ShapeDtypeStruct((D, S), bf16),
        in_specs=[hbm, hbm, hbm, hbm, hbm, vmem, vmem, hbm, hbm, hbm],
        out_specs=hbm,
        scratch_shapes=scratch,
        compiler_params=pltpu.CompilerParams(vmem_limit_bytes=100 * 1024 * 1024),
    )(xT, A_wq, A_wk, A_wv, A_wo, A_beta, B_w_r, B_w_gate, B_w_up, B_w_down.T)
    return outT.T.reshape(1, S, D)
```

```python
import contextlib
import functools
import os

import jax
import jax.numpy as jnp
from jax import lax
import jax.experimental.pallas as pl
import jax.experimental.pallas.tpu as pltpu

S = 2048
D = 576
H = 32
DH = 18
NSEG = 4
L = 512
NT = S // 128
F = 4608
HPW = 7
NW = 5
WL = HPW * DH
RS = 20
MROWS = 144
VWORDS = 80
LOG2E = 1.4426950408889634
NEG = -1e9 * LOG2E
QSCALE = (DH ** -0.5) * LOG2E
EPS = 1e-5
MID_ORDER = os.environ.get('MID_ORDER', 'ukqvor')
WFILL = int(os.environ.get('WFILL', '1'))
LNPOS = int(os.environ.get('LNPOS', '0'))
GROUP = int(os.environ.get('GROUP', '0'))
BFIRST = int(os.environ.get('BFIRST', '0'))
PRO = int(os.environ.get('PRO', '1'))
OSPLIT = int(os.environ.get('OSPLIT', '0'))
LNSPLIT = int(os.environ.get('LNSPLIT', '0'))

_PROF = bool(os.environ.get("PROF"))


def _scope(name):
    return jax.named_scope(name) if _PROF else contextlib.nullcontext()


f32 = jnp.float32
bf16 = jnp.bfloat16
u32 = jnp.uint32


def _nh(w):
    return HPW if w < NW - 1 else H - HPW * (NW - 1)


def _pack(x):
    return pltpu.bitcast(x.astype(bf16), u32)


def _unpack(x):
    return pltpu.bitcast(x, bf16)


def _phi(t):
    return jnp.where(t > 0, t + 1.0, jnp.exp(t))


RC = 16
NCH = D // RC


class _Acc:
    def __init__(self, n=2):
        self.parts = [None] * n
        self.i = 0

    def add(self, x):
        k = self.i % len(self.parts)
        self.parts[k] = x if self.parts[k] is None else self.parts[k] + x
        self.i += 1

    def total(self):
        t = self.parts[0]
        for p in self.parts[1:]:
            t = t + p
        return jnp.sum(t, axis=0, keepdims=True)


def _ln_stats(chunk):
    x0 = chunk(0)
    c = x0[0:1]
    s1, s2 = _Acc(), _Acc()
    for i in range(NCH):
        d = (x0 if i == 0 else chunk(i)) - c
        s1.add(d)
        s2.add(d * d)
    mu = s1.total() * (1.0 / D)
    var = jnp.maximum(s2.total() * (1.0 / D) - mu * mu, 0.0)
    return c + mu, lax.rsqrt(var + EPS)


def _sigmoid(x):
    return 1.0 / (1.0 + jnp.exp(-x))


def _kernel(xT_hbm, wq_hbm, wk_hbm, wv_hbm, wo_hbm, beta_ref, wr_ref, wg_hbm, wu_hbm, wdT_hbm,
            out_hbm,
            x_v, wq_v, wk_v, wv_v, wo_v, wg_v, wu_v, wdT_v,
            wT, woT, wd_s, g_s, wr_s,
            xn_s, k_s, phikT_s, qT_s, phiqT_s, vT_s, mt_s, mtb_s, am_s,
            s_scr, m_scr, oT_s, out_v, h_s, st_s, r_s, xs_keep,
            sem_x, sem_w, sem_o):
    def x_copy(s):
        return pltpu.make_async_copy(xT_hbm.at[:, pl.ds(s * L, L)], x_v.at[s], sem_x.at[s])

    def o_copy(t):
        return pltpu.make_async_copy(out_v.at[t], out_hbm.at[:, pl.ds(pl.multiple_of(t * 128, 128), 128)],
                                     sem_o.at[t])

    w_copies = [pltpu.make_async_copy(src, dst, sem_w.at[i]) for i, (src, dst) in enumerate(
        [(wk_hbm, wk_v), (wq_hbm, wq_v), (wv_hbm, wv_v), (wo_hbm, wo_v),
         (wdT_hbm, wdT_v), (wg_hbm, wg_v), (wu_hbm, wu_v)])]

    def ln1_chunk(seg, t, i):
        cols = pl.ds(pl.multiple_of(t * 128, 128), 128)
        return x_v[seg, RC * i:RC * (i + 1), cols].astype(f32)

    def ln1_stats(seg, t):
        return _ln_stats(functools.partial(ln1_chunk, seg, t))

    def ln1_norm(seg, t, stats):
        mean, rstd = stats
        for i in range(NCH):
            xn_s[t, RC * i:RC * (i + 1), :] = ((ln1_chunk(seg, t, i) - mean) * rstd).astype(bf16)

    def ln1_tile(seg, t):
        ln1_norm(seg, t, ln1_stats(seg, t))

    def proj(i):
        xn = jnp.concatenate([xn_s[t] for t in range(4)], axis=1)
        r = jnp.dot(wT[D * i:D * (i + 1), :], xn, preferred_element_type=f32)
        return jnp.concatenate([r, jnp.zeros((64, L), f32)], axis=0)

    def post_k(r):
        for t in range(4):
            for w in range(NW):
                kk = r[WL * w:WL * w + 128, 128 * t:128 * (t + 1)]
                k_s[w, 64 * t:64 * (t + 1), :] = pltpu.bitcast(kk.astype(bf16).T, u32)
                phikT_s[w, t] = _pack(_phi(kk))

    def post_v(r):
        rr = lax.broadcasted_iota(jnp.int32, (RS, 128), 0)
        ones_row = jnp.where(rr == DH, 1.0, 0.0).astype(f32)
        for t in range(4):
            for w in range(NW):
                nh = _nh(w)
                vs = [jnp.where(rr < DH,
                                r[DH * (HPW * w + a):DH * (HPW * w + a) + RS, 128 * t:128 * (t + 1)], ones_row)
                      for a in range(nh)]
                if (nh * RS) % 16:
                    vs.append(jnp.zeros((16 - (nh * RS) % 16, 128), f32))
                vv = _pack(jnp.concatenate(vs, axis=0))
                vT_s[w, t, 0:vv.shape[0], :] = vv

    def post_q(r):
        for t in range(4):
            for w in range(NW):
                q = r[WL * w:WL * w + 128, 128 * t:128 * (t + 1)]
                qT_s[w, t] = _pack(q * QSCALE)
                phiqT_s[w, t] = _pack(_phi(q))

    def mem_update(ws=range(NW)):
        r = lax.broadcasted_iota(jnp.int32, (MROWS, 128), 0)
        c = lax.broadcasted_iota(jnp.int32, (MROWS, 128), 1)
        for w in ws:
            vt = jnp.concatenate([_unpack(vT_s[w, t, 0:MROWS // 2, :]) for t in range(4)], axis=1)
            pk = jnp.concatenate([_unpack(phikT_s[w, t]) for t in range(4)], axis=1)
            upd = lax.dot_general(vt, pk, (((1,), (1,)), ((), ())), preferred_element_type=f32)
            mt = mt_s[w] + upd
            mt_s[w] = mt
            keep = jnp.zeros((MROWS, 128), jnp.bool_)
            for a in range(_nh(w)):
                keep = keep | ((r >= RS * a) & (r < RS * (a + 1)) & (c >= DH * a) & (c < DH * (a + 1)))
            mtb_s[w] = _pack(jnp.where(keep, mt, 0.0))

    def mem_retrieve():
        for w in range(NW):
            for j in range(4):
                am = jnp.dot(_unpack(mtb_s[w]), _unpack(phiqT_s[w, j]), preferred_element_type=f32)
                for a in range(_nh(w)):
                    ama = am[RS * a:RS * a + 24]
                    g = g_s[w, a:a + 1, :]
                    om = ama * (g / (ama[DH:DH + 1] + 1e-6))
                    am_s[j, WL * w + DH * a:WL * w + DH * (a + 1), :] = om[0:DH]

    def phase_a(w, heads, j, buf):
        n = 128 * (j + 1)
        nh = len(heads)
        cols = slice(128 * heads[0], 128 * (heads[-1] + 1))
        rows = lax.broadcasted_iota(jnp.int32, (64, 128), 0)
        qw = qT_s[w, j]
        qbd = jnp.concatenate(
            [jnp.where((rows >= 9 * a) & (rows < 9 * a + 9), qw, jnp.uint32(0)) for a in heads], axis=1)
        s = jnp.dot(_unpack(k_s[w, 0:n // 2, :]), _unpack(qbd), preferred_element_type=f32)
        kr = lax.broadcasted_iota(jnp.int32, (128, 128), 0)
        qc = lax.broadcasted_iota(jnp.int32, (128, 128), 1)
        causal = kr <= qc
        sd = jnp.concatenate(
            [jnp.where(causal, s[n - 128:n, 128 * a:128 * (a + 1)], NEG) for a in range(nh)], axis=1)
        s_scr[buf, n - 128:n, cols] = sd
        m = jnp.max(sd, axis=0, keepdims=True)
        if j > 0:
            s_scr[buf, 0:n - 128, cols] = s[0:n - 128]
            m = jnp.maximum(m, jnp.max(s[0:n - 128], axis=0, keepdims=True))
        m_scr[buf, :, cols] = jnp.broadcast_to(m, (8, 128 * nh))

    def phase_b(w, heads, j, buf):
        n = 128 * (j + 1)
        for a in heads:
            m = m_scr[buf, 0:1, 128 * a:128 * (a + 1)]
            p = jnp.exp2(s_scr[buf, 0:n, 128 * a:128 * (a + 1)] - m).astype(bf16)
            vt = jnp.concatenate([_unpack(vT_s[w, t, (RS // 2) * a:(RS // 2) * a + 16, :]) for t in range(j + 1)], axis=1)
            o = jnp.dot(vt, p, preferred_element_type=f32)
            g = g_s[w, a:a + 1, :]
            od = o[0:24] * ((1.0 - g) / o[DH:DH + 1])
            row0 = WL * w + DH * a
            oT_s[j, pl.ds(row0, DH), :] = (od + am_s[j, pl.ds(row0, 24), :])[0:DH]

    def groups(w):
        nh = _nh(w)
        if GROUP == 0 or nh <= GROUP:
            return [list(range(nh))]
        return [list(range(0, GROUP)), list(range(GROUP, nh))]

    def window(w, nxt, fillers):
        order = [3, 2, 1, 0]
        for t in range(4):
            for fn in fillers.get(t, ()):
                fn()
            ga = groups(w) if t < 3 else (groups(nxt) if nxt is not None else [])
            gb = groups(w)
            for i in range(max(len(ga), len(gb))):
                if BFIRST and i < len(gb):
                    phase_b(w, gb[i], order[t], t % 2)
                if i < len(ga):
                    if t < 3:
                        phase_a(w, ga[i], order[t + 1], (t + 1) % 2)
                    else:
                        phase_a(nxt, ga[i], order[0], 0)
                if t == 3 and nxt is None and i == 0:
                    mem_update(range(WFILL))
                if not BFIRST and i < len(gb):
                    phase_b(w, gb[i], order[t], t % 2)

    def outproj(seg):
        oT = jnp.concatenate([oT_s[t] for t in range(4)], axis=1).astype(bf16)
        if OSPLIT:
            rem = jnp.dot(woT[:, 512:D], oT[512:D], preferred_element_type=f32)
            attn = rem + jnp.dot(woT[:, 0:512], oT[0:512], preferred_element_type=f32)
        else:
            attn = jnp.dot(woT[...], oT, preferred_element_type=f32)
        for t in range(4):
            cols = slice(128 * t, 128 * (t + 1))
            tile = 4 * seg + t
            c = None
            s1, s2, s3 = _Acc(), _Acc(), _Acc()
            for i in range(NCH):
                rows = slice(RC * i, RC * (i + 1))
                h = x_v[seg, rows, cols].astype(f32) + attn[rows, cols]
                h_s[tile, rows, :] = h
                if c is None:
                    c = h[0:1]
                d = h - c
                s1.add(d)
                s2.add(d * d)
                s3.add(d * wr_s[rows, :])
            mu = s1.total() * (1.0 / D)
            var = jnp.maximum(s2.total() * (1.0 / D) - mu * mu, 0.0)
            rstd = lax.rsqrt(var + EPS)
            mean = c + mu
            st_s[tile, 0:1, :] = mean
            st_s[tile, 1:2, :] = rstd
            r_s[pl.ds(tile, 1), :] = (s3.total() - mu * wr_s[D:D + 1, :]) * rstd
            ga = 1.0 + rstd
            gb = mean * rstd
            for i in range(NCH):
                rows = slice(RC * i, RC * (i + 1))
                out_v[tile, rows, :] = (h_s[tile, rows, :] * ga - gb).astype(bf16)

    def transpose_wd(seg):
        nblk = F // 128 // (NSEG - 1)
        for i in range(nblk):
            c0 = pl.multiple_of((seg * nblk + i) * 128, 128)
            wd_s[pl.ds(c0, 128), :] = wdT_v[:, pl.ds(c0, 128)].T

    def project_segment():
        post_k(proj(0))
        post_q(proj(1))
        post_v(proj(2))

    with _scope("setup"):
        x_copy(0).start()
        if PRO == 0:
            w_copies[0].start()
        beta = beta_ref[...].astype(f32).reshape(1, H)
        hrow = lax.broadcasted_iota(jnp.int32, (8 * NW, H), 0)
        hcol = lax.broadcasted_iota(jnp.int32, (8 * NW, H), 1)
        sel = (hcol == HPW * (hrow >> 3) + (hrow & 7)) & ((hrow & 7) < HPW)
        bcol = jnp.sum(jnp.where(sel, beta, 0.0), axis=1, keepdims=True)
        g_s[...] = jnp.broadcast_to(_sigmoid(bcol), (8 * NW, 128)).reshape(NW, 8, 128)
        wr_row = wr_ref[...].astype(f32).reshape(1, D)
        wr_pad = jnp.concatenate([wr_row, jnp.zeros((1, 64), f32)], axis=1)
        wr_s[...] = jnp.broadcast_to(wr_pad, (128, D + 64)).T
        wr_s[D:D + 1, :] = jnp.broadcast_to(jnp.sum(wr_row, axis=1, keepdims=True), (1, 128))

        if PRO == 1:
            w_copies[0].start()
        mt_s[...] = jnp.zeros(mt_s.shape, f32)
        vT_s[...] = jnp.zeros(vT_s.shape, u32)
        am_s[...] = jnp.zeros(am_s.shape, f32)
        s_scr[:, 0:8, 0:128] = jnp.zeros((2, 8, 128), f32)
        m_scr[...] = jnp.zeros(m_scr.shape, f32)

        if PRO == 2:
            w_copies[0].start()
        x_copy(0).wait()
        w_copies[1].start()
        for t in range(4):
            ln1_tile(0, t)
    with _scope("proj0"):
        w_copies[0].wait()
        w_copies[2].start()
        wT[0:D, :] = wk_v[...].T
        post_k(proj(0))
        w_copies[1].wait()
        w_copies[2].wait()
        w_copies[3].start()
        for s in range(1, NSEG):
            x_copy(s).start()
        wT[D:2 * D, :] = wq_v[...].T
        wT[2 * D:3 * D, :] = wv_v[...].T
        post_q(proj(1))
        post_v(proj(2))
        w_copies[3].wait()
        for s in range(1, NSEG):
            x_copy(s).wait()
        w_copies[4].start()

    def segment(seg, carry):
        nseg = jnp.minimum(seg + 1, NSEG - 1)

        with _scope("windows"):
            for hs in groups(0):
                phase_a(0, hs, 3, 0)
            stats = {}

            def do_stats(t):
                stats[t] = ln1_stats(nseg, t)

            def do_norm(t):
                ln1_norm(nseg, t, stats[t])

            if LNSPLIT:
                do_stats(0)
            for w in range(NW):
                fillers = {}
                if not LNSPLIT:
                    if w < 4:
                        fillers = {LNPOS: [functools.partial(do_stats, w), functools.partial(do_norm, w)]}
                else:
                    fl = []
                    if w < 4:
                        fl.append(functools.partial(do_norm, w))
                    if w + 1 < 4:
                        fl.append(functools.partial(do_stats, w + 1))
                    fillers = {LNPOS: fl}
                window(w, w + 1 if w + 1 < NW else None, fillers)

        @pl.when(seg < NSEG - 1)
        def _():
            @pl.when(seg == 0)
            def _():
                w_copies[4].wait()
                for c in w_copies[5:]:
                    c.start()

            with _scope("mid"):
                woT[...] = wo_v[...].T
                transpose_wd(seg)
                steps = {
                    "u": lambda: mem_update(range(WFILL, NW)),
                    "o": lambda: outproj(seg),
                    "k": lambda: post_k(proj(0)),
                    "q": lambda: post_q(proj(1)),
                    "v": lambda: post_v(proj(2)),
                    "r": mem_retrieve,
                }
                for c in MID_ORDER:
                    steps[c]()
                for t in range(4):
                    o_copy(4 * seg + t).start()
        return carry

    lax.fori_loop(0, NSEG, segment, 0)
    with _scope("last_out"):
        xs_keep[...] = s_scr[0, 0:8, 0:128] + s_scr[1, 0:8, 0:128] + m_scr[0, :, 0:128] + m_scr[1, :, 0:128]
        outproj(NSEG - 1)
        for t in range(4):
            o_copy(4 * (NSEG - 1) + t).start()

    with _scope("ffn"):
        r = r_s[...]
        rmax = jnp.max(r)
        tok = (lax.broadcasted_iota(jnp.int32, (NT, 128), 0) * 128
               + lax.broadcasted_iota(jnp.int32, (NT, 128), 1))
        idx = jnp.minimum(jnp.min(jnp.where(r == rmax, tok, S)), S - 1)
        tile = idx >> 7
        lane = idx & 127
        hn = ((h_s[tile] - st_s[tile, 0:1, :]) * st_s[tile, 1:2, :]).astype(bf16)
        onehot = jnp.where(lax.broadcasted_iota(jnp.int32, (16, 128), 1) == lane, 1.0, 0.0).astype(bf16)
        xs = lax.dot_general(onehot, hn, (((1,), (1,)), ((), ())), preferred_element_type=f32)
        for c in w_copies[5:]:
            c.wait()
        xm = xs[:, 0:512].astype(bf16)
        xr = xs[:, 512:D]
        row = lax.broadcasted_iota(jnp.int32, (16, 64), 0)
        x2 = jnp.concatenate([jnp.where(row == 0, xr, 0.0), jnp.where(row == 1, xr, 0.0)], axis=1).astype(bf16)
        wrem = jnp.concatenate([wg_v[512:D, :], wu_v[512:D, :]], axis=0)
        rem = jnp.dot(x2, wrem, preferred_element_type=f32)
        gate = jnp.dot(xm, wg_v[0:512, :], preferred_element_type=f32)[0:1] + rem[0:1]
        up = jnp.dot(xm, wu_v[0:512, :], preferred_element_type=f32)[0:1] + rem[1:2]
        act = jnp.broadcast_to(gate * _sigmoid(gate) * up, (16, F)).astype(bf16)
        y = jnp.dot(act, wd_s[...], preferred_element_type=f32)
        y = y[0:1] * _sigmoid(jnp.full((1, 1), rmax, f32))
        ypad = jnp.concatenate([y, jnp.zeros((1, 64), f32)], axis=1)
        ycol = jnp.broadcast_to(ypad, (128, D + 64)).T[0:D]
        for t in range(NT):
            o_copy(t).wait()
        lanes = lax.broadcasted_iota(jnp.int32, (D, 128), 1)
        blk = out_v[tile].astype(f32)
        out_v[tile] = jnp.where(lanes == lane, blk + ycol, blk).astype(bf16)
        fix = o_copy(tile)
        fix.start()
        fix.wait()


@jax.jit
def pallas_sequential_preLN__memory_aug_infini_attn__moe_arch_mod__prompt_kernel(
    A_x: jax.Array,
    A_wq: jax.Array,
    A_wk: jax.Array,
    A_wv: jax.Array,
    A_wo: jax.Array,
    A_beta: jax.Array,
    B_x: jax.Array,
    B_w_r: jax.Array,
    B_w_gate: jax.Array,
    B_w_up: jax.Array,
    B_w_down: jax.Array,
):
    del B_x
    xT = A_x.reshape(S, D).T
    wdT = B_w_down.T

    hbm = pl.BlockSpec(memory_space=pltpu.HBM)
    vmem = pl.BlockSpec(memory_space=pltpu.VMEM)
    scratch = [
        pltpu.VMEM((NSEG, D, L), bf16),
        pltpu.VMEM((D, D), bf16),
        pltpu.VMEM((D, D), bf16),
        pltpu.VMEM((D, D), bf16),
        pltpu.VMEM((D, D), bf16),
        pltpu.VMEM((D, F), bf16),
        pltpu.VMEM((D, F), bf16),
        pltpu.VMEM((D, F), bf16),
        pltpu.VMEM((3 * D, D), bf16),
        pltpu.VMEM((D, D), bf16),
        pltpu.VMEM((F, D), bf16),
        pltpu.VMEM((NW, 8, 128), f32),
        pltpu.VMEM((D + 64, 128), f32),
        pltpu.VMEM((4, D, 128), bf16),
        pltpu.VMEM((NW, L // 2, 128), u32),
        pltpu.VMEM((NW, 4, 64, 128), u32),
        pltpu.VMEM((NW, 4, 64, 128), u32),
        pltpu.VMEM((NW, 4, 64, 128), u32),
        pltpu.VMEM((NW, 4, VWORDS, 128), u32),
        pltpu.VMEM((NW, MROWS, 128), f32),
        pltpu.VMEM((NW, MROWS // 2, 128), u32),
        pltpu.VMEM((4, D + 8, 128), f32),
        pltpu.VMEM((2, L, 128 * HPW), f32),
        pltpu.VMEM((2, 8, 128 * HPW), f32),
        pltpu.VMEM((4, D, 128), f32),
        pltpu.VMEM((NT, D, 128), bf16),
        pltpu.VMEM((NT, D, 128), f32),
        pltpu.VMEM((NT, 8, 128), f32),
        pltpu.VMEM((NT, 128), f32),
        pltpu.VMEM((8, 128), f32),
        pltpu.SemaphoreType.DMA((NSEG,)),
        pltpu.SemaphoreType.DMA((7,)),
        pltpu.SemaphoreType.DMA((NT,)),
    ]
    outT = pl.pallas_call(
        _kernel,
        out_shape=jax.ShapeDtypeStruct((D, S), bf16),
        in_specs=[hbm, hbm, hbm, hbm, hbm, vmem, vmem, hbm, hbm, hbm],
        out_specs=hbm,
        scratch_shapes=scratch,
        compiler_params=pltpu.CompilerParams(vmem_limit_bytes=100 * 1024 * 1024),
    )(xT, A_wq, A_wk, A_wv, A_wo, A_beta, B_w_r, B_w_gate, B_w_up, B_w_down.T)
    return outT.T.reshape(1, S, D)
```

```python
import contextlib
import functools
import os

import jax
import jax.numpy as jnp
from jax import lax
import jax.experimental.pallas as pl
import jax.experimental.pallas.tpu as pltpu

S = 2048
D = 576
H = 32
DH = 18
NSEG = 4
L = 512
NT = S // 128
F = 4608
HPW = 7
NW = 5
WL = HPW * DH
RS = 20
MROWS = 144
VWORDS = 80
LOG2E = 1.4426950408889634
NEG = -1e9 * LOG2E
QSCALE = (DH ** -0.5) * LOG2E
EPS = 1e-5
MID_ORDER = os.environ.get('MID_ORDER', 'ukqvor')
WFILL = int(os.environ.get('WFILL', '1'))
LNPOS = int(os.environ.get('LNPOS', '0'))
GROUP = int(os.environ.get('GROUP', '0'))
BFIRST = int(os.environ.get('BFIRST', '0'))
PRO = int(os.environ.get('PRO', '1'))
OSPLIT = int(os.environ.get('OSPLIT', '0'))
LNPARTS = int(os.environ.get('LNPARTS', '4'))
LNSLOTS = [int(c) for c in os.environ.get('LNSLOTS', '0123')]
LNMAX = int(os.environ.get('LNMAX', '99'))

_PROF = bool(os.environ.get("PROF"))


def _scope(name):
    return jax.named_scope(name) if _PROF else contextlib.nullcontext()


f32 = jnp.float32
bf16 = jnp.bfloat16
u32 = jnp.uint32


def _nh(w):
    return HPW if w < NW - 1 else H - HPW * (NW - 1)


def _pack(x):
    return pltpu.bitcast(x.astype(bf16), u32)


def _unpack(x):
    return pltpu.bitcast(x, bf16)


def _phi(t):
    return jnp.where(t > 0, t + 1.0, jnp.exp(t))


RC = 16
NCH = D // RC


class _Acc:
    def __init__(self, n=2):
        self.parts = [None] * n
        self.i = 0

    def add(self, x):
        k = self.i % len(self.parts)
        self.parts[k] = x if self.parts[k] is None else self.parts[k] + x
        self.i += 1

    def total(self):
        t = self.parts[0]
        for p in self.parts[1:]:
            t = t + p
        return jnp.sum(t, axis=0, keepdims=True)


def _ln_stats(chunk):
    x0 = chunk(0)
    c = x0[0:1]
    s1, s2 = _Acc(), _Acc()
    for i in range(NCH):
        d = (x0 if i == 0 else chunk(i)) - c
        s1.add(d)
        s2.add(d * d)
    mu = s1.total() * (1.0 / D)
    var = jnp.maximum(s2.total() * (1.0 / D) - mu * mu, 0.0)
    return c + mu, lax.rsqrt(var + EPS)


def _sigmoid(x):
    return 1.0 / (1.0 + jnp.exp(-x))


def _kernel(xT_hbm, wq_hbm, wk_hbm, wv_hbm, wo_hbm, beta_ref, wr_ref, wg_hbm, wu_hbm, wdT_hbm,
            out_hbm,
            x_v, wq_v, wk_v, wv_v, wo_v, wg_v, wu_v, wdT_v,
            wT, woT, wd_s, g_s, wr_s,
            xn_s, k_s, phikT_s, qT_s, phiqT_s, vT_s, mt_s, mtb_s, am_s,
            s_scr, m_scr, oT_s, out_v, h_s, st_s, r_s, xs_keep,
            sem_x, sem_w, sem_o):
    def x_copy(s):
        return pltpu.make_async_copy(xT_hbm.at[:, pl.ds(s * L, L)], x_v.at[s], sem_x.at[s])

    def o_copy(t):
        return pltpu.make_async_copy(out_v.at[t], out_hbm.at[:, pl.ds(pl.multiple_of(t * 128, 128), 128)],
                                     sem_o.at[t])

    w_copies = [pltpu.make_async_copy(src, dst, sem_w.at[i]) for i, (src, dst) in enumerate(
        [(wk_hbm, wk_v), (wq_hbm, wq_v), (wv_hbm, wv_v), (wo_hbm, wo_v),
         (wdT_hbm, wdT_v), (wg_hbm, wg_v), (wu_hbm, wu_v)])]

    def ln1_chunk(seg, t, i):
        cols = pl.ds(pl.multiple_of(t * 128, 128), 128)
        return x_v[seg, RC * i:RC * (i + 1), cols].astype(f32)

    def ln1_units(seg, t, nparts):
        st = {}
        bounds = [NCH * i // nparts for i in range(nparts + 1)]

        def stats_part(k):
            if k == 0:
                x0 = ln1_chunk(seg, t, 0)
                st["x0"], st["c"] = x0, x0[0:1]
                st["s1"], st["s2"] = _Acc(), _Acc()
            for i in range(bounds[k], bounds[k + 1]):
                d = (st["x0"] if i == 0 else ln1_chunk(seg, t, i)) - st["c"]
                st["s1"].add(d)
                st["s2"].add(d * d)
            if k == nparts - 1:
                mu = st["s1"].total() * (1.0 / D)
                var = jnp.maximum(st["s2"].total() * (1.0 / D) - mu * mu, 0.0)
                st["mean"], st["rstd"] = st["c"] + mu, lax.rsqrt(var + EPS)

        def norm_part(k):
            for i in range(bounds[k], bounds[k + 1]):
                xn = (ln1_chunk(seg, t, i) - st["mean"]) * st["rstd"]
                xn_s[t, RC * i:RC * (i + 1), :] = xn.astype(bf16)

        return ([functools.partial(stats_part, k) for k in range(nparts)],
                [functools.partial(norm_part, k) for k in range(nparts)])

    def ln1_tile(seg, t):
        stats, norm = ln1_units(seg, t, 1)
        for fn in stats + norm:
            fn()

    def proj(i):
        xn = jnp.concatenate([xn_s[t] for t in range(4)], axis=1)
        r = jnp.dot(wT[D * i:D * (i + 1), :], xn, preferred_element_type=f32)
        return jnp.concatenate([r, jnp.zeros((64, L), f32)], axis=0)

    def post_k(r):
        for t in range(4):
            for w in range(NW):
                kk = r[WL * w:WL * w + 128, 128 * t:128 * (t + 1)]
                k_s[w, 64 * t:64 * (t + 1), :] = pltpu.bitcast(kk.astype(bf16).T, u32)
                phikT_s[w, t] = _pack(_phi(kk))

    def post_v(r):
        rr = lax.broadcasted_iota(jnp.int32, (RS, 128), 0)
        ones_row = jnp.where(rr == DH, 1.0, 0.0).astype(f32)
        for t in range(4):
            for w in range(NW):
                nh = _nh(w)
                vs = [jnp.where(rr < DH,
                                r[DH * (HPW * w + a):DH * (HPW * w + a) + RS, 128 * t:128 * (t + 1)], ones_row)
                      for a in range(nh)]
                if (nh * RS) % 16:
                    vs.append(jnp.zeros((16 - (nh * RS) % 16, 128), f32))
                vv = _pack(jnp.concatenate(vs, axis=0))
                vT_s[w, t, 0:vv.shape[0], :] = vv

    def post_q(r):
        for t in range(4):
            for w in range(NW):
                q = r[WL * w:WL * w + 128, 128 * t:128 * (t + 1)]
                qT_s[w, t] = _pack(q * QSCALE)
                phiqT_s[w, t] = _pack(_phi(q))

    def mem_update(ws=range(NW)):
        r = lax.broadcasted_iota(jnp.int32, (MROWS, 128), 0)
        c = lax.broadcasted_iota(jnp.int32, (MROWS, 128), 1)
        for w in ws:
            vt = jnp.concatenate([_unpack(vT_s[w, t, 0:MROWS // 2, :]) for t in range(4)], axis=1)
            pk = jnp.concatenate([_unpack(phikT_s[w, t]) for t in range(4)], axis=1)
            upd = lax.dot_general(vt, pk, (((1,), (1,)), ((), ())), preferred_element_type=f32)
            mt = mt_s[w] + upd
            mt_s[w] = mt
            keep = jnp.zeros((MROWS, 128), jnp.bool_)
            for a in range(_nh(w)):
                keep = keep | ((r >= RS * a) & (r < RS * (a + 1)) & (c >= DH * a) & (c < DH * (a + 1)))
            mtb_s[w] = _pack(jnp.where(keep, mt, 0.0))

    def mem_retrieve():
        for w in range(NW):
            for j in range(4):
                am = jnp.dot(_unpack(mtb_s[w]), _unpack(phiqT_s[w, j]), preferred_element_type=f32)
                for a in range(_nh(w)):
                    ama = am[RS * a:RS * a + 24]
                    g = g_s[w, a:a + 1, :]
                    om = ama * (g / (ama[DH:DH + 1] + 1e-6))
                    am_s[j, WL * w + DH * a:WL * w + DH * (a + 1), :] = om[0:DH]

    def phase_a(w, heads, j, buf):
        n = 128 * (j + 1)
        nh = len(heads)
        cols = slice(128 * heads[0], 128 * (heads[-1] + 1))
        rows = lax.broadcasted_iota(jnp.int32, (64, 128), 0)
        qw = qT_s[w, j]
        qbd = jnp.concatenate(
            [jnp.where((rows >= 9 * a) & (rows < 9 * a + 9), qw, jnp.uint32(0)) for a in heads], axis=1)
        s = jnp.dot(_unpack(k_s[w, 0:n // 2, :]), _unpack(qbd), preferred_element_type=f32)
        kr = lax.broadcasted_iota(jnp.int32, (128, 128), 0)
        qc = lax.broadcasted_iota(jnp.int32, (128, 128), 1)
        causal = kr <= qc
        sd = jnp.concatenate(
            [jnp.where(causal, s[n - 128:n, 128 * a:128 * (a + 1)], NEG) for a in range(nh)], axis=1)
        s_scr[buf, n - 128:n, cols] = sd
        m = jnp.max(sd, axis=0, keepdims=True)
        if j > 0:
            s_scr[buf, 0:n - 128, cols] = s[0:n - 128]
            m = jnp.maximum(m, jnp.max(s[0:n - 128], axis=0, keepdims=True))
        m_scr[buf, :, cols] = jnp.broadcast_to(m, (8, 128 * nh))

    def phase_b(w, heads, j, buf):
        n = 128 * (j + 1)
        for a in heads:
            m = m_scr[buf, 0:1, 128 * a:128 * (a + 1)]
            p = jnp.exp2(s_scr[buf, 0:n, 128 * a:128 * (a + 1)] - m).astype(bf16)
            vt = jnp.concatenate([_unpack(vT_s[w, t, (RS // 2) * a:(RS // 2) * a + 16, :]) for t in range(j + 1)], axis=1)
            o = jnp.dot(vt, p, preferred_element_type=f32)
            g = g_s[w, a:a + 1, :]
            od = o[0:24] * ((1.0 - g) / o[DH:DH + 1])
            row0 = WL * w + DH * a
            oT_s[j, pl.ds(row0, DH), :] = (od + am_s[j, pl.ds(row0, 24), :])[0:DH]

    def groups(w):
        nh = _nh(w)
        if GROUP == 0 or nh <= GROUP:
            return [list(range(nh))]
        return [list(range(0, GROUP)), list(range(GROUP, nh))]

    def window(w, nxt, fillers):
        order = [3, 2, 1, 0]
        for t in range(4):
            for fn in fillers.get(t, ()):
                fn()
            ga = groups(w) if t < 3 else (groups(nxt) if nxt is not None else [])
            gb = groups(w)
            for i in range(max(len(ga), len(gb))):
                if BFIRST and i < len(gb):
                    phase_b(w, gb[i], order[t], t % 2)
                if i < len(ga):
                    if t < 3:
                        phase_a(w, ga[i], order[t + 1], (t + 1) % 2)
                    else:
                        phase_a(nxt, ga[i], order[0], 0)
                if t == 3 and nxt is None and i == 0:
                    mem_update(range(WFILL))
                if not BFIRST and i < len(gb):
                    phase_b(w, gb[i], order[t], t % 2)

    def outproj(seg):
        oT = jnp.concatenate([oT_s[t] for t in range(4)], axis=1).astype(bf16)
        if OSPLIT:
            rem = jnp.dot(woT[:, 512:D], oT[512:D], preferred_element_type=f32)
            attn = rem + jnp.dot(woT[:, 0:512], oT[0:512], preferred_element_type=f32)
        else:
            attn = jnp.dot(woT[...], oT, preferred_element_type=f32)
        for t in range(4):
            cols = slice(128 * t, 128 * (t + 1))
            tile = 4 * seg + t
            c = None
            s1, s2, s3 = _Acc(), _Acc(), _Acc()
            for i in range(NCH):
                rows = slice(RC * i, RC * (i + 1))
                h = x_v[seg, rows, cols].astype(f32) + attn[rows, cols]
                h_s[tile, rows, :] = h
                if c is None:
                    c = h[0:1]
                d = h - c
                s1.add(d)
                s2.add(d * d)
                s3.add(d * wr_s[rows, :])
            mu = s1.total() * (1.0 / D)
            var = jnp.maximum(s2.total() * (1.0 / D) - mu * mu, 0.0)
            rstd = lax.rsqrt(var + EPS)
            mean = c + mu
            st_s[tile, 0:1, :] = mean
            st_s[tile, 1:2, :] = rstd
            r_s[pl.ds(tile, 1), :] = (s3.total() - mu * wr_s[D:D + 1, :]) * rstd
            ga = 1.0 + rstd
            gb = mean * rstd
            for i in range(NCH):
                rows = slice(RC * i, RC * (i + 1))
                out_v[tile, rows, :] = (h_s[tile, rows, :] * ga - gb).astype(bf16)

    def transpose_wd(seg):
        nblk = F // 128 // (NSEG - 1)
        for i in range(nblk):
            c0 = pl.multiple_of((seg * nblk + i) * 128, 128)
            wd_s[pl.ds(c0, 128), :] = wdT_v[:, pl.ds(c0, 128)].T

    def project_segment():
        post_k(proj(0))
        post_q(proj(1))
        post_v(proj(2))

    with _scope("setup"):
        x_copy(0).start()
        if PRO == 0:
            w_copies[0].start()
        beta = beta_ref[...].astype(f32).reshape(1, H)
        hrow = lax.broadcasted_iota(jnp.int32, (8 * NW, H), 0)
        hcol = lax.broadcasted_iota(jnp.int32, (8 * NW, H), 1)
        sel = (hcol == HPW * (hrow >> 3) + (hrow & 7)) & ((hrow & 7) < HPW)
        bcol = jnp.sum(jnp.where(sel, beta, 0.0), axis=1, keepdims=True)
        g_s[...] = jnp.broadcast_to(_sigmoid(bcol), (8 * NW, 128)).reshape(NW, 8, 128)
        wr_row = wr_ref[...].astype(f32).reshape(1, D)
        wr_pad = jnp.concatenate([wr_row, jnp.zeros((1, 64), f32)], axis=1)
        wr_s[...] = jnp.broadcast_to(wr_pad, (128, D + 64)).T
        wr_s[D:D + 1, :] = jnp.broadcast_to(jnp.sum(wr_row, axis=1, keepdims=True), (1, 128))

        if PRO == 1:
            w_copies[0].start()
        mt_s[...] = jnp.zeros(mt_s.shape, f32)
        vT_s[...] = jnp.zeros(vT_s.shape, u32)
        am_s[...] = jnp.zeros(am_s.shape, f32)
        s_scr[:, 0:8, 0:128] = jnp.zeros((2, 8, 128), f32)
        m_scr[...] = jnp.zeros(m_scr.shape, f32)

        if PRO == 2:
            w_copies[0].start()
        x_copy(0).wait()
        w_copies[1].start()
        for t in range(4):
            ln1_tile(0, t)
    with _scope("proj0"):
        w_copies[0].wait()
        w_copies[2].start()
        wT[0:D, :] = wk_v[...].T
        post_k(proj(0))
        w_copies[1].wait()
        w_copies[2].wait()
        w_copies[3].start()
        for s in range(1, NSEG):
            x_copy(s).start()
        wT[D:2 * D, :] = wq_v[...].T
        wT[2 * D:3 * D, :] = wv_v[...].T
        post_q(proj(1))
        post_v(proj(2))
        w_copies[3].wait()
        for s in range(1, NSEG):
            x_copy(s).wait()
        w_copies[4].start()

    def segment(seg, carry):
        nseg = jnp.minimum(seg + 1, NSEG - 1)

        with _scope("windows"):
            for hs in groups(0):
                phase_a(0, hs, 3, 0)
            units = []
            for t in range(4):
                st, nm = ln1_units(nseg, t, LNPARTS)
                units += st + nm
            slots = [(w, t) for w in range(NW) for t in range(4) if t in LNSLOTS][:LNMAX]
            plan = {}
            for k, fn in enumerate(units):
                plan.setdefault(slots[k * len(slots) // len(units)], []).append(fn)
            for w in range(NW):
                fillers = {t: plan.get((w, t), []) for t in range(4)}
                window(w, w + 1 if w + 1 < NW else None, fillers)

        @pl.when(seg < NSEG - 1)
        def _():
            @pl.when(seg == 0)
            def _():
                w_copies[4].wait()
                for c in w_copies[5:]:
                    c.start()

            with _scope("mid"):
                woT[...] = wo_v[...].T
                transpose_wd(seg)
                steps = {
                    "u": lambda: mem_update(range(WFILL, NW)),
                    "o": lambda: outproj(seg),
                    "k": lambda: post_k(proj(0)),
                    "q": lambda: post_q(proj(1)),
                    "v": lambda: post_v(proj(2)),
                    "r": mem_retrieve,
                }
                for c in MID_ORDER:
                    steps[c]()
                for t in range(4):
                    o_copy(4 * seg + t).start()
        return carry

    lax.fori_loop(0, NSEG, segment, 0)
    with _scope("last_out"):
        xs_keep[...] = s_scr[0, 0:8, 0:128] + s_scr[1, 0:8, 0:128] + m_scr[0, :, 0:128] + m_scr[1, :, 0:128]
        outproj(NSEG - 1)
        for t in range(4):
            o_copy(4 * (NSEG - 1) + t).start()

    with _scope("ffn"):
        r = r_s[...]
        rmax = jnp.max(r)
        tok = (lax.broadcasted_iota(jnp.int32, (NT, 128), 0) * 128
               + lax.broadcasted_iota(jnp.int32, (NT, 128), 1))
        idx = jnp.minimum(jnp.min(jnp.where(r == rmax, tok, S)), S - 1)
        tile = idx >> 7
        lane = idx & 127
        hn = ((h_s[tile] - st_s[tile, 0:1, :]) * st_s[tile, 1:2, :]).astype(bf16)
        onehot = jnp.where(lax.broadcasted_iota(jnp.int32, (16, 128), 1) == lane, 1.0, 0.0).astype(bf16)
        xs = lax.dot_general(onehot, hn, (((1,), (1,)), ((), ())), preferred_element_type=f32)
        for c in w_copies[5:]:
            c.wait()
        xm = xs[:, 0:512].astype(bf16)
        xr = xs[:, 512:D]
        row = lax.broadcasted_iota(jnp.int32, (16, 64), 0)
        x2 = jnp.concatenate([jnp.where(row == 0, xr, 0.0), jnp.where(row == 1, xr, 0.0)], axis=1).astype(bf16)
        wrem = jnp.concatenate([wg_v[512:D, :], wu_v[512:D, :]], axis=0)
        rem = jnp.dot(x2, wrem, preferred_element_type=f32)
        gate = jnp.dot(xm, wg_v[0:512, :], preferred_element_type=f32)[0:1] + rem[0:1]
        up = jnp.dot(xm, wu_v[0:512, :], preferred_element_type=f32)[0:1] + rem[1:2]
        act = jnp.broadcast_to(gate * _sigmoid(gate) * up, (16, F)).astype(bf16)
        y = jnp.dot(act, wd_s[...], preferred_element_type=f32)
        y = y[0:1] * _sigmoid(jnp.full((1, 1), rmax, f32))
        ypad = jnp.concatenate([y, jnp.zeros((1, 64), f32)], axis=1)
        ycol = jnp.broadcast_to(ypad, (128, D + 64)).T[0:D]
        for t in range(NT):
            o_copy(t).wait()
        lanes = lax.broadcasted_iota(jnp.int32, (D, 128), 1)
        blk = out_v[tile].astype(f32)
        out_v[tile] = jnp.where(lanes == lane, blk + ycol, blk).astype(bf16)
        fix = o_copy(tile)
        fix.start()
        fix.wait()


@jax.jit
def pallas_sequential_preLN__memory_aug_infini_attn__moe_arch_mod__prompt_kernel(
    A_x: jax.Array,
    A_wq: jax.Array,
    A_wk: jax.Array,
    A_wv: jax.Array,
    A_wo: jax.Array,
    A_beta: jax.Array,
    B_x: jax.Array,
    B_w_r: jax.Array,
    B_w_gate: jax.Array,
    B_w_up: jax.Array,
    B_w_down: jax.Array,
):
    del B_x
    xT = A_x.reshape(S, D).T
    wdT = B_w_down.T

    hbm = pl.BlockSpec(memory_space=pltpu.HBM)
    vmem = pl.BlockSpec(memory_space=pltpu.VMEM)
    scratch = [
        pltpu.VMEM((NSEG, D, L), bf16),
        pltpu.VMEM((D, D), bf16),
        pltpu.VMEM((D, D), bf16),
        pltpu.VMEM((D, D), bf16),
        pltpu.VMEM((D, D), bf16),
        pltpu.VMEM((D, F), bf16),
        pltpu.VMEM((D, F), bf16),
        pltpu.VMEM((D, F), bf16),
        pltpu.VMEM((3 * D, D), bf16),
        pltpu.VMEM((D, D), bf16),
        pltpu.VMEM((F, D), bf16),
        pltpu.VMEM((NW, 8, 128), f32),
        pltpu.VMEM((D + 64, 128), f32),
        pltpu.VMEM((4, D, 128), bf16),
        pltpu.VMEM((NW, L // 2, 128), u32),
        pltpu.VMEM((NW, 4, 64, 128), u32),
        pltpu.VMEM((NW, 4, 64, 128), u32),
        pltpu.VMEM((NW, 4, 64, 128), u32),
        pltpu.VMEM((NW, 4, VWORDS, 128), u32),
        pltpu.VMEM((NW, MROWS, 128), f32),
        pltpu.VMEM((NW, MROWS // 2, 128), u32),
        pltpu.VMEM((4, D + 8, 128), f32),
        pltpu.VMEM((2, L, 128 * HPW), f32),
        pltpu.VMEM((2, 8, 128 * HPW), f32),
        pltpu.VMEM((4, D, 128), f32),
        pltpu.VMEM((NT, D, 128), bf16),
        pltpu.VMEM((NT, D, 128), f32),
        pltpu.VMEM((NT, 8, 128), f32),
        pltpu.VMEM((NT, 128), f32),
        pltpu.VMEM((8, 128), f32),
        pltpu.SemaphoreType.DMA((NSEG,)),
        pltpu.SemaphoreType.DMA((7,)),
        pltpu.SemaphoreType.DMA((NT,)),
    ]
    outT = pl.pallas_call(
        _kernel,
        out_shape=jax.ShapeDtypeStruct((D, S), bf16),
        in_specs=[hbm, hbm, hbm, hbm, hbm, vmem, vmem, hbm, hbm, hbm],
        out_specs=hbm,
        scratch_shapes=scratch,
        compiler_params=pltpu.CompilerParams(vmem_limit_bytes=100 * 1024 * 1024),
    )(xT, A_wq, A_wk, A_wv, A_wo, A_beta, B_w_r, B_w_gate, B_w_up, B_w_down.T)
    return outT.T.reshape(1, S, D)
```

```python
import contextlib
import functools
import os

import jax
import jax.numpy as jnp
from jax import lax
import jax.experimental.pallas as pl
import jax.experimental.pallas.tpu as pltpu

S = 2048
D = 576
H = 32
DH = 18
NSEG = 4
L = 512
NT = S // 128
F = 4608
HPW = 7
NW = 5
WL = HPW * DH
RS = 20
MROWS = 144
VWORDS = 80
LOG2E = 1.4426950408889634
NEG = -1e9 * LOG2E
QSCALE = (DH ** -0.5) * LOG2E
EPS = 1e-5
MID_ORDER = os.environ.get('MID_ORDER', 'wabcukqvor0123')
WFILL = int(os.environ.get('WFILL', '1'))
LNPOS = int(os.environ.get('LNPOS', '0'))
GROUP = int(os.environ.get('GROUP', '0'))
BFIRST = int(os.environ.get('BFIRST', '0'))
PRO = int(os.environ.get('PRO', '1'))
LNPARTS = int(os.environ.get('LNPARTS', '4'))
LNSLOTS = [int(c) for c in os.environ.get('LNSLOTS', '0123')]
LNMAX = int(os.environ.get('LNMAX', '99'))

_PROF = bool(os.environ.get("PROF"))


def _scope(name):
    return jax.named_scope(name) if _PROF else contextlib.nullcontext()


f32 = jnp.float32
bf16 = jnp.bfloat16
u32 = jnp.uint32


def _nh(w):
    return HPW if w < NW - 1 else H - HPW * (NW - 1)


def _pack(x):
    return pltpu.bitcast(x.astype(bf16), u32)


def _unpack(x):
    return pltpu.bitcast(x, bf16)


def _phi(t):
    return jnp.where(t > 0, t + 1.0, jnp.exp(t))


RC = 16
NCH = D // RC


class _Acc:
    def __init__(self, n=2):
        self.parts = [None] * n
        self.i = 0

    def add(self, x):
        k = self.i % len(self.parts)
        self.parts[k] = x if self.parts[k] is None else self.parts[k] + x
        self.i += 1

    def total(self):
        t = self.parts[0]
        for p in self.parts[1:]:
            t = t + p
        return jnp.sum(t, axis=0, keepdims=True)


def _ln_stats(chunk):
    x0 = chunk(0)
    c = x0[0:1]
    s1, s2 = _Acc(), _Acc()
    for i in range(NCH):
        d = (x0 if i == 0 else chunk(i)) - c
        s1.add(d)
        s2.add(d * d)
    mu = s1.total() * (1.0 / D)
    var = jnp.maximum(s2.total() * (1.0 / D) - mu * mu, 0.0)
    return c + mu, lax.rsqrt(var + EPS)


def _sigmoid(x):
    return 1.0 / (1.0 + jnp.exp(-x))


def _kernel(xT_hbm, wq_hbm, wk_hbm, wv_hbm, wo_hbm, beta_ref, wr_ref, wg_hbm, wu_hbm, wdT_hbm,
            out_hbm,
            x_v, wq_v, wk_v, wv_v, wo_v, wg_v, wu_v, wdT_v,
            wT, woT, wd_s, g_s, wr_s,
            xn_s, k_s, phikT_s, qT_s, phiqT_s, vT_s, mt_s, mtb_s, am_s,
            s_scr, m_scr, oT_s, out_v, h_s, st_s, r_s, xs_keep,
            sem_x, sem_w, sem_o):
    def x_copy(s):
        return pltpu.make_async_copy(xT_hbm.at[:, pl.ds(s * L, L)], x_v.at[s], sem_x.at[s])

    def o_copy(t):
        return pltpu.make_async_copy(out_v.at[t], out_hbm.at[:, pl.ds(pl.multiple_of(t * 128, 128), 128)],
                                     sem_o.at[t])

    w_copies = [pltpu.make_async_copy(src, dst, sem_w.at[i]) for i, (src, dst) in enumerate(
        [(wk_hbm, wk_v), (wq_hbm, wq_v), (wv_hbm, wv_v), (wo_hbm, wo_v),
         (wdT_hbm, wdT_v), (wg_hbm, wg_v), (wu_hbm, wu_v)])]

    def ln1_chunk(seg, t, i):
        cols = pl.ds(pl.multiple_of(t * 128, 128), 128)
        return x_v[seg, RC * i:RC * (i + 1), cols].astype(f32)

    def ln1_units(seg, t, nparts):
        st = {}
        bounds = [NCH * i // nparts for i in range(nparts + 1)]

        def stats_part(k):
            if k == 0:
                x0 = ln1_chunk(seg, t, 0)
                st["x0"], st["c"] = x0, x0[0:1]
                st["s1"], st["s2"] = _Acc(), _Acc()
            for i in range(bounds[k], bounds[k + 1]):
                d = (st["x0"] if i == 0 else ln1_chunk(seg, t, i)) - st["c"]
                st["s1"].add(d)
                st["s2"].add(d * d)
            if k == nparts - 1:
                mu = st["s1"].total() * (1.0 / D)
                var = jnp.maximum(st["s2"].total() * (1.0 / D) - mu * mu, 0.0)
                st["mean"], st["rstd"] = st["c"] + mu, lax.rsqrt(var + EPS)

        def norm_part(k):
            for i in range(bounds[k], bounds[k + 1]):
                xn = (ln1_chunk(seg, t, i) - st["mean"]) * st["rstd"]
                xn_s[t, RC * i:RC * (i + 1), :] = xn.astype(bf16)

        return ([functools.partial(stats_part, k) for k in range(nparts)],
                [functools.partial(norm_part, k) for k in range(nparts)])

    def ln1_tile(seg, t):
        stats, norm = ln1_units(seg, t, 1)
        for fn in stats + norm:
            fn()

    def proj(i):
        xn = jnp.concatenate([xn_s[t] for t in range(4)], axis=1)
        r = jnp.dot(wT[D * i:D * (i + 1), :], xn, preferred_element_type=f32)
        return jnp.concatenate([r, jnp.zeros((64, L), f32)], axis=0)

    def post_k(r):
        for t in range(4):
            for w in range(NW):
                kk = r[WL * w:WL * w + 128, 128 * t:128 * (t + 1)]
                k_s[w, 64 * t:64 * (t + 1), :] = pltpu.bitcast(kk.astype(bf16).T, u32)
                phikT_s[w, t] = _pack(_phi(kk))

    def post_v(r):
        rr = lax.broadcasted_iota(jnp.int32, (RS, 128), 0)
        ones_row = jnp.where(rr == DH, 1.0, 0.0).astype(f32)
        for t in range(4):
            for w in range(NW):
                nh = _nh(w)
                vs = [jnp.where(rr < DH,
                                r[DH * (HPW * w + a):DH * (HPW * w + a) + RS, 128 * t:128 * (t + 1)], ones_row)
                      for a in range(nh)]
                if (nh * RS) % 16:
                    vs.append(jnp.zeros((16 - (nh * RS) % 16, 128), f32))
                vv = _pack(jnp.concatenate(vs, axis=0))
                vT_s[w, t, 0:vv.shape[0], :] = vv

    def post_q(r):
        for t in range(4):
            for w in range(NW):
                q = r[WL * w:WL * w + 128, 128 * t:128 * (t + 1)]
                qT_s[w, t] = _pack(q * QSCALE)
                phiqT_s[w, t] = _pack(_phi(q))

    def mem_update(ws=range(NW)):
        r = lax.broadcasted_iota(jnp.int32, (MROWS, 128), 0)
        c = lax.broadcasted_iota(jnp.int32, (MROWS, 128), 1)
        for w in ws:
            vt = jnp.concatenate([_unpack(vT_s[w, t, 0:MROWS // 2, :]) for t in range(4)], axis=1)
            pk = jnp.concatenate([_unpack(phikT_s[w, t]) for t in range(4)], axis=1)
            upd = lax.dot_general(vt, pk, (((1,), (1,)), ((), ())), preferred_element_type=f32)
            mt = mt_s[w] + upd
            mt_s[w] = mt
            keep = jnp.zeros((MROWS, 128), jnp.bool_)
            for a in range(_nh(w)):
                keep = keep | ((r >= RS * a) & (r < RS * (a + 1)) & (c >= DH * a) & (c < DH * (a + 1)))
            mtb_s[w] = _pack(jnp.where(keep, mt, 0.0))

    def mem_retrieve():
        for w in range(NW):
            for j in range(4):
                am = jnp.dot(_unpack(mtb_s[w]), _unpack(phiqT_s[w, j]), preferred_element_type=f32)
                for a in range(_nh(w)):
                    ama = am[RS * a:RS * a + 24]
                    g = g_s[w, a:a + 1, :]
                    om = ama * (g / (ama[DH:DH + 1] + 1e-6))
                    am_s[j, WL * w + DH * a:WL * w + DH * (a + 1), :] = om[0:DH]

    def phase_a(w, heads, j, buf):
        n = 128 * (j + 1)
        nh = len(heads)
        cols = slice(128 * heads[0], 128 * (heads[-1] + 1))
        rows = lax.broadcasted_iota(jnp.int32, (64, 128), 0)
        qw = qT_s[w, j]
        qbd = jnp.concatenate(
            [jnp.where((rows >= 9 * a) & (rows < 9 * a + 9), qw, jnp.uint32(0)) for a in heads], axis=1)
        s = jnp.dot(_unpack(k_s[w, 0:n // 2, :]), _unpack(qbd), preferred_element_type=f32)
        kr = lax.broadcasted_iota(jnp.int32, (128, 128), 0)
        qc = lax.broadcasted_iota(jnp.int32, (128, 128), 1)
        causal = kr <= qc
        sd = jnp.concatenate(
            [jnp.where(causal, s[n - 128:n, 128 * a:128 * (a + 1)], NEG) for a in range(nh)], axis=1)
        s_scr[buf, n - 128:n, cols] = sd
        m = jnp.max(sd, axis=0, keepdims=True)
        if j > 0:
            s_scr[buf, 0:n - 128, cols] = s[0:n - 128]
            m = jnp.maximum(m, jnp.max(s[0:n - 128], axis=0, keepdims=True))
        m_scr[buf, :, cols] = jnp.broadcast_to(m, (8, 128 * nh))

    def phase_b(w, heads, j, buf):
        n = 128 * (j + 1)
        for a in heads:
            m = m_scr[buf, 0:1, 128 * a:128 * (a + 1)]
            p = jnp.exp2(s_scr[buf, 0:n, 128 * a:128 * (a + 1)] - m).astype(bf16)
            vt = jnp.concatenate([_unpack(vT_s[w, t, (RS // 2) * a:(RS // 2) * a + 16, :]) for t in range(j + 1)], axis=1)
            o = jnp.dot(vt, p, preferred_element_type=f32)
            g = g_s[w, a:a + 1, :]
            od = o[0:24] * ((1.0 - g) / o[DH:DH + 1])
            row0 = WL * w + DH * a
            oT_s[j, pl.ds(row0, DH), :] = (od + am_s[j, pl.ds(row0, 24), :])[0:DH]

    def groups(w):
        nh = _nh(w)
        if GROUP == 0 or nh <= GROUP:
            return [list(range(nh))]
        return [list(range(0, GROUP)), list(range(GROUP, nh))]

    def window(w, nxt, fillers):
        order = [3, 2, 1, 0]
        for t in range(4):
            for fn in fillers.get(t, ()):
                fn()
            ga = groups(w) if t < 3 else (groups(nxt) if nxt is not None else [])
            gb = groups(w)
            for i in range(max(len(ga), len(gb))):
                if BFIRST and i < len(gb):
                    phase_b(w, gb[i], order[t], t % 2)
                if i < len(ga):
                    if t < 3:
                        phase_a(w, ga[i], order[t + 1], (t + 1) % 2)
                    else:
                        phase_a(nxt, ga[i], order[0], 0)
                if t == 3 and nxt is None and i == 0:
                    mem_update(range(WFILL))
                if not BFIRST and i < len(gb):
                    phase_b(w, gb[i], order[t], t % 2)

    def ln2_out(tile):
        mean = st_s[tile, 0:1, :]
        rstd = st_s[tile, 1:2, :]
        ga = 1.0 + rstd
        gb = mean * rstd
        for i in range(NCH):
            rows = slice(RC * i, RC * (i + 1))
            out_v[tile, rows, :] = (h_s[tile, rows, :] * ga - gb).astype(bf16)

    def outproj(seg):
        oT = jnp.concatenate([oT_s[t] for t in range(4)], axis=1).astype(bf16)
        attn = jnp.dot(woT[...], oT, preferred_element_type=f32)
        for t in range(4):
            cols = slice(128 * t, 128 * (t + 1))
            tile = 4 * seg + t
            c = None
            s1, s2, s3 = _Acc(), _Acc(), _Acc()
            for i in range(NCH):
                rows = slice(RC * i, RC * (i + 1))
                h = x_v[seg, rows, cols].astype(f32) + attn[rows, cols]
                h_s[tile, rows, :] = h
                if c is None:
                    c = h[0:1]
                d = h - c
                s1.add(d)
                s2.add(d * d)
                s3.add(d * wr_s[rows, :])
            mu = s1.total() * (1.0 / D)
            var = jnp.maximum(s2.total() * (1.0 / D) - mu * mu, 0.0)
            rstd = lax.rsqrt(var + EPS)
            st_s[tile, 0:1, :] = c + mu
            st_s[tile, 1:2, :] = rstd
            r_s[pl.ds(tile, 1), :] = (s3.total() - mu * wr_s[D:D + 1, :]) * rstd

    def transpose_wd(seg, lo, hi):
        nblk = F // 128 // (NSEG - 1)
        for i in range(lo, hi):
            c0 = pl.multiple_of((seg * nblk + i) * 128, 128)
            wd_s[pl.ds(c0, 128), :] = wdT_v[:, pl.ds(c0, 128)].T

    def project_segment():
        post_k(proj(0))
        post_q(proj(1))
        post_v(proj(2))

    with _scope("setup"):
        x_copy(0).start()
        if PRO == 0:
            w_copies[0].start()
        beta = beta_ref[...].astype(f32).reshape(1, H)
        hrow = lax.broadcasted_iota(jnp.int32, (8 * NW, H), 0)
        hcol = lax.broadcasted_iota(jnp.int32, (8 * NW, H), 1)
        sel = (hcol == HPW * (hrow >> 3) + (hrow & 7)) & ((hrow & 7) < HPW)
        bcol = jnp.sum(jnp.where(sel, beta, 0.0), axis=1, keepdims=True)
        g_s[...] = jnp.broadcast_to(_sigmoid(bcol), (8 * NW, 128)).reshape(NW, 8, 128)
        wr_row = wr_ref[...].astype(f32).reshape(1, D)
        wr_pad = jnp.concatenate([wr_row, jnp.zeros((1, 64), f32)], axis=1)
        wr_s[...] = jnp.broadcast_to(wr_pad, (128, D + 64)).T
        wr_s[D:D + 1, :] = jnp.broadcast_to(jnp.sum(wr_row, axis=1, keepdims=True), (1, 128))

        if PRO == 1:
            w_copies[0].start()
        mt_s[...] = jnp.zeros(mt_s.shape, f32)
        vT_s[...] = jnp.zeros(vT_s.shape, u32)
        am_s[...] = jnp.zeros(am_s.shape, f32)
        s_scr[:, 0:8, 0:128] = jnp.zeros((2, 8, 128), f32)
        m_scr[...] = jnp.zeros(m_scr.shape, f32)

        if PRO == 2:
            w_copies[0].start()
        x_copy(0).wait()
        w_copies[1].start()
        for t in range(4):
            ln1_tile(0, t)
    with _scope("proj0"):
        w_copies[0].wait()
        w_copies[2].start()
        wT[0:D, :] = wk_v[...].T
        post_k(proj(0))
        w_copies[1].wait()
        w_copies[2].wait()
        w_copies[3].start()
        for s in range(1, NSEG):
            x_copy(s).start()
        wT[D:2 * D, :] = wq_v[...].T
        wT[2 * D:3 * D, :] = wv_v[...].T
        post_q(proj(1))
        post_v(proj(2))
        w_copies[3].wait()
        for s in range(1, NSEG):
            x_copy(s).wait()
        w_copies[4].start()

    def segment(seg, carry):
        nseg = jnp.minimum(seg + 1, NSEG - 1)

        with _scope("windows"):
            for hs in groups(0):
                phase_a(0, hs, 3, 0)
            units = []
            for t in range(4):
                st, nm = ln1_units(nseg, t, LNPARTS)
                units += st + nm
            slots = [(w, t) for w in range(NW) for t in range(4) if t in LNSLOTS][:LNMAX]
            plan = {}
            for k, fn in enumerate(units):
                plan.setdefault(slots[k * len(slots) // len(units)], []).append(fn)
            for w in range(NW):
                fillers = {t: plan.get((w, t), []) for t in range(4)}
                window(w, w + 1 if w + 1 < NW else None, fillers)

        @pl.when(seg < NSEG - 1)
        def _():
            @pl.when(seg == 0)
            def _():
                w_copies[4].wait()
                for c in w_copies[5:]:
                    c.start()

            with _scope("mid"):
                nblk = F // 128 // (NSEG - 1)

                def t_wo():
                    woT[...] = wo_v[...].T

                steps = {
                    "w": t_wo,
                    "a": lambda: transpose_wd(seg, 0, nblk // 3),
                    "b": lambda: transpose_wd(seg, nblk // 3, 2 * nblk // 3),
                    "c": lambda: transpose_wd(seg, 2 * nblk // 3, nblk),
                    "u": lambda: mem_update(range(WFILL, NW)),
                    "o": lambda: outproj(seg),
                    "k": lambda: post_k(proj(0)),
                    "q": lambda: post_q(proj(1)),
                    "v": lambda: post_v(proj(2)),
                    "r": mem_retrieve,
                    "0": lambda: ln2_out(4 * seg),
                    "1": lambda: ln2_out(4 * seg + 1),
                    "2": lambda: ln2_out(4 * seg + 2),
                    "3": lambda: ln2_out(4 * seg + 3),
                }
                for c in MID_ORDER:
                    steps[c]()
                for t in range(4):
                    o_copy(4 * seg + t).start()
        return carry

    lax.fori_loop(0, NSEG, segment, 0)
    with _scope("last_out"):
        xs_keep[...] = s_scr[0, 0:8, 0:128] + s_scr[1, 0:8, 0:128] + m_scr[0, :, 0:128] + m_scr[1, :, 0:128]
        outproj(NSEG - 1)
        for t in range(4):
            ln2_out(4 * (NSEG - 1) + t)
            o_copy(4 * (NSEG - 1) + t).start()

    with _scope("ffn"):
        r = r_s[...]
        rmax = jnp.max(r)
        tok = (lax.broadcasted_iota(jnp.int32, (NT, 128), 0) * 128
               + lax.broadcasted_iota(jnp.int32, (NT, 128), 1))
        idx = jnp.minimum(jnp.min(jnp.where(r == rmax, tok, S)), S - 1)
        tile = idx >> 7
        lane = idx & 127
        hn = ((h_s[tile] - st_s[tile, 0:1, :]) * st_s[tile, 1:2, :]).astype(bf16)
        onehot = jnp.where(lax.broadcasted_iota(jnp.int32, (16, 128), 1) == lane, 1.0, 0.0).astype(bf16)
        xs = lax.dot_general(onehot, hn, (((1,), (1,)), ((), ())), preferred_element_type=f32)
        for c in w_copies[5:]:
            c.wait()
        xm = xs[:, 0:512].astype(bf16)
        xr = xs[:, 512:D]
        row = lax.broadcasted_iota(jnp.int32, (16, 64), 0)
        x2 = jnp.concatenate([jnp.where(row == 0, xr, 0.0), jnp.where(row == 1, xr, 0.0)], axis=1).astype(bf16)
        wrem = jnp.concatenate([wg_v[512:D, :], wu_v[512:D, :]], axis=0)
        rem = jnp.dot(x2, wrem, preferred_element_type=f32)
        gate = jnp.dot(xm, wg_v[0:512, :], preferred_element_type=f32)[0:1] + rem[0:1]
        up = jnp.dot(xm, wu_v[0:512, :], preferred_element_type=f32)[0:1] + rem[1:2]
        act = jnp.broadcast_to(gate * _sigmoid(gate) * up, (16, F)).astype(bf16)
        y = jnp.dot(act, wd_s[...], preferred_element_type=f32)
        y = y[0:1] * _sigmoid(jnp.full((1, 1), rmax, f32))
        ypad = jnp.concatenate([y, jnp.zeros((1, 64), f32)], axis=1)
        ycol = jnp.broadcast_to(ypad, (128, D + 64)).T[0:D]
        for t in range(NT):
            o_copy(t).wait()
        lanes = lax.broadcasted_iota(jnp.int32, (D, 128), 1)
        blk = out_v[tile].astype(f32)
        out_v[tile] = jnp.where(lanes == lane, blk + ycol, blk).astype(bf16)
        fix = o_copy(tile)
        fix.start()
        fix.wait()


@jax.jit
def pallas_sequential_preLN__memory_aug_infini_attn__moe_arch_mod__prompt_kernel(
    A_x: jax.Array,
    A_wq: jax.Array,
    A_wk: jax.Array,
    A_wv: jax.Array,
    A_wo: jax.Array,
    A_beta: jax.Array,
    B_x: jax.Array,
    B_w_r: jax.Array,
    B_w_gate: jax.Array,
    B_w_up: jax.Array,
    B_w_down: jax.Array,
):
    del B_x
    xT = A_x.reshape(S, D).T
    wdT = B_w_down.T

    hbm = pl.BlockSpec(memory_space=pltpu.HBM)
    vmem = pl.BlockSpec(memory_space=pltpu.VMEM)
    scratch = [
        pltpu.VMEM((NSEG, D, L), bf16),
        pltpu.VMEM((D, D), bf16),
        pltpu.VMEM((D, D), bf16),
        pltpu.VMEM((D, D), bf16),
        pltpu.VMEM((D, D), bf16),
        pltpu.VMEM((D, F), bf16),
        pltpu.VMEM((D, F), bf16),
        pltpu.VMEM((D, F), bf16),
        pltpu.VMEM((3 * D, D), bf16),
        pltpu.VMEM((D, D), bf16),
        pltpu.VMEM((F, D), bf16),
        pltpu.VMEM((NW, 8, 128), f32),
        pltpu.VMEM((D + 64, 128), f32),
        pltpu.VMEM((4, D, 128), bf16),
        pltpu.VMEM((NW, L // 2, 128), u32),
        pltpu.VMEM((NW, 4, 64, 128), u32),
        pltpu.VMEM((NW, 4, 64, 128), u32),
        pltpu.VMEM((NW, 4, 64, 128), u32),
        pltpu.VMEM((NW, 4, VWORDS, 128), u32),
        pltpu.VMEM((NW, MROWS, 128), f32),
        pltpu.VMEM((NW, MROWS // 2, 128), u32),
        pltpu.VMEM((4, D + 8, 128), f32),
        pltpu.VMEM((2, L, 128 * HPW), f32),
        pltpu.VMEM((2, 8, 128 * HPW), f32),
        pltpu.VMEM((4, D, 128), f32),
        pltpu.VMEM((NT, D, 128), bf16),
        pltpu.VMEM((NT, D, 128), f32),
        pltpu.VMEM((NT, 8, 128), f32),
        pltpu.VMEM((NT, 128), f32),
        pltpu.VMEM((8, 128), f32),
        pltpu.SemaphoreType.DMA((NSEG,)),
        pltpu.SemaphoreType.DMA((7,)),
        pltpu.SemaphoreType.DMA((NT,)),
    ]
    outT = pl.pallas_call(
        _kernel,
        out_shape=jax.ShapeDtypeStruct((D, S), bf16),
        in_specs=[hbm, hbm, hbm, hbm, hbm, vmem, vmem, hbm, hbm, hbm],
        out_specs=hbm,
        scratch_shapes=scratch,
        compiler_params=pltpu.CompilerParams(vmem_limit_bytes=100 * 1024 * 1024),
    )(xT, A_wq, A_wk, A_wv, A_wo, A_beta, B_w_r, B_w_gate, B_w_up, B_w_down.T)
    return outT.T.reshape(1, S, D)
```

```python
import contextlib
import functools
import os

import jax
import jax.numpy as jnp
from jax import lax
import jax.experimental.pallas as pl
import jax.experimental.pallas.tpu as pltpu

S = 2048
D = 576
H = 32
DH = 18
NSEG = 4
L = 512
NT = S // 128
F = 4608
HPW = 7
NW = 5
WL = HPW * DH
RS = 20
MROWS = 144
VWORDS = 80
LOG2E = 1.4426950408889634
NEG = -1e9 * LOG2E
QSCALE = (DH ** -0.5) * LOG2E
EPS = 1e-5
MID_ORDER = os.environ.get('MID_ORDER', 'wabcukqvor0123')
UPD_PLAN = {}
for _e in os.environ.get('UPD', '42:0,43:1').split(','):
    if _e:
        UPD_PLAN.setdefault((int(_e[0]), int(_e[1])), []).append(int(_e[3]))
UPD_IN_W = [u for v in UPD_PLAN.values() for u in v]
LNPOS = int(os.environ.get('LNPOS', '0'))
RECIP = int(os.environ.get('RECIP', '0'))
OUTW = int(os.environ.get('OUTW', '0'))
PRO = int(os.environ.get('PRO', '1'))
LNPARTS = int(os.environ.get('LNPARTS', '4'))
LNSLOTS = [int(c) for c in os.environ.get('LNSLOTS', '0123')]
LNMAX = int(os.environ.get('LNMAX', '99'))

_PROF = bool(os.environ.get("PROF"))


def _scope(name):
    return jax.named_scope(name) if _PROF else contextlib.nullcontext()


f32 = jnp.float32
bf16 = jnp.bfloat16
u32 = jnp.uint32


def _nh(w):
    return HPW if w < NW - 1 else H - HPW * (NW - 1)


def _pack(x):
    return pltpu.bitcast(x.astype(bf16), u32)


def _unpack(x):
    return pltpu.bitcast(x, bf16)


def _phi(t):
    return jnp.where(t > 0, t + 1.0, jnp.exp(t))


RC = int(os.environ.get('RC', '16'))
NCH = D // RC


class _Acc:
    def __init__(self, n=int(os.environ.get('NACC', '2'))):
        self.parts = [None] * n
        self.i = 0

    def add(self, x):
        k = self.i % len(self.parts)
        self.parts[k] = x if self.parts[k] is None else self.parts[k] + x
        self.i += 1

    def total(self):
        t = self.parts[0]
        for p in self.parts[1:]:
            t = t + p
        return jnp.sum(t, axis=0, keepdims=True)


def _ln_stats(chunk):
    x0 = chunk(0)
    c = x0[0:1]
    s1, s2 = _Acc(), _Acc()
    for i in range(NCH):
        d = (x0 if i == 0 else chunk(i)) - c
        s1.add(d)
        s2.add(d * d)
    mu = s1.total() * (1.0 / D)
    var = jnp.maximum(s2.total() * (1.0 / D) - mu * mu, 0.0)
    return c + mu, lax.rsqrt(var + EPS)


def _recip(x):
    if RECIP == 0:
        return 1.0 / x
    r = pl.reciprocal(x, approx=True)
    return r * (2.0 - x * r)


def _sigmoid(x):
    return 1.0 / (1.0 + jnp.exp(-x))


def _kernel(xT_hbm, wq_hbm, wk_hbm, wv_hbm, wo_hbm, beta_ref, wr_ref, wg_hbm, wu_hbm, wdT_hbm,
            out_hbm,
            x_v, wq_v, wk_v, wv_v, wo_v, wg_v, wu_v, wdT_v,
            wT, woT, wd_s, g_s, wr_s,
            xn_s, k_s, phikT_s, qT_s, phiqT_s, vT_s, mt_s, mtb_s, am_s,
            s_scr, m_scr, oT_s, out_v, h_s, st_s, r_s, xs_keep,
            sem_x, sem_w, sem_o):
    def x_copy(s):
        return pltpu.make_async_copy(xT_hbm.at[:, pl.ds(s * L, L)], x_v.at[s], sem_x.at[s])

    def o_copy(t):
        return pltpu.make_async_copy(out_v.at[t], out_hbm.at[:, pl.ds(pl.multiple_of(t * 128, 128), 128)],
                                     sem_o.at[t])

    w_copies = [pltpu.make_async_copy(src, dst, sem_w.at[i]) for i, (src, dst) in enumerate(
        [(wk_hbm, wk_v), (wq_hbm, wq_v), (wv_hbm, wv_v), (wo_hbm, wo_v),
         (wdT_hbm, wdT_v), (wg_hbm, wg_v), (wu_hbm, wu_v)])]

    def ln1_chunk(seg, t, i):
        cols = pl.ds(pl.multiple_of(t * 128, 128), 128)
        return x_v[seg, RC * i:RC * (i + 1), cols].astype(f32)

    def ln1_units(seg, t, nparts):
        st = {}
        bounds = [NCH * i // nparts for i in range(nparts + 1)]

        def stats_part(k):
            if k == 0:
                x0 = ln1_chunk(seg, t, 0)
                st["x0"], st["c"] = x0, x0[0:1]
                st["s1"], st["s2"] = _Acc(), _Acc()
            for i in range(bounds[k], bounds[k + 1]):
                d = (st["x0"] if i == 0 else ln1_chunk(seg, t, i)) - st["c"]
                st["s1"].add(d)
                st["s2"].add(d * d)
            if k == nparts - 1:
                mu = st["s1"].total() * (1.0 / D)
                var = jnp.maximum(st["s2"].total() * (1.0 / D) - mu * mu, 0.0)
                st["mean"], st["rstd"] = st["c"] + mu, lax.rsqrt(var + EPS)

        def norm_part(k):
            for i in range(bounds[k], bounds[k + 1]):
                xn = (ln1_chunk(seg, t, i) - st["mean"]) * st["rstd"]
                xn_s[t, RC * i:RC * (i + 1), :] = xn.astype(bf16)

        return ([functools.partial(stats_part, k) for k in range(nparts)],
                [functools.partial(norm_part, k) for k in range(nparts)])

    def ln1_tile(seg, t):
        stats, norm = ln1_units(seg, t, 1)
        for fn in stats + norm:
            fn()

    def proj(i):
        xn = jnp.concatenate([xn_s[t] for t in range(4)], axis=1)
        r = jnp.dot(wT[D * i:D * (i + 1), :], xn, preferred_element_type=f32)
        return jnp.concatenate([r, jnp.zeros((64, L), f32)], axis=0)

    def post_k(r):
        for t in range(4):
            for w in range(NW):
                kk = r[WL * w:WL * w + 128, 128 * t:128 * (t + 1)]
                k_s[w, 64 * t:64 * (t + 1), :] = pltpu.bitcast(kk.astype(bf16).T, u32)
                phikT_s[w, t] = _pack(_phi(kk))

    def post_v(r):
        rr = lax.broadcasted_iota(jnp.int32, (RS, 128), 0)
        ones_row = jnp.where(rr == DH, 1.0, 0.0).astype(f32)
        for t in range(4):
            for w in range(NW):
                nh = _nh(w)
                vs = [jnp.where(rr < DH,
                                r[DH * (HPW * w + a):DH * (HPW * w + a) + RS, 128 * t:128 * (t + 1)], ones_row)
                      for a in range(nh)]
                if (nh * RS) % 16:
                    vs.append(jnp.zeros((16 - (nh * RS) % 16, 128), f32))
                vv = _pack(jnp.concatenate(vs, axis=0))
                vT_s[w, t, 0:vv.shape[0], :] = vv

    def post_q(r):
        for t in range(4):
            for w in range(NW):
                q = r[WL * w:WL * w + 128, 128 * t:128 * (t + 1)]
                qT_s[w, t] = _pack(q * QSCALE)
                phiqT_s[w, t] = _pack(_phi(q))

    def mem_update(ws=range(NW)):
        r = lax.broadcasted_iota(jnp.int32, (MROWS, 128), 0)
        c = lax.broadcasted_iota(jnp.int32, (MROWS, 128), 1)
        for w in ws:
            vt = jnp.concatenate([_unpack(vT_s[w, t, 0:MROWS // 2, :]) for t in range(4)], axis=1)
            pk = jnp.concatenate([_unpack(phikT_s[w, t]) for t in range(4)], axis=1)
            upd = lax.dot_general(vt, pk, (((1,), (1,)), ((), ())), preferred_element_type=f32)
            mt = mt_s[w] + upd
            mt_s[w] = mt
            keep = jnp.zeros((MROWS, 128), jnp.bool_)
            for a in range(_nh(w)):
                keep = keep | ((r >= RS * a) & (r < RS * (a + 1)) & (c >= DH * a) & (c < DH * (a + 1)))
            mtb_s[w] = _pack(jnp.where(keep, mt, 0.0))

    def mem_retrieve():
        for w in range(NW):
            for j in range(4):
                am = jnp.dot(_unpack(mtb_s[w]), _unpack(phiqT_s[w, j]), preferred_element_type=f32)
                for a in range(_nh(w)):
                    ama = am[RS * a:RS * a + 24]
                    g = g_s[w, a:a + 1, :]
                    om = ama * (g * _recip(ama[DH:DH + 1] + 1e-6))
                    am_s[j, WL * w + DH * a:WL * w + DH * (a + 1), :] = om[0:DH]

    def phase_a(w, heads, j, buf):
        n = 128 * (j + 1)
        nh = len(heads)
        cols = slice(128 * heads[0], 128 * (heads[-1] + 1))
        rows = lax.broadcasted_iota(jnp.int32, (64, 128), 0)
        qw = qT_s[w, j]
        qbd = jnp.concatenate(
            [jnp.where((rows >= 9 * a) & (rows < 9 * a + 9), qw, jnp.uint32(0)) for a in heads], axis=1)
        s = jnp.dot(_unpack(k_s[w, 0:n // 2, :]), _unpack(qbd), preferred_element_type=f32)
        kr = lax.broadcasted_iota(jnp.int32, (128, 128), 0)
        qc = lax.broadcasted_iota(jnp.int32, (128, 128), 1)
        causal = kr <= qc
        sd = jnp.concatenate(
            [jnp.where(causal, s[n - 128:n, 128 * a:128 * (a + 1)], NEG) for a in range(nh)], axis=1)
        s_scr[buf, n - 128:n, cols] = sd
        m = jnp.max(sd, axis=0, keepdims=True)
        if j > 0:
            s_scr[buf, 0:n - 128, cols] = s[0:n - 128]
            m = jnp.maximum(m, jnp.max(s[0:n - 128], axis=0, keepdims=True))
        m_scr[buf, :, cols] = jnp.broadcast_to(m, (8, 128 * nh))

    def phase_b(w, heads, j, buf):
        n = 128 * (j + 1)
        for a in heads:
            m = m_scr[buf, 0:1, 128 * a:128 * (a + 1)]
            p = jnp.exp2(s_scr[buf, 0:n, 128 * a:128 * (a + 1)] - m).astype(bf16)
            vt = jnp.concatenate([_unpack(vT_s[w, t, (RS // 2) * a:(RS // 2) * a + 16, :]) for t in range(j + 1)], axis=1)
            o = jnp.dot(vt, p, preferred_element_type=f32)
            g = g_s[w, a:a + 1, :]
            od = o[0:24] * ((1.0 - g) * _recip(o[DH:DH + 1]))
            row0 = WL * w + DH * a
            oT_s[j, pl.ds(row0, DH), :] = (od + am_s[j, pl.ds(row0, 24), :])[0:DH]

    def window(w, nxt, fillers):
        order = [3, 2, 1, 0]
        heads = list(range(_nh(w)))
        for t in range(4):
            for fn in fillers.get(t, ()):
                fn()
            if t < 3:
                phase_a(w, heads, order[t + 1], (t + 1) % 2)
            elif nxt is not None:
                phase_a(nxt, list(range(_nh(nxt))), order[0], 0)
            ws = UPD_PLAN.get((w, t), [])
            if ws:
                mem_update(ws)
            phase_b(w, heads, order[t], t % 2)

    def ln2_out(tile, lo=0, hi=NCH):
        mean = st_s[tile, 0:1, :]
        rstd = st_s[tile, 1:2, :]
        ga = 1.0 + rstd
        gb = mean * rstd
        for i in range(lo, hi):
            rows = slice(RC * i, RC * (i + 1))
            out_v[tile, rows, :] = (h_s[tile, rows, :] * ga - gb).astype(bf16)

    def outproj(seg):
        oT = jnp.concatenate([oT_s[t] for t in range(4)], axis=1).astype(bf16)
        attn = jnp.dot(woT[...], oT, preferred_element_type=f32)
        for t in range(4):
            cols = slice(128 * t, 128 * (t + 1))
            tile = 4 * seg + t
            c = None
            s1, s2, s3 = _Acc(), _Acc(), _Acc()
            for i in range(NCH):
                rows = slice(RC * i, RC * (i + 1))
                h = x_v[seg, rows, cols].astype(f32) + attn[rows, cols]
                h_s[tile, rows, :] = h
                if c is None:
                    c = h[0:1]
                d = h - c
                s1.add(d)
                s2.add(d * d)
                s3.add(d * wr_s[rows, :])
            mu = s1.total() * (1.0 / D)
            var = jnp.maximum(s2.total() * (1.0 / D) - mu * mu, 0.0)
            rstd = lax.rsqrt(var + EPS)
            st_s[tile, 0:1, :] = c + mu
            st_s[tile, 1:2, :] = rstd
            r_s[pl.ds(tile, 1), :] = (s3.total() - mu * wr_s[D:D + 1, :]) * rstd

    def transpose_wd(seg, lo, hi):
        nblk = F // 128 // (NSEG - 1)
        for i in range(lo, hi):
            c0 = pl.multiple_of((seg * nblk + i) * 128, 128)
            wd_s[pl.ds(c0, 128), :] = wdT_v[:, pl.ds(c0, 128)].T

    def project_segment():
        post_k(proj(0))
        post_q(proj(1))
        post_v(proj(2))

    with _scope("setup"):
        x_copy(0).start()
        if PRO == 0:
            w_copies[0].start()
        beta = beta_ref[...].astype(f32).reshape(1, H)
        hrow = lax.broadcasted_iota(jnp.int32, (8 * NW, H), 0)
        hcol = lax.broadcasted_iota(jnp.int32, (8 * NW, H), 1)
        sel = (hcol == HPW * (hrow >> 3) + (hrow & 7)) & ((hrow & 7) < HPW)
        bcol = jnp.sum(jnp.where(sel, beta, 0.0), axis=1, keepdims=True)
        g_s[...] = jnp.broadcast_to(_sigmoid(bcol), (8 * NW, 128)).reshape(NW, 8, 128)
        wr_row = wr_ref[...].astype(f32).reshape(1, D)
        wr_pad = jnp.concatenate([wr_row, jnp.zeros((1, 64), f32)], axis=1)
        wr_s[...] = jnp.broadcast_to(wr_pad, (128, D + 64)).T
        wr_s[D:D + 1, :] = jnp.broadcast_to(jnp.sum(wr_row, axis=1, keepdims=True), (1, 128))

        if PRO == 1:
            w_copies[0].start()
        mt_s[...] = jnp.zeros(mt_s.shape, f32)
        vT_s[...] = jnp.zeros(vT_s.shape, u32)
        am_s[...] = jnp.zeros(am_s.shape, f32)
        if OUTW:
            h_s[0:4] = jnp.zeros((4, D, 128), f32)
            st_s[0:4] = jnp.zeros((4, 8, 128), f32)
        s_scr[:, 0:8, 0:128] = jnp.zeros((2, 8, 128), f32)
        m_scr[...] = jnp.zeros(m_scr.shape, f32)

        if PRO == 2:
            w_copies[0].start()
        x_copy(0).wait()
        w_copies[1].start()
        for t in range(4):
            ln1_tile(0, t)
    with _scope("proj0"):
        w_copies[0].wait()
        w_copies[2].start()
        wT[0:D, :] = wk_v[...].T
        post_k(proj(0))
        w_copies[1].wait()
        w_copies[2].wait()
        w_copies[3].start()
        for s in range(1, NSEG):
            x_copy(s).start()
        wT[D:2 * D, :] = wq_v[...].T
        wT[2 * D:3 * D, :] = wv_v[...].T
        post_q(proj(1))
        post_v(proj(2))
        w_copies[3].wait()
        for s in range(1, NSEG):
            x_copy(s).wait()
        w_copies[4].start()

    def segment(seg, carry):
        nseg = jnp.minimum(seg + 1, NSEG - 1)
        pseg = jnp.maximum(seg - 1, 0)

        with _scope("windows"):
            phase_a(0, list(range(HPW)), 3, 0)
            units = []
            for t in range(4):
                st, nm = ln1_units(nseg, t, LNPARTS)
                units += st + nm
            if OUTW:
                outs = [functools.partial(ln2_out, 4 * pseg + t, NCH * k // 2, NCH * (k + 1) // 2)
                        for t in range(4) for k in range(2)]
                merged = []
                for k, fn in enumerate(units):
                    merged.append(fn)
                    if k % 4 == 3:
                        merged.append(outs[k // 4])
                units = merged
            slots = [(w, t) for w in range(NW) for t in range(4) if t in LNSLOTS][:LNMAX]
            plan = {}
            for k, fn in enumerate(units):
                plan.setdefault(slots[k * len(slots) // len(units)], []).append(fn)
            for w in range(NW):
                fillers = {t: plan.get((w, t), []) for t in range(4)}
                window(w, w + 1 if w + 1 < NW else None, fillers)

        if OUTW:
            @pl.when(seg > 0)
            def _():
                for t in range(4):
                    o_copy(4 * pseg + t).start()

        @pl.when(seg < NSEG - 1)
        def _():
            @pl.when(seg == 0)
            def _():
                w_copies[4].wait()
                for c in w_copies[5:]:
                    c.start()

            with _scope("mid"):
                nblk = F // 128 // (NSEG - 1)

                def t_wo():
                    woT[...] = wo_v[...].T

                steps = {
                    "w": t_wo,
                    "a": lambda: transpose_wd(seg, 0, nblk // 3),
                    "b": lambda: transpose_wd(seg, nblk // 3, 2 * nblk // 3),
                    "c": lambda: transpose_wd(seg, 2 * nblk // 3, nblk),
                    "u": lambda: mem_update([w for w in range(NW) if w not in UPD_IN_W]),
                    "o": lambda: outproj(seg),
                    "k": lambda: post_k(proj(0)),
                    "q": lambda: post_q(proj(1)),
                    "v": lambda: post_v(proj(2)),
                    "r": mem_retrieve,
                    "0": lambda: ln2_out(4 * seg),
                    "1": lambda: ln2_out(4 * seg + 1),
                    "2": lambda: ln2_out(4 * seg + 2),
                    "3": lambda: ln2_out(4 * seg + 3),
                }
                for c in MID_ORDER:
                    if not (OUTW and c in "0123"):
                        steps[c]()
                if not OUTW:
                    for t in range(4):
                        o_copy(4 * seg + t).start()
        return carry

    lax.fori_loop(0, NSEG, segment, 0)
    with _scope("last_out"):
        xs_keep[...] = s_scr[0, 0:8, 0:128] + s_scr[1, 0:8, 0:128] + m_scr[0, :, 0:128] + m_scr[1, :, 0:128]
        outproj(NSEG - 1)
        for t in range(4):
            ln2_out(4 * (NSEG - 1) + t)
            o_copy(4 * (NSEG - 1) + t).start()

    with _scope("ffn"):
        r = r_s[...]
        rmax = jnp.max(r)
        tok = (lax.broadcasted_iota(jnp.int32, (NT, 128), 0) * 128
               + lax.broadcasted_iota(jnp.int32, (NT, 128), 1))
        idx = jnp.minimum(jnp.min(jnp.where(r == rmax, tok, S)), S - 1)
        tile = idx >> 7
        lane = idx & 127
        hn = ((h_s[tile] - st_s[tile, 0:1, :]) * st_s[tile, 1:2, :]).astype(bf16)
        onehot = jnp.where(lax.broadcasted_iota(jnp.int32, (16, 128), 1) == lane, 1.0, 0.0).astype(bf16)
        xs = lax.dot_general(onehot, hn, (((1,), (1,)), ((), ())), preferred_element_type=f32)
        for c in w_copies[5:]:
            c.wait()
        xm = xs[:, 0:512].astype(bf16)
        xr = xs[:, 512:D]
        row = lax.broadcasted_iota(jnp.int32, (16, 64), 0)
        x2 = jnp.concatenate([jnp.where(row == 0, xr, 0.0), jnp.where(row == 1, xr, 0.0)], axis=1).astype(bf16)
        wrem = jnp.concatenate([wg_v[512:D, :], wu_v[512:D, :]], axis=0)
        rem = jnp.dot(x2, wrem, preferred_element_type=f32)
        gate = jnp.dot(xm, wg_v[0:512, :], preferred_element_type=f32)[0:1] + rem[0:1]
        up = jnp.dot(xm, wu_v[0:512, :], preferred_element_type=f32)[0:1] + rem[1:2]
        act = jnp.broadcast_to(gate * _sigmoid(gate) * up, (16, F)).astype(bf16)
        y = jnp.dot(act, wd_s[...], preferred_element_type=f32)
        y = y[0:1] * _sigmoid(jnp.full((1, 1), rmax, f32))
        ypad = jnp.concatenate([y, jnp.zeros((1, 64), f32)], axis=1)
        ycol = jnp.broadcast_to(ypad, (128, D + 64)).T[0:D]
        for t in range(NT):
            o_copy(t).wait()
        lanes = lax.broadcasted_iota(jnp.int32, (D, 128), 1)
        blk = out_v[tile].astype(f32)
        out_v[tile] = jnp.where(lanes == lane, blk + ycol, blk).astype(bf16)
        fix = o_copy(tile)
        fix.start()
        fix.wait()


@jax.jit
def pallas_sequential_preLN__memory_aug_infini_attn__moe_arch_mod__prompt_kernel(
    A_x: jax.Array,
    A_wq: jax.Array,
    A_wk: jax.Array,
    A_wv: jax.Array,
    A_wo: jax.Array,
    A_beta: jax.Array,
    B_x: jax.Array,
    B_w_r: jax.Array,
    B_w_gate: jax.Array,
    B_w_up: jax.Array,
    B_w_down: jax.Array,
):
    del B_x
    xT = A_x.reshape(S, D).T
    wdT = B_w_down.T

    hbm = pl.BlockSpec(memory_space=pltpu.HBM)
    vmem = pl.BlockSpec(memory_space=pltpu.VMEM)
    scratch = [
        pltpu.VMEM((NSEG, D, L), bf16),
        pltpu.VMEM((D, D), bf16),
        pltpu.VMEM((D, D), bf16),
        pltpu.VMEM((D, D), bf16),
        pltpu.VMEM((D, D), bf16),
        pltpu.VMEM((D, F), bf16),
        pltpu.VMEM((D, F), bf16),
        pltpu.VMEM((D, F), bf16),
        pltpu.VMEM((3 * D, D), bf16),
        pltpu.VMEM((D, D), bf16),
        pltpu.VMEM((F, D), bf16),
        pltpu.VMEM((NW, 8, 128), f32),
        pltpu.VMEM((D + 64, 128), f32),
        pltpu.VMEM((4, D, 128), bf16),
        pltpu.VMEM((NW, L // 2, 128), u32),
        pltpu.VMEM((NW, 4, 64, 128), u32),
        pltpu.VMEM((NW, 4, 64, 128), u32),
        pltpu.VMEM((NW, 4, 64, 128), u32),
        pltpu.VMEM((NW, 4, VWORDS, 128), u32),
        pltpu.VMEM((NW, MROWS, 128), f32),
        pltpu.VMEM((NW, MROWS // 2, 128), u32),
        pltpu.VMEM((4, D + 8, 128), f32),
        pltpu.VMEM((2, L, 128 * HPW), f32),
        pltpu.VMEM((2, 8, 128 * HPW), f32),
        pltpu.VMEM((4, D, 128), f32),
        pltpu.VMEM((NT, D, 128), bf16),
        pltpu.VMEM((NT, D, 128), f32),
        pltpu.VMEM((NT, 8, 128), f32),
        pltpu.VMEM((NT, 128), f32),
        pltpu.VMEM((8, 128), f32),
        pltpu.SemaphoreType.DMA((NSEG,)),
        pltpu.SemaphoreType.DMA((7,)),
        pltpu.SemaphoreType.DMA((NT,)),
    ]
    outT = pl.pallas_call(
        _kernel,
        out_shape=jax.ShapeDtypeStruct((D, S), bf16),
        in_specs=[hbm, hbm, hbm, hbm, hbm, vmem, vmem, hbm, hbm, hbm],
        out_specs=hbm,
        scratch_shapes=scratch,
        compiler_params=pltpu.CompilerParams(vmem_limit_bytes=100 * 1024 * 1024),
    )(xT, A_wq, A_wk, A_wv, A_wo, A_beta, B_w_r, B_w_gate, B_w_up, B_w_down.T)
    return outT.T.reshape(1, S, D)
```

```python
import contextlib
import functools
import os

import jax
import jax.numpy as jnp
from jax import lax
import jax.experimental.pallas as pl
import jax.experimental.pallas.tpu as pltpu

S = 2048
D = 576
H = 32
DH = 18
NSEG = 4
L = 512
NT = S // 128
F = 4608
HPW = 7
NW = 5
WL = HPW * DH
RS = 20
MROWS = 144
VWORDS = 80
LOG2E = 1.4426950408889634
NEG = -1e9 * LOG2E
QSCALE = (DH ** -0.5) * LOG2E
EPS = 1e-5
MID_ORDER = os.environ.get('MID_ORDER', 'wabcukqvor0123')
UPD_PLAN = {}
for _e in os.environ.get('UPD', '42:0,43:1').split(','):
    if _e:
        UPD_PLAN.setdefault((int(_e[0]), int(_e[1])), []).append(int(_e[3]))
UPD_IN_W = [u for v in UPD_PLAN.values() for u in v]
LNPOS = int(os.environ.get('LNPOS', '0'))
NV = int(os.environ.get('NV', '10'))
RECIP = int(os.environ.get('RECIP', '0'))
OUTW = int(os.environ.get('OUTW', '0'))
PRO = int(os.environ.get('PRO', '1'))
LNPARTS = int(os.environ.get('LNPARTS', '4'))
LNSLOTS = [int(c) for c in os.environ.get('LNSLOTS', '0123')]
LNMAX = int(os.environ.get('LNMAX', '99'))

_PROF = bool(os.environ.get("PROF"))


def _scope(name):
    return jax.named_scope(name) if _PROF else contextlib.nullcontext()


f32 = jnp.float32
bf16 = jnp.bfloat16
u32 = jnp.uint32


def _nh(w):
    return HPW if w < NW - 1 else H - HPW * (NW - 1)


def _pack(x):
    return pltpu.bitcast(x.astype(bf16), u32)


def _unpack(x):
    return pltpu.bitcast(x, bf16)


def _phi(t):
    return jnp.where(t > 0, t + 1.0, jnp.exp(t))


RC = int(os.environ.get('RC', '16'))
NCH = D // RC


class _Acc:
    def __init__(self, n=int(os.environ.get('NACC', '2'))):
        self.parts = [None] * n
        self.i = 0

    def add(self, x):
        k = self.i % len(self.parts)
        self.parts[k] = x if self.parts[k] is None else self.parts[k] + x
        self.i += 1

    def total(self):
        t = self.parts[0]
        for p in self.parts[1:]:
            t = t + p
        return jnp.sum(t, axis=0, keepdims=True)


def _ln_stats(chunk):
    x0 = chunk(0)
    c = x0[0:1]
    s1, s2 = _Acc(), _Acc()
    for i in range(NCH):
        d = (x0 if i == 0 else chunk(i)) - c
        s1.add(d)
        s2.add(d * d)
    mu = s1.total() * (1.0 / D)
    var = jnp.maximum(s2.total() * (1.0 / D) - mu * mu, 0.0)
    return c + mu, lax.rsqrt(var + EPS)


def _recip(x):
    if RECIP == 0:
        return 1.0 / x
    r = pl.reciprocal(x, approx=True)
    return r * (2.0 - x * r)


def _sigmoid(x):
    return 1.0 / (1.0 + jnp.exp(-x))


def _kernel(xT_hbm, wq_hbm, wk_hbm, wv_hbm, wo_hbm, beta_ref, wr_ref, wg_hbm, wu_hbm, wdT_hbm,
            out_hbm,
            x_v, wq_v, wk_v, wv_v, wo_v, wg_v, wu_v, wdT_v,
            wT, woT, wd_s, g_s, wr_s,
            xn_s, k_s, phikT_s, qT_s, phiqT_s, vT_s, mt_s, mtb_s, am_s,
            s_scr, m_scr, oT_s, out_v, h_s, st_s, r_s, xs_keep, xb_s,
            sem_x, sem_w, sem_o):
    def x_copy(s):
        return pltpu.make_async_copy(xT_hbm.at[:, pl.ds(s * L, L)], x_v.at[s], sem_x.at[s])

    def o_copy(t):
        return pltpu.make_async_copy(out_v.at[t], out_hbm.at[:, pl.ds(pl.multiple_of(t * 128, 128), 128)],
                                     sem_o.at[t])

    w_copies = [pltpu.make_async_copy(src, dst, sem_w.at[i]) for i, (src, dst) in enumerate(
        [(wk_hbm, wk_v), (wq_hbm, wq_v), (wv_hbm, wv_v), (wo_hbm, wo_v),
         (wdT_hbm, wdT_v), (wg_hbm, wg_v), (wu_hbm, wu_v)])]

    def ln1_chunk(seg, t, i):
        cols = pl.ds(pl.multiple_of(t * 128, 128), 128)
        return x_v[seg, RC * i:RC * (i + 1), cols].astype(f32)

    def ln1_units(seg, t, nparts):
        st = {}
        bounds = [NCH * i // nparts for i in range(nparts + 1)]

        def stats_part(k):
            if k == 0:
                x0 = ln1_chunk(seg, t, 0)
                st["x0"], st["c"] = x0, x0[0:1]
                st["s1"], st["s2"] = _Acc(), _Acc()
            for i in range(bounds[k], bounds[k + 1]):
                d = (st["x0"] if i == 0 else ln1_chunk(seg, t, i)) - st["c"]
                st["s1"].add(d)
                st["s2"].add(d * d)
            if k == nparts - 1:
                mu = st["s1"].total() * (1.0 / D)
                var = jnp.maximum(st["s2"].total() * (1.0 / D) - mu * mu, 0.0)
                st["mean"], st["rstd"] = st["c"] + mu, lax.rsqrt(var + EPS)

        def norm_part(k):
            for i in range(bounds[k], bounds[k + 1]):
                xn = (ln1_chunk(seg, t, i) - st["mean"]) * st["rstd"]
                xn_s[t, RC * i:RC * (i + 1), :] = xn.astype(bf16)

        return ([functools.partial(stats_part, k) for k in range(nparts)],
                [functools.partial(norm_part, k) for k in range(nparts)])

    def ln1_tile(seg, t):
        stats, norm = ln1_units(seg, t, 1)
        for fn in stats + norm:
            fn()

    def proj(i):
        xn = jnp.concatenate([xn_s[t] for t in range(4)], axis=1)
        r = jnp.dot(wT[D * i:D * (i + 1), :], xn, preferred_element_type=f32)
        return jnp.concatenate([r, jnp.zeros((64, L), f32)], axis=0)

    def post_k(r):
        for t in range(4):
            for w in range(NW):
                kk = r[WL * w:WL * w + 128, 128 * t:128 * (t + 1)]
                k_s[w, 64 * t:64 * (t + 1), :] = pltpu.bitcast(kk.astype(bf16).T, u32)
                phikT_s[w, t] = _pack(_phi(kk))

    def post_v(r):
        rr = lax.broadcasted_iota(jnp.int32, (RS, 128), 0)
        ones_row = jnp.where(rr == DH, 1.0, 0.0).astype(f32)
        for t in range(4):
            for w in range(NW):
                nh = _nh(w)
                vs = [jnp.where(rr < DH,
                                r[DH * (HPW * w + a):DH * (HPW * w + a) + RS, 128 * t:128 * (t + 1)], ones_row)
                      for a in range(nh)]
                if (nh * RS) % 16:
                    vs.append(jnp.zeros((16 - (nh * RS) % 16, 128), f32))
                vv = _pack(jnp.concatenate(vs, axis=0))
                vT_s[w, t, 0:vv.shape[0], :] = vv

    def post_q(r):
        for t in range(4):
            for w in range(NW):
                q = r[WL * w:WL * w + 128, 128 * t:128 * (t + 1)]
                qT_s[w, t] = _pack(q * QSCALE)
                phiqT_s[w, t] = _pack(_phi(q))

    def mem_update(ws=range(NW)):
        r = lax.broadcasted_iota(jnp.int32, (MROWS, 128), 0)
        c = lax.broadcasted_iota(jnp.int32, (MROWS, 128), 1)
        for w in ws:
            vt = jnp.concatenate([_unpack(vT_s[w, t, 0:MROWS // 2, :]) for t in range(4)], axis=1)
            pk = jnp.concatenate([_unpack(phikT_s[w, t]) for t in range(4)], axis=1)
            upd = lax.dot_general(vt, pk, (((1,), (1,)), ((), ())), preferred_element_type=f32)
            mt = mt_s[w] + upd
            mt_s[w] = mt
            keep = jnp.zeros((MROWS, 128), jnp.bool_)
            for a in range(_nh(w)):
                keep = keep | ((r >= RS * a) & (r < RS * (a + 1)) & (c >= DH * a) & (c < DH * (a + 1)))
            mtb_s[w] = _pack(jnp.where(keep, mt, 0.0))

    def mem_retrieve():
        for w in range(NW):
            for j in range(4):
                am = jnp.dot(_unpack(mtb_s[w]), _unpack(phiqT_s[w, j]), preferred_element_type=f32)
                for a in range(_nh(w)):
                    ama = am[RS * a:RS * a + 24]
                    g = g_s[w, a:a + 1, :]
                    om = ama * (g * _recip(ama[DH:DH + 1] + 1e-6))
                    am_s[j, WL * w + DH * a:WL * w + DH * (a + 1), :] = om[0:DH]

    def phase_a(w, heads, j, buf):
        n = 128 * (j + 1)
        nh = len(heads)
        cols = slice(128 * heads[0], 128 * (heads[-1] + 1))
        rows = lax.broadcasted_iota(jnp.int32, (64, 128), 0)
        qw = qT_s[w, j]
        qbd = jnp.concatenate(
            [jnp.where((rows >= 9 * a) & (rows < 9 * a + 9), qw, jnp.uint32(0)) for a in heads], axis=1)
        s = jnp.dot(_unpack(k_s[w, 0:n // 2, :]), _unpack(qbd), preferred_element_type=f32)
        kr = lax.broadcasted_iota(jnp.int32, (128, 128), 0)
        qc = lax.broadcasted_iota(jnp.int32, (128, 128), 1)
        causal = kr <= qc
        sd = jnp.concatenate(
            [jnp.where(causal, s[n - 128:n, 128 * a:128 * (a + 1)], NEG) for a in range(nh)], axis=1)
        s_scr[buf, n - 128:n, cols] = sd
        m = jnp.max(sd, axis=0, keepdims=True)
        if j > 0:
            s_scr[buf, 0:n - 128, cols] = s[0:n - 128]
            m = jnp.maximum(m, jnp.max(s[0:n - 128], axis=0, keepdims=True))
        m_scr[buf, :, cols] = jnp.broadcast_to(m, (8, 128 * nh))

    def phase_b(w, heads, j, buf):
        n = 128 * (j + 1)
        for a in heads:
            m = m_scr[buf, 0:1, 128 * a:128 * (a + 1)]
            p = jnp.exp2(s_scr[buf, 0:n, 128 * a:128 * (a + 1)] - m).astype(bf16)
            vt = jnp.concatenate([_unpack(vT_s[w, t, (RS // 2) * a:(RS // 2) * a + 16, :]) for t in range(j + 1)], axis=1)
            o = jnp.dot(vt, p, preferred_element_type=f32)
            g = g_s[w, a:a + 1, :]
            od = o[0:24] * ((1.0 - g) * _recip(o[DH:DH + 1]))
            row0 = WL * w + DH * a
            oT_s[j, pl.ds(row0, DH), :] = (od + am_s[j, pl.ds(row0, 24), :])[0:DH]

    def window(w, nxt, fillers):
        order = [3, 2, 1, 0]
        heads = list(range(_nh(w)))
        for t in range(4):
            for fn in fillers.get(t, ()):
                fn()
            if t < 3:
                phase_a(w, heads, order[t + 1], (t + 1) % 2)
            elif nxt is not None:
                phase_a(nxt, list(range(_nh(nxt))), order[0], 0)
            ws = UPD_PLAN.get((w, t), [])
            if ws:
                mem_update(ws)
            phase_b(w, heads, order[t], t % 2)

    def ln2_out(tile, lo=0, hi=NCH):
        mean = st_s[tile, 0:1, :]
        rstd = st_s[tile, 1:2, :]
        ga = 1.0 + rstd
        gb = mean * rstd
        for i in range(lo, hi):
            rows = slice(RC * i, RC * (i + 1))
            out_v[tile, rows, :] = (h_s[tile, rows, :] * ga - gb).astype(bf16)

    def outproj(seg):
        oT = jnp.concatenate([oT_s[t] for t in range(4)], axis=1).astype(bf16)
        attn = jnp.dot(woT[...], oT, preferred_element_type=f32)
        for t in range(4):
            cols = slice(128 * t, 128 * (t + 1))
            tile = 4 * seg + t
            c = None
            s1, s2, s3 = _Acc(), _Acc(), _Acc()
            for i in range(NCH):
                rows = slice(RC * i, RC * (i + 1))
                h = x_v[seg, rows, cols].astype(f32) + attn[rows, cols]
                h_s[tile, rows, :] = h
                if c is None:
                    c = h[0:1]
                d = h - c
                s1.add(d)
                s2.add(d * d)
                s3.add(d * wr_s[rows, :])
            mu = s1.total() * (1.0 / D)
            var = jnp.maximum(s2.total() * (1.0 / D) - mu * mu, 0.0)
            rstd = lax.rsqrt(var + EPS)
            st_s[tile, 0:1, :] = c + mu
            st_s[tile, 1:2, :] = rstd
            r_s[pl.ds(tile, 1), :] = (s3.total() - mu * wr_s[D:D + 1, :]) * rstd

    def transpose_wd(seg, lo, hi):
        nblk = F // 128 // (NSEG - 1)
        for i in range(lo, hi):
            c0 = pl.multiple_of((seg * nblk + i) * 128, 128)
            wd_s[pl.ds(c0, 128), :] = wdT_v[:, pl.ds(c0, 128)].T

    def project_segment():
        post_k(proj(0))
        post_q(proj(1))
        post_v(proj(2))

    with _scope("setup"):
        x_copy(0).start()
        if PRO == 0:
            w_copies[0].start()
        beta = beta_ref[...].astype(f32).reshape(1, H)
        hrow = lax.broadcasted_iota(jnp.int32, (8 * NW, H), 0)
        hcol = lax.broadcasted_iota(jnp.int32, (8 * NW, H), 1)
        sel = (hcol == HPW * (hrow >> 3) + (hrow & 7)) & ((hrow & 7) < HPW)
        bcol = jnp.sum(jnp.where(sel, beta, 0.0), axis=1, keepdims=True)
        g_s[...] = jnp.broadcast_to(_sigmoid(bcol), (8 * NW, 128)).reshape(NW, 8, 128)
        wr_row = wr_ref[...].astype(f32).reshape(1, D)
        wr_pad = jnp.concatenate([wr_row, jnp.zeros((1, 64), f32)], axis=1)
        wr_s[...] = jnp.broadcast_to(wr_pad, (128, D + 64)).T
        wr_s[D:D + 1, :] = jnp.broadcast_to(jnp.sum(wr_row, axis=1, keepdims=True), (1, 128))

        if PRO == 1:
            w_copies[0].start()
        mt_s[...] = jnp.zeros(mt_s.shape, f32)
        vT_s[...] = jnp.zeros(vT_s.shape, u32)
        am_s[...] = jnp.zeros(am_s.shape, f32)
        if OUTW:
            h_s[0:4] = jnp.zeros((4, D, 128), f32)
            st_s[0:4] = jnp.zeros((4, 8, 128), f32)
        s_scr[:, 0:8, 0:128] = jnp.zeros((2, 8, 128), f32)
        m_scr[...] = jnp.zeros(m_scr.shape, f32)

        if PRO == 2:
            w_copies[0].start()
        x_copy(0).wait()
        w_copies[1].start()
        for t in range(4):
            ln1_tile(0, t)
    with _scope("proj0"):
        w_copies[0].wait()
        w_copies[2].start()
        wT[0:D, :] = wk_v[...].T
        post_k(proj(0))
        w_copies[1].wait()
        w_copies[2].wait()
        w_copies[3].start()
        for s in range(1, NSEG):
            x_copy(s).start()
        wT[D:2 * D, :] = wq_v[...].T
        wT[2 * D:3 * D, :] = wv_v[...].T
        post_q(proj(1))
        post_v(proj(2))
        w_copies[3].wait()
        for s in range(1, NSEG):
            x_copy(s).wait()
        w_copies[4].start()

    def segment(seg, carry):
        nseg = jnp.minimum(seg + 1, NSEG - 1)
        pseg = jnp.maximum(seg - 1, 0)

        with _scope("windows"):
            phase_a(0, list(range(HPW)), 3, 0)
            units = []
            for t in range(4):
                st, nm = ln1_units(nseg, t, LNPARTS)
                units += st + nm
            if OUTW:
                outs = [functools.partial(ln2_out, 4 * pseg + t, NCH * k // 2, NCH * (k + 1) // 2)
                        for t in range(4) for k in range(2)]
                merged = []
                for k, fn in enumerate(units):
                    merged.append(fn)
                    if k % 4 == 3:
                        merged.append(outs[k // 4])
                units = merged
            slots = [(w, t) for w in range(NW) for t in range(4) if t in LNSLOTS][:LNMAX]
            plan = {}
            for k, fn in enumerate(units):
                plan.setdefault(slots[k * len(slots) // len(units)], []).append(fn)
            for w in range(NW):
                fillers = {t: plan.get((w, t), []) for t in range(4)}
                window(w, w + 1 if w + 1 < NW else None, fillers)

        if OUTW:
            @pl.when(seg > 0)
            def _():
                for t in range(4):
                    o_copy(4 * pseg + t).start()

        @pl.when(seg < NSEG - 1)
        def _():
            @pl.when(seg == 0)
            def _():
                w_copies[4].wait()
                for c in w_copies[5:]:
                    c.start()

            with _scope("mid"):
                nblk = F // 128 // (NSEG - 1)

                def t_wo():
                    woT[...] = wo_v[...].T

                steps = {
                    "w": t_wo,
                    "a": lambda: transpose_wd(seg, 0, nblk // 3),
                    "b": lambda: transpose_wd(seg, nblk // 3, 2 * nblk // 3),
                    "c": lambda: transpose_wd(seg, 2 * nblk // 3, nblk),
                    "u": lambda: mem_update([w for w in range(NW) if w not in UPD_IN_W]),
                    "o": lambda: outproj(seg),
                    "k": lambda: post_k(proj(0)),
                    "q": lambda: post_q(proj(1)),
                    "v": lambda: post_v(proj(2)),
                    "r": mem_retrieve,
                    "0": lambda: ln2_out(4 * seg),
                    "1": lambda: ln2_out(4 * seg + 1),
                    "2": lambda: ln2_out(4 * seg + 2),
                    "3": lambda: ln2_out(4 * seg + 3),
                }
                for c in MID_ORDER:
                    if not (OUTW and c in "0123"):
                        steps[c]()
                if not OUTW:
                    for t in range(4):
                        o_copy(4 * seg + t).start()
        return carry

    lax.fori_loop(0, NSEG, segment, 0)
    for c in w_copies[5:]:
        c.wait()
    with _scope("last_out"):
        xs_keep[...] = s_scr[0, 0:8, 0:128] + s_scr[1, 0:8, 0:128] + m_scr[0, :, 0:128] + m_scr[1, :, 0:128]
        outproj(NSEG - 1)
        for t in range(4):
            ln2_out(4 * (NSEG - 1) + t)
            o_copy(4 * (NSEG - 1) + t).start()

    with _scope("ffn"):
        r = r_s[...]
        rmax = jnp.max(r)
        tok = (lax.broadcasted_iota(jnp.int32, (NT, 128), 0) * 128
               + lax.broadcasted_iota(jnp.int32, (NT, 128), 1))
        idx = jnp.minimum(jnp.min(jnp.where(r == rmax, tok, S)), S - 1)
        tile = idx >> 7
        lane = idx & 127
        hn = ((h_s[tile] - st_s[tile, 0:1, :]) * st_s[tile, 1:2, :]).astype(bf16)
        onehot = jnp.where(lax.broadcasted_iota(jnp.int32, (16, 128), 1) == lane, 1.0, 0.0).astype(bf16)
        xs = lax.dot_general(onehot, hn, (((1,), (1,)), ((), ())), preferred_element_type=f32)
        fm = F - 128 * NV
        xm = xs[:, 0:512].astype(bf16)
        xr = xs[:, 512:D]
        row = lax.broadcasted_iota(jnp.int32, (16, 64), 0)
        x2 = jnp.concatenate([jnp.where(row == 0, xr, 0.0), jnp.where(row == 1, xr, 0.0)], axis=1).astype(bf16)
        wrem = jnp.concatenate([wg_v[512:D, 0:fm], wu_v[512:D, 0:fm]], axis=0)
        if NV:
            sel_mat = jnp.where(lax.broadcasted_iota(jnp.int32, (128, 128), 0) == lane, 1.0, 0.0).astype(bf16)
            xb_s[...] = jnp.dot(hn, sel_mat, preferred_element_type=f32)
        rem = jnp.dot(x2, wrem, preferred_element_type=f32)
        gate = jnp.dot(xm, wg_v[0:512, 0:fm], preferred_element_type=f32)[0:1] + rem[0:1]
        up = jnp.dot(xm, wu_v[0:512, 0:fm], preferred_element_type=f32)[0:1] + rem[1:2]
        if NV:
            accs = [None] * (2 * NV)
            for i in range(NCH):
                rows = slice(RC * i, RC * (i + 1))
                xb = xb_s[rows, :]
                for c in range(2 * NV):
                    wsrc = wg_v if c < NV else wu_v
                    c0 = fm + 128 * (c % NV)
                    t = wsrc[rows, c0:c0 + 128].astype(f32) * xb
                    accs[c] = t if accs[c] is None else accs[c] + t
            sums = [jnp.sum(a, axis=0, keepdims=True) for a in accs]
            gate = jnp.concatenate([gate] + sums[:NV], axis=1)
            up = jnp.concatenate([up] + sums[NV:], axis=1)
        act = jnp.broadcast_to(gate * _sigmoid(gate) * up, (16, F)).astype(bf16)
        y = jnp.dot(act, wd_s[...], preferred_element_type=f32)
        y = y[0:1] * _sigmoid(jnp.full((1, 1), rmax, f32))
        ypad = jnp.concatenate([y, jnp.zeros((1, 64), f32)], axis=1)
        ycol = jnp.broadcast_to(ypad, (128, D + 64)).T[0:D]
        for t in range(NT):
            o_copy(t).wait()
        lanes = lax.broadcasted_iota(jnp.int32, (D, 128), 1)
        blk = out_v[tile].astype(f32)
        out_v[tile] = jnp.where(lanes == lane, blk + ycol, blk).astype(bf16)
        fix = o_copy(tile)
        fix.start()
        fix.wait()


@jax.jit
def pallas_sequential_preLN__memory_aug_infini_attn__moe_arch_mod__prompt_kernel(
    A_x: jax.Array,
    A_wq: jax.Array,
    A_wk: jax.Array,
    A_wv: jax.Array,
    A_wo: jax.Array,
    A_beta: jax.Array,
    B_x: jax.Array,
    B_w_r: jax.Array,
    B_w_gate: jax.Array,
    B_w_up: jax.Array,
    B_w_down: jax.Array,
):
    del B_x
    xT = A_x.reshape(S, D).T
    wdT = B_w_down.T

    hbm = pl.BlockSpec(memory_space=pltpu.HBM)
    vmem = pl.BlockSpec(memory_space=pltpu.VMEM)
    scratch = [
        pltpu.VMEM((NSEG, D, L), bf16),
        pltpu.VMEM((D, D), bf16),
        pltpu.VMEM((D, D), bf16),
        pltpu.VMEM((D, D), bf16),
        pltpu.VMEM((D, D), bf16),
        pltpu.VMEM((D, F), bf16),
        pltpu.VMEM((D, F), bf16),
        pltpu.VMEM((D, F), bf16),
        pltpu.VMEM((3 * D, D), bf16),
        pltpu.VMEM((D, D), bf16),
        pltpu.VMEM((F, D), bf16),
        pltpu.VMEM((NW, 8, 128), f32),
        pltpu.VMEM((D + 64, 128), f32),
        pltpu.VMEM((4, D, 128), bf16),
        pltpu.VMEM((NW, L // 2, 128), u32),
        pltpu.VMEM((NW, 4, 64, 128), u32),
        pltpu.VMEM((NW, 4, 64, 128), u32),
        pltpu.VMEM((NW, 4, 64, 128), u32),
        pltpu.VMEM((NW, 4, VWORDS, 128), u32),
        pltpu.VMEM((NW, MROWS, 128), f32),
        pltpu.VMEM((NW, MROWS // 2, 128), u32),
        pltpu.VMEM((4, D + 8, 128), f32),
        pltpu.VMEM((2, L, 128 * HPW), f32),
        pltpu.VMEM((2, 8, 128 * HPW), f32),
        pltpu.VMEM((4, D, 128), f32),
        pltpu.VMEM((NT, D, 128), bf16),
        pltpu.VMEM((NT, D, 128), f32),
        pltpu.VMEM((NT, 8, 128), f32),
        pltpu.VMEM((NT, 128), f32),
        pltpu.VMEM((8, 128), f32),
        pltpu.VMEM((D, 128), f32),
        pltpu.SemaphoreType.DMA((NSEG,)),
        pltpu.SemaphoreType.DMA((7,)),
        pltpu.SemaphoreType.DMA((NT,)),
    ]
    outT = pl.pallas_call(
        _kernel,
        out_shape=jax.ShapeDtypeStruct((D, S), bf16),
        in_specs=[hbm, hbm, hbm, hbm, hbm, vmem, vmem, hbm, hbm, hbm],
        out_specs=hbm,
        scratch_shapes=scratch,
        compiler_params=pltpu.CompilerParams(vmem_limit_bytes=100 * 1024 * 1024),
    )(xT, A_wq, A_wk, A_wv, A_wo, A_beta, B_w_r, B_w_gate, B_w_up, B_w_down.T)
    return outT.T.reshape(1, S, D)
```

```python
import contextlib
import functools
import os

import jax
import jax.numpy as jnp
from jax import lax
import jax.experimental.pallas as pl
import jax.experimental.pallas.tpu as pltpu

S = 2048
D = 576
H = 32
DH = 18
NSEG = 4
L = 512
NT = S // 128
F = 4608
HPW = 7
NW = 5
WL = HPW * DH
RS = 20
MROWS = 144
VWORDS = 80
LOG2E = 1.4426950408889634
NEG = -1e9 * LOG2E
QSCALE = (DH ** -0.5) * LOG2E
EPS = 1e-5
MID_ORDER = os.environ.get('MID_ORDER', 'wabcukqvor0123')
UPD_PLAN = {}
for _e in os.environ.get('UPD', '12:0,22:1,32:2,42:3,43:4').split(','):
    if _e:
        UPD_PLAN.setdefault((int(_e[0]), int(_e[1])), []).append(int(_e[3]))
UPD_IN_W = [u for v in UPD_PLAN.values() for u in v]
LNPOS = int(os.environ.get('LNPOS', '0'))
BARRIER = int(os.environ.get('BARRIER', '3'))
NV = int(os.environ.get('NV', '10'))
RECIP = int(os.environ.get('RECIP', '0'))
OUTW = int(os.environ.get('OUTW', '0'))
PRO = int(os.environ.get('PRO', '1'))
LNPARTS = int(os.environ.get('LNPARTS', '4'))
LNSLOTS = [int(c) for c in os.environ.get('LNSLOTS', '0123')]
LNMAX = int(os.environ.get('LNMAX', '99'))

_PROF = bool(os.environ.get("PROF"))


def _scope(name):
    return jax.named_scope(name) if _PROF else contextlib.nullcontext()


f32 = jnp.float32
bf16 = jnp.bfloat16
u32 = jnp.uint32


def _nh(w):
    return HPW if w < NW - 1 else H - HPW * (NW - 1)


def _pack(x):
    return pltpu.bitcast(x.astype(bf16), u32)


def _unpack(x):
    return pltpu.bitcast(x, bf16)


def _phi(t):
    return jnp.where(t > 0, t + 1.0, jnp.exp(t))


RC = int(os.environ.get('RC', '16'))
NCH = D // RC


class _Acc:
    def __init__(self, n=int(os.environ.get('NACC', '2'))):
        self.parts = [None] * n
        self.i = 0

    def add(self, x):
        k = self.i % len(self.parts)
        self.parts[k] = x if self.parts[k] is None else self.parts[k] + x
        self.i += 1

    def total(self):
        t = self.parts[0]
        for p in self.parts[1:]:
            t = t + p
        return jnp.sum(t, axis=0, keepdims=True)


def _ln_stats(chunk):
    x0 = chunk(0)
    c = x0[0:1]
    s1, s2 = _Acc(), _Acc()
    for i in range(NCH):
        d = (x0 if i == 0 else chunk(i)) - c
        s1.add(d)
        s2.add(d * d)
    mu = s1.total() * (1.0 / D)
    var = jnp.maximum(s2.total() * (1.0 / D) - mu * mu, 0.0)
    return c + mu, lax.rsqrt(var + EPS)


def _recip(x):
    if RECIP == 0:
        return 1.0 / x
    r = pl.reciprocal(x, approx=True)
    return r * (2.0 - x * r)


def _sigmoid(x):
    return 1.0 / (1.0 + jnp.exp(-x))


def _kernel(xT_hbm, wq_hbm, wk_hbm, wv_hbm, wo_hbm, beta_ref, wr_ref, wg_hbm, wu_hbm, wdT_hbm,
            out_hbm,
            x_v, wq_v, wk_v, wv_v, wo_v, wg_v, wu_v, wdT_v,
            wT, woT, wd_s, g_s, wr_s,
            xn_s, k_s, phikT_s, qT_s, phiqT_s, vT_s, mt_s, mtb_s, am_s,
            s_scr, m_scr, oT_s, out_v, h_s, st_s, r_s, xs_keep, xb_s, zero_s,
            sem_x, sem_w, sem_o):
    def x_copy(s):
        return pltpu.make_async_copy(xT_hbm.at[:, pl.ds(s * L, L)], x_v.at[s], sem_x.at[s])

    def o_copy(t):
        return pltpu.make_async_copy(out_v.at[t], out_hbm.at[:, pl.ds(pl.multiple_of(t * 128, 128), 128)],
                                     sem_o.at[t])

    w_copies = [pltpu.make_async_copy(src, dst, sem_w.at[i]) for i, (src, dst) in enumerate(
        [(wk_hbm, wk_v), (wq_hbm, wq_v), (wv_hbm, wv_v), (wo_hbm, wo_v),
         (wdT_hbm, wdT_v), (wg_hbm, wg_v), (wu_hbm, wu_v)])]

    def ln1_chunk(seg, t, i):
        cols = pl.ds(pl.multiple_of(t * 128, 128), 128)
        return x_v[seg, RC * i:RC * (i + 1), cols].astype(f32)

    def ln1_units(seg, t, nparts):
        st = {}
        bounds = [NCH * i // nparts for i in range(nparts + 1)]

        def stats_part(k):
            if k == 0:
                x0 = ln1_chunk(seg, t, 0)
                st["x0"], st["c"] = x0, x0[0:1]
                st["s1"], st["s2"] = _Acc(), _Acc()
            for i in range(bounds[k], bounds[k + 1]):
                d = (st["x0"] if i == 0 else ln1_chunk(seg, t, i)) - st["c"]
                st["s1"].add(d)
                st["s2"].add(d * d)
            if k == nparts - 1:
                mu = st["s1"].total() * (1.0 / D)
                var = jnp.maximum(st["s2"].total() * (1.0 / D) - mu * mu, 0.0)
                st["mean"], st["rstd"] = st["c"] + mu, lax.rsqrt(var + EPS)

        def norm_part(k):
            for i in range(bounds[k], bounds[k + 1]):
                xn = (ln1_chunk(seg, t, i) - st["mean"]) * st["rstd"]
                xn_s[t, RC * i:RC * (i + 1), :] = xn.astype(bf16)

        return ([functools.partial(stats_part, k) for k in range(nparts)],
                [functools.partial(norm_part, k) for k in range(nparts)])

    def ln1_tile(seg, t):
        stats, norm = ln1_units(seg, t, 1)
        for fn in stats + norm:
            fn()

    def proj(i):
        xn = jnp.concatenate([xn_s[t] for t in range(4)], axis=1)
        r = jnp.dot(wT[D * i:D * (i + 1), :], xn, preferred_element_type=f32)
        return jnp.concatenate([r, jnp.zeros((64, L), f32)], axis=0)

    def post_k(r):
        for t in range(4):
            for w in range(NW):
                kk = r[WL * w:WL * w + 128, 128 * t:128 * (t + 1)]
                k_s[w, 64 * t:64 * (t + 1), :] = pltpu.bitcast(kk.astype(bf16).T, u32)
                phikT_s[w, t] = _pack(_phi(kk))

    def post_v(r):
        rr = lax.broadcasted_iota(jnp.int32, (RS, 128), 0)
        ones_row = jnp.where(rr == DH, 1.0, 0.0).astype(f32)
        for t in range(4):
            for w in range(NW):
                nh = _nh(w)
                vs = [jnp.where(rr < DH,
                                r[DH * (HPW * w + a):DH * (HPW * w + a) + RS, 128 * t:128 * (t + 1)], ones_row)
                      for a in range(nh)]
                if (nh * RS) % 16:
                    vs.append(jnp.zeros((16 - (nh * RS) % 16, 128), f32))
                vv = _pack(jnp.concatenate(vs, axis=0))
                vT_s[w, t, 0:vv.shape[0], :] = vv

    def post_q(r):
        for t in range(4):
            for w in range(NW):
                q = r[WL * w:WL * w + 128, 128 * t:128 * (t + 1)]
                qT_s[w, t] = _pack(q * QSCALE)
                phiqT_s[w, t] = _pack(_phi(q))

    def mem_update(ws=range(NW)):
        r = lax.broadcasted_iota(jnp.int32, (MROWS, 128), 0)
        c = lax.broadcasted_iota(jnp.int32, (MROWS, 128), 1)
        for w in ws:
            vt = jnp.concatenate([_unpack(vT_s[w, t, 0:MROWS // 2, :]) for t in range(4)], axis=1)
            pk = jnp.concatenate([_unpack(phikT_s[w, t]) for t in range(4)], axis=1)
            upd = lax.dot_general(vt, pk, (((1,), (1,)), ((), ())), preferred_element_type=f32)
            mt = mt_s[w] + upd
            mt_s[w] = mt
            keep = jnp.zeros((MROWS, 128), jnp.bool_)
            for a in range(_nh(w)):
                keep = keep | ((r >= RS * a) & (r < RS * (a + 1)) & (c >= DH * a) & (c < DH * (a + 1)))
            mtb_s[w] = _pack(jnp.where(keep, mt, 0.0))

    def mem_retrieve():
        for w in range(NW):
            for j in range(4):
                am = jnp.dot(_unpack(mtb_s[w]), _unpack(phiqT_s[w, j]), preferred_element_type=f32)
                for a in range(_nh(w)):
                    ama = am[RS * a:RS * a + 24]
                    g = g_s[w, a:a + 1, :]
                    om = ama * (g * _recip(ama[DH:DH + 1] + 1e-6))
                    am_s[j, WL * w + DH * a:WL * w + DH * (a + 1), :] = om[0:DH]

    def phase_a(w, heads, j, buf):
        n = 128 * (j + 1)
        nh = len(heads)
        cols = slice(128 * heads[0], 128 * (heads[-1] + 1))
        rows = lax.broadcasted_iota(jnp.int32, (64, 128), 0)
        qw = qT_s[w, j]
        qbd = jnp.concatenate(
            [jnp.where((rows >= 9 * a) & (rows < 9 * a + 9), qw, jnp.uint32(0)) for a in heads], axis=1)
        s = jnp.dot(_unpack(k_s[w, 0:n // 2, :]), _unpack(qbd), preferred_element_type=f32)
        kr = lax.broadcasted_iota(jnp.int32, (128, 128), 0)
        qc = lax.broadcasted_iota(jnp.int32, (128, 128), 1)
        causal = kr <= qc
        sd = jnp.concatenate(
            [jnp.where(causal, s[n - 128:n, 128 * a:128 * (a + 1)], NEG) for a in range(nh)], axis=1)
        s_scr[buf, n - 128:n, cols] = sd
        m = jnp.max(sd, axis=0, keepdims=True)
        if j > 0:
            s_scr[buf, 0:n - 128, cols] = s[0:n - 128]
            m = jnp.maximum(m, jnp.max(s[0:n - 128], axis=0, keepdims=True))
        m_scr[buf, :, cols] = jnp.broadcast_to(m, (8, 128 * nh))

    def phase_b(w, heads, j, buf):
        n = 128 * (j + 1)
        for a in heads:
            m = m_scr[buf, 0:1, 128 * a:128 * (a + 1)]
            p = jnp.exp2(s_scr[buf, 0:n, 128 * a:128 * (a + 1)] - m).astype(bf16)
            vt = jnp.concatenate([_unpack(vT_s[w, t, (RS // 2) * a:(RS // 2) * a + 16, :]) for t in range(j + 1)], axis=1)
            o = jnp.dot(vt, p, preferred_element_type=f32)
            g = g_s[w, a:a + 1, :]
            od = o[0:24] * ((1.0 - g) * _recip(o[DH:DH + 1]))
            row0 = WL * w + DH * a
            oT_s[j, pl.ds(row0, DH), :] = (od + am_s[j, pl.ds(row0, 24), :])[0:DH]

    def window(w, nxt, fillers, upd_plan):
        order = [3, 2, 1, 0]
        heads = list(range(_nh(w)))
        for t in range(4):
            for fn in fillers.get(t, ()):
                fn()
            if t < 3:
                phase_a(w, heads, order[t + 1], (t + 1) % 2)
            elif nxt is not None:
                phase_a(nxt, list(range(_nh(nxt))), order[0], 0)
            ws = upd_plan.get((w, t), [])
            if ws:
                mem_update(ws)
            phase_b(w, heads, order[t], t % 2)

    def ln2_out(tile, lo=0, hi=NCH):
        mean = st_s[tile, 0:1, :]
        rstd = st_s[tile, 1:2, :]
        ga = 1.0 + rstd
        gb = mean * rstd
        for i in range(lo, hi):
            rows = slice(RC * i, RC * (i + 1))
            out_v[tile, rows, :] = (h_s[tile, rows, :] * ga - gb).astype(bf16)

    def outproj(seg):
        oT = jnp.concatenate([oT_s[t] for t in range(4)], axis=1).astype(bf16)
        attn = jnp.dot(woT[...], oT, preferred_element_type=f32)
        for t in range(4):
            cols = slice(128 * t, 128 * (t + 1))
            tile = 4 * seg + t
            c = None
            s1, s2, s3 = _Acc(), _Acc(), _Acc()
            for i in range(NCH):
                rows = slice(RC * i, RC * (i + 1))
                h = x_v[seg, rows, cols].astype(f32) + attn[rows, cols]
                h_s[tile, rows, :] = h
                if c is None:
                    c = h[0:1]
                d = h - c
                s1.add(d)
                s2.add(d * d)
                s3.add(d * wr_s[rows, :])
            mu = s1.total() * (1.0 / D)
            var = jnp.maximum(s2.total() * (1.0 / D) - mu * mu, 0.0)
            rstd = lax.rsqrt(var + EPS)
            st_s[tile, 0:1, :] = c + mu
            st_s[tile, 1:2, :] = rstd
            r_s[pl.ds(tile, 1), :] = (s3.total() - mu * wr_s[D:D + 1, :]) * rstd

    def transpose_wd(lo, hi):
        for i in range(lo, hi):
            wd_s[128 * i:128 * (i + 1), :] = wdT_v[:, 128 * i:128 * (i + 1)].T

    def project_segment():
        post_k(proj(0))
        post_q(proj(1))
        post_v(proj(2))

    with _scope("setup"):
        x_copy(0).start()
        if PRO == 0:
            w_copies[0].start()
        beta = beta_ref[...].astype(f32).reshape(1, H)
        hrow = lax.broadcasted_iota(jnp.int32, (8 * NW, H), 0)
        hcol = lax.broadcasted_iota(jnp.int32, (8 * NW, H), 1)
        sel = (hcol == HPW * (hrow >> 3) + (hrow & 7)) & ((hrow & 7) < HPW)
        bcol = jnp.sum(jnp.where(sel, beta, 0.0), axis=1, keepdims=True)
        g_s[...] = jnp.broadcast_to(_sigmoid(bcol), (8 * NW, 128)).reshape(NW, 8, 128)
        wr_row = wr_ref[...].astype(f32).reshape(1, D)
        wr_pad = jnp.concatenate([wr_row, jnp.zeros((1, 64), f32)], axis=1)
        wr_s[...] = jnp.broadcast_to(wr_pad, (128, D + 64)).T
        wr_s[D:D + 1, :] = jnp.broadcast_to(jnp.sum(wr_row, axis=1, keepdims=True), (1, 128))

        if PRO == 1:
            w_copies[0].start()
        zero_s[0] = 0
        mt_s[...] = jnp.zeros(mt_s.shape, f32)
        vT_s[...] = jnp.zeros(vT_s.shape, u32)
        am_s[...] = jnp.zeros(am_s.shape, f32)
        if OUTW:
            h_s[0:4] = jnp.zeros((4, D, 128), f32)
            st_s[0:4] = jnp.zeros((4, 8, 128), f32)
        s_scr[:, 0:8, 0:128] = jnp.zeros((2, 8, 128), f32)
        m_scr[...] = jnp.zeros(m_scr.shape, f32)

        if PRO == 2:
            w_copies[0].start()
        x_copy(0).wait()
        w_copies[1].start()
        for t in range(4):
            ln1_tile(0, t)
    with _scope("proj0"):
        w_copies[0].wait()
        w_copies[2].start()
        wT[0:D, :] = wk_v[...].T
        post_k(proj(0))
        w_copies[1].wait()
        w_copies[2].wait()
        w_copies[3].start()
        for s in range(1, NSEG):
            x_copy(s).start()
        wT[D:2 * D, :] = wq_v[...].T
        wT[2 * D:3 * D, :] = wv_v[...].T
        post_q(proj(1))
        post_v(proj(2))
        w_copies[3].wait()
        for s in range(1, NSEG):
            x_copy(s).wait()
        for c in w_copies[4:]:
            c.start()

    def windows(units, upd_plan):
        phase_a(0, list(range(HPW)), 3, 0)
        slots = [(w, t) for w in range(NW) for t in range(4)]
        plan = {}
        for k, fn in enumerate(units):
            plan.setdefault(slots[k * len(slots) // len(units)], []).append(fn)
        for w in range(NW):
            fillers = {t: plan.get((w, t), []) for t in range(4)}
            window(w, w + 1 if w + 1 < NW else None, fillers, upd_plan)

    def t_wo():
        woT[...] = wo_v[...].T

    def barrier():
        @pl.when(zero_s[0] != 0)
        def _():
            xs_keep[...] = s_scr[0, 0:8, 0:128]

    def segment(seg, carry):
        with _scope("windows"):
            units = []
            for t in range(4):
                st, nm = ln1_units(seg + 1, t, LNPARTS)
                units += st + nm
            windows(units, UPD_PLAN)
        if BARRIER & 1:
            barrier()

        with _scope("mid"):
            steps = {
                "w": t_wo,
                "u": lambda: mem_update([w for w in range(NW) if w not in UPD_IN_W]),
                "o": lambda: outproj(seg),
                "k": lambda: post_k(proj(0)),
                "q": lambda: post_q(proj(1)),
                "v": lambda: post_v(proj(2)),
                "r": mem_retrieve,
                "0": lambda: ln2_out(4 * seg),
                "1": lambda: ln2_out(4 * seg + 1),
                "2": lambda: ln2_out(4 * seg + 2),
                "3": lambda: ln2_out(4 * seg + 3),
            }
            for c in MID_ORDER:
                if c in steps:
                    steps[c]()
            for t in range(4):
                o_copy(4 * seg + t).start()
        return carry

    lax.fori_loop(0, NSEG - 1, segment, 0)
    for c in w_copies[4:]:
        c.wait()
    with _scope("windows_last"):
        nb = F // 128
        windows([functools.partial(transpose_wd, i, i + 1) for i in range(nb)], {})
    if BARRIER & 2:
        barrier()
    with _scope("last_out"):
        xs_keep[...] = s_scr[0, 0:8, 0:128] + s_scr[1, 0:8, 0:128] + m_scr[0, :, 0:128] + m_scr[1, :, 0:128]
        outproj(NSEG - 1)
        for t in range(4):
            ln2_out(4 * (NSEG - 1) + t)
            o_copy(4 * (NSEG - 1) + t).start()

    if BARRIER & 4:
        barrier()
    with _scope("ffn"):
        r = r_s[...]
        rmax = jnp.max(r)
        tok = (lax.broadcasted_iota(jnp.int32, (NT, 128), 0) * 128
               + lax.broadcasted_iota(jnp.int32, (NT, 128), 1))
        idx = jnp.minimum(jnp.min(jnp.where(r == rmax, tok, S)), S - 1)
        tile = idx >> 7
        lane = idx & 127
        hn = ((h_s[tile] - st_s[tile, 0:1, :]) * st_s[tile, 1:2, :]).astype(bf16)
        onehot = jnp.where(lax.broadcasted_iota(jnp.int32, (16, 128), 1) == lane, 1.0, 0.0).astype(bf16)
        xs = lax.dot_general(onehot, hn, (((1,), (1,)), ((), ())), preferred_element_type=f32)
        fm = F - 128 * NV
        xm = xs[:, 0:512].astype(bf16)
        xr = xs[:, 512:D]
        row = lax.broadcasted_iota(jnp.int32, (16, 64), 0)
        x2 = jnp.concatenate([jnp.where(row == 0, xr, 0.0), jnp.where(row == 1, xr, 0.0)], axis=1).astype(bf16)
        wrem = jnp.concatenate([wg_v[512:D, 0:fm], wu_v[512:D, 0:fm]], axis=0)
        if NV:
            sel_mat = jnp.where(lax.broadcasted_iota(jnp.int32, (128, 128), 0) == lane, 1.0, 0.0).astype(bf16)
            xb_s[...] = jnp.dot(hn, sel_mat, preferred_element_type=f32)
        rem = jnp.dot(x2, wrem, preferred_element_type=f32)
        gate = jnp.dot(xm, wg_v[0:512, 0:fm], preferred_element_type=f32)[0:1] + rem[0:1]
        up = jnp.dot(xm, wu_v[0:512, 0:fm], preferred_element_type=f32)[0:1] + rem[1:2]
        if NV:
            accs = [None] * (2 * NV)
            for i in range(NCH):
                rows = slice(RC * i, RC * (i + 1))
                xb = xb_s[rows, :]
                for c in range(2 * NV):
                    wsrc = wg_v if c < NV else wu_v
                    c0 = fm + 128 * (c % NV)
                    t = wsrc[rows, c0:c0 + 128].astype(f32) * xb
                    accs[c] = t if accs[c] is None else accs[c] + t
            sums = [jnp.sum(a, axis=0, keepdims=True) for a in accs]
            gate = jnp.concatenate([gate] + sums[:NV], axis=1)
            up = jnp.concatenate([up] + sums[NV:], axis=1)
        act = jnp.broadcast_to(gate * _sigmoid(gate) * up, (16, F)).astype(bf16)
        y = jnp.dot(act, wd_s[...], preferred_element_type=f32)
        y = y[0:1] * _sigmoid(jnp.full((1, 1), rmax, f32))
        ypad = jnp.concatenate([y, jnp.zeros((1, 64), f32)], axis=1)
        ycol = jnp.broadcast_to(ypad, (128, D + 64)).T[0:D]
        for t in range(NT):
            o_copy(t).wait()
        lanes = lax.broadcasted_iota(jnp.int32, (D, 128), 1)
        blk = out_v[tile].astype(f32)
        out_v[tile] = jnp.where(lanes == lane, blk + ycol, blk).astype(bf16)
        fix = o_copy(tile)
        fix.start()
        fix.wait()


@jax.jit
def pallas_sequential_preLN__memory_aug_infini_attn__moe_arch_mod__prompt_kernel(
    A_x: jax.Array,
    A_wq: jax.Array,
    A_wk: jax.Array,
    A_wv: jax.Array,
    A_wo: jax.Array,
    A_beta: jax.Array,
    B_x: jax.Array,
    B_w_r: jax.Array,
    B_w_gate: jax.Array,
    B_w_up: jax.Array,
    B_w_down: jax.Array,
):
    del B_x
    xT = A_x.reshape(S, D).T
    wdT = B_w_down.T

    hbm = pl.BlockSpec(memory_space=pltpu.HBM)
    vmem = pl.BlockSpec(memory_space=pltpu.VMEM)
    scratch = [
        pltpu.VMEM((NSEG, D, L), bf16),
        pltpu.VMEM((D, D), bf16),
        pltpu.VMEM((D, D), bf16),
        pltpu.VMEM((D, D), bf16),
        pltpu.VMEM((D, D), bf16),
        pltpu.VMEM((D, F), bf16),
        pltpu.VMEM((D, F), bf16),
        pltpu.VMEM((D, F), bf16),
        pltpu.VMEM((3 * D, D), bf16),
        pltpu.VMEM((D, D), bf16),
        pltpu.VMEM((F, D), bf16),
        pltpu.VMEM((NW, 8, 128), f32),
        pltpu.VMEM((D + 64, 128), f32),
        pltpu.VMEM((4, D, 128), bf16),
        pltpu.VMEM((NW, L // 2, 128), u32),
        pltpu.VMEM((NW, 4, 64, 128), u32),
        pltpu.VMEM((NW, 4, 64, 128), u32),
        pltpu.VMEM((NW, 4, 64, 128), u32),
        pltpu.VMEM((NW, 4, VWORDS, 128), u32),
        pltpu.VMEM((NW, MROWS, 128), f32),
        pltpu.VMEM((NW, MROWS // 2, 128), u32),
        pltpu.VMEM((4, D + 8, 128), f32),
        pltpu.VMEM((2, L, 128 * HPW), f32),
        pltpu.VMEM((2, 8, 128 * HPW), f32),
        pltpu.VMEM((4, D, 128), f32),
        pltpu.VMEM((NT, D, 128), bf16),
        pltpu.VMEM((NT, D, 128), f32),
        pltpu.VMEM((NT, 8, 128), f32),
        pltpu.VMEM((NT, 128), f32),
        pltpu.VMEM((8, 128), f32),
        pltpu.VMEM((D, 128), f32),
        pltpu.SMEM((1,), jnp.int32),
        pltpu.SemaphoreType.DMA((NSEG,)),
        pltpu.SemaphoreType.DMA((7,)),
        pltpu.SemaphoreType.DMA((NT,)),
    ]
    outT = pl.pallas_call(
        _kernel,
        out_shape=jax.ShapeDtypeStruct((D, S), bf16),
        in_specs=[hbm, hbm, hbm, hbm, hbm, vmem, vmem, hbm, hbm, hbm],
        out_specs=hbm,
        scratch_shapes=scratch,
        compiler_params=pltpu.CompilerParams(vmem_limit_bytes=100 * 1024 * 1024),
    )(xT, A_wq, A_wk, A_wv, A_wo, A_beta, B_w_r, B_w_gate, B_w_up, B_w_down.T)
    return outT.T.reshape(1, S, D)
```

```python
import functools

import jax
import jax.numpy as jnp
from jax import lax
import jax.experimental.pallas as pl
import jax.experimental.pallas.tpu as pltpu

S = 2048
D = 576
H = 32
DH = 18
NSEG = 4
L = 512
NT = S // 128
F = 4608
HPW = 7
NW = 5
WL = HPW * DH
RS = 20
MROWS = 144
VWORDS = 80
LOG2E = 1.4426950408889634
NEG = -1e9 * LOG2E
QSCALE = (DH ** -0.5) * LOG2E
EPS = 1e-5
RC = 16
NCH = D // RC
LNPARTS = 4
NV = 10
UPD_PLAN = {(1, 2): [0], (2, 2): [1], (3, 2): [2], (4, 2): [3], (4, 3): [4]}

f32 = jnp.float32
bf16 = jnp.bfloat16
u32 = jnp.uint32


def _nh(w):
    return HPW if w < NW - 1 else H - HPW * (NW - 1)


def _pack(x):
    return pltpu.bitcast(x.astype(bf16), u32)


def _unpack(x):
    return pltpu.bitcast(x, bf16)


def _phi(t):
    return jnp.where(t > 0, t + 1.0, jnp.exp(t))


class _Acc:
    def __init__(self, n=2):
        self.parts = [None] * n
        self.i = 0

    def add(self, x):
        k = self.i % len(self.parts)
        self.parts[k] = x if self.parts[k] is None else self.parts[k] + x
        self.i += 1

    def total(self):
        t = self.parts[0]
        for p in self.parts[1:]:
            t = t + p
        return jnp.sum(t, axis=0, keepdims=True)


def _sigmoid(x):
    return 1.0 / (1.0 + jnp.exp(-x))


def _kernel(xT_hbm, wq_hbm, wk_hbm, wv_hbm, wo_hbm, beta_ref, wr_ref, wg_hbm, wu_hbm, wdT_hbm,
            out_hbm,
            x_v, wq_v, wk_v, wv_v, wo_v, wg_v, wu_v, wdT_v,
            wT, woT, wd_s, g_s, wr_s,
            xn_s, k_s, phikT_s, qT_s, phiqT_s, vT_s, mt_s, mtb_s, am_s,
            s_scr, m_scr, oT_s, out_v, h_s, st_s, r_s, xs_keep, xb_s, zero_s,
            sem_x, sem_w, sem_o):
    def x_copy(s):
        return pltpu.make_async_copy(xT_hbm.at[:, pl.ds(s * L, L)], x_v.at[s], sem_x.at[s])

    def o_copy(t):
        return pltpu.make_async_copy(out_v.at[t], out_hbm.at[:, pl.ds(pl.multiple_of(t * 128, 128), 128)],
                                     sem_o.at[t])

    w_copies = [pltpu.make_async_copy(src, dst, sem_w.at[i]) for i, (src, dst) in enumerate(
        [(wk_hbm, wk_v), (wq_hbm, wq_v), (wv_hbm, wv_v), (wo_hbm, wo_v),
         (wdT_hbm, wdT_v), (wg_hbm, wg_v), (wu_hbm, wu_v)])]

    def ln1_chunk(seg, t, i):
        cols = pl.ds(pl.multiple_of(t * 128, 128), 128)
        return x_v[seg, RC * i:RC * (i + 1), cols].astype(f32)

    def ln1_units(seg, t, nparts):
        st = {}
        bounds = [NCH * i // nparts for i in range(nparts + 1)]

        def stats_part(k):
            if k == 0:
                x0 = ln1_chunk(seg, t, 0)
                st["x0"], st["c"] = x0, x0[0:1]
                st["s1"], st["s2"] = _Acc(), _Acc()
            for i in range(bounds[k], bounds[k + 1]):
                d = (st["x0"] if i == 0 else ln1_chunk(seg, t, i)) - st["c"]
                st["s1"].add(d)
                st["s2"].add(d * d)
            if k == nparts - 1:
                mu = st["s1"].total() * (1.0 / D)
                var = jnp.maximum(st["s2"].total() * (1.0 / D) - mu * mu, 0.0)
                st["mean"], st["rstd"] = st["c"] + mu, lax.rsqrt(var + EPS)

        def norm_part(k):
            for i in range(bounds[k], bounds[k + 1]):
                xn = (ln1_chunk(seg, t, i) - st["mean"]) * st["rstd"]
                xn_s[t, RC * i:RC * (i + 1), :] = xn.astype(bf16)

        return ([functools.partial(stats_part, k) for k in range(nparts)],
                [functools.partial(norm_part, k) for k in range(nparts)])

    def ln1_tile(seg, t):
        stats, norm = ln1_units(seg, t, 1)
        for fn in stats + norm:
            fn()

    def proj(i):
        xn = jnp.concatenate([xn_s[t] for t in range(4)], axis=1)
        r = jnp.dot(wT[D * i:D * (i + 1), :], xn, preferred_element_type=f32)
        return jnp.concatenate([r, jnp.zeros((64, L), f32)], axis=0)

    def post_k(r):
        for w in range(NW):
            for t in range(4):
                kk = r[WL * w:WL * w + 128, 128 * t:128 * (t + 1)]
                k_s[w, 64 * t:64 * (t + 1), :] = pltpu.bitcast(kk.astype(bf16).T, u32)
                phikT_s[w, t] = _pack(_phi(kk))

    def post_v(r):
        rr = lax.broadcasted_iota(jnp.int32, (RS, 128), 0)
        ones_row = jnp.where(rr == DH, 1.0, 0.0).astype(f32)
        for w in range(NW):
            for t in range(4):
                nh = _nh(w)
                vs = [jnp.where(rr < DH,
                                r[DH * (HPW * w + a):DH * (HPW * w + a) + RS, 128 * t:128 * (t + 1)], ones_row)
                      for a in range(nh)]
                if (nh * RS) % 16:
                    vs.append(jnp.zeros((16 - (nh * RS) % 16, 128), f32))
                vv = _pack(jnp.concatenate(vs, axis=0))
                vT_s[w, t, 0:vv.shape[0], :] = vv

    def post_q(r):
        for w in range(NW):
            for t in range(4):
                q = r[WL * w:WL * w + 128, 128 * t:128 * (t + 1)]
                qT_s[w, t] = _pack(q * QSCALE)
                phiqT_s[w, t] = _pack(_phi(q))

    def mem_update(ws=range(NW)):
        r = lax.broadcasted_iota(jnp.int32, (MROWS, 128), 0)
        c = lax.broadcasted_iota(jnp.int32, (MROWS, 128), 1)
        for w in ws:
            vt = jnp.concatenate([_unpack(vT_s[w, t, 0:MROWS // 2, :]) for t in range(4)], axis=1)
            pk = jnp.concatenate([_unpack(phikT_s[w, t]) for t in range(4)], axis=1)
            upd = lax.dot_general(vt, pk, (((1,), (1,)), ((), ())), preferred_element_type=f32)
            mt = mt_s[w] + upd
            mt_s[w] = mt
            keep = jnp.zeros((MROWS, 128), jnp.bool_)
            for a in range(_nh(w)):
                keep = keep | ((r >= RS * a) & (r < RS * (a + 1)) & (c >= DH * a) & (c < DH * (a + 1)))
            mtb_s[w] = _pack(jnp.where(keep, mt, 0.0))

    def mem_retrieve():
        for w in range(NW):
            for j in range(4):
                am = jnp.dot(_unpack(mtb_s[w]), _unpack(phiqT_s[w, j]), preferred_element_type=f32)
                for a in range(_nh(w)):
                    ama = am[RS * a:RS * a + 24]
                    g = g_s[w, a:a + 1, :]
                    om = ama * (g / (ama[DH:DH + 1] + 1e-6))
                    am_s[j, WL * w + DH * a:WL * w + DH * (a + 1), :] = om[0:DH]

    def phase_a(w, heads, j, buf):
        n = 128 * (j + 1)
        nh = len(heads)
        cols = slice(128 * heads[0], 128 * (heads[-1] + 1))
        rows = lax.broadcasted_iota(jnp.int32, (64, 128), 0)
        qw = qT_s[w, j]
        qbd = jnp.concatenate(
            [jnp.where((rows >= 9 * a) & (rows < 9 * a + 9), qw, jnp.uint32(0)) for a in heads], axis=1)
        s = jnp.dot(_unpack(k_s[w, 0:n // 2, :]), _unpack(qbd), preferred_element_type=f32)
        kr = lax.broadcasted_iota(jnp.int32, (128, 128), 0)
        qc = lax.broadcasted_iota(jnp.int32, (128, 128), 1)
        causal = kr <= qc
        sd = jnp.concatenate(
            [jnp.where(causal, s[n - 128:n, 128 * a:128 * (a + 1)], NEG) for a in range(nh)], axis=1)
        s_scr[buf, n - 128:n, cols] = sd
        m = jnp.max(sd, axis=0, keepdims=True)
        if j > 0:
            s_scr[buf, 0:n - 128, cols] = s[0:n - 128]
            m = jnp.maximum(m, jnp.max(s[0:n - 128], axis=0, keepdims=True))
        m_scr[buf, :, cols] = jnp.broadcast_to(m, (8, 128 * nh))

    def phase_b(w, heads, j, buf):
        n = 128 * (j + 1)
        for a in heads:
            m = m_scr[buf, 0:1, 128 * a:128 * (a + 1)]
            p = jnp.exp2(s_scr[buf, 0:n, 128 * a:128 * (a + 1)] - m).astype(bf16)
            vt = jnp.concatenate([_unpack(vT_s[w, t, (RS // 2) * a:(RS // 2) * a + 16, :]) for t in range(j + 1)], axis=1)
            o = jnp.dot(vt, p, preferred_element_type=f32)
            g = g_s[w, a:a + 1, :]
            od = o[0:24] * ((1.0 - g) / o[DH:DH + 1])
            row0 = WL * w + DH * a
            oT_s[j, pl.ds(row0, DH), :] = (od + am_s[j, pl.ds(row0, 24), :])[0:DH]

    def window(w, nxt, fillers, upd_plan):
        order = [3, 2, 1, 0]
        heads = list(range(_nh(w)))
        for t in range(4):
            for fn in fillers.get(t, ()):
                fn()
            if t < 3:
                phase_a(w, heads, order[t + 1], (t + 1) % 2)
            elif nxt is not None:
                phase_a(nxt, list(range(_nh(nxt))), order[0], 0)
            ws = upd_plan.get((w, t), [])
            if ws:
                mem_update(ws)
            phase_b(w, heads, order[t], t % 2)

    def ln2_out(tile, lo=0, hi=NCH):
        mean = st_s[tile, 0:1, :]
        rstd = st_s[tile, 1:2, :]
        ga = 1.0 + rstd
        gb = mean * rstd
        for i in range(lo, hi):
            rows = slice(RC * i, RC * (i + 1))
            out_v[tile, rows, :] = (h_s[tile, rows, :] * ga - gb).astype(bf16)

    def outproj(seg):
        oT = jnp.concatenate([oT_s[t] for t in range(4)], axis=1).astype(bf16)
        attn = jnp.dot(woT[...], oT, preferred_element_type=f32)
        for t in range(4):
            cols = slice(128 * t, 128 * (t + 1))
            tile = 4 * seg + t
            c = None
            s1, s2, s3 = _Acc(), _Acc(), _Acc()
            for i in range(NCH):
                rows = slice(RC * i, RC * (i + 1))
                h = x_v[seg, rows, cols].astype(f32) + attn[rows, cols]
                h_s[tile, rows, :] = h
                if c is None:
                    c = h[0:1]
                d = h - c
                s1.add(d)
                s2.add(d * d)
                s3.add(d * wr_s[rows, :])
            mu = s1.total() * (1.0 / D)
            var = jnp.maximum(s2.total() * (1.0 / D) - mu * mu, 0.0)
            rstd = lax.rsqrt(var + EPS)
            st_s[tile, 0:1, :] = c + mu
            st_s[tile, 1:2, :] = rstd
            r_s[pl.ds(tile, 1), :] = (s3.total() - mu * wr_s[D:D + 1, :]) * rstd

    def transpose_wd(lo, hi):
        for i in range(lo, hi):
            wd_s[128 * i:128 * (i + 1), :] = wdT_v[:, 128 * i:128 * (i + 1)].T

    x_copy(0).start()
    beta = beta_ref[...].astype(f32).reshape(1, H)
    hrow = lax.broadcasted_iota(jnp.int32, (8 * NW, H), 0)
    hcol = lax.broadcasted_iota(jnp.int32, (8 * NW, H), 1)
    sel = (hcol == HPW * (hrow >> 3) + (hrow & 7)) & ((hrow & 7) < HPW)
    bcol = jnp.sum(jnp.where(sel, beta, 0.0), axis=1, keepdims=True)
    g_s[...] = jnp.broadcast_to(_sigmoid(bcol), (8 * NW, 128)).reshape(NW, 8, 128)
    wr_row = wr_ref[...].astype(f32).reshape(1, D)
    wr_pad = jnp.concatenate([wr_row, jnp.zeros((1, 64), f32)], axis=1)
    wr_s[...] = jnp.broadcast_to(wr_pad, (128, D + 64)).T
    wr_s[D:D + 1, :] = jnp.broadcast_to(jnp.sum(wr_row, axis=1, keepdims=True), (1, 128))

    w_copies[0].start()
    zero_s[0] = 0
    mt_s[...] = jnp.zeros(mt_s.shape, f32)
    vT_s[...] = jnp.zeros(vT_s.shape, u32)
    am_s[...] = jnp.zeros(am_s.shape, f32)
    s_scr[:, 0:8, 0:128] = jnp.zeros((2, 8, 128), f32)
    m_scr[...] = jnp.zeros(m_scr.shape, f32)

    x_copy(0).wait()
    w_copies[1].start()
    for t in range(4):
        ln1_tile(0, t)
    w_copies[0].wait()
    w_copies[2].start()
    wT[0:D, :] = wk_v[...].T
    post_k(proj(0))
    w_copies[1].wait()
    w_copies[2].wait()
    w_copies[3].start()
    for s in range(1, NSEG):
        x_copy(s).start()
    wT[D:2 * D, :] = wq_v[...].T
    wT[2 * D:3 * D, :] = wv_v[...].T
    post_q(proj(1))
    post_v(proj(2))
    w_copies[3].wait()
    for s in range(1, NSEG):
        x_copy(s).wait()
    for c in w_copies[4:]:
        c.start()

    def windows(units, upd_plan):
        phase_a(0, list(range(HPW)), 3, 0)
        slots = [(w, t) for w in range(NW) for t in range(4)]
        plan = {}
        for k, fn in enumerate(units):
            plan.setdefault(slots[k * len(slots) // len(units)], []).append(fn)
        for w in range(NW):
            fillers = {t: plan.get((w, t), []) for t in range(4)}
            window(w, w + 1 if w + 1 < NW else None, fillers, upd_plan)

    def t_wo():
        woT[...] = wo_v[...].T

    def barrier():
        @pl.when(zero_s[0] != 0)
        def _():
            xs_keep[...] = s_scr[0, 0:8, 0:128]

    def segment(seg, carry):
        units = []
        for t in range(4):
            st, nm = ln1_units(seg + 1, t, LNPARTS)
            units += st + nm
        windows(units, UPD_PLAN)
        barrier()

        t_wo()
        post_k(proj(0))
        post_q(proj(1))
        post_v(proj(2))
        outproj(seg)
        mem_retrieve()
        for t in range(4):
            ln2_out(4 * seg + t)
        for t in range(4):
            o_copy(4 * seg + t).start()
        return carry

    lax.fori_loop(0, NSEG - 1, segment, 0)
    for c in w_copies[4:]:
        c.wait()
    nb = F // 128
    windows([functools.partial(transpose_wd, i, i + 1) for i in range(nb)], {})
    barrier()
    for t in range(4 * (NSEG - 1)):
        o_copy(t).wait()
    xs_keep[...] = s_scr[0, 0:8, 0:128] + s_scr[1, 0:8, 0:128] + m_scr[0, :, 0:128] + m_scr[1, :, 0:128]
    outproj(NSEG - 1)
    for t in range(4):
        ln2_out(4 * (NSEG - 1) + t)
        o_copy(4 * (NSEG - 1) + t).start()

    r = r_s[...]
    rmax = jnp.max(r)
    tok = (lax.broadcasted_iota(jnp.int32, (NT, 128), 0) * 128
           + lax.broadcasted_iota(jnp.int32, (NT, 128), 1))
    idx = jnp.minimum(jnp.min(jnp.where(r == rmax, tok, S)), S - 1)
    tile = idx >> 7
    lane = idx & 127
    hn = ((h_s[tile] - st_s[tile, 0:1, :]) * st_s[tile, 1:2, :]).astype(bf16)
    onehot = jnp.where(lax.broadcasted_iota(jnp.int32, (16, 128), 1) == lane, 1.0, 0.0).astype(bf16)
    xs = lax.dot_general(onehot, hn, (((1,), (1,)), ((), ())), preferred_element_type=f32)
    fm = F - 128 * NV
    xm = xs[:, 0:512].astype(bf16)
    xr = xs[:, 512:D]
    row = lax.broadcasted_iota(jnp.int32, (16, 64), 0)
    x2 = jnp.concatenate([jnp.where(row == 0, xr, 0.0), jnp.where(row == 1, xr, 0.0)], axis=1).astype(bf16)
    wrem = jnp.concatenate([wg_v[512:D, 0:fm], wu_v[512:D, 0:fm]], axis=0)
    if NV:
        sel_mat = jnp.where(lax.broadcasted_iota(jnp.int32, (128, 128), 0) == lane, 1.0, 0.0).astype(bf16)
        xb_s[...] = jnp.dot(hn, sel_mat, preferred_element_type=f32)
    rem = jnp.dot(x2, wrem, preferred_element_type=f32)
    gate = jnp.dot(xm, wg_v[0:512, 0:fm], preferred_element_type=f32)[0:1] + rem[0:1]
    up = jnp.dot(xm, wu_v[0:512, 0:fm], preferred_element_type=f32)[0:1] + rem[1:2]
    if NV:
        accs = [None] * (2 * NV)
        for i in range(NCH):
            rows = slice(RC * i, RC * (i + 1))
            xb = xb_s[rows, :]
            for c in range(2 * NV):
                wsrc = wg_v if c < NV else wu_v
                c0 = fm + 128 * (c % NV)
                t = wsrc[rows, c0:c0 + 128].astype(f32) * xb
                accs[c] = t if accs[c] is None else accs[c] + t
        sums = [jnp.sum(a, axis=0, keepdims=True) for a in accs]
        gate = jnp.concatenate([gate] + sums[:NV], axis=1)
        up = jnp.concatenate([up] + sums[NV:], axis=1)
    act = jnp.broadcast_to(gate * _sigmoid(gate) * up, (16, F)).astype(bf16)
    y = jnp.dot(act, wd_s[...], preferred_element_type=f32)
    y = y[0:1] * _sigmoid(jnp.full((1, 1), rmax, f32))
    ypad = jnp.concatenate([y, jnp.zeros((1, 64), f32)], axis=1)
    ycol = jnp.broadcast_to(ypad, (128, D + 64)).T[0:D]
    for t in range(4 * (NSEG - 1), NT):
        o_copy(t).wait()
    lanes = lax.broadcasted_iota(jnp.int32, (D, 128), 1)
    blk = out_v[tile].astype(f32)
    out_v[tile] = jnp.where(lanes == lane, blk + ycol, blk).astype(bf16)
    fix = o_copy(tile)
    fix.start()
    fix.wait()


@jax.jit
def pallas_sequential_preLN__memory_aug_infini_attn__moe_arch_mod__prompt_kernel(
    A_x: jax.Array,
    A_wq: jax.Array,
    A_wk: jax.Array,
    A_wv: jax.Array,
    A_wo: jax.Array,
    A_beta: jax.Array,
    B_x: jax.Array,
    B_w_r: jax.Array,
    B_w_gate: jax.Array,
    B_w_up: jax.Array,
    B_w_down: jax.Array,
):
    del B_x
    xT = A_x.reshape(S, D).T

    hbm = pl.BlockSpec(memory_space=pltpu.HBM)
    vmem = pl.BlockSpec(memory_space=pltpu.VMEM)
    scratch = [
        pltpu.VMEM((NSEG, D, L), bf16),
        pltpu.VMEM((D, D), bf16),
        pltpu.VMEM((D, D), bf16),
        pltpu.VMEM((D, D), bf16),
        pltpu.VMEM((D, D), bf16),
        pltpu.VMEM((D, F), bf16),
        pltpu.VMEM((D, F), bf16),
        pltpu.VMEM((D, F), bf16),
        pltpu.VMEM((3 * D, D), bf16),
        pltpu.VMEM((D, D), bf16),
        pltpu.VMEM((F, D), bf16),
        pltpu.VMEM((NW, 8, 128), f32),
        pltpu.VMEM((D + 64, 128), f32),
        pltpu.VMEM((4, D, 128), bf16),
        pltpu.VMEM((NW, L // 2, 128), u32),
        pltpu.VMEM((NW, 4, 64, 128), u32),
        pltpu.VMEM((NW, 4, 64, 128), u32),
        pltpu.VMEM((NW, 4, 64, 128), u32),
        pltpu.VMEM((NW, 4, VWORDS, 128), u32),
        pltpu.VMEM((NW, MROWS, 128), f32),
        pltpu.VMEM((NW, MROWS // 2, 128), u32),
        pltpu.VMEM((4, D + 8, 128), f32),
        pltpu.VMEM((2, L, 128 * HPW), f32),
        pltpu.VMEM((2, 8, 128 * HPW), f32),
        pltpu.VMEM((4, D, 128), f32),
        pltpu.VMEM((NT, D, 128), bf16),
        pltpu.VMEM((NT, D, 128), f32),
        pltpu.VMEM((NT, 8, 128), f32),
        pltpu.VMEM((NT, 128), f32),
        pltpu.VMEM((8, 128), f32),
        pltpu.VMEM((D, 128), f32),
        pltpu.SMEM((1,), jnp.int32),
        pltpu.SemaphoreType.DMA((NSEG,)),
        pltpu.SemaphoreType.DMA((7,)),
        pltpu.SemaphoreType.DMA((NT,)),
    ]
    outT = pl.pallas_call(
        _kernel,
        out_shape=jax.ShapeDtypeStruct((D, S), bf16),
        in_specs=[hbm, hbm, hbm, hbm, hbm, vmem, vmem, hbm, hbm, hbm],
        out_specs=hbm,
        scratch_shapes=scratch,
        compiler_params=pltpu.CompilerParams(vmem_limit_bytes=100 * 1024 * 1024),
    )(xT, A_wq, A_wk, A_wv, A_wo, A_beta, B_w_r, B_w_gate, B_w_up, B_w_down.T)
    return outT.T.reshape(1, S, D)
```

```python
import functools

import jax
import jax.numpy as jnp
from jax import lax
import jax.experimental.pallas as pl
import jax.experimental.pallas.tpu as pltpu

S = 2048
D = 576
H = 32
DH = 18
NSEG = 4
L = 512
NT = S // 128
F = 4608
HPW = 7
NW = 5
WL = HPW * DH
RS = 20
MROWS = 144
VWORDS = 80
LOG2E = 1.4426950408889634
NEG = -1e9 * LOG2E
QSCALE = (DH ** -0.5) * LOG2E
EPS = 1e-5
RC = 16
NCH = D // RC
LNPARTS = 4
NV = 10
UPD_PLAN = {(1, 2): [0], (2, 2): [1], (3, 2): [2], (4, 2): [3], (4, 3): [4]}

f32 = jnp.float32
bf16 = jnp.bfloat16
u32 = jnp.uint32


def _nh(w):
    return HPW if w < NW - 1 else H - HPW * (NW - 1)


def _pack(x):
    return pltpu.bitcast(x.astype(bf16), u32)


def _unpack(x):
    return pltpu.bitcast(x, bf16)


def _phi(t):
    return jnp.where(t > 0, t + 1.0, jnp.exp(t))


class _Acc:
    def __init__(self, n=2):
        self.parts = [None] * n
        self.i = 0

    def add(self, x):
        k = self.i % len(self.parts)
        self.parts[k] = x if self.parts[k] is None else self.parts[k] + x
        self.i += 1

    def total(self):
        t = self.parts[0]
        for p in self.parts[1:]:
            t = t + p
        return jnp.sum(t, axis=0, keepdims=True)


def _sigmoid(x):
    return 1.0 / (1.0 + jnp.exp(-x))


def _kernel(xT_hbm, wq_hbm, wk_hbm, wv_hbm, wo_hbm, beta_hbm, wr_hbm, wg_hbm, wu_hbm, wdT_hbm,
            out_hbm,
            x_v, wq_v, wk_v, wv_v, wo_v, wg_v, wu_v, wdT_v, beta_ref, wr_ref,
            wT, woT, wd_s, g_s, wr_s,
            xn_s, k_s, phikT_s, qT_s, phiqT_s, vT_s, mt_s, mtb_s, am_s,
            s_scr, m_scr, oT_s, out_v, h_s, st_s, r_s, xs_keep, xb_s, zero_s,
            sem_x, sem_w, sem_o, sem_s):
    def x_copy(s):
        return pltpu.make_async_copy(xT_hbm.at[:, pl.ds(s * L, L)], x_v.at[s], sem_x.at[s])

    def o_copy(t):
        return pltpu.make_async_copy(out_v.at[t], out_hbm.at[:, pl.ds(pl.multiple_of(t * 128, 128), 128)],
                                     sem_o.at[t])

    w_copies = [pltpu.make_async_copy(src, dst, sem_w.at[i]) for i, (src, dst) in enumerate(
        [(wk_hbm, wk_v), (wq_hbm, wq_v), (wv_hbm, wv_v), (wo_hbm, wo_v),
         (wdT_hbm, wdT_v), (wg_hbm, wg_v), (wu_hbm, wu_v)])]

    def ln1_chunk(seg, t, i):
        cols = pl.ds(pl.multiple_of(t * 128, 128), 128)
        return x_v[seg, RC * i:RC * (i + 1), cols].astype(f32)

    def ln1_units(seg, t, nparts):
        st = {}
        bounds = [NCH * i // nparts for i in range(nparts + 1)]

        def stats_part(k):
            if k == 0:
                x0 = ln1_chunk(seg, t, 0)
                st["x0"], st["c"] = x0, x0[0:1]
                st["s1"], st["s2"] = _Acc(), _Acc()
            for i in range(bounds[k], bounds[k + 1]):
                d = (st["x0"] if i == 0 else ln1_chunk(seg, t, i)) - st["c"]
                st["s1"].add(d)
                st["s2"].add(d * d)
            if k == nparts - 1:
                mu = st["s1"].total() * (1.0 / D)
                var = jnp.maximum(st["s2"].total() * (1.0 / D) - mu * mu, 0.0)
                st["mean"], st["rstd"] = st["c"] + mu, lax.rsqrt(var + EPS)

        def norm_part(k):
            for i in range(bounds[k], bounds[k + 1]):
                xn = (ln1_chunk(seg, t, i) - st["mean"]) * st["rstd"]
                xn_s[t, RC * i:RC * (i + 1), :] = xn.astype(bf16)

        return ([functools.partial(stats_part, k) for k in range(nparts)],
                [functools.partial(norm_part, k) for k in range(nparts)])

    def ln1_tile(seg, t):
        stats, norm = ln1_units(seg, t, 1)
        for fn in stats + norm:
            fn()

    def proj(i):
        xn = jnp.concatenate([xn_s[t] for t in range(4)], axis=1)
        r = jnp.dot(wT[D * i:D * (i + 1), :], xn, preferred_element_type=f32)
        return jnp.concatenate([r, jnp.zeros((64, L), f32)], axis=0)

    def post_k(r):
        for w in range(NW):
            for t in range(4):
                kk = r[WL * w:WL * w + 128, 128 * t:128 * (t + 1)]
                k_s[w, 64 * t:64 * (t + 1), :] = pltpu.bitcast(kk.astype(bf16).T, u32)
                phikT_s[w, t] = _pack(_phi(kk))

    def post_v(r):
        rr = lax.broadcasted_iota(jnp.int32, (RS, 128), 0)
        ones_row = jnp.where(rr == DH, 1.0, 0.0).astype(f32)
        for w in range(NW):
            for t in range(4):
                nh = _nh(w)
                vs = [jnp.where(rr < DH,
                                r[DH * (HPW * w + a):DH * (HPW * w + a) + RS, 128 * t:128 * (t + 1)], ones_row)
                      for a in range(nh)]
                if (nh * RS) % 16:
                    vs.append(jnp.zeros((16 - (nh * RS) % 16, 128), f32))
                vv = _pack(jnp.concatenate(vs, axis=0))
                vT_s[w, t, 0:vv.shape[0], :] = vv

    def post_q(r):
        for w in range(NW):
            for t in range(4):
                q = r[WL * w:WL * w + 128, 128 * t:128 * (t + 1)]
                qT_s[w, t] = _pack(q * QSCALE)
                phiqT_s[w, t] = _pack(_phi(q))

    def mem_update(ws=range(NW)):
        r = lax.broadcasted_iota(jnp.int32, (MROWS, 128), 0)
        c = lax.broadcasted_iota(jnp.int32, (MROWS, 128), 1)
        for w in ws:
            vt = jnp.concatenate([_unpack(vT_s[w, t, 0:MROWS // 2, :]) for t in range(4)], axis=1)
            pk = jnp.concatenate([_unpack(phikT_s[w, t]) for t in range(4)], axis=1)
            upd = lax.dot_general(vt, pk, (((1,), (1,)), ((), ())), preferred_element_type=f32)
            mt = mt_s[w] + upd
            mt_s[w] = mt
            keep = jnp.zeros((MROWS, 128), jnp.bool_)
            for a in range(_nh(w)):
                keep = keep | ((r >= RS * a) & (r < RS * (a + 1)) & (c >= DH * a) & (c < DH * (a + 1)))
            mtb_s[w] = _pack(jnp.where(keep, mt, 0.0))

    def mem_retrieve():
        for w in range(NW):
            for j in range(4):
                am = jnp.dot(_unpack(mtb_s[w]), _unpack(phiqT_s[w, j]), preferred_element_type=f32)
                for a in range(_nh(w)):
                    ama = am[RS * a:RS * a + 24]
                    g = g_s[w, a:a + 1, :]
                    om = ama * (g / (ama[DH:DH + 1] + 1e-6))
                    am_s[j, WL * w + DH * a:WL * w + DH * (a + 1), :] = om[0:DH]

    def phase_a(w, heads, j, buf):
        n = 128 * (j + 1)
        nh = len(heads)
        cols = slice(128 * heads[0], 128 * (heads[-1] + 1))
        rows = lax.broadcasted_iota(jnp.int32, (64, 128), 0)
        qw = qT_s[w, j]
        qbd = jnp.concatenate(
            [jnp.where((rows >= 9 * a) & (rows < 9 * a + 9), qw, jnp.uint32(0)) for a in heads], axis=1)
        s = jnp.dot(_unpack(k_s[w, 0:n // 2, :]), _unpack(qbd), preferred_element_type=f32)
        kr = lax.broadcasted_iota(jnp.int32, (128, 128), 0)
        qc = lax.broadcasted_iota(jnp.int32, (128, 128), 1)
        causal = kr <= qc
        sd = jnp.concatenate(
            [jnp.where(causal, s[n - 128:n, 128 * a:128 * (a + 1)], NEG) for a in range(nh)], axis=1)
        s_scr[buf, n - 128:n, cols] = sd
        m = jnp.max(sd, axis=0, keepdims=True)
        if j > 0:
            s_scr[buf, 0:n - 128, cols] = s[0:n - 128]
            m = jnp.maximum(m, jnp.max(s[0:n - 128], axis=0, keepdims=True))
        m_scr[buf, :, cols] = jnp.broadcast_to(m, (8, 128 * nh))

    def phase_b(w, heads, j, buf):
        n = 128 * (j + 1)
        for a in heads:
            m = m_scr[buf, 0:1, 128 * a:128 * (a + 1)]
            p = jnp.exp2(s_scr[buf, 0:n, 128 * a:128 * (a + 1)] - m).astype(bf16)
            vt = jnp.concatenate([_unpack(vT_s[w, t, (RS // 2) * a:(RS // 2) * a + 16, :]) for t in range(j + 1)], axis=1)
            o = jnp.dot(vt, p, preferred_element_type=f32)
            g = g_s[w, a:a + 1, :]
            od = o[0:24] * ((1.0 - g) / o[DH:DH + 1])
            row0 = WL * w + DH * a
            oT_s[j, pl.ds(row0, DH), :] = (od + am_s[j, pl.ds(row0, 24), :])[0:DH]

    def window(w, nxt, fillers, upd_plan):
        order = [3, 2, 1, 0]
        heads = list(range(_nh(w)))
        for t in range(4):
            for fn in fillers.get(t, ()):
                fn()
            if t < 3:
                phase_a(w, heads, order[t + 1], (t + 1) % 2)
            elif nxt is not None:
                phase_a(nxt, list(range(_nh(nxt))), order[0], 0)
            ws = upd_plan.get((w, t), [])
            if ws:
                mem_update(ws)
            phase_b(w, heads, order[t], t % 2)

    def ln2_out(tile, lo=0, hi=NCH):
        mean = st_s[tile, 0:1, :]
        rstd = st_s[tile, 1:2, :]
        ga = 1.0 + rstd
        gb = mean * rstd
        for i in range(lo, hi):
            rows = slice(RC * i, RC * (i + 1))
            out_v[tile, rows, :] = (h_s[tile, rows, :] * ga - gb).astype(bf16)

    def outproj(seg):
        oT = jnp.concatenate([oT_s[t] for t in range(4)], axis=1).astype(bf16)
        attn = jnp.dot(woT[...], oT, preferred_element_type=f32)
        for t in range(4):
            cols = slice(128 * t, 128 * (t + 1))
            tile = 4 * seg + t
            c = None
            s1, s2, s3 = _Acc(), _Acc(), _Acc()
            for i in range(NCH):
                rows = slice(RC * i, RC * (i + 1))
                h = x_v[seg, rows, cols].astype(f32) + attn[rows, cols]
                h_s[tile, rows, :] = h
                if c is None:
                    c = h[0:1]
                d = h - c
                s1.add(d)
                s2.add(d * d)
                s3.add(d * wr_s[rows, :])
            mu = s1.total() * (1.0 / D)
            var = jnp.maximum(s2.total() * (1.0 / D) - mu * mu, 0.0)
            rstd = lax.rsqrt(var + EPS)
            st_s[tile, 0:1, :] = c + mu
            st_s[tile, 1:2, :] = rstd
            r_s[pl.ds(tile, 1), :] = (s3.total() - mu * wr_s[D:D + 1, :]) * rstd

    def transpose_wd(lo, hi):
        for i in range(lo, hi):
            wd_s[128 * i:128 * (i + 1), :] = wdT_v[:, 128 * i:128 * (i + 1)].T

    x_copy(0).start()
    w_copies[1].start()
    small = [pltpu.make_async_copy(beta_hbm, beta_ref, sem_s.at[0]),
             pltpu.make_async_copy(wr_hbm, wr_ref, sem_s.at[1])]
    for c in small:
        c.start()
    zero_s[0] = 0
    mt_s[...] = jnp.zeros(mt_s.shape, f32)
    vT_s[...] = jnp.zeros(vT_s.shape, u32)
    am_s[...] = jnp.zeros(am_s.shape, f32)
    s_scr[:, 0:8, 0:128] = jnp.zeros((2, 8, 128), f32)
    m_scr[...] = jnp.zeros(m_scr.shape, f32)

    x_copy(0).wait()
    w_copies[0].start()
    for t in range(4):
        ln1_tile(0, t)
    for c in small:
        c.wait()
    beta = beta_ref[...].astype(f32).reshape(1, H)
    hrow = lax.broadcasted_iota(jnp.int32, (8 * NW, H), 0)
    hcol = lax.broadcasted_iota(jnp.int32, (8 * NW, H), 1)
    sel = (hcol == HPW * (hrow >> 3) + (hrow & 7)) & ((hrow & 7) < HPW)
    bcol = jnp.sum(jnp.where(sel, beta, 0.0), axis=1, keepdims=True)
    g_s[...] = jnp.broadcast_to(_sigmoid(bcol), (8 * NW, 128)).reshape(NW, 8, 128)
    wr_row = wr_ref[...].astype(f32).reshape(1, D)
    wr_pad = jnp.concatenate([wr_row, jnp.zeros((1, 64), f32)], axis=1)
    wr_s[...] = jnp.broadcast_to(wr_pad, (128, D + 64)).T
    wr_s[D:D + 1, :] = jnp.broadcast_to(jnp.sum(wr_row, axis=1, keepdims=True), (1, 128))

    w_copies[1].wait()
    w_copies[2].start()
    wT[D:2 * D, :] = wq_v[...].T
    post_q(proj(1))
    w_copies[0].wait()
    w_copies[2].wait()
    w_copies[3].start()
    for s in range(1, NSEG):
        x_copy(s).start()
    wT[0:D, :] = wk_v[...].T
    wT[2 * D:3 * D, :] = wv_v[...].T
    post_k(proj(0))
    post_v(proj(2))
    w_copies[3].wait()
    for s in range(1, NSEG):
        x_copy(s).wait()
    for c in w_copies[4:]:
        c.start()

    def windows(units, upd_plan):
        phase_a(0, list(range(HPW)), 3, 0)
        slots = [(w, t) for w in range(NW) for t in range(4)]
        plan = {}
        for k, fn in enumerate(units):
            plan.setdefault(slots[k * len(slots) // len(units)], []).append(fn)
        for w in range(NW):
            fillers = {t: plan.get((w, t), []) for t in range(4)}
            window(w, w + 1 if w + 1 < NW else None, fillers, upd_plan)

    def t_wo():
        woT[...] = wo_v[...].T

    def barrier():
        @pl.when(zero_s[0] != 0)
        def _():
            xs_keep[...] = s_scr[0, 0:8, 0:128]

    def segment(seg, carry):
        units = []
        for t in range(4):
            st, nm = ln1_units(seg + 1, t, LNPARTS)
            units += st + nm
        windows(units, UPD_PLAN)
        barrier()

        t_wo()
        post_k(proj(0))
        post_q(proj(1))
        post_v(proj(2))
        outproj(seg)
        mem_retrieve()
        for t in range(4):
            ln2_out(4 * seg + t)
        for t in range(4):
            o_copy(4 * seg + t).start()
        return carry

    lax.fori_loop(0, NSEG - 1, segment, 0)
    for c in w_copies[4:]:
        c.wait()
    nb = F // 128
    windows([functools.partial(transpose_wd, i, i + 1) for i in range(nb)], {})
    barrier()
    for t in range(4 * (NSEG - 1)):
        o_copy(t).wait()
    xs_keep[...] = s_scr[0, 0:8, 0:128] + s_scr[1, 0:8, 0:128] + m_scr[0, :, 0:128] + m_scr[1, :, 0:128]
    outproj(NSEG - 1)
    for t in range(4):
        ln2_out(4 * (NSEG - 1) + t)
        o_copy(4 * (NSEG - 1) + t).start()

    r = r_s[...]
    rmax = jnp.max(jnp.max(r, axis=0, keepdims=True), axis=1, keepdims=True)
    tok = (lax.broadcasted_iota(jnp.int32, (NT, 128), 0) * 128
           + lax.broadcasted_iota(jnp.int32, (NT, 128), 1))
    idx = jnp.minimum(jnp.min(jnp.where(r == rmax, tok, S)), S - 1)
    tile = idx >> 7
    lane = idx & 127
    hn = ((h_s[tile] - st_s[tile, 0:1, :]) * st_s[tile, 1:2, :]).astype(bf16)
    onehot = jnp.where(lax.broadcasted_iota(jnp.int32, (16, 128), 1) == lane, 1.0, 0.0).astype(bf16)
    xs = lax.dot_general(onehot, hn, (((1,), (1,)), ((), ())), preferred_element_type=f32)
    fm = F - 128 * NV
    xm = xs[:, 0:512].astype(bf16)
    xr = xs[:, 512:D]
    row = lax.broadcasted_iota(jnp.int32, (16, 64), 0)
    x2 = jnp.concatenate([jnp.where(row == 0, xr, 0.0), jnp.where(row == 1, xr, 0.0)], axis=1).astype(bf16)
    wrem = jnp.concatenate([wg_v[512:D, 0:fm], wu_v[512:D, 0:fm]], axis=0)
    if NV:
        sel_mat = jnp.where(lax.broadcasted_iota(jnp.int32, (128, 128), 0) == lane, 1.0, 0.0).astype(bf16)
        xb_s[...] = jnp.dot(hn, sel_mat, preferred_element_type=f32)
    rem = jnp.dot(x2, wrem, preferred_element_type=f32)
    gate = jnp.dot(xm, wg_v[0:512, 0:fm], preferred_element_type=f32)[0:1] + rem[0:1]
    up = jnp.dot(xm, wu_v[0:512, 0:fm], preferred_element_type=f32)[0:1] + rem[1:2]
    if NV:
        accs = [None] * (2 * NV)
        for i in range(NCH):
            rows = slice(RC * i, RC * (i + 1))
            xb = xb_s[rows, :]
            for c in range(2 * NV):
                wsrc = wg_v if c < NV else wu_v
                c0 = fm + 128 * (c % NV)
                t = wsrc[rows, c0:c0 + 128].astype(f32) * xb
                accs[c] = t if accs[c] is None else accs[c] + t
        sums = [jnp.sum(a, axis=0, keepdims=True) for a in accs]
        gate = jnp.concatenate([gate] + sums[:NV], axis=1)
        up = jnp.concatenate([up] + sums[NV:], axis=1)
    act = jnp.broadcast_to(gate * _sigmoid(gate) * up, (16, F)).astype(bf16)
    y = jnp.dot(act, wd_s[...], preferred_element_type=f32)
    y = y[0:1] * _sigmoid(rmax)
    ypad = jnp.concatenate([y, jnp.zeros((1, 64), f32)], axis=1)
    ycol = jnp.broadcast_to(ypad, (128, D + 64)).T[0:D]
    for t in range(4 * (NSEG - 1), NT):
        o_copy(t).wait()
    lanes = lax.broadcasted_iota(jnp.int32, (D, 128), 1)
    blk = out_v[tile].astype(f32)
    out_v[tile] = jnp.where(lanes == lane, blk + ycol, blk).astype(bf16)
    fix = o_copy(tile)
    fix.start()
    fix.wait()


@jax.jit
def pallas_sequential_preLN__memory_aug_infini_attn__moe_arch_mod__prompt_kernel(
    A_x: jax.Array,
    A_wq: jax.Array,
    A_wk: jax.Array,
    A_wv: jax.Array,
    A_wo: jax.Array,
    A_beta: jax.Array,
    B_x: jax.Array,
    B_w_r: jax.Array,
    B_w_gate: jax.Array,
    B_w_up: jax.Array,
    B_w_down: jax.Array,
):
    del B_x
    xT = A_x.reshape(S, D).T

    hbm = pl.BlockSpec(memory_space=pltpu.HBM)
    scratch = [
        pltpu.VMEM((NSEG, D, L), bf16),
        pltpu.VMEM((D, D), bf16),
        pltpu.VMEM((D, D), bf16),
        pltpu.VMEM((D, D), bf16),
        pltpu.VMEM((D, D), bf16),
        pltpu.VMEM((D, F), bf16),
        pltpu.VMEM((D, F), bf16),
        pltpu.VMEM((D, F), bf16),
        pltpu.VMEM((H,), bf16),
        pltpu.VMEM((D,), bf16),
        pltpu.VMEM((3 * D, D), bf16),
        pltpu.VMEM((D, D), bf16),
        pltpu.VMEM((F, D), bf16),
        pltpu.VMEM((NW, 8, 128), f32),
        pltpu.VMEM((D + 64, 128), f32),
        pltpu.VMEM((4, D, 128), bf16),
        pltpu.VMEM((NW, L // 2, 128), u32),
        pltpu.VMEM((NW, 4, 64, 128), u32),
        pltpu.VMEM((NW, 4, 64, 128), u32),
        pltpu.VMEM((NW, 4, 64, 128), u32),
        pltpu.VMEM((NW, 4, VWORDS, 128), u32),
        pltpu.VMEM((NW, MROWS, 128), f32),
        pltpu.VMEM((NW, MROWS // 2, 128), u32),
        pltpu.VMEM((4, D + 8, 128), f32),
        pltpu.VMEM((2, L, 128 * HPW), f32),
        pltpu.VMEM((2, 8, 128 * HPW), f32),
        pltpu.VMEM((4, D, 128), f32),
        pltpu.VMEM((NT, D, 128), bf16),
        pltpu.VMEM((NT, D, 128), f32),
        pltpu.VMEM((NT, 8, 128), f32),
        pltpu.VMEM((NT, 128), f32),
        pltpu.VMEM((8, 128), f32),
        pltpu.VMEM((D, 128), f32),
        pltpu.SMEM((1,), jnp.int32),
        pltpu.SemaphoreType.DMA((NSEG,)),
        pltpu.SemaphoreType.DMA((7,)),
        pltpu.SemaphoreType.DMA((NT,)),
        pltpu.SemaphoreType.DMA((2,)),
    ]
    outT = pl.pallas_call(
        _kernel,
        out_shape=jax.ShapeDtypeStruct((D, S), bf16),
        in_specs=[hbm] * 10,
        out_specs=hbm,
        scratch_shapes=scratch,
        compiler_params=pltpu.CompilerParams(vmem_limit_bytes=100 * 1024 * 1024),
    )(xT, A_wq, A_wk, A_wv, A_wo, A_beta, B_w_r, B_w_gate, B_w_up, B_w_down.T)
    return outT.T.reshape(1, S, D)
```

```python
import functools

import jax
import jax.numpy as jnp
from jax import lax
import jax.experimental.pallas as pl
import jax.experimental.pallas.tpu as pltpu

S = 2048
D = 576
H = 32
DH = 18
NSEG = 4
L = 512
NT = S // 128
F = 4608
HPW = 7
NW = 5
WL = HPW * DH
RS = 20
MROWS = 144
VWORDS = 80
LOG2E = 1.4426950408889634
NEG = -1e9 * LOG2E
QSCALE = (DH ** -0.5) * LOG2E
EPS = 1e-5
RC = 16
NCH = D // RC
LNPARTS = 4
OP_PLAN = [(3, 3), (4, 3)]
NOP = len(OP_PLAN)
NV = 10
UPD_PLAN = {(1, 2): [0], (2, 2): [1], (3, 2): [2], (4, 2): [3], (4, 3): [4]}

f32 = jnp.float32
bf16 = jnp.bfloat16
u32 = jnp.uint32


def _nh(w):
    return HPW if w < NW - 1 else H - HPW * (NW - 1)


def _pack(x):
    return pltpu.bitcast(x.astype(bf16), u32)


def _unpack(x):
    return pltpu.bitcast(x, bf16)


def _phi(t):
    return jnp.where(t > 0, t + 1.0, jnp.exp(t))


class _Acc:
    def __init__(self, n=2):
        self.parts = [None] * n
        self.i = 0

    def add(self, x):
        k = self.i % len(self.parts)
        self.parts[k] = x if self.parts[k] is None else self.parts[k] + x
        self.i += 1

    def total(self):
        t = self.parts[0]
        for p in self.parts[1:]:
            t = t + p
        return jnp.sum(t, axis=0, keepdims=True)


def _sigmoid(x):
    return 1.0 / (1.0 + jnp.exp(-x))


def _kernel(xT_hbm, wq_hbm, wk_hbm, wv_hbm, wo_hbm, beta_hbm, wr_hbm, wg_hbm, wu_hbm, wdT_hbm,
            out_hbm,
            x_v, wq_v, wk_v, wv_v, wo_v, wg_v, wu_v, wdT_v, beta_ref, wr_ref,
            wT, woT, wd_s, g_s, wr_s,
            xn_s, k_s, phikT_s, qT_s, phiqT_s, vT_s, mt_s, mtb_s, am_s,
            s_scr, m_scr, oT_s, out_v, h_s, st_s, r_s, xs_keep, xb_s, acc_s, zero_s,
            sem_x, sem_w, sem_o, sem_s):
    def x_copy(s):
        return pltpu.make_async_copy(xT_hbm.at[:, pl.ds(s * L, L)], x_v.at[s], sem_x.at[s])

    def o_copy(t):
        return pltpu.make_async_copy(out_v.at[t], out_hbm.at[:, pl.ds(pl.multiple_of(t * 128, 128), 128)],
                                     sem_o.at[t])

    w_copies = [pltpu.make_async_copy(src, dst, sem_w.at[i]) for i, (src, dst) in enumerate(
        [(wk_hbm, wk_v), (wq_hbm, wq_v), (wv_hbm, wv_v), (wo_hbm, wo_v),
         (wdT_hbm, wdT_v), (wg_hbm, wg_v), (wu_hbm, wu_v)])]

    def ln1_chunk(seg, t, i):
        cols = pl.ds(pl.multiple_of(t * 128, 128), 128)
        return x_v[seg, RC * i:RC * (i + 1), cols].astype(f32)

    def ln1_units(seg, t, nparts):
        st = {}
        bounds = [NCH * i // nparts for i in range(nparts + 1)]

        def stats_part(k):
            if k == 0:
                x0 = ln1_chunk(seg, t, 0)
                st["x0"], st["c"] = x0, x0[0:1]
                st["s1"], st["s2"] = _Acc(), _Acc()
            for i in range(bounds[k], bounds[k + 1]):
                d = (st["x0"] if i == 0 else ln1_chunk(seg, t, i)) - st["c"]
                st["s1"].add(d)
                st["s2"].add(d * d)
            if k == nparts - 1:
                mu = st["s1"].total() * (1.0 / D)
                var = jnp.maximum(st["s2"].total() * (1.0 / D) - mu * mu, 0.0)
                st["mean"], st["rstd"] = st["c"] + mu, lax.rsqrt(var + EPS)

        def norm_part(k):
            for i in range(bounds[k], bounds[k + 1]):
                xn = (ln1_chunk(seg, t, i) - st["mean"]) * st["rstd"]
                xn_s[t, RC * i:RC * (i + 1), :] = xn.astype(bf16)

        return ([functools.partial(stats_part, k) for k in range(nparts)],
                [functools.partial(norm_part, k) for k in range(nparts)])

    def ln1_tile(seg, t):
        stats, norm = ln1_units(seg, t, 1)
        for fn in stats + norm:
            fn()

    def proj(i):
        xn = jnp.concatenate([xn_s[t] for t in range(4)], axis=1)
        r = jnp.dot(wT[D * i:D * (i + 1), :], xn, preferred_element_type=f32)
        return jnp.concatenate([r, jnp.zeros((64, L), f32)], axis=0)

    def post_k(r):
        for w in range(NW):
            for t in range(4):
                kk = r[WL * w:WL * w + 128, 128 * t:128 * (t + 1)]
                k_s[w, 64 * t:64 * (t + 1), :] = pltpu.bitcast(kk.astype(bf16).T, u32)
                phikT_s[w, t] = _pack(_phi(kk))

    def post_v(r):
        rr = lax.broadcasted_iota(jnp.int32, (RS, 128), 0)
        ones_row = jnp.where(rr == DH, 1.0, 0.0).astype(f32)
        for w in range(NW):
            for t in range(4):
                nh = _nh(w)
                vs = [jnp.where(rr < DH,
                                r[DH * (HPW * w + a):DH * (HPW * w + a) + RS, 128 * t:128 * (t + 1)], ones_row)
                      for a in range(nh)]
                if (nh * RS) % 16:
                    vs.append(jnp.zeros((16 - (nh * RS) % 16, 128), f32))
                vv = _pack(jnp.concatenate(vs, axis=0))
                vT_s[w, t, 0:vv.shape[0], :] = vv

    def post_q(r):
        for w in range(NW):
            for t in range(4):
                q = r[WL * w:WL * w + 128, 128 * t:128 * (t + 1)]
                qT_s[w, t] = _pack(q * QSCALE)
                phiqT_s[w, t] = _pack(_phi(q))

    def mem_update(ws=range(NW)):
        r = lax.broadcasted_iota(jnp.int32, (MROWS, 128), 0)
        c = lax.broadcasted_iota(jnp.int32, (MROWS, 128), 1)
        for w in ws:
            vt = jnp.concatenate([_unpack(vT_s[w, t, 0:MROWS // 2, :]) for t in range(4)], axis=1)
            pk = jnp.concatenate([_unpack(phikT_s[w, t]) for t in range(4)], axis=1)
            upd = lax.dot_general(vt, pk, (((1,), (1,)), ((), ())), preferred_element_type=f32)
            mt = mt_s[w] + upd
            mt_s[w] = mt
            keep = jnp.zeros((MROWS, 128), jnp.bool_)
            for a in range(_nh(w)):
                keep = keep | ((r >= RS * a) & (r < RS * (a + 1)) & (c >= DH * a) & (c < DH * (a + 1)))
            mtb_s[w] = _pack(jnp.where(keep, mt, 0.0))

    def mem_retrieve():
        for w in range(NW):
            for j in range(4):
                am = jnp.dot(_unpack(mtb_s[w]), _unpack(phiqT_s[w, j]), preferred_element_type=f32)
                for a in range(_nh(w)):
                    ama = am[RS * a:RS * a + 24]
                    g = g_s[w, a:a + 1, :]
                    om = ama * (g / (ama[DH:DH + 1] + 1e-6))
                    am_s[j, WL * w + DH * a:WL * w + DH * (a + 1), :] = om[0:DH]

    def phase_a(w, heads, j, buf):
        n = 128 * (j + 1)
        nh = len(heads)
        cols = slice(128 * heads[0], 128 * (heads[-1] + 1))
        rows = lax.broadcasted_iota(jnp.int32, (64, 128), 0)
        qw = qT_s[w, j]
        qbd = jnp.concatenate(
            [jnp.where((rows >= 9 * a) & (rows < 9 * a + 9), qw, jnp.uint32(0)) for a in heads], axis=1)
        s = jnp.dot(_unpack(k_s[w, 0:n // 2, :]), _unpack(qbd), preferred_element_type=f32)
        kr = lax.broadcasted_iota(jnp.int32, (128, 128), 0)
        qc = lax.broadcasted_iota(jnp.int32, (128, 128), 1)
        causal = kr <= qc
        sd = jnp.concatenate(
            [jnp.where(causal, s[n - 128:n, 128 * a:128 * (a + 1)], NEG) for a in range(nh)], axis=1)
        s_scr[buf, n - 128:n, cols] = sd
        m = jnp.max(sd, axis=0, keepdims=True)
        if j > 0:
            s_scr[buf, 0:n - 128, cols] = s[0:n - 128]
            m = jnp.maximum(m, jnp.max(s[0:n - 128], axis=0, keepdims=True))
        m_scr[buf, :, cols] = jnp.broadcast_to(m, (8, 128 * nh))

    def phase_b(w, heads, j, buf):
        n = 128 * (j + 1)
        for a in heads:
            m = m_scr[buf, 0:1, 128 * a:128 * (a + 1)]
            p = jnp.exp2(s_scr[buf, 0:n, 128 * a:128 * (a + 1)] - m).astype(bf16)
            vt = jnp.concatenate([_unpack(vT_s[w, t, (RS // 2) * a:(RS // 2) * a + 16, :]) for t in range(j + 1)], axis=1)
            o = jnp.dot(vt, p, preferred_element_type=f32)
            g = g_s[w, a:a + 1, :]
            od = o[0:24] * ((1.0 - g) / o[DH:DH + 1])
            row0 = WL * w + DH * a
            oT_s[j, pl.ds(row0, DH), :] = (od + am_s[j, pl.ds(row0, 24), :])[0:DH]

    def window(w, nxt, fillers, upd_plan):
        order = [3, 2, 1, 0]
        heads = list(range(_nh(w)))
        for t in range(4):
            for fn in fillers.get(t, ()):
                fn()
            if t < 3:
                phase_a(w, heads, order[t + 1], (t + 1) % 2)
            elif nxt is not None:
                phase_a(nxt, list(range(_nh(nxt))), order[0], 0)
            for fn in upd_plan.get((w, t), ()):
                fn()
            phase_b(w, heads, order[t], t % 2)

    def ln2_out(tile, lo=0, hi=NCH):
        mean = st_s[tile, 0:1, :]
        rstd = st_s[tile, 1:2, :]
        ga = 1.0 + rstd
        gb = mean * rstd
        for i in range(lo, hi):
            rows = slice(RC * i, RC * (i + 1))
            out_v[tile, rows, :] = (h_s[tile, rows, :] * ga - gb).astype(bf16)

    def outproj_part(k):
        rows = slice(128 * k, 128 * (k + 1))
        oT = jnp.concatenate([oT_s[t, rows, :] for t in range(4)], axis=1).astype(bf16)
        part = jnp.dot(woT[:, rows], oT, preferred_element_type=f32)
        for t in range(4):
            cols = slice(128 * t, 128 * (t + 1))
            acc_s[t] = part[:, cols] if k == 0 else acc_s[t] + part[:, cols]

    def outproj(seg, k0=0):
        oT = jnp.concatenate([oT_s[t, 128 * k0:D, :] for t in range(4)], axis=1).astype(bf16)
        attn = jnp.dot(woT[:, 128 * k0:D], oT, preferred_element_type=f32)
        if k0:
            attn = attn + jnp.concatenate([acc_s[t] for t in range(4)], axis=1)
        for t in range(4):
            cols = slice(128 * t, 128 * (t + 1))
            tile = 4 * seg + t
            c = None
            s1, s2, s3 = _Acc(), _Acc(), _Acc()
            for i in range(NCH):
                rows = slice(RC * i, RC * (i + 1))
                h = x_v[seg, rows, cols].astype(f32) + attn[rows, cols]
                h_s[tile, rows, :] = h
                if c is None:
                    c = h[0:1]
                d = h - c
                s1.add(d)
                s2.add(d * d)
                s3.add(d * wr_s[rows, :])
            mu = s1.total() * (1.0 / D)
            var = jnp.maximum(s2.total() * (1.0 / D) - mu * mu, 0.0)
            rstd = lax.rsqrt(var + EPS)
            st_s[tile, 0:1, :] = c + mu
            st_s[tile, 1:2, :] = rstd
            r_s[pl.ds(tile, 1), :] = (s3.total() - mu * wr_s[D:D + 1, :]) * rstd

    def transpose_wd(lo, hi):
        for i in range(lo, hi):
            wd_s[128 * i:128 * (i + 1), :] = wdT_v[:, 128 * i:128 * (i + 1)].T

    x_copy(0).start()
    w_copies[1].start()
    small = [pltpu.make_async_copy(beta_hbm, beta_ref, sem_s.at[0]),
             pltpu.make_async_copy(wr_hbm, wr_ref, sem_s.at[1])]
    for c in small:
        c.start()
    zero_s[0] = 0
    mt_s[...] = jnp.zeros(mt_s.shape, f32)
    vT_s[...] = jnp.zeros(vT_s.shape, u32)
    am_s[...] = jnp.zeros(am_s.shape, f32)
    s_scr[:, 0:8, 0:128] = jnp.zeros((2, 8, 128), f32)
    m_scr[...] = jnp.zeros(m_scr.shape, f32)

    x_copy(0).wait()
    w_copies[0].start()
    for t in range(4):
        ln1_tile(0, t)
    for c in small:
        c.wait()
    beta = beta_ref[...].astype(f32).reshape(1, H)
    hrow = lax.broadcasted_iota(jnp.int32, (8 * NW, H), 0)
    hcol = lax.broadcasted_iota(jnp.int32, (8 * NW, H), 1)
    sel = (hcol == HPW * (hrow >> 3) + (hrow & 7)) & ((hrow & 7) < HPW)
    bcol = jnp.sum(jnp.where(sel, beta, 0.0), axis=1, keepdims=True)
    g_s[...] = jnp.broadcast_to(_sigmoid(bcol), (8 * NW, 128)).reshape(NW, 8, 128)
    wr_row = wr_ref[...].astype(f32).reshape(1, D)
    wr_pad = jnp.concatenate([wr_row, jnp.zeros((1, 64), f32)], axis=1)
    wr_s[...] = jnp.broadcast_to(wr_pad, (128, D + 64)).T
    wr_s[D:D + 1, :] = jnp.broadcast_to(jnp.sum(wr_row, axis=1, keepdims=True), (1, 128))

    w_copies[1].wait()
    w_copies[2].start()
    wT[D:2 * D, :] = wq_v[...].T
    post_q(proj(1))
    w_copies[0].wait()
    w_copies[2].wait()
    w_copies[3].start()
    for s in range(1, NSEG):
        x_copy(s).start()
    wT[0:D, :] = wk_v[...].T
    wT[2 * D:3 * D, :] = wv_v[...].T
    post_k(proj(0))
    post_v(proj(2))
    w_copies[3].wait()
    for s in range(1, NSEG):
        x_copy(s).wait()
    for c in w_copies[4:]:
        c.start()

    def windows(units, upd_plan):
        phase_a(0, list(range(HPW)), 3, 0)
        slots = [(w, t) for w in range(NW) for t in range(4)]
        plan = {}
        for k, fn in enumerate(units):
            plan.setdefault(slots[k * len(slots) // len(units)], []).append(fn)
        for w in range(NW):
            fillers = {t: plan.get((w, t), []) for t in range(4)}
            window(w, w + 1 if w + 1 < NW else None, fillers, upd_plan)

    def t_wo():
        woT[...] = wo_v[...].T

    def barrier():
        @pl.when(zero_s[0] != 0)
        def _():
            xs_keep[...] = s_scr[0, 0:8, 0:128]

    def segment(seg, carry):
        units = []
        for t in range(4):
            st, nm = ln1_units(seg + 1, t, LNPARTS)
            units += st + nm
        windows(units, {k: [functools.partial(mem_update, v)] for k, v in UPD_PLAN.items()})
        barrier()

        t_wo()
        post_k(proj(0))
        post_q(proj(1))
        post_v(proj(2))
        outproj(seg)
        mem_retrieve()
        for t in range(4):
            ln2_out(4 * seg + t)
        for t in range(4):
            o_copy(4 * seg + t).start()
        return carry

    lax.fori_loop(0, NSEG - 1, segment, 0)
    for c in w_copies[4:]:
        c.wait()
    nb = F // 128
    windows([functools.partial(transpose_wd, i, i + 1) for i in range(nb)],
            {OP_PLAN[k]: [functools.partial(outproj_part, k)] for k in range(NOP)})
    barrier()
    for t in range(4 * (NSEG - 1)):
        o_copy(t).wait()
    xs_keep[...] = s_scr[0, 0:8, 0:128] + s_scr[1, 0:8, 0:128] + m_scr[0, :, 0:128] + m_scr[1, :, 0:128]
    outproj(NSEG - 1, NOP)
    for t in range(4):
        ln2_out(4 * (NSEG - 1) + t)
        o_copy(4 * (NSEG - 1) + t).start()

    r = r_s[...]
    rmax = jnp.max(jnp.max(r, axis=0, keepdims=True), axis=1, keepdims=True)
    tok = (lax.broadcasted_iota(jnp.int32, (NT, 128), 0) * 128
           + lax.broadcasted_iota(jnp.int32, (NT, 128), 1))
    idx = jnp.minimum(jnp.min(jnp.where(r == rmax, tok, S)), S - 1)
    tile = idx >> 7
    lane = idx & 127
    hn = ((h_s[tile] - st_s[tile, 0:1, :]) * st_s[tile, 1:2, :]).astype(bf16)
    onehot = jnp.where(lax.broadcasted_iota(jnp.int32, (16, 128), 1) == lane, 1.0, 0.0).astype(bf16)
    xs = lax.dot_general(onehot, hn, (((1,), (1,)), ((), ())), preferred_element_type=f32)
    fm = F - 128 * NV
    xm = xs[:, 0:512].astype(bf16)
    xr = xs[:, 512:D]
    row = lax.broadcasted_iota(jnp.int32, (16, 64), 0)
    x2 = jnp.concatenate([jnp.where(row == 0, xr, 0.0), jnp.where(row == 1, xr, 0.0)], axis=1).astype(bf16)
    wrem = jnp.concatenate([wg_v[512:D, 0:fm], wu_v[512:D, 0:fm]], axis=0)
    if NV:
        sel_mat = jnp.where(lax.broadcasted_iota(jnp.int32, (128, 128), 0) == lane, 1.0, 0.0).astype(bf16)
        xb_s[...] = jnp.dot(hn, sel_mat, preferred_element_type=f32)
    rem = jnp.dot(x2, wrem, preferred_element_type=f32)
    gate = jnp.dot(xm, wg_v[0:512, 0:fm], preferred_element_type=f32)[0:1] + rem[0:1]
    up = jnp.dot(xm, wu_v[0:512, 0:fm], preferred_element_type=f32)[0:1] + rem[1:2]
    if NV:
        accs = [None] * (2 * NV)
        for i in range(NCH):
            rows = slice(RC * i, RC * (i + 1))
            xb = xb_s[rows, :]
            for c in range(2 * NV):
                wsrc = wg_v if c < NV else wu_v
                c0 = fm + 128 * (c % NV)
                t = wsrc[rows, c0:c0 + 128].astype(f32) * xb
                accs[c] = t if accs[c] is None else accs[c] + t
        sums = [jnp.sum(a, axis=0, keepdims=True) for a in accs]
        gate = jnp.concatenate([gate] + sums[:NV], axis=1)
        up = jnp.concatenate([up] + sums[NV:], axis=1)
    act = jnp.broadcast_to(gate * _sigmoid(gate) * up, (16, F)).astype(bf16)
    y = jnp.dot(act, wd_s[...], preferred_element_type=f32)
    y = y[0:1] * _sigmoid(rmax)
    ypad = jnp.concatenate([y, jnp.zeros((1, 64), f32)], axis=1)
    ycol = jnp.broadcast_to(ypad, (128, D + 64)).T[0:D]
    for t in range(4 * (NSEG - 1), NT):
        o_copy(t).wait()
    lanes = lax.broadcasted_iota(jnp.int32, (D, 128), 1)
    blk = out_v[tile].astype(f32)
    out_v[tile] = jnp.where(lanes == lane, blk + ycol, blk).astype(bf16)
    fix = o_copy(tile)
    fix.start()
    fix.wait()


@jax.jit
def pallas_sequential_preLN__memory_aug_infini_attn__moe_arch_mod__prompt_kernel(
    A_x: jax.Array,
    A_wq: jax.Array,
    A_wk: jax.Array,
    A_wv: jax.Array,
    A_wo: jax.Array,
    A_beta: jax.Array,
    B_x: jax.Array,
    B_w_r: jax.Array,
    B_w_gate: jax.Array,
    B_w_up: jax.Array,
    B_w_down: jax.Array,
):
    del B_x
    xT = A_x.reshape(S, D).T

    hbm = pl.BlockSpec(memory_space=pltpu.HBM)
    scratch = [
        pltpu.VMEM((NSEG, D, L), bf16),
        pltpu.VMEM((D, D), bf16),
        pltpu.VMEM((D, D), bf16),
        pltpu.VMEM((D, D), bf16),
        pltpu.VMEM((D, D), bf16),
        pltpu.VMEM((D, F), bf16),
        pltpu.VMEM((D, F), bf16),
        pltpu.VMEM((D, F), bf16),
        pltpu.VMEM((H,), bf16),
        pltpu.VMEM((D,), bf16),
        pltpu.VMEM((3 * D, D), bf16),
        pltpu.VMEM((D, D), bf16),
        pltpu.VMEM((F, D), bf16),
        pltpu.VMEM((NW, 8, 128), f32),
        pltpu.VMEM((D + 64, 128), f32),
        pltpu.VMEM((4, D, 128), bf16),
        pltpu.VMEM((NW, L // 2, 128), u32),
        pltpu.VMEM((NW, 4, 64, 128), u32),
        pltpu.VMEM((NW, 4, 64, 128), u32),
        pltpu.VMEM((NW, 4, 64, 128), u32),
        pltpu.VMEM((NW, 4, VWORDS, 128), u32),
        pltpu.VMEM((NW, MROWS, 128), f32),
        pltpu.VMEM((NW, MROWS // 2, 128), u32),
        pltpu.VMEM((4, D + 8, 128), f32),
        pltpu.VMEM((2, L, 128 * HPW), f32),
        pltpu.VMEM((2, 8, 128 * HPW), f32),
        pltpu.VMEM((4, D, 128), f32),
        pltpu.VMEM((NT, D, 128), bf16),
        pltpu.VMEM((NT, D, 128), f32),
        pltpu.VMEM((NT, 8, 128), f32),
        pltpu.VMEM((NT, 128), f32),
        pltpu.VMEM((8, 128), f32),
        pltpu.VMEM((D, 128), f32),
        pltpu.VMEM((4, D, 128), f32),
        pltpu.SMEM((1,), jnp.int32),
        pltpu.SemaphoreType.DMA((NSEG,)),
        pltpu.SemaphoreType.DMA((7,)),
        pltpu.SemaphoreType.DMA((NT,)),
        pltpu.SemaphoreType.DMA((2,)),
    ]
    outT = pl.pallas_call(
        _kernel,
        out_shape=jax.ShapeDtypeStruct((D, S), bf16),
        in_specs=[hbm] * 10,
        out_specs=hbm,
        scratch_shapes=scratch,
        compiler_params=pltpu.CompilerParams(vmem_limit_bytes=100 * 1024 * 1024),
    )(xT, A_wq, A_wk, A_wv, A_wo, A_beta, B_w_r, B_w_gate, B_w_up, B_w_down.T)
    return outT.T.reshape(1, S, D)
```
